```python
import jax
import jax.numpy as jnp

def _softmax(x, axis=-1):
    return jax.nn.softmax(x, axis=axis)
def _gelu(x):
    return jax.nn.gelu(x, approximate=True)
def _silu(x):
    return jax.nn.silu(x)
def _sigmoid(x):
    return jax.nn.sigmoid(x)
def _layernorm(x, axis=-1, eps=1e-5):
    m = jnp.mean(x, axis=axis, keepdims=True)
    v = jnp.var(x, axis=axis, keepdims=True)
    return (x - m) / jnp.sqrt(v + eps)
def _scatter_add(tgt, idx, src, axis=0):
    return tgt.at[idx].add(src)
def _segment_sum(src, seg, n):
    return jax.ops.segment_sum(src, seg, n)
class _Rng:
    def __init__(self, key):
        self._k = key
    def _next(self):
        self._k, sub = jax.random.split(self._k)
        return sub
    def normal(self, shape):
        return jax.random.normal(self._next(), shape, dtype=jnp.bfloat16)
    def randint(self, lo, hi, shape):
        return jax.random.randint(self._next(), shape, lo, hi, dtype=jnp.int32)
    def uniform(self, shape, lo=0.0, hi=1.0):
        return jax.random.uniform(self._next(), shape, jnp.bfloat16, lo, hi)
    def permutation(self, n):
        return jax.random.permutation(self._next(), n)


kernel_name = 'interleave_layers__ssm_conv_s4__sliding_local_dilated__prompt'

def setup_inputs():
    _rng = _Rng(jax.random.key(int.from_bytes(__import__("os").urandom(4), "little")))
    _w = (lambda a: (lambda t: t.astype(jnp.bfloat16) if jnp.issubdtype(t.dtype, jnp.floating) else t)(jnp.asarray(a)))
    def _A_setup():
        B, L, D, N = 1, 2048, 512, 128
        A_re = -jnp.exp((lambda *s: _rng.normal(s) * 0.05)(D, N))
        A_im = jnp.pi * (lambda *s: _rng.normal(s) * 0.05)(D, N)
        B_re = (lambda *s: _rng.normal(s) * 0.05)(D, N)
        B_im = (lambda *s: _rng.normal(s) * 0.05)(D, N)
        C_re = (lambda *s: _rng.normal(s) * 0.05)(D, N)
        C_im = (lambda *s: _rng.normal(s) * 0.05)(D, N)
        log_dt = (lambda *s: _rng.normal(s) * 0.05)(D) * 0.5 - 4.0
        Dskip = (lambda *s: _rng.normal(s) * 0.05)(D)
        return {
            "u": _w((lambda *s: _rng.normal(s) * 0.05)(B, L, D)),
            "A_re": _w(A_re),
            "A_im": _w(A_im),
            "B_re": _w(B_re),
            "B_im": _w(B_im),
            "C_re": _w(C_re),
            "C_im": _w(C_im),
            "log_dt": _w(log_dt),
            "Dskip": _w(Dskip),
        }
    _A_in = _A_setup()

    def _B_setup():
        B, S, D = 1, 2048, 512
        return {
            "x": _w((lambda *s: _rng.normal(s) * 0.05)(B, S, D)),
            "wqkv": _w((lambda *s: _rng.normal(s) * 0.05)(D, 3 * D)),
            "wo": _w((lambda *s: _rng.normal(s) * 0.05)(D, D)),
        }
    _B_in = _B_setup()

    return {
        "A_u": _A_in["u"],
        "A_A_re": _A_in["A_re"],
        "A_A_im": _A_in["A_im"],
        "A_B_re": _A_in["B_re"],
        "A_B_im": _A_in["B_im"],
        "A_C_re": _A_in["C_re"],
        "A_C_im": _A_in["C_im"],
        "A_log_dt": _A_in["log_dt"],
        "A_Dskip": _A_in["Dskip"],
        "B_x": _B_in["x"],
        "B_wqkv": _B_in["wqkv"],
        "B_wo": _B_in["wo"],
    }

def reference(A_u, A_A_re, A_A_im, A_B_re, A_B_im, A_C_re, A_C_im, A_log_dt, A_Dskip, B_x, B_wqkv, B_wo):
    def _A_ref(u, A_re, A_im, B_re, B_im, C_re, C_im, log_dt, Dskip):
        Bsz, L, D = u.shape
        dt = jnp.exp(log_dt)[:, None]
        A = A_re + 1j * A_im
        Bc = B_re + 1j * B_im
        Cc = C_re + 1j * C_im
        logdA = dt * A
        dB = dt * Bc
        l = (lambda x, dt: x.astype(dt))(jnp.arange(L), A_re.dtype)
        P = jnp.exp(logdA[:, :, None] * l[None, None, :])
        K = jnp.einsum("dn,dnl,dn->dl", Cc, P, dB).real
        L2 = 2 * L
        Kp = jnp.pad(K, ((0, 0), (0, L)))
        up = (lambda x, *d: x.transpose(*d))(u, 0, 2, 1)
        up = jnp.pad(up, ((0, 0), (0, 0), (0, L)))
        Kf = (lambda x, axes=(-2,-1): jnp.fft.rfft2(x.astype(jnp.float32), axes=axes))(Kp[:, None, :], axes=(-2, -1))
        Uf = (lambda x, axes=(-2,-1): jnp.fft.rfft2(x.astype(jnp.float32), axes=axes))(up[:, :, None, :], axes=(-2, -1))
        Yf = Uf * Kf[None, :, :, :]
        y = (lambda x, s, axes=(-2,-1): jnp.fft.irfft2(x, s=s, axes=axes).astype(jnp.bfloat16))(Yf, (1, L2), axes=(-2, -1))[:, :, 0, :L]
        y = (lambda x, *d: x.transpose(*d))(y, 0, 2, 1) + u * Dskip[None, None, :]
        return y

    def _B_ref(x, wqkv, wo):
        B, S, D = x.shape
        H = 32; Dh = D // H
        W, dil = 8, 2
        qkv = (lambda x, *d: x.transpose(*d))((x @ wqkv).reshape(B, S, 3, H, Dh), 2, 0, 3, 1, 4)
        q, k, v = qkv[0], qkv[1], qkv[2]
        scale = Dh ** -0.5
        pos = jnp.arange(S)
        off = jnp.arange(W) * dil
        idx = pos[:, None] - off[None, :]
        mask = idx >= 0
        idx_c = jnp.where(mask, idx, 0).reshape(-1)
        kg = k[:, :, idx_c, :].reshape(B, H, S, W, Dh)
        vg = v[:, :, idx_c, :].reshape(B, H, S, W, Dh)
        logits = jnp.einsum("bhsd,bhswd->bhsw", q, kg) * scale
        logits = jnp.where(mask[None, None, :, :], logits, -1e9)
        attn = _softmax(logits, axis=-1)
        o = jnp.einsum("bhsw,bhswd->bhsd", attn, vg)
        return (lambda x, *d: x.transpose(*d))(o, 0, 2, 1, 3).reshape(B, S, D) @ wo

    x = A_u
    x = x + _A_ref(_layernorm(x, axis=-1), A_A_re, A_A_im, A_B_re, A_B_im, A_C_re, A_C_im, A_log_dt, A_Dskip)
    x = x + _B_ref(_layernorm(x, axis=-1), B_wqkv, B_wo)
    x = x + _A_ref(_layernorm(x, axis=-1), A_A_re, A_A_im, A_B_re, A_B_im, A_C_re, A_C_im, A_log_dt, A_Dskip)
    x = x + _B_ref(_layernorm(x, axis=-1), B_wqkv, B_wo)
    return x
```

```python
import jax
import jax.numpy as jnp
import ml_dtypes
import numpy as np
from jax import lax
import jax.experimental.pallas as pl
import jax.experimental.pallas.tpu as pltpu

L, D, N = 2048, 512, 128
R0, R1 = 16, 128
W, DH = 8, 16
F32, BF16 = jnp.float32, jnp.bfloat16
NT = (((1,), (1,)), ((), ()))


def _constants():
    n0 = np.arange(R0)[:, None, None]
    n1 = np.arange(R1)[None, :, None]
    k1 = np.arange(R1)[None, None, :]
    ang = 2.0 * np.pi * (k1 + 0.25) * (R0 * n1 + n0) / L
    f = np.concatenate([np.cos(ang), np.sin(ang)], axis=2)
    g = f.transpose(0, 2, 1)
    bf = ml_dtypes.bfloat16
    lr = np.arange(L).astype(np.float32).astype(bf).astype(np.int64).reshape(8, 16, R0)
    r = lr - (256 * np.arange(8)[:, None, None] + 16 * np.arange(16)[None, :, None])
    assert (r == r[:, :1, :]).all()
    return f.astype(bf), np.ascontiguousarray(g).astype(bf), r[:, 0, :].tolist()


_F, _G, _RND = _constants()


def _cmul(a, b):
    return a[0] * b[0] - a[1] * b[1], a[0] * b[1] + a[1] * b[0]


def _csq(a):
    t = a[0] * a[1]
    return (a[0] + a[1]) * (a[0] - a[1]), t + t


def _dft4(x, sign):
    (ar, ai), (br, bi), (cr, ci), (dr, di) = x
    sr, si, tr, ti = ar + cr, ai + ci, ar - cr, ai - ci
    ur, ui, vr, vi = br + dr, bi + di, br - dr, bi - di
    p, m = (tr - vi, ti + vr), (tr + vi, ti - vr)
    if sign < 0:
        p, m = m, p
    return [(sr + ur, si + ui), p, (sr - ur, si - ui), m]


def _twiddle(v, e):
    e %= 16
    re, im = v
    h = float(np.sqrt(0.5))
    if e == 0:
        return v
    if e == 4:
        return -im, re
    if e == 12:
        return im, -re
    if e == 2:
        return (re - im) * h, (re + im) * h
    if e == 14:
        return (re + im) * h, (im - re) * h
    if e == 6:
        return (re + im) * -h, (re - im) * h
    if e == 10:
        return (im - re) * h, (re + im) * -h
    c, s = float(np.cos(np.pi * e / 8)), float(np.sin(np.pi * e / 8))
    return re * c - im * s, re * s + im * c


def _dft16_groups(x):
    s = [_dft4([x(a + 4 * m) for m in range(4)], 1) for a in range(4)]
    for b in range(4):
        yield b, _dft4([_twiddle(s[a][b], a * b) for a in range(4)], 1)


def _layernorm(x):
    m = jnp.sum(x, axis=0, keepdims=True) * (1.0 / D)
    c = x - m
    v = jnp.sum(c * c, axis=0, keepdims=True) * (1.0 / D)
    return (c * lax.rsqrt(v + 1e-5)).astype(BF16)


def _kernel(x_ref, are_ref, aim_ref, bre_ref, bim_ref, cre_ref, cim_ref, ldt_ref, dsk_ref,
            wqkv_ref, wo_ref, f_ref, g_ref, out_ref,
            xs, io, par, kt, kf, u1, ub, wt, wot, qb, kb, vb, ob):

    def col(ref):
        v = ref[...].astype(F32).reshape(1, D)
        return jnp.broadcast_to(v, (128, D)).T

    with jax.named_scope("setup"):
        dt = jnp.exp(col(ldt_ref)).astype(BF16).astype(F32)
        mag = jnp.exp(dt * are_ref[...].astype(F32))
        ang = dt * aim_ref[...].astype(F32)
        par[0] = mag * jnp.cos(ang)
        par[1] = mag * jnp.sin(ang)
        wr, wi = _cmul((cre_ref[...].astype(F32), cim_ref[...].astype(F32)),
                       (dt * bre_ref[...].astype(F32), dt * bim_ref[...].astype(F32)))
        par[2] = wr * (1.0 / L)
        par[3] = wi * (-1.0 / L)
        par[4] = col(dsk_ref) * (1.0 / L)

    lags = sorted({(c, r) for c in range(8) for r in _RND[c]})

    def kgen(i, carry):
        rows = pl.ds(pl.multiple_of(i * 8, 8), 8)
        z = {0: (jnp.ones((8, N), F32), jnp.zeros((8, N), F32)), 1: (par[0, rows, :], par[1, rows, :])}
        for e in range(2, 17):
            z[e] = _csq(z[e // 2]) if e % 2 == 0 else _cmul(z[e - 1], z[1])
        for e in (32, 64, 128, 256):
            z[e] = _csq(z[e // 2])
        for c in range(2, 8):
            z[256 * c] = _csq(z[128 * c]) if c % 2 == 0 else _cmul(z[256 * (c - 1)], z[256])
        b = [(par[2, rows, :], par[3, rows, :])]
        for e in (16, 32, 64, 128):
            zc = (z[e][0], -z[e][1])
            b += [_cmul(v, zc) for v in b]
        a = [z[256 * c + r] if (c == 0 or r == 0) else _cmul(z[256 * c], z[r]) for c, r in lags]
        a.append(a[-1])
        stack = lambda vs: jnp.concatenate(
            [jnp.concatenate([v[0] for v in vs], 0), jnp.concatenate([v[1] for v in vs], 0)], 1).astype(BF16)
        o = lax.dot_general(stack(a), stack(b), NT, preferred_element_type=F32)
        lane = lax.broadcasted_iota(jnp.int32, (8, 128), 1)
        src = (lane & 15) * 8 + lax.broadcasted_iota(jnp.int32, (8, 128), 0)
        piece = {}
        for t, (c, r) in enumerate(lags):
            piece[c, r] = jnp.take_along_axis(o[8 * t:8 * t + 8], src, axis=1, mode="promise_in_bounds")
        lane_c = lane >> 4
        memo = {}

        def merged(c, rs):
            if (c, rs) not in memo:
                memo[c, rs] = (piece[c, rs[0]] if c == 7 else
                               jnp.where(lane_c == c, piece[c, rs[0]], merged(c + 1, rs[1:])))
            return memo[c, rs]

        for n0 in range(R0):
            kt[n0, rows, :] = merged(0, tuple(_RND[c][n0] for c in range(8)))
        return carry

    with jax.named_scope("kgen"):
        lax.fori_loop(0, D // 8, kgen, 0)

    def kfwd(n0, carry):
        u1[n0] = jnp.dot(kt[n0].astype(BF16), f_ref[n0], preferred_element_type=F32)
        return carry

    def kdft(i, carry):
        rows = pl.ds(pl.multiple_of(i * 8, 8), 8)
        skip = par[4, rows, :]
        for b, xk in _dft16_groups(lambda n: (u1[n, rows, :128], u1[n, rows, 128:])):
            for m in range(4):
                kf[b + 4 * m, rows, :128] = xk[m][0] + skip
                kf[b + 4 * m, rows, 128:] = xk[m][1]
        return carry

    with jax.named_scope("kfwd"):
        lax.fori_loop(0, R0, kfwd, 0)
    with jax.named_scope("kdft"):
        lax.fori_loop(0, D // 8, kdft, 0)

    with jax.named_scope("wprep"):
        ri = lax.broadcasted_iota(jnp.int32, (128, 128), 0)
        ci = lax.broadcasted_iota(jnp.int32, (128, 128), 1)
        perm = jnp.where(ci == (ri & 7) * DH + (ri >> 3), 1.0, 0.0).astype(BF16)
        for g in range(4):
            for t in range(3):
                blk = wqkv_ref[:, t * D + g * 128:t * D + (g + 1) * 128]
                v = lax.dot_general(perm, blk, NT, preferred_element_type=F32)
                if t == 0:
                    v = v * DH ** -0.5
                wt[g, t * 128:(t + 1) * 128, :] = v.astype(BF16)
            v = jnp.dot(perm, wo_ref[g * 128:(g + 1) * 128, :], preferred_element_type=F32)
            wot[:, g * 128:(g + 1) * 128] = v.T.astype(BF16)

    with jax.named_scope("xin"):
        for c in range(4):
            io[c] = pltpu.bitcast(x_ref[:, c * 128:(c + 1) * 128], jnp.uint32)

        def xin(j, carry):
            for c in range(4):
                t = io[c, pl.ds(j, R1, stride=8), :].T
                xs[2 * j, c * 128:(c + 1) * 128, :] = pltpu.bitcast(t << 16, F32)
                xs[2 * j + 1, c * 128:(c + 1) * 128, :] = pltpu.bitcast(t & jnp.uint32(0xFFFF0000), F32)
            return carry

        lax.fori_loop(0, R0 // 2, xin, 0)

    def fwd(n0, carry):
        u1[n0] = jnp.dot(_layernorm(xs[n0]), f_ref[n0], preferred_element_type=F32)
        return carry

    def mid(i, carry):
        rows = pl.ds(pl.multiple_of(i * 8, 8), 8)
        t = []
        for b, xk in _dft16_groups(lambda n: (u1[n, rows, :128], u1[n, rows, 128:])):
            y = [_cmul(xk[m], (kf[b + 4 * m, rows, :128], kf[b + 4 * m, rows, 128:])) for m in range(4)]
            t.append([_twiddle(v, -a * b) for a, v in enumerate(_dft4(y, -1))])
        for a in range(4):
            for m, v in enumerate(_dft4([t[b][a] for b in range(4)], -1)):
                u1[a + 4 * m, rows, :128] = v[0]
                u1[a + 4 * m, rows, 128:] = v[1]
        return carry

    def inv(n0, carry):
        x = xs[n0] + jnp.dot(u1[n0].astype(BF16), g_ref[n0], preferred_element_type=F32)
        xs[n0] = x
        ub[n0] = _layernorm(x)
        return carry

    def unit(i, carry):
        p, g = i >> 2, i & 3
        for m in range(8):
            r = jnp.dot(wt[g], ub[2 * m + p], preferred_element_type=F32)
            qb[m] = r[:128]
            kb[m + 7] = r[128:256]
            vb[m + 7] = r[256:]
            if m:
                kb[m - 1] = pltpu.roll(r[128:256], 1, 1)
                vb[m - 1] = pltpu.roll(r[256:], 1, 1)
        first = lax.broadcasted_iota(jnp.int32, (8, 128), 1) == 0
        for m in range(8):
            s = [None] * W
            for d in range(DH):
                q = qb[m, 8 * d:8 * d + 8, :]
                for w in range(W):
                    t = q * kb[m + 7 - w, 8 * d:8 * d + 8, :]
                    s[w] = t if d == 0 else s[w] + t
            s = [jnp.where(first, -1e9, s[w]) if w > m else s[w] for w in range(W)]
            mx = s[0]
            for w in range(1, W):
                mx = jnp.maximum(mx, s[w])
            e = [jnp.exp(v - mx) for v in s]
            den = e[0]
            for w in range(1, W):
                den = den + e[w]
            rs = 1.0 / den
            e = [v * rs for v in e]
            for d in range(0, DH, 2):
                o = []
                for dd in (d, d + 1):
                    acc = e[0] * vb[m + 7, 8 * dd:8 * dd + 8, :]
                    for w in range(1, W):
                        acc = acc + e[w] * vb[m + 7 - w, 8 * dd:8 * dd + 8, :]
                    o.append(acc)
                ob[2 * m + p, pl.ds(pl.multiple_of(g * 128 + 8 * d, 16), 16), :] = (
                    jnp.concatenate(o, 0).astype(BF16))
        return carry

    def oproj(n0, carry):
        xs[n0] = xs[n0] + jnp.dot(wot[...], ob[n0], preferred_element_type=F32)
        return carry

    def layer(_, carry):
        with jax.named_scope("fwd"):
            lax.fori_loop(0, R0, fwd, 0)
        with jax.named_scope("mid"):
            lax.fori_loop(0, D // 8, mid, 0)
        with jax.named_scope("inv"):
            lax.fori_loop(0, R0, inv, 0)
        with jax.named_scope("unit"):
            lax.fori_loop(0, 8, unit, 0)
        with jax.named_scope("oproj"):
            lax.fori_loop(0, R0, oproj, 0)
        return carry

    lax.fori_loop(0, 2, layer, 0)

    with jax.named_scope("xout"):
        def xout(j, carry):
            for c in range(4):
                lo = xs[2 * j, c * 128:(c + 1) * 128, :].astype(BF16).astype(F32)
                hi = xs[2 * j + 1, c * 128:(c + 1) * 128, :].astype(BF16).astype(F32)
                t = (pltpu.bitcast(lo, jnp.uint32) >> 16) | pltpu.bitcast(hi, jnp.uint32)
                io[c, pl.ds(j, R1, stride=8), :] = t.T
            return carry

        lax.fori_loop(0, R0 // 2, xout, 0)
        for c in range(4):
            out_ref[:, c * 128:(c + 1) * 128] = pltpu.bitcast(io[c], BF16)


@jax.jit
def pallas_interleave_layers__ssm_conv_s4__sliding_local_dilated__prompt_kernel(
    A_u: jax.Array,
    A_A_re: jax.Array,
    A_A_im: jax.Array,
    A_B_re: jax.Array,
    A_B_im: jax.Array,
    A_C_re: jax.Array,
    A_C_im: jax.Array,
    A_log_dt: jax.Array,
    A_Dskip: jax.Array,
    B_x: jax.Array,
    B_wqkv: jax.Array,
    B_wo: jax.Array,
):
    del B_x
    out = pl.pallas_call(
        _kernel,
        out_shape=jax.ShapeDtypeStruct((L, D), BF16),
        scratch_shapes=[
            pltpu.VMEM((R0, D, R1), F32),
            pltpu.VMEM((4, L // 2, 128), jnp.uint32),
            pltpu.VMEM((5, D, N), F32),
            pltpu.VMEM((R0, D, R1), F32),
            pltpu.VMEM((R0, D, 2 * R1), F32),
            pltpu.VMEM((R0, D, 2 * R1), F32),
            pltpu.VMEM((R0, D, R1), BF16),
            pltpu.VMEM((4, 384, D), BF16),
            pltpu.VMEM((D, D), BF16),
            pltpu.VMEM((8, 128, R1), F32),
            pltpu.VMEM((15, 128, R1), F32),
            pltpu.VMEM((15, 128, R1), F32),
            pltpu.VMEM((R0, D, R1), BF16),
        ],
        compiler_params=pltpu.CompilerParams(vmem_limit_bytes=100 * 1024 * 1024),
    )(A_u.reshape(L, D), A_A_re, A_A_im, A_B_re, A_B_im, A_C_re, A_C_im, A_log_dt, A_Dskip,
      B_wqkv, B_wo, _F, _G)
    return out.reshape(1, L, D)
```

```python
import jax
import jax.numpy as jnp
import ml_dtypes
import numpy as np
from jax import lax
import jax.experimental.pallas as pl
import jax.experimental.pallas.tpu as pltpu

L, D, N = 2048, 512, 128
R0, R1 = 16, 128
W, DH = 8, 16
F32, BF16, U32 = jnp.float32, jnp.bfloat16, jnp.uint32
KPER = 2
NB = D // 128
NT = (((1,), (1,)), ((), ()))


def _constants():
    n0 = np.arange(R0)[:, None, None]
    n1 = np.arange(R1)[None, :, None]
    k1 = np.arange(R1)[None, None, :]
    ang = 2.0 * np.pi * (k1 + 0.25) * (R0 * n1 + n0) / L
    f = np.concatenate([np.cos(ang), np.sin(ang)], axis=2)
    g = f.transpose(0, 2, 1)
    bf = ml_dtypes.bfloat16
    lr = np.arange(L).astype(np.float32).astype(bf).astype(np.int64).reshape(8, 16, R0)
    r = lr - (256 * np.arange(8)[:, None, None] + 16 * np.arange(16)[None, :, None])
    assert (r == r[:, :1, :]).all()

    def words(m):
        h = np.ascontiguousarray(m).astype(bf).view(np.uint16).astype(np.uint32)
        return h[:, 0::2] | (h[:, 1::2] << 16)

    return words(f), words(g), r[:, 0, :].tolist()


_F, _G, _RND = _constants()


def _cmul(a, b):
    return a[0] * b[0] - a[1] * b[1], a[0] * b[1] + a[1] * b[0]


def _csq(a):
    t = a[0] * a[1]
    return (a[0] + a[1]) * (a[0] - a[1]), t + t


def _dft4(x, sign):
    (ar, ai), (br, bi), (cr, ci), (dr, di) = x
    sr, si, tr, ti = ar + cr, ai + ci, ar - cr, ai - ci
    ur, ui, vr, vi = br + dr, bi + di, br - dr, bi - di
    p, m = (tr - vi, ti + vr), (tr + vi, ti - vr)
    if sign < 0:
        p, m = m, p
    return [(sr + ur, si + ui), p, (sr - ur, si - ui), m]


def _twiddle(v, e):
    e %= 16
    re, im = v
    h = float(np.sqrt(0.5))
    if e == 0:
        return v
    if e == 4:
        return -im, re
    if e == 12:
        return im, -re
    if e == 2:
        return (re - im) * h, (re + im) * h
    if e == 14:
        return (re + im) * h, (im - re) * h
    if e == 6:
        return (re + im) * -h, (re - im) * h
    if e == 10:
        return (im - re) * h, (re + im) * -h
    c, s = float(np.cos(np.pi * e / 8)), float(np.sin(np.pi * e / 8))
    return re * c - im * s, re * s + im * c


def _bf(x):
    return pltpu.bitcast(x, BF16)


def _tree(op, v):
    while len(v) > 1:
        v = [op(v[i], v[i + 1]) if i + 1 < len(v) else v[i] for i in range(0, len(v), 2)]
    return v[0]


def _run(*streams):
    order = sorted(((i + 0.5) / len(s), k, i) for k, s in enumerate(streams) for i in range(len(s)))
    for _, k, i in order:
        streams[k][i]()


def _pipeline(streams, hooks=None):
    hooks = hooks or {}
    cuts = sorted({e for _, a, n in streams for e in (a, a + n)} | set(hooks))
    for lo, hi in zip(cuts, cuts[1:]):
        def body(s, carry, lo=lo):
            for fn, a, n in streams:
                if a <= lo < a + n:
                    fn(s - a)
            return carry

        if lo in hooks:
            hooks[lo]()
        if hi - lo == 1:
            body(lo, 0)
        else:
            lax.fori_loop(lo, hi, body, 0)


def _rows(i, n):
    return pl.ds(i * n if isinstance(i, int) else pl.multiple_of(i * n, n), n)


def _kernel(zero_ref, x_hbm, are_ref, aim_ref, bre_ref, bim_ref, cre_ref, cim_ref, ldt_ref, dsk_ref,
            wqkv_hbm, wo_hbm, f_hbm, g_hbm, out_hbm,
            xs, kf, ua, ub, uc, yb, par, zw, lag, qa, ka, va, qb, kb, vb, xio, io, wqkv, wo, fm, gm, kt, un, wt, wot, ob, sems):
    step = lambda fn, *a: (lambda: fn(*a))
    qs, ks, vs = (qa, qb), (ka, kb), (va, vb)
    loads = [pltpu.make_async_copy(s, d, sems.at[i]) for i, (s, d) in enumerate(
        ((x_hbm, xio), (f_hbm, fm), (wo_hbm, wo), (g_hbm, gm),
         *((wqkv_hbm.at[:, pl.ds(128 * j, 128)], wqkv.at[j]) for j in range(12))))]
    for c in loads:
        c.start()
    high = jnp.uint32(0xFFFF0000)
    halves = lambda t: (pltpu.bitcast(t << 16, F32), pltpu.bitcast(t & high, F32))

    def col(ref):
        v = ref[...].astype(F32).reshape(1, D)
        return jnp.broadcast_to(v, (128, D)).T

    par[0] = jnp.exp(col(ldt_ref))
    par[1] = col(dsk_ref) * (1.0 / L)

    def setup(i):
        get = lambda ref: jnp.concatenate(halves(pltpu.bitcast(ref[_rows(i, 16), :], U32)), 0)
        dt = jnp.concatenate(halves(pltpu.bitcast(par[0, _rows(i, 16), :].astype(BF16), U32)), 0)
        mag = jnp.exp(dt * get(are_ref))
        ang = dt * get(aim_ref)
        wr, wi = _cmul((get(cre_ref), get(cim_ref)), (dt * get(bre_ref), dt * get(bim_ref)))
        scale = (1.0 + 1.5 * 2.0 ** -9) / L
        for k, v in enumerate((mag * jnp.cos(ang), mag * jnp.sin(ang), wr * scale, wi * -scale)):
            zw[i, k] = v

    lags = sorted({(c, r) for c in range(8) for r in _RND[c] if r < 16}) + [(8, 0)]

    def powers(i, h):
        zr, zi, wr, wi = (zw[i, k, 8 * h:8 * h + 8, :] for k in range(4))
        z = {0: (jnp.ones((8, N), F32), jnp.zeros((8, N), F32)), 1: (zr, zi)}
        for e in (2, 4, 8, 16, 32, 64, 128, 256):
            z[e] = _csq(z[e // 2])
        b = [(wr, wi)]
        for e in (16, 32, 64, 128):
            zc = (z[e][0], -z[e][1])
            b += [_cmul(v, zc) for v in b]

        def power(e):
            if e not in z:
                low = e % 256 if e > 256 and e % 256 else e & -e
                z[e] = _csq(z[e // 2]) if e // 2 in z and e % 2 == 0 else _cmul(power(e - low), power(low))
            return z[e]

        a = [power(256 * c + r) for c, r in lags + lags[-1:]]
        stack = lambda vs: jnp.concatenate(
            [jnp.concatenate([v[k] for v in vs], 0) for k in range(2)], 1).astype(BF16)
        return pltpu.bitcast(lax.dot_general(stack(a), stack(b), NT, preferred_element_type=F32), U32)

    def lagsums(i, k):
        lag[k] = (powers(i, 0) >> 16) | (powers(i, 1) & high)

    def kgen(i, k):
        lane = lax.broadcasted_iota(jnp.int32, (8, 128), 1)
        src = (lane & 15) * 8 + lax.broadcasted_iota(jnp.int32, (8, 128), 0)
        piece = {}
        for t, cr in enumerate(lags):
            piece[cr] = jnp.take_along_axis(lag[k, 8 * t:8 * t + 8, :], src, axis=1, mode="promise_in_bounds")
        memo = {}

        def merged(c, rs):
            if (c, rs) not in memo:
                memo[c, rs] = (piece[c, rs[0]] if c == 7 or min(rs) == 16 else
                               jnp.where(lane >> 4 == c, piece[c, rs[0]], merged(c + 1, rs[1:])))
            return memo[c, rs]

        nxt = pltpu.roll(jnp.where(lane == 0, piece[8, 0], merged(0, (0,) * 8)), 127, 1)
        piece.update({(c, 16): nxt for c in range(8)})
        for n0 in range(R0):
            kt[n0, _rows(i, 8), :] = merged(0, tuple(_RND[c][n0] for c in range(8)))

    get = lambda ref, n, rows: (ref[n, 0, rows, :], ref[n, 1, rows, :])

    def put(ref, n, rows, v):
        ref[n, 0, rows, :], ref[n, 1, rows, :] = v

    def outer(src, a, rows):
        return [_twiddle(v, a * b) for b, v in enumerate(_dft4([get(src, a + 4 * m, rows) for m in range(4)], 1))]

    def transform(lhs, dst, n0, rows):
        r = jnp.dot(lhs, _bf(fm[n0]), preferred_element_type=F32)
        put(dst, n0, rows, (r[:, :128], r[:, 128:]))

    def kfwd(n0, r):
        transform(_bf(kt[n0, _rows(r, 128), :]), ub, n0, _rows(r, 256))

    def kdft(i):
        rows = _rows(i, 8)
        t = [outer(ub, a, rows) for a in range(4)]
        for b in range(4):
            for m, v in enumerate(_dft4([t[a][b] for a in range(4)], 1)):
                put(kf, b + 4 * m, rows, (v[0] + par[1, rows, :], v[1]))

    def fwd(n0, r):
        transform(un[n0, _rows(r, MR[fwd]), :], ua, n0, _rows(r, MR[fwd]))

    def pre(a, i):
        for b, v in enumerate(outer(ua, a, _rows(i, 8))):
            put(ub, a + 4 * b, _rows(i, 8), v)

    def mid(i):
        out = []
        for rows in (_rows(2 * i, 8), _rows(2 * i + 1, 8)):
            t = []
            for b, v in enumerate(outer(ua, 0, rows)):
                x = _dft4([v] + [get(ub, a + 4 * b, rows) for a in range(1, 4)], 1)
                y = _dft4([_cmul(x[m], get(kf, b + 4 * m, rows)) for m in range(4)], -1)
                t.append(y[0])
                for a in range(1, 4):
                    put(uc, a + 4 * b, rows, y[a])
            out.append(_dft4(t, -1))
        for m, (v, w) in enumerate(zip(*out)):
            put(yb, 4 * m, _rows(i, 16), [jnp.concatenate([v[k], w[k]], 0).astype(BF16) for k in range(2)])

    def post(a, i):
        rows = _rows(i, 16)
        for m, v in enumerate(_dft4([_twiddle(get(uc, a + 4 * b, rows), -a * b) for b in range(4)], -1)):
            put(yb, a + 4 * m, rows, (v[0].astype(BF16), v[1].astype(BF16)))

    def inv(n0, r):
        rows = _rows(r, MR[inv])
        y = jnp.concatenate(get(yb, n0, rows), 1)
        xs[n0, rows, :] = xs[n0, rows, :] + jnp.dot(y, _bf(gm[n0]), preferred_element_type=F32)

    def wprep(g, t):
        ri = lax.broadcasted_iota(jnp.int32, (128, 128), 0)
        ci = lax.broadcasted_iota(jnp.int32, (128, 128), 1)
        perm = jnp.where(ci == (ri & 7) * DH + (ri >> 3), DH ** -0.5 if t == 0 else 1.0, 0.0).astype(BF16)
        if t < 3:
            blk = wqkv[4 * t + g]
            wt[g, t * 64:(t + 1) * 64, :] = pltpu.bitcast(lax.dot_general(
                perm, blk, NT, preferred_element_type=F32).astype(BF16), U32)
        else:
            v = jnp.dot(perm, wo[_rows(g, 128), :], preferred_element_type=F32)
            wot[g] = pltpu.bitcast(v.T.astype(BF16), U32)

    def xwords(i):
        for c in range(NB):
            io[c, _rows(i, 128), :] = pltpu.bitcast(xio[_rows(i, 256), c * 128:(c + 1) * 128], U32)

    def xin(j):
        for c in range(NB):
            xs[2 * j, _rows(c, 128), :], xs[2 * j + 1, _rows(c, 128), :] = halves(io[c, pl.ds(j, R1, stride=8), :].T)

    def norm(n0):
        def mean(v):
            acc = [v[8 * i:8 * i + 8] for i in range(4)]
            for i in range(4, D // 8):
                acc[i % 4] = acc[i % 4] + v[8 * i:8 * i + 8]
            return jnp.sum(_tree(jnp.add, acc), axis=0, keepdims=True) * (1.0 / D)

        def scale():
            un[n0] = ((xs[n0] - stat[0]) * lax.rsqrt(stat[1] + 1e-5)).astype(BF16)

        stat = []
        return (lambda: stat.append(mean(xs[n0])), lambda: stat.append(mean(jnp.square(xs[n0] - stat[0]))), scale)

    def proj(i, slot, m, t):
        p, g = i >> 2, i & 3
        r = jnp.dot(_bf(wt[g, _rows(t, 64), :]), un[2 * m + p], preferred_element_type=F32)
        (qs, ks, vs)[t][slot][m + 7 * (t > 0)] = r
        if t and m:
            (qs, ks, vs)[t][slot][m - 1] = pltpu.roll(r, 1, 1)

    def attn(i, slot, m0):
        p, g = i >> 2, i & 3
        first = lax.broadcasted_iota(jnp.int32, (8, 128), 1) == 0
        window = lambda ref, d: {e: ref[slot][e, 8 * d:8 * d + 8, :] for e in range(m0, m0 + W + 1)}
        s = {}

        def logits(d):
            k = window(ks, d)
            for m in (m0, m0 + 1):
                q = qs[slot][m, 8 * d:8 * d + 8, :]
                for w in range(W):
                    t = q * k[m + 7 - w]
                    s[m, w] = t if d == 0 else s[m, w] + t

        def softmax(m):
            t = [jnp.where(first, -1e9, s[m, w]) if w > m else s[m, w] for w in range(W)]
            mx = _tree(jnp.maximum, t)
            e = [jnp.exp(v - mx) for v in t]
            rs = 1.0 / _tree(jnp.add, e)
            s.update({(m, w): e[w] * rs for w in range(W)})

        def values(d):
            v = window(vs, d)
            for m in (m0, m0 + 1):
                s[m, W + d % 2] = _tree(jnp.add, [s[m, w] * v[m + 7 - w] for w in range(W)])
                if d % 2:
                    ob[2 * m + p, g, 8 * d - 8:8 * d + 8, :] = jnp.concatenate(
                        [s[m, W], s[m, W + 1]], 0).astype(BF16)

        return ([step(logits, d) for d in range(DH)] + [step(softmax, m0), step(softmax, m0 + 1)]
                + [step(values, d) for d in range(DH)])

    wo_rows = lambda rows: jnp.concatenate([_bf(wot[g, rows, :]) for g in range(4)], 1)

    def oproj(n0, r):
        rows = _rows(r, MR[oproj])
        xs[n0, rows, :] = xs[n0, rows, :] + jnp.dot(
            wo_rows(_rows(r, MR[oproj] // 2)), ob[n0].reshape(D, R1), preferred_element_type=F32)

    def xout(c, j):
        r = jnp.dot(wo_rows(slice(c * 64, (c + 1) * 64)), ob[2 * j + 1].reshape(D, R1),
                    preferred_element_type=F32)
        lo = xs[2 * j, _rows(c, 128), :].astype(BF16).astype(F32)
        hi = (xs[2 * j + 1, _rows(c, 128), :] + r).astype(BF16).astype(F32)
        io[c, pl.ds(j, R1, stride=8), :] = ((pltpu.bitcast(lo, U32) >> 16) | pltpu.bitcast(hi, U32)).T

    MR = {fwd: 256, inv: 256, oproj: 128}
    four = lambda fn, *aa: [step(fn, a + 4 * m, r) for a in aa for m in range(4) for r in range(D // MR[fn])]
    rowwise = lambda fn, a, n: [step(fn, a, i) for i in range(D // n)]

    regions, zero = [], zero_ref[0]

    def slot(*streams):
        regions.append(None)
        pl.when(zero < len(regions))(lambda: _run(*streams))

    norms = lambda *aa: [f for a in aa for stage in zip(*[norm(a + 4 * m) for m in range(4)]) for f in stage]
    pres = lambda a: rowwise(pre, a, 8)
    posts = lambda a: rowwise(post, a, 16)
    projs = lambda i, s, ms: [step(proj, i, s, m, t) for m in ms for t in range(3)]
    attns = lambda i, s: [f for m in range(0, 8, 2) for f in attn(i, s, m)]

    with jax.named_scope("kgen"):
        ng = D // 16 // KPER
        each = lambda fn: (lambda i: [fn(KPER * i + k, k) for k in range(KPER)])
        _pipeline([(each(kgen), 2, ng), (each(lagsums), 1, ng), (each(lambda i, k: setup(i)), 0, ng),
                   (xwords, ng - 8, 8)], {ng - 8: loads[0].wait})
    with jax.named_scope("kfwd"):
        loads[1].wait()
        lax.fori_loop(0, 4, lambda i, c: ([(kfwd(2 * i + k, 0), xin(2 * i + k), kfwd(2 * i + k, 1)) for k in range(2)], c)[-1], 0)
        slot([step(kfwd, n0, r) for n0 in range(8, R0) for r in range(2)], norms(2, 1, 3, 0))
        for c in loads[2:]:
            c.wait()

        def spectrum(g, c):
            _run([step(wprep, g, k) for k in range(4)] + [step(fwd, 2 + 4 * g, r) for r in range(D // MR[fwd])],
                 [step(kdft, 16 * g + i) for i in range(16)])
            return c

        lax.fori_loop(0, 4, spectrum, 0)
        slot(four(fwd, 1), pres(2))

    def layer(li, carry):
        with jax.named_scope("conv"):
            slot(four(fwd, 3), pres(1))
            slot(four(fwd, 0), pres(3))
            lax.fori_loop(0, D // 16, lambda i, c: (mid(i), c)[-1], 0)
            slot(four(inv, 0), posts(2))
            slot(four(inv, 2), norms(0))
            slot(projs(0, 0, range(0, 8, 2)), norms(2) + posts(1))
            slot(four(inv, 1), posts(3))
            slot(four(inv, 3), norms(1))
            slot(projs(0, 0, range(1, 8, 2)), norms(3))
        with jax.named_scope("attn"):
            both = lambda i, s: slot(projs(i + 1, 1 - s, range(8)), attns(i, s))
            lax.fori_loop(0, 3, lambda j, c: (both(2 * j, 0), both(2 * j + 1, 1), c)[-1], 0)
            both(6, 0)
            slot(four(oproj, 2, 0), attns(7, 1))

        @pl.when(li == 0)
        def _():
            slot(four(oproj, 1), norms(2, 0))
            slot(four(fwd, 2), norms(1))
            slot(four(oproj, 3), pres(2))
            slot(four(fwd, 1), norms(3))

        return carry

    lax.fori_loop(0, 2, layer, 0)

    with jax.named_scope("xout"):
        stores = []
        for c in range(NB):
            for j in range(8):
                xout(c, j)
            cols = pl.ds(c * 128, 128)
            xio[:, cols] = _bf(io[c])
            stores.append(pltpu.make_async_copy(xio.at[:, cols], out_hbm.at[:, cols], sems.at[c]))
            stores[-1].start()
        for c in stores:
            c.wait()


@jax.jit
def pallas_interleave_layers__ssm_conv_s4__sliding_local_dilated__prompt_kernel(
    A_u: jax.Array,
    A_A_re: jax.Array,
    A_A_im: jax.Array,
    A_B_re: jax.Array,
    A_B_im: jax.Array,
    A_C_re: jax.Array,
    A_C_im: jax.Array,
    A_log_dt: jax.Array,
    A_Dskip: jax.Array,
    B_x: jax.Array,
    B_wqkv: jax.Array,
    B_wo: jax.Array,
):
    del B_x
    hbm, vmem = pl.BlockSpec(memory_space=pl.ANY), pl.BlockSpec(memory_space=pltpu.VMEM)
    tiles = lambda *n: pltpu.VMEM((*n, 128, 128), F32)
    out = pl.pallas_call(
        _kernel,
        out_shape=jax.ShapeDtypeStruct((L, D), BF16),
        in_specs=[pl.BlockSpec(memory_space=pltpu.SMEM), hbm] + [vmem] * 8 + [hbm] * 4,
        out_specs=hbm,
        scratch_shapes=[
            pltpu.VMEM((R0, D, R1), F32),
            *[pltpu.VMEM((R0, 2, D, R1), F32)] * 4,
            pltpu.VMEM((R0, 2, D, R1), BF16),
            pltpu.VMEM((2, D, N), F32),
            pltpu.VMEM((D // 16, 4, 16, N), F32),
            pltpu.VMEM((KPER, 336, 128), U32),
            *[tiles(n) for n in (8, 15, 15) * 2],
            pltpu.VMEM((L, D), BF16),
            pltpu.VMEM((NB, L // 2, 128), U32),
            pltpu.VMEM((12, D, 128), BF16),
            pltpu.VMEM((D, D), BF16),
            pltpu.VMEM(_F.shape, U32),
            pltpu.VMEM(_G.shape, U32),
            pltpu.VMEM((R0, D // 2, R1), U32),
            pltpu.VMEM((R0, D, R1), BF16),
            pltpu.VMEM((4, 192, D), U32),
            pltpu.VMEM((4, D // 2, 128), U32),
            pltpu.VMEM((R0, 4, 128, R1), BF16),
            pltpu.SemaphoreType.DMA((16,)),
        ],
        compiler_params=pltpu.CompilerParams(vmem_limit_bytes=100 * 1024 * 1024),
    )(np.zeros((2,), np.int32), A_u.reshape(L, D), A_A_re, A_A_im, A_B_re, A_B_im, A_C_re, A_C_im, A_log_dt, A_Dskip,
      B_wqkv, B_wo, _F, _G)
    return out.reshape(1, L, D)
```

```python
import jax
import jax.numpy as jnp
import ml_dtypes
import numpy as np
from jax import lax
import jax.experimental.pallas as pl
import jax.experimental.pallas.tpu as pltpu

L, D, N = 2048, 512, 128
R0, R1 = 16, 128
W, DH = 8, 16
F32, BF16, U32 = jnp.float32, jnp.bfloat16, jnp.uint32
CUT = (0, 20, 42)
KPER = 4
NB = D // 128
NT = (((1,), (1,)), ((), ()))


def _constants():
    n0 = np.arange(R0)[:, None, None]
    n1 = np.arange(R1)[None, :, None]
    k1 = np.arange(R1)[None, None, :]
    ang = 2.0 * np.pi * (k1 + 0.25) * (R0 * n1 + n0) / L
    f = np.concatenate([np.cos(ang), np.sin(ang)], axis=2)
    g = f.transpose(0, 2, 1)
    bf = ml_dtypes.bfloat16
    lr = np.arange(L).astype(np.float32).astype(bf).astype(np.int64).reshape(8, 16, R0)
    r = lr - (256 * np.arange(8)[:, None, None] + 16 * np.arange(16)[None, :, None])
    assert (r == r[:, :1, :]).all()

    def words(m):
        h = np.ascontiguousarray(m).astype(bf).view(np.uint16).astype(np.uint32)
        return h[:, 0::2] | (h[:, 1::2] << 16)

    return words(f), words(g), r[:, 0, :].tolist()


_F, _G, _RND = _constants()


def _cmul(a, b):
    return a[0] * b[0] - a[1] * b[1], a[0] * b[1] + a[1] * b[0]


def _csq(a):
    t = a[0] * a[1]
    return (a[0] + a[1]) * (a[0] - a[1]), t + t


def _dft4(x, sign):
    (ar, ai), (br, bi), (cr, ci), (dr, di) = x
    sr, si, tr, ti = ar + cr, ai + ci, ar - cr, ai - ci
    ur, ui, vr, vi = br + dr, bi + di, br - dr, bi - di
    p, m = (tr - vi, ti + vr), (tr + vi, ti - vr)
    if sign < 0:
        p, m = m, p
    return [(sr + ur, si + ui), p, (sr - ur, si - ui), m]


def _twiddle(v, e):
    e %= 16
    re, im = v
    h = float(np.sqrt(0.5))
    if e == 0:
        return v
    if e == 4:
        return -im, re
    if e == 12:
        return im, -re
    if e == 2:
        return (re - im) * h, (re + im) * h
    if e == 14:
        return (re + im) * h, (im - re) * h
    if e == 6:
        return (re + im) * -h, (re - im) * h
    if e == 10:
        return (im - re) * h, (re + im) * -h
    c, s = float(np.cos(np.pi * e / 8)), float(np.sin(np.pi * e / 8))
    return re * c - im * s, re * s + im * c


def _bf(x):
    return pltpu.bitcast(x, BF16)


def _tree(op, v):
    while len(v) > 1:
        v = [op(v[i], v[i + 1]) if i + 1 < len(v) else v[i] for i in range(0, len(v), 2)]
    return v[0]


def _run(*streams):
    order = sorted(((i + 0.5 * (k > 0)) / len(s), k, i) for k, s in enumerate(streams) for i in range(len(s)))
    for _, k, i in order:
        streams[k][i]()


def _pipeline(streams, hooks=None):
    hooks = hooks or {}
    cuts = sorted({e for _, a, n in streams for e in (a, a + n)} | set(hooks))
    for lo, hi in zip(cuts, cuts[1:]):
        def body(s, carry, lo=lo):
            _run(*[fn(s - a) for fn, a, n in streams if a <= lo < a + n])
            return carry

        if lo in hooks:
            hooks[lo]()
        if hi - lo == 1:
            body(lo, 0)
        else:
            lax.fori_loop(lo, hi, body, 0)


def _rows(i, n):
    return pl.ds(i * n if isinstance(i, int) else pl.multiple_of(i * n, n), n)


def _kernel(zero_ref, x_hbm, are_ref, aim_ref, bre_ref, bim_ref, cre_ref, cim_ref, ldt_ref, dsk_ref,
            wqkv_hbm, wo_hbm, f_hbm, g_hbm, out_hbm,
            xs, kf, ua, ub, uc, yb, par, zw, lag, qa, ka, va, qb, kb, vb, io, perm, wqkv, wo, fm, gm, kt, un, wt, us, wot, ob, sems):
    step = lambda fn, *a: (lambda: fn(*a))
    qs, ks, vs = (qa, qb), (ka, kb), (va, vb)
    loads = [pltpu.make_async_copy(s, d, sems.at[i]) for i, (s, d) in enumerate(
        (*((x_hbm.bitcast(U32).at[:, pl.ds(128 * c, 128)], io.at[c]) for c in range(NB)),
         (f_hbm, fm), (wo_hbm, wo), (g_hbm, gm),
         *((wqkv_hbm.at[:, pl.ds(128 * j, 128)], wqkv.at[j]) for j in range(12))))]
    for c in loads:
        c.start()
    high = jnp.uint32(0xFFFF0000)
    halves = lambda t: (pltpu.bitcast(t << 16, F32), pltpu.bitcast(t & high, F32))

    def col(ref):
        v = ref[...].astype(F32).reshape(1, D)
        return jnp.broadcast_to(v, (128, D)).T

    par[0] = jnp.exp(col(ldt_ref))
    par[1] = col(dsk_ref) * (1.0 / L)

    ri = lax.broadcasted_iota(jnp.int32, (128, 128), 0)
    ci = lax.broadcasted_iota(jnp.int32, (128, 128), 1)
    perm[...] = pltpu.bitcast(jnp.where(ci == (ri & 7) * DH + (ri >> 3), 1.0, 0.0).astype(BF16), U32)

    def setup(i):
        get = lambda ref: halves(pltpu.bitcast(ref[_rows(i, 16), :], U32))
        dt = halves(pltpu.bitcast(par[0, _rows(i, 16), :].astype(BF16), U32))

        def pole(h):
            mag, ang = jnp.exp(dt[h] * get(are_ref)[h]), dt[h] * get(aim_ref)[h]
            zw[i, h, 0], zw[i, h, 1] = mag * jnp.cos(ang), mag * jnp.sin(ang)

        def weight():
            scale = (1.0 + 1.5 * 2.0 ** -9) / L
            for h, (cr, ci, br, bi) in enumerate(zip(*map(get, (cre_ref, cim_ref, bre_ref, bim_ref)))):
                wr, wi = _cmul((cr, ci), (dt[h] * br, dt[h] * bi))
                zw[i, h, 2], zw[i, h, 3] = wr * scale, wi * -scale

        return [step(pole, 0), weight, step(pole, 1)]

    lags = sorted({(c, r) for c in range(8) for r in _RND[c] if r < 16}) + [(8, 0)]
    stack = lambda vs: jnp.concatenate([jnp.concatenate([v[k] for v in vs], 0) for k in range(2)], 1).astype(BF16)

    def lagsums(i):
        start = [[zw[i, h, c] for c in range(4)] for h in range(2)]
        zs, rhs, even = [], [], []

        def right(h):
            zr, zi, wr, wi = start[h]
            z = {0: (jnp.ones((8, N), F32), jnp.zeros((8, N), F32)), 1: (zr, zi)}
            for e in (2, 4, 8, 16, 32, 64, 128, 256):
                z[e] = _csq(z[e // 2])
            b = [(wr, wi)]
            for e in (16, 32, 64, 128):
                zc = (z[e][0], -z[e][1])
                b += [_cmul(v, zc) for v in b]
            zs.append(z)
            rhs.append(stack(b))

        def left(t, h):
            z = zs[h]

            def power(e):
                if e not in z:
                    low = e % 256 if e > 256 and e % 256 else e & -e
                    z[e] = _csq(z[e // 2]) if e // 2 in z and e % 2 == 0 else _cmul(power(e - low), power(low))
                return z[e]

            a = [power(256 * c + r) for c, r in (lags + lags[-1:])[CUT[t]:CUT[t + 1]]]
            o = pltpu.bitcast(lax.dot_general(stack(a), rhs[h], NT, preferred_element_type=F32), U32)
            if h:
                lag[i, 8 * CUT[t]:8 * CUT[t + 1], :] = even[t] | (o & high)
            else:
                even.append(o >> 16)

        return [f for h in range(2) for f in [step(right, h)] + [step(left, t, h) for t in range(len(CUT) - 1)]]

    def kgen(i):
        lane = lax.broadcasted_iota(jnp.int32, (8, 128), 1)
        src = (lane & 15) * 8 + lax.broadcasted_iota(jnp.int32, (8, 128), 0)

        memo = {}

        def piece(c, r):
            if r == 16:
                c = 0
            if (c, r) not in memo:
                memo[c, r] = (
                    pltpu.roll(jnp.where(lane == 0, piece(8, 0), merged(0, (0,) * 8)), 127, 1) if r == 16 else
                    jnp.take_along_axis(lag[i, _rows(lags.index((c, r)), 8), :], src, axis=1,
                                        mode="promise_in_bounds"))
            return memo[c, r]

        def merged(c, rs):
            if (c, rs) not in memo:
                memo[c, rs] = (piece(c, rs[0]) if c == 7 or min(rs) == 16 else
                               jnp.where(lane >> 4 == c, piece(c, rs[0]), merged(c + 1, rs[1:])))
            return memo[c, rs]

        for n0 in range(R0):
            kt[n0, _rows(i, 8), :] = merged(0, tuple(_RND[c][n0] for c in range(8)))

    get = lambda ref, n, rows: (ref[n, 0, rows, :], ref[n, 1, rows, :])

    def put(ref, n, rows, v):
        ref[n, 0, rows, :], ref[n, 1, rows, :] = v

    def outer(src, a, rows):
        return [_twiddle(v, a * b) for b, v in enumerate(_dft4([get(src, a + 4 * m, rows) for m in range(4)], 1))]

    def transform(lhs, dst, n0, rows):
        r = jnp.dot(lhs, _bf(fm[n0]), preferred_element_type=F32)
        put(dst, n0, rows, (r[:, :128], r[:, 128:]))

    def kfwd(n0, r):
        transform(_bf(kt[n0, _rows(r, 64), :]), ub, n0, _rows(r, 128))

    def kdft(i):
        rows, t = _rows(i, 8), []

        def inner(b):
            for m, v in enumerate(_dft4([t[a][b] for a in range(4)], 1)):
                put(kf, b + 4 * m, rows, (v[0] + par[1, rows, :], v[1]))

        return [lambda a=a: t.append(outer(ub, a, rows)) for a in range(4)] + [step(inner, b) for b in range(4)]

    def fwd(n0, r):
        transform(un[n0, _rows(r, 128), :], ua, n0, _rows(r, 128))

    def pre(a, i):
        for b, v in enumerate(outer(ua, a, _rows(i, 8))):
            put(ub, a + 4 * b, _rows(i, 8), v)

    def mid(i):
        out = []
        for rows in (_rows(2 * i, 8), _rows(2 * i + 1, 8)):
            t = []
            for b, v in enumerate(outer(ua, 0, rows)):
                x = _dft4([v] + [get(ub, a + 4 * b, rows) for a in range(1, 4)], 1)
                y = _dft4([_cmul(x[m], get(kf, b + 4 * m, rows)) for m in range(4)], -1)
                t.append(y[0])
                for a in range(1, 4):
                    put(uc, a + 4 * b, rows, y[a])
            out.append(_dft4(t, -1))
        for m, (v, w) in enumerate(zip(*out)):
            put(yb, 4 * m, _rows(i, 16), [jnp.concatenate([v[k], w[k]], 0).astype(BF16) for k in range(2)])

    def post(a, i):
        rows = _rows(i, 16)
        for m, v in enumerate(_dft4([_twiddle(get(uc, a + 4 * b, rows), -a * b) for b in range(4)], -1)):
            put(yb, a + 4 * m, rows, (v[0].astype(BF16), v[1].astype(BF16)))

    def inv(n0, r):
        rows = _rows(r, 128)
        y = jnp.concatenate(get(yb, n0, rows), 1)
        xs[n0, rows, :] = xs[n0, rows, :] + jnp.dot(y, _bf(gm[n0]), preferred_element_type=F32)

    def wprep(g, t):
        if t < 3:
            v = lax.dot_general(_bf(perm[...]), wqkv[4 * t + g], NT, preferred_element_type=F32)
            v = v if t else v * DH ** -0.5
            a11, a12, a21, a22 = v[:64, :256], v[:64, 256:], v[64:, :256], v[64:, 256:]
            for k, a in enumerate((a11 + a22, a21 + a22, a11, a22, a11 + a12, a21 - a11, a12 - a22)):
                wt[g, k, _rows(t, 32), :] = pltpu.bitcast(a.astype(BF16), U32)
        else:
            v = jnp.dot(_bf(perm[...]), wo[_rows(g, 128), :], preferred_element_type=F32)
            wot[g] = pltpu.bitcast(v.T.astype(BF16), U32)

    def xin(j, c):
        xs[2 * j, _rows(c, 128), :], xs[2 * j + 1, _rows(c, 128), :] = halves(io[c, pl.ds(j, R1, stride=8), :].T)

    def norm(n0):
        acc, stat = {}, []

        def moment(k, c):
            for i in range(16 * c, 16 * c + 16):
                v = xs[n0, 8 * i:8 * i + 8, :]
                v = jnp.square(v - stat[0]) if k else v
                acc[i % 4] = v if i < 4 else acc[i % 4] + v
            if c == 3:
                v = jnp.sum(_tree(jnp.add, list(acc.values())), axis=0, keepdims=True) * (1.0 / D)
                stat.append(lax.rsqrt(v + 1e-5) if k else v)

        def scale(c):
            rows = _rows(c, 128)
            un[n0, rows, :] = get(rows).astype(BF16)

        get = lambda rows: (xs[n0, rows, :] - stat[0]) * stat[1]
        return [[step(fn, *k, c) for c in range(4)] for fn, *k in ((moment, 0), (moment, 1), (scale,))], get

    def norms(*aa):
        return [f for a in aa for stage in zip(*[norm(a + 4 * m)[0] for m in range(4)])
                for steps in stage for f in steps]

    def pair_norms(a):
        stages, get = zip(*[norm(a + 4 * m) for m in range(4)])

        def operands(j, c):
            (b11, b21), (b12, b22) = ((f(_rows(c, 32)), f(_rows(c + 8, 32))) for f in get[2 * j:2 * j + 2])
            for k, b in enumerate((b11 + b22, b11, b12 - b22, b21 - b11, b22, b11 + b12, b21 + b22)):
                us[2 * a + j, k, _rows(c, 32), :] = b.astype(BF16)

        return ([f for k in range(2) for st in stages for f in st[k]]
                + [step(operands, j, c) for j in range(2) for c in range(8)])

    def proj(i, slot, m):
        p, g = i >> 2, i & 3
        c = {}

        def product(k):
            return jnp.dot(_bf(wt[g, k - 1]), us[2 * p + 4 * (m & 1) + (m >> 2), k - 1],
                           preferred_element_type=F32)

        def emit(half, mm, r):
            for t, ref in enumerate((qs[slot], ks[slot], vs[slot])):
                ref[mm + 7 * (t > 0), _rows(half, 64), :] = r[64 * t:64 * t + 64]
                if t and mm:
                    ref[mm - 1, _rows(half, 64), :] = pltpu.roll(r[64 * t:64 * t + 64], 1, 1)

        def run(k):
            c[k] = r = product(k)
            if k == 4:
                emit(1, m, c[2] + r)
            elif k == 1:
                c[11], c[22] = r + c[4], r - c[2]
            elif k == 7:
                c[11] = c[11] + r
            elif k == 5:
                emit(0, m, c[11] - r)
            elif k == 3:
                emit(0, m + 2, c[5] + r)
                c[22] = c[22] + r
            elif k == 6:
                emit(1, m + 2, c[22] + r)

        return [step(run, k) for k in (2, 4, 1, 7, 5, 3, 6)]

    def attn(i, slot, m0):
        p, g = i >> 2, i & 3
        first = lax.broadcasted_iota(jnp.int32, (8, 128), 1) == 0
        window = lambda ref, d: {e: ref[slot][e, 8 * d:8 * d + 8, :] for e in range(m0, m0 + W + 1)}
        s = {}

        def logits(d):
            k = window(ks, d)
            for m in (m0, m0 + 1):
                q = qs[slot][m, 8 * d:8 * d + 8, :]
                for w in range(W):
                    t = q * k[m + 7 - w]
                    s[m, w] = t if d == 0 else s[m, w] + t

        def softmax(m):
            t = [jnp.where(first, -1e9, s[m, w]) if w > m else s[m, w] for w in range(W)]
            mx = _tree(jnp.maximum, t)
            e = [jnp.exp(v - mx) for v in t]
            rs = 1.0 / _tree(jnp.add, e)
            s.update({(m, w): e[w] * rs for w in range(W)})

        def values(d):
            v = window(vs, d)
            for m in (m0, m0 + 1):
                s[m, W + d % 2] = _tree(jnp.add, [s[m, w] * v[m + 7 - w] for w in range(W)])
                if d % 2:
                    ob[2 * m + p, g, 8 * d - 8:8 * d + 8, :] = jnp.concatenate(
                        [s[m, W], s[m, W + 1]], 0).astype(BF16)

        return ([step(logits, d) for d in range(DH)] + [step(softmax, m0), step(softmax, m0 + 1)]
                + [step(values, d) for d in range(DH)])

    wo_rows = lambda rows: jnp.concatenate([_bf(wot[g, rows, :]) for g in range(4)], 1)

    def oproj(n0, r):
        rows = _rows(r, 128)
        xs[n0, rows, :] = xs[n0, rows, :] + jnp.dot(
            wo_rows(_rows(r, 64)), ob[n0].reshape(D, R1), preferred_element_type=F32)

    def xout(c, j):
        lo, hi = (pltpu.bitcast(xs[2 * j + k, _rows(c, 128), :].astype(BF16).astype(F32), U32) for k in range(2))
        io[c, pl.ds(j, R1, stride=8), :] = ((lo >> 16) | hi).T

    four = lambda fn, *aa: [step(fn, a + 4 * m, r) for a in aa for m in range(4) for r in range(NB)]
    rowwise = lambda fn, a, n: [step(fn, a, i) for i in range(D // n)]

    regions, zero = [], zero_ref[0]

    def slot(*streams):
        regions.append(None)
        pl.when(zero < len(regions))(lambda: _run(*streams))

    pres = lambda a: rowwise(pre, a, 8)
    posts = lambda a: rowwise(post, a, 16)
    projs = lambda i, s, ms: [f for m in ms for f in proj(i, s, m)]
    attns = lambda i, s: [f for m in range(0, 8, 2) for f in attn(i, s, m)]

    with jax.named_scope("kgen"):
        ng = D // 16 // KPER
        each = lambda fn: (lambda i: [f for k in range(KPER) for f in fn(KPER * i + k)])
        _pipeline([(lambda i: [lambda: [kgen(KPER * i + k) for k in range(KPER)]], 2, ng),
                   (each(lagsums), 1, ng), (each(setup), 0, ng),
                   (lambda j: [step(xin, j * KPER // 2 + k, c) for k in range(KPER // 2) for c in range(NB)],
                    ng // 2, ng // 2)],
                  {ng // 2: lambda: [c.wait() for c in loads[:NB]]})
    with jax.named_scope("kfwd"):
        for c in loads[NB:]:
            c.wait()
        kdfts = lambda r: [f for i in range(16) for f in kdft(16 * r + i)]
        for r, other in enumerate((norms(2, 1), norms(3), norms(0), [])):
            slot([f for k in range(4) for f in [step(wprep, r, k)] + [step(kfwd, 4 * k + n, r) for n in range(4)]],
                 kdfts(r - 1) if r else [], other)
        slot(four(fwd, 2), kdfts(NB - 1))
        slot(four(fwd, 1), pres(2))

    def layer(li, carry):
        with jax.named_scope("conv"):
            slot(four(fwd, 3), pres(1))
            slot(four(fwd, 0), pres(3))
            lax.fori_loop(0, D // 16, lambda i, c: (mid(i), c)[-1], 0)
            slot(four(inv, 0), posts(2))
            slot(four(inv, 2), pair_norms(0))
            slot(projs(0, 0, (0, 4)), pair_norms(2) + posts(1))
            slot(four(inv, 1), posts(3))
            slot(four(inv, 3), pair_norms(1))
            slot(projs(0, 0, (1, 5)), pair_norms(3))
        with jax.named_scope("attn"):
            both = lambda i, s: slot(projs(i + 1, 1 - s, (0, 1, 4, 5)), attns(i, s))
            lax.fori_loop(0, 3, lambda j, c: (both(2 * j, 0), both(2 * j + 1, 1), c)[-1], 0)
            both(6, 0)
            slot(four(oproj, 2, 0), attns(7, 1))

        @pl.when(li == 0)
        def _():
            slot(four(oproj, 1), norms(2, 0))
            slot(four(fwd, 2), norms(1))
            slot(four(oproj, 3), pres(2))
            slot(four(fwd, 1), norms(3))

        return carry

    lax.fori_loop(0, 2, layer, 0)

    with jax.named_scope("xout"):
        stores = [pltpu.make_async_copy(io.at[c], out_hbm.bitcast(U32).at[:, pl.ds(c * 128, 128)], sems.at[c])
                  for c in range(NB)]
        for c in range(NB + 1):
            slot([step(oproj, 2 * j + 1, c) for j in range(8)] if c < NB else [],
                 [step(xout, c - 1, j) for j in range(8)] if c else [])
            if c:
                stores[c - 1].start()
        for c in stores:
            c.wait()


@jax.jit
def pallas_interleave_layers__ssm_conv_s4__sliding_local_dilated__prompt_kernel(
    A_u: jax.Array,
    A_A_re: jax.Array,
    A_A_im: jax.Array,
    A_B_re: jax.Array,
    A_B_im: jax.Array,
    A_C_re: jax.Array,
    A_C_im: jax.Array,
    A_log_dt: jax.Array,
    A_Dskip: jax.Array,
    B_x: jax.Array,
    B_wqkv: jax.Array,
    B_wo: jax.Array,
):
    del B_x
    hbm, vmem = pl.BlockSpec(memory_space=pl.ANY), pl.BlockSpec(memory_space=pltpu.VMEM)
    tiles = lambda *n: pltpu.VMEM((*n, 128, 128), F32)
    out = pl.pallas_call(
        _kernel,
        out_shape=jax.ShapeDtypeStruct((L, D), BF16),
        in_specs=[pl.BlockSpec(memory_space=pltpu.SMEM), hbm] + [vmem] * 8 + [hbm] * 4,
        out_specs=hbm,
        scratch_shapes=[
            pltpu.VMEM((R0, D, R1), F32),
            *[pltpu.VMEM((R0, 2, D, R1), F32)] * 4,
            pltpu.VMEM((R0, 2, D, R1), BF16),
            pltpu.VMEM((2, D, N), F32),
            pltpu.VMEM((D // 16, 2, 4, 8, N), F32),
            pltpu.VMEM((D // 16, 336, 128), U32),
            *[tiles(n) for n in (8, 15, 15) * 2],
            pltpu.VMEM((NB, L // 2, 128), U32),
            pltpu.VMEM((64, 128), U32),
            pltpu.VMEM((12, D, 128), BF16),
            pltpu.VMEM((D, D), BF16),
            pltpu.VMEM(_F.shape, U32),
            pltpu.VMEM(_G.shape, U32),
            pltpu.VMEM((R0, D // 2, R1), U32),
            pltpu.VMEM((R0, D, R1), BF16),
            pltpu.VMEM((4, 7, 96, D // 2), U32),
            pltpu.VMEM((8, 7, D // 2, R1), BF16),
            pltpu.VMEM((4, D // 2, 128), U32),
            pltpu.VMEM((R0, 4, 128, R1), BF16),
            pltpu.SemaphoreType.DMA((19,)),
        ],
        compiler_params=pltpu.CompilerParams(vmem_limit_bytes=100 * 1024 * 1024),
    )(np.zeros((2,), np.int32), A_u.reshape(L, D), A_A_re, A_A_im, A_B_re, A_B_im, A_C_re, A_C_im, A_log_dt, A_Dskip,
      B_wqkv, B_wo, _F, _G)
    return out.reshape(1, L, D)
```

```python
import jax
import jax.numpy as jnp
import ml_dtypes
import numpy as np
from jax import lax
import jax.experimental.pallas as pl
import jax.experimental.pallas.tpu as pltpu

L, D, N = 2048, 512, 128
R0, R1 = 16, 128
W, DH = 8, 16
F32, BF16, U32 = jnp.float32, jnp.bfloat16, jnp.uint32
CUT = (0, 20, 42)
KPER = 4
NB = D // 128
NT = (((1,), (1,)), ((), ()))


def _constants():
    n0 = np.arange(R0)[:, None, None]
    n1 = np.arange(R1)[None, :, None]
    k1 = np.arange(R1)[None, None, :]
    ang = 2.0 * np.pi * (k1 + 0.25) * (R0 * n1 + n0) / L
    f = np.concatenate([np.cos(ang), np.sin(ang)], axis=2)
    g = f.transpose(0, 2, 1)
    bf = ml_dtypes.bfloat16
    lr = np.arange(L).astype(np.float32).astype(bf).astype(np.int64).reshape(8, 16, R0)
    r = lr - (256 * np.arange(8)[:, None, None] + 16 * np.arange(16)[None, :, None])
    assert (r == r[:, :1, :]).all()

    def words(m):
        h = np.ascontiguousarray(m).astype(bf).view(np.uint16).astype(np.uint32)
        return h[:, 0::2] | (h[:, 1::2] << 16)

    return words(f), words(g), r[:, 0, :].tolist()


_F, _G, _RND = _constants()


def _cmul(a, b):
    return a[0] * b[0] - a[1] * b[1], a[0] * b[1] + a[1] * b[0]


def _csq(a):
    t = a[0] * a[1]
    return (a[0] + a[1]) * (a[0] - a[1]), t + t


def _dft4(x, sign):
    (ar, ai), (br, bi), (cr, ci), (dr, di) = x
    sr, si, tr, ti = ar + cr, ai + ci, ar - cr, ai - ci
    ur, ui, vr, vi = br + dr, bi + di, br - dr, bi - di
    p, m = (tr - vi, ti + vr), (tr + vi, ti - vr)
    if sign < 0:
        p, m = m, p
    return [(sr + ur, si + ui), p, (sr - ur, si - ui), m]


def _twiddle(v, e):
    e %= 16
    re, im = v
    h = float(np.sqrt(0.5))
    if e == 0:
        return v
    if e == 4:
        return -im, re
    if e == 12:
        return im, -re
    if e == 2:
        return (re - im) * h, (re + im) * h
    if e == 14:
        return (re + im) * h, (im - re) * h
    if e == 6:
        return (re + im) * -h, (re - im) * h
    if e == 10:
        return (im - re) * h, (re + im) * -h
    c, s = float(np.cos(np.pi * e / 8)), float(np.sin(np.pi * e / 8))
    return re * c - im * s, re * s + im * c


def _bf(x):
    return pltpu.bitcast(x, BF16)


def _tree(op, v):
    while len(v) > 1:
        v = [op(v[i], v[i + 1]) if i + 1 < len(v) else v[i] for i in range(0, len(v), 2)]
    return v[0]


def _run(*streams):
    order = sorted(((i + 0.5 * (k > 0)) / len(s), k, i) for k, s in enumerate(streams) for i in range(len(s)))
    for _, k, i in order:
        streams[k][i]()


def _pipeline(streams, hooks=None):
    hooks = hooks or {}
    cuts = sorted({e for _, a, n in streams for e in (a, a + n)} | set(hooks))
    for lo, hi in zip(cuts, cuts[1:]):
        def body(s, carry, lo=lo):
            _run(*[fn(s - a) for fn, a, n in streams if a <= lo < a + n])
            return carry

        if lo in hooks:
            hooks[lo]()
        if hi - lo == 1:
            body(lo, 0)
        else:
            lax.fori_loop(lo, hi, body, 0)


def _left(a11, a12, a21, a22):
    return a21 + a22, a22, a11 + a22, a12 - a22, a11 + a12, a11, a21 - a11


def _right(b11, b12, b21, b22):
    return b11, b21 - b11, b11 + b22, b21 + b22, b22, b12 - b22, b11 + b12


def _strassen(product, emit):
    c = {}

    def run(k):
        c[k] = r = product(k)
        if k == 1:
            emit(1, 0, c[0] + r)
        elif k == 2:
            c[11], c[22] = r + c[1], r - c[0]
        elif k == 3:
            c[11] = c[11] + r
        elif k == 4:
            emit(0, 0, c[11] - r)
        elif k == 5:
            emit(0, 1, c[4] + r)
            c[22] = c[22] + r
        elif k == 6:
            emit(1, 1, c[22] + r)

    return [lambda k=k: run(k) for k in range(7)]


def _rows(i, n):
    return pl.ds(i * n if isinstance(i, int) else pl.multiple_of(i * n, n), n)


def _kernel(zero_ref, x_hbm, are_ref, aim_ref, bre_ref, bim_ref, cre_ref, cim_ref, ldt_ref, dsk_ref,
            wqkv_hbm, wo_hbm, f_hbm, g_hbm, out_hbm,
            xs, kf, ua, ub, uc, yb, par, zw, lag, qa, ka, va, qb, kb, vb, io, perm, wqkv, wo, fm, gm, kt, un, wt, us, wot, ob, sems):
    step = lambda fn, *a: (lambda: fn(*a))
    qs, ks, vs = (qa, qb), (ka, kb), (va, vb)
    loads = [pltpu.make_async_copy(s, d, sems.at[i]) for i, (s, d) in enumerate(
        (*((x_hbm.bitcast(U32).at[:, pl.ds(128 * c, 128)], io.at[c]) for c in range(NB)),
         (f_hbm, fm), (wo_hbm, wo), (g_hbm, gm),
         *((wqkv_hbm.at[:, pl.ds(128 * j, 128)], wqkv.at[j]) for j in range(12))))]
    for c in loads:
        c.start()
    high = jnp.uint32(0xFFFF0000)
    halves = lambda t: (pltpu.bitcast(t << 16, F32), pltpu.bitcast(t & high, F32))

    def col(ref):
        v = ref[...].astype(F32).reshape(1, D)
        return jnp.broadcast_to(v, (128, D)).T

    par[0] = jnp.exp(col(ldt_ref))
    par[1] = col(dsk_ref) * (1.0 / L)

    ri = lax.broadcasted_iota(jnp.int32, (128, 128), 0)
    ci = lax.broadcasted_iota(jnp.int32, (128, 128), 1)
    perm[...] = pltpu.bitcast(jnp.where(ci == (ri & 7) * DH + (ri >> 3), 1.0, 0.0).astype(BF16), U32)

    def setup(i):
        get = lambda ref: halves(pltpu.bitcast(ref[_rows(i, 16), :], U32))
        dt = halves(pltpu.bitcast(par[0, _rows(i, 16), :].astype(BF16), U32))

        def pole(h):
            mag, ang = jnp.exp(dt[h] * get(are_ref)[h]), dt[h] * get(aim_ref)[h]
            zw[i, h, 0], zw[i, h, 1] = mag * jnp.cos(ang), mag * jnp.sin(ang)

        def weight():
            scale = (1.0 + 1.5 * 2.0 ** -9) / L
            for h, (cr, ci, br, bi) in enumerate(zip(*map(get, (cre_ref, cim_ref, bre_ref, bim_ref)))):
                wr, wi = _cmul((cr, ci), (dt[h] * br, dt[h] * bi))
                zw[i, h, 2], zw[i, h, 3] = wr * scale, wi * -scale

        return [step(pole, 0), weight, step(pole, 1)]

    lags = sorted({(c, r) for c in range(8) for r in _RND[c] if r < 16}) + [(8, 0)]
    stack = lambda vs: jnp.concatenate([jnp.concatenate([v[k] for v in vs], 0) for k in range(2)], 1).astype(BF16)

    def lagsums(i):
        start = [[zw[i, h, c] for c in range(4)] for h in range(2)]
        zs, rhs, even = [], [], []

        def right(h):
            zr, zi, wr, wi = start[h]
            z = {0: (jnp.ones((8, N), F32), jnp.zeros((8, N), F32)), 1: (zr, zi)}
            for e in (2, 4, 8, 16, 32, 64, 128, 256):
                z[e] = _csq(z[e // 2])
            b = [(wr, wi)]
            for e in (16, 32, 64, 128):
                zc = (z[e][0], -z[e][1])
                b += [_cmul(v, zc) for v in b]
            zs.append(z)
            rhs.append(stack(b))

        def left(t, h):
            z = zs[h]

            def power(e):
                if e not in z:
                    low = e % 256 if e > 256 and e % 256 else e & -e
                    z[e] = _csq(z[e // 2]) if e // 2 in z and e % 2 == 0 else _cmul(power(e - low), power(low))
                return z[e]

            a = [power(256 * c + r) for c, r in (lags + lags[-1:])[CUT[t]:CUT[t + 1]]]
            o = pltpu.bitcast(lax.dot_general(stack(a), rhs[h], NT, preferred_element_type=F32), U32)
            if h:
                lag[i, 8 * CUT[t]:8 * CUT[t + 1], :] = even[t] | (o & high)
            else:
                even.append(o >> 16)

        return [f for h in range(2) for f in [step(right, h)] + [step(left, t, h) for t in range(len(CUT) - 1)]]

    def kgen(i):
        lane = lax.broadcasted_iota(jnp.int32, (8, 128), 1)
        src = (lane & 15) * 8 + lax.broadcasted_iota(jnp.int32, (8, 128), 0)

        memo = {}

        def piece(c, r):
            if r == 16:
                c = 0
            if (c, r) not in memo:
                memo[c, r] = (
                    pltpu.roll(jnp.where(lane == 0, piece(8, 0), merged(0, (0,) * 8)), 127, 1) if r == 16 else
                    jnp.take_along_axis(lag[i, _rows(lags.index((c, r)), 8), :], src, axis=1,
                                        mode="promise_in_bounds"))
            return memo[c, r]

        def merged(c, rs):
            if (c, rs) not in memo:
                memo[c, rs] = (piece(c, rs[0]) if c == 7 or min(rs) == 16 else
                               jnp.where(lane >> 4 == c, piece(c, rs[0]), merged(c + 1, rs[1:])))
            return memo[c, rs]

        for n0 in range(R0):
            kt[n0, _rows(i, 8), :] = merged(0, tuple(_RND[c][n0] for c in range(8)))

    get = lambda ref, n, rows: (ref[n, 0, rows, :], ref[n, 1, rows, :])

    def put(ref, n, rows, v):
        ref[n, 0, rows, :], ref[n, 1, rows, :] = v

    def outer(src, a, rows):
        return [_twiddle(v, a * b) for b, v in enumerate(_dft4([get(src, a + 4 * m, rows) for m in range(4)], 1))]

    def transform(lhs, dst, n0, rows):
        r = jnp.dot(lhs, _bf(fm[n0]), preferred_element_type=F32)
        put(dst, n0, rows, (r[:, :128], r[:, 128:]))

    def kfwd(n0, r):
        transform(_bf(kt[n0, _rows(r, 64), :]), ub, n0, _rows(r, 128))

    def kdft(i):
        rows, t = _rows(i, 8), []

        def inner(b):
            for m, v in enumerate(_dft4([t[a][b] for a in range(4)], 1)):
                put(kf, b + 4 * m, rows, (v[0] + par[1, rows, :], v[1]))

        return [lambda a=a: t.append(outer(ub, a, rows)) for a in range(4)] + [step(inner, b) for b in range(4)]

    def fwd(n0, r):
        transform(un[n0, _rows(r, 128), :], ua, n0, _rows(r, 128))

    def pre(a, i):
        for b, v in enumerate(outer(ua, a, _rows(i, 8))):
            put(ub, a + 4 * b, _rows(i, 8), v)

    def mid(i):
        out = []
        for rows in (_rows(2 * i, 8), _rows(2 * i + 1, 8)):
            t = []
            for b, v in enumerate(outer(ua, 0, rows)):
                x = _dft4([v] + [get(ub, a + 4 * b, rows) for a in range(1, 4)], 1)
                y = _dft4([_cmul(x[m], get(kf, b + 4 * m, rows)) for m in range(4)], -1)
                t.append(y[0])
                for a in range(1, 4):
                    put(uc, a + 4 * b, rows, y[a])
            out.append(_dft4(t, -1))
        for m, (v, w) in enumerate(zip(*out)):
            put(yb, 4 * m, _rows(i, 16), [jnp.concatenate([v[k], w[k]], 0).astype(BF16) for k in range(2)])

    def post(a, i):
        rows = _rows(i, 16)
        for m, v in enumerate(_dft4([_twiddle(get(uc, a + 4 * b, rows), -a * b) for b in range(4)], -1)):
            put(yb, a + 4 * m, rows, (v[0].astype(BF16), v[1].astype(BF16)))

    def inv(n0, r):
        rows = _rows(r, 128)
        y = jnp.concatenate(get(yb, n0, rows), 1)
        xs[n0, rows, :] = xs[n0, rows, :] + jnp.dot(y, _bf(gm[n0]), preferred_element_type=F32)

    def wprep(g, t):
        if t < 3:
            v = lax.dot_general(_bf(perm[...]), wqkv[4 * t + g], NT, preferred_element_type=F32)
            v = v if t else v * DH ** -0.5
            for k, a in enumerate(_left(v[:64, :256], v[:64, 256:], v[64:, :256], v[64:, 256:])):
                wt[g, k, _rows(t, 32), :] = pltpu.bitcast(a.astype(BF16), U32)
        else:
            v = [jnp.dot(_bf(perm[...]), wo[_rows(e, 128), _rows(g, 128)], preferred_element_type=F32)
                 for e in range(4)]
            lo, hi = (jnp.concatenate([u[64 * h:64 * h + 64] for u in v], 0).T for h in range(2))
            for k, a in enumerate(_left(lo[:64], hi[:64], lo[64:], hi[64:])):
                wot[k, _rows(g, 32), :] = pltpu.bitcast(a.astype(BF16), U32)

    def xin(j, c):
        xs[2 * j, _rows(c, 128), :], xs[2 * j + 1, _rows(c, 128), :] = halves(io[c, pl.ds(j, R1, stride=8), :].T)

    def norm(n0):
        acc, stat = {}, []

        def moment(k, c):
            for i in range(16 * c, 16 * c + 16):
                v = xs[n0, 8 * i:8 * i + 8, :]
                v = jnp.square(v - stat[0]) if k else v
                acc[i % 4] = v if i < 4 else acc[i % 4] + v
            if c == 3:
                v = jnp.sum(_tree(jnp.add, list(acc.values())), axis=0, keepdims=True) * (1.0 / D)
                stat.append(lax.rsqrt(v + 1e-5) if k else v)

        def scale(c):
            rows = _rows(c, 128)
            un[n0, rows, :] = get(rows).astype(BF16)

        get = lambda rows: (xs[n0, rows, :] - stat[0]) * stat[1]
        return [[step(fn, *k, c) for c in range(4)] for fn, *k in ((moment, 0), (moment, 1), (scale,))], get

    def norms(*aa):
        return [f for a in aa for stage in zip(*[norm(a + 4 * m)[0] for m in range(4)])
                for steps in stage for f in steps]

    def pair_norms(a):
        stages, get = zip(*[norm(a + 4 * m) for m in range(4)])

        def operands(j, c):
            (b11, b21), (b12, b22) = ((f(_rows(c, 32)), f(_rows(c + 8, 32))) for f in get[2 * j:2 * j + 2])
            for k, b in enumerate(_right(b11, b12, b21, b22)):
                us[2 * a + j, k, _rows(c, 32), :] = b.astype(BF16)

        return ([f for k in range(2) for st in stages for f in st[k]]
                + [step(operands, j, c) for j in range(2) for c in range(8)])

    def proj(i, slot, m, t):
        p, g, ref = i >> 2, i & 3, (qs, ks, vs)[t][slot]

        def emit(half, j, r):
            ref[m + 2 * j + 7 * (t > 0), _rows(half, 64), :] = r
            if t and m + j:
                ref[m + 2 * j - 1, _rows(half, 64), :] = pltpu.roll(r, 1, 1)

        return _strassen(lambda k: jnp.dot(_bf(wt[g, k, _rows(t, 32), :]), us[2 * p + 4 * (m & 1) + (m >> 2), k],
                                           preferred_element_type=F32), emit)

    def attn(i, slot, m0):
        p, g = i >> 2, i & 3
        first = lax.broadcasted_iota(jnp.int32, (8, 128), 1) == 0
        window = lambda ref, d: {e: ref[slot][e, 8 * d:8 * d + 8, :] for e in range(m0, m0 + W + 1)}
        s, o = {}, {}

        def logits(d):
            k = window(ks, d)
            for m in (m0, m0 + 1):
                q = qs[slot][m, 8 * d:8 * d + 8, :]
                for w in range(W):
                    t = q * k[m + 7 - w]
                    s[m, w] = t if d == 0 else s[m, w] + t

        def softmax(m):
            t = [jnp.where(first, -1e9, s[m, w]) if w > m else s[m, w] for w in range(W)]
            mx = _tree(jnp.maximum, t)
            e = [jnp.exp(v - mx) for v in t]
            rs = 1.0 / _tree(jnp.add, e)
            s.update({(m, w): e[w] * rs for w in range(W)})

        def values(d):
            v = window(vs, d)
            for m in (m0, m0 + 1):
                o[m, d] = _tree(jnp.add, [s[m, w] * v[m + 7 - w] for w in range(W)])
            if d % 2 and d > 8:
                blocks = [jnp.concatenate([o[m, e - 1], o[m, e]], 0) for e in (d - 8, d) for m in (m0, m0 + 1)]
                for k, b in enumerate(_right(*blocks)):
                    ob[m0 + p, k, g, 8 * d - 72:8 * d - 56, :] = b.astype(BF16)

        return ([step(logits, d) for d in range(DH)] + [step(softmax, m0), step(softmax, m0 + 1)]
                + [step(values, d + e) for d in range(0, 8, 2) for e in (0, 1, 8, 9)])

    def oproj(p, c, n):
        def pair(m0):
            def emit(half, j, r):
                for i in range(n):
                    at = (2 * (m0 + j) + p, _rows(2 * (c + i) + half, 64))
                    xs[at] = xs[at] + r[64 * i:64 * i + 64]

            return _strassen(lambda k: jnp.dot(_bf(wot[k, 32 * c:32 * (c + n), :]), ob[m0 + p, k].reshape(D // 2, R1),
                                               preferred_element_type=F32), emit)

        return [f for m0 in range(0, 8, 2) for f in pair(m0)]

    def xout(c, j):
        lo, hi = (pltpu.bitcast(xs[2 * j + k, _rows(c, 128), :].astype(BF16).astype(F32), U32) for k in range(2))
        io[c, pl.ds(j, R1, stride=8), :] = ((lo >> 16) | hi).T

    four = lambda fn, *aa: [step(fn, a + 4 * m, r) for a in aa for m in range(4) for r in range(NB)]
    rowwise = lambda fn, a, n: [step(fn, a, i) for i in range(D // n)]

    regions, zero = [], zero_ref[0]

    def slot(*streams):
        regions.append(None)
        pl.when(zero < len(regions))(lambda: _run(*streams))

    pres = lambda a: rowwise(pre, a, 8)
    posts = lambda a: rowwise(post, a, 16)
    projs = lambda i, s, ms: [f for t in (1, 2, 0) for m in ms for f in proj(i, s, m, t)]
    attns = lambda i, s: [f for m in range(0, 8, 2) for f in attn(i, s, m)]

    with jax.named_scope("kgen"):
        ng = D // 16 // KPER
        each = lambda fn: (lambda i: [f for k in range(KPER) for f in fn(KPER * i + k)])
        _pipeline([(lambda i: [lambda: [kgen(KPER * i + k) for k in range(KPER)]], 2, ng),
                   (each(lagsums), 1, ng), (each(setup), 0, ng),
                   (lambda j: [step(xin, j * KPER // 2 + k, c) for k in range(KPER // 2) for c in range(NB)],
                    ng // 2, ng // 2)],
                  {ng // 2: lambda: [c.wait() for c in loads[:NB]]})
    with jax.named_scope("kfwd"):
        for c in loads[NB:]:
            c.wait()
        kdfts = lambda r: [f for i in range(16) for f in kdft(16 * r + i)]
        for r, other in enumerate((norms(2, 1), norms(3), norms(0), [])):
            slot([f for k in range(4) for f in [step(wprep, r, k)] + [step(kfwd, 4 * k + n, r) for n in range(4)]],
                 kdfts(r - 1) if r else [], other)
        slot(four(fwd, 2), kdfts(NB - 1))
        slot(four(fwd, 1), pres(2))

    def layer(li, carry):
        with jax.named_scope("conv"):
            slot(four(fwd, 3), pres(1))
            slot(four(fwd, 0), pres(3))
            lax.fori_loop(0, D // 16, lambda i, c: (mid(i), c)[-1], 0)
            slot(four(inv, 0), posts(2))
            slot(four(inv, 2), pair_norms(0))
            slot(projs(0, 0, (0, 4)), pair_norms(2))
            slot(projs(0, 0, (1, 5)), posts(1) + posts(3))
        with jax.named_scope("attn"):
            slot(four(inv, 1, 3), attns(0, 0))
            slot(projs(1, 1, (0, 1, 4, 5)), pair_norms(1) + pair_norms(3))
            both = lambda i, s: slot(projs(i + 1, 1 - s, (0, 1, 4, 5)), attns(i, s))
            lax.fori_loop(0, 3, lambda j, c: (both(2 * j + 1, 1), both(2 * j + 2, 0), c)[-1], 0)
            slot(oproj(0, 0, 2) + oproj(0, 2, 2), attns(7, 1))

        @pl.when(li == 0)
        def _():
            slot(oproj(1, 0, 2) + oproj(1, 2, 2), norms(2, 0))
            slot(four(fwd, 2), norms(1))
            slot(four(fwd, 1), norms(3), pres(2))

        return carry

    lax.fori_loop(0, 2, layer, 0)

    with jax.named_scope("xout"):
        stores = [pltpu.make_async_copy(io.at[c], out_hbm.bitcast(U32).at[:, pl.ds(c * 128, 128)], sems.at[c])
                  for c in range(NB)]
        for c in range(NB + 1):
            slot(oproj(1, c, 1) if c < NB else [],
                 [step(xout, c - 1, j) for j in range(8)] if c else [])
            if c:
                stores[c - 1].start()
        for c in stores:
            c.wait()


@jax.jit
def pallas_interleave_layers__ssm_conv_s4__sliding_local_dilated__prompt_kernel(
    A_u: jax.Array,
    A_A_re: jax.Array,
    A_A_im: jax.Array,
    A_B_re: jax.Array,
    A_B_im: jax.Array,
    A_C_re: jax.Array,
    A_C_im: jax.Array,
    A_log_dt: jax.Array,
    A_Dskip: jax.Array,
    B_x: jax.Array,
    B_wqkv: jax.Array,
    B_wo: jax.Array,
):
    del B_x
    hbm, vmem = pl.BlockSpec(memory_space=pl.ANY), pl.BlockSpec(memory_space=pltpu.VMEM)
    tiles = lambda *n: pltpu.VMEM((*n, 128, 128), F32)
    out = pl.pallas_call(
        _kernel,
        out_shape=jax.ShapeDtypeStruct((L, D), BF16),
        in_specs=[pl.BlockSpec(memory_space=pltpu.SMEM), hbm] + [vmem] * 8 + [hbm] * 4,
        out_specs=hbm,
        scratch_shapes=[
            pltpu.VMEM((R0, D, R1), F32),
            *[pltpu.VMEM((R0, 2, D, R1), F32)] * 4,
            pltpu.VMEM((R0, 2, D, R1), BF16),
            pltpu.VMEM((2, D, N), F32),
            pltpu.VMEM((D // 16, 2, 4, 8, N), F32),
            pltpu.VMEM((D // 16, 336, 128), U32),
            *[tiles(n) for n in (8, 15, 15) * 2],
            pltpu.VMEM((NB, L // 2, 128), U32),
            pltpu.VMEM((64, 128), U32),
            pltpu.VMEM((12, D, 128), BF16),
            pltpu.VMEM((D, D), BF16),
            pltpu.VMEM(_F.shape, U32),
            pltpu.VMEM(_G.shape, U32),
            pltpu.VMEM((R0, D // 2, R1), U32),
            pltpu.VMEM((R0, D, R1), BF16),
            pltpu.VMEM((4, 7, 96, D // 2), U32),
            pltpu.VMEM((8, 7, D // 2, R1), BF16),
            pltpu.VMEM((7, D // 4, D // 2), U32),
            pltpu.VMEM((8, 7, 4, 64, R1), BF16),
            pltpu.SemaphoreType.DMA((19,)),
        ],
        compiler_params=pltpu.CompilerParams(vmem_limit_bytes=100 * 1024 * 1024),
    )(np.zeros((2,), np.int32), A_u.reshape(L, D), A_A_re, A_A_im, A_B_re, A_B_im, A_C_re, A_C_im, A_log_dt, A_Dskip,
      B_wqkv, B_wo, _F, _G)
    return out.reshape(1, L, D)
```

```python
import jax
import jax.numpy as jnp
import ml_dtypes
import numpy as np
from jax import lax
import jax.experimental.pallas as pl
import jax.experimental.pallas.tpu as pltpu

L, D, N = 2048, 512, 128
R0, R1 = 16, 128
W, DH = 8, 16
F32, BF16, U32 = jnp.float32, jnp.bfloat16, jnp.uint32
CUT = (0, 20, 42)
KPER = 4
NB = D // 128
NT = (((1,), (1,)), ((), ()))


def _constants():
    n0 = np.arange(R0)[:, None, None]
    n1 = np.arange(R1)[None, :, None]
    k1 = np.arange(R1)[None, None, :]
    ang = 2.0 * np.pi * (k1 + 0.25) * (R0 * n1 + n0) / L
    f = np.concatenate([np.cos(ang), np.sin(ang)], axis=2)
    g = f.transpose(0, 2, 1)
    bf = ml_dtypes.bfloat16
    lr = np.arange(L).astype(np.float32).astype(bf).astype(np.int64).reshape(8, 16, R0)
    r = lr - (256 * np.arange(8)[:, None, None] + 16 * np.arange(16)[None, :, None])
    assert (r == r[:, :1, :]).all()

    def words(m):
        h = np.ascontiguousarray(m).astype(bf).view(np.uint16).astype(np.uint32)
        return h[:, 0::2] | (h[:, 1::2] << 16)

    return words(f), words(g), r[:, 0, :].tolist()


_F, _G, _RND = _constants()


def _cmul(a, b):
    return a[0] * b[0] - a[1] * b[1], a[0] * b[1] + a[1] * b[0]


def _csq(a):
    t = a[0] * a[1]
    return (a[0] + a[1]) * (a[0] - a[1]), t + t


def _dft4(x, sign):
    (ar, ai), (br, bi), (cr, ci), (dr, di) = x
    sr, si, tr, ti = ar + cr, ai + ci, ar - cr, ai - ci
    ur, ui, vr, vi = br + dr, bi + di, br - dr, bi - di
    p, m = (tr - vi, ti + vr), (tr + vi, ti - vr)
    if sign < 0:
        p, m = m, p
    return [(sr + ur, si + ui), p, (sr - ur, si - ui), m]


def _twiddle(v, e):
    e %= 16
    re, im = v
    h = float(np.sqrt(0.5))
    if e == 0:
        return v
    if e == 4:
        return -im, re
    if e == 12:
        return im, -re
    if e == 2:
        return (re - im) * h, (re + im) * h
    if e == 14:
        return (re + im) * h, (im - re) * h
    if e == 6:
        return (re + im) * -h, (re - im) * h
    if e == 10:
        return (im - re) * h, (re + im) * -h
    c, s = float(np.cos(np.pi * e / 8)), float(np.sin(np.pi * e / 8))
    return re * c - im * s, re * s + im * c


def _bf(x):
    return pltpu.bitcast(x, BF16)


def _tree(op, v):
    while len(v) > 1:
        v = [op(v[i], v[i + 1]) if i + 1 < len(v) else v[i] for i in range(0, len(v), 2)]
    return v[0]


def _run(*streams):
    order = sorted(((i + 0.5 * (k > 0)) / len(s), k, i) for k, s in enumerate(streams) for i in range(len(s)))
    for _, k, i in order:
        streams[k][i]()


def _pipeline(streams, hooks=None):
    hooks = hooks or {}
    cuts = sorted({e for _, a, n in streams for e in (a, a + n)} | set(hooks))
    for lo, hi in zip(cuts, cuts[1:]):
        def body(s, carry, lo=lo):
            _run(*[fn(s - a) for fn, a, n in streams if a <= lo < a + n])
            return carry

        if lo in hooks:
            hooks[lo]()
        if hi - lo == 1:
            body(lo, 0)
        else:
            lax.fori_loop(lo, hi, body, 0)


def _left(a11, a12, a21, a22):
    return a21 + a22, a22, a11 + a22, a12 - a22, a11 + a12, a11, a21 - a11


def _right(b11, b12, b21, b22):
    return b11, b21 - b11, b11 + b22, b21 + b22, b22, b12 - b22, b11 + b12


def _strassen(product, emit):
    c = {}

    def run(k):
        c[k] = r = product(k)
        if k == 1:
            emit(1, 0, c[0] + r)
        elif k == 2:
            c[11], c[22] = r + c[1], r - c[0]
        elif k == 3:
            c[11] = c[11] + r
        elif k == 4:
            emit(0, 0, c[11] - r)
        elif k == 5:
            emit(0, 1, c[4] + r)
            c[22] = c[22] + r
        elif k == 6:
            emit(1, 1, c[22] + r)

    return [lambda k=k: run(k) for k in range(7)]


def _rows(i, n):
    return pl.ds(i * n if isinstance(i, int) else pl.multiple_of(i * n, n), n)


def _kernel(zero_ref, x_hbm, are_ref, aim_ref, bre_ref, bim_ref, cre_ref, cim_ref, ldt_ref, dsk_ref,
            wqkv_hbm, wo_hbm, f_hbm, g_hbm, out_hbm,
            xs, kf, ua, ub, uc, yb, par, zw, lag, qa, ka, va, qb, kb, vb, io, perm, wqkv, wo, fm, gm, kt, un, wt, us, wot, ob, sems):
    step = lambda fn, *a: (lambda: fn(*a))
    qs, ks, vs = (qa, qb), (ka, kb), (va, vb)
    loads = [pltpu.make_async_copy(s, d, sems.at[i]) for i, (s, d) in enumerate(
        (*((x_hbm.bitcast(U32).at[:, pl.ds(128 * c, 128)], io.at[c]) for c in range(NB)),
         (f_hbm, fm), (wo_hbm, wo), (g_hbm, gm),
         *((wqkv_hbm.at[:, pl.ds(128 * j, 128)], wqkv.at[j]) for j in range(12))))]
    for c in loads:
        c.start()
    high = jnp.uint32(0xFFFF0000)
    halves = lambda t: (pltpu.bitcast(t << 16, F32), pltpu.bitcast(t & high, F32))

    def col(ref):
        v = ref[...].astype(F32).reshape(1, D)
        return jnp.broadcast_to(v, (128, D)).T

    par[0] = jnp.exp(col(ldt_ref))
    par[1] = col(dsk_ref) * (1.0 / L)

    ri = lax.broadcasted_iota(jnp.int32, (128, 128), 0)
    ci = lax.broadcasted_iota(jnp.int32, (128, 128), 1)
    perm[...] = pltpu.bitcast(jnp.where(ci == (ri & 7) * DH + (ri >> 3), 1.0, 0.0).astype(BF16), U32)

    def setup(i):
        get = lambda ref: halves(pltpu.bitcast(ref[_rows(i, 16), :], U32))
        dt = halves(pltpu.bitcast(par[0, _rows(i, 16), :].astype(BF16), U32))

        def pole(h):
            mag, ang = jnp.exp(dt[h] * get(are_ref)[h]), dt[h] * get(aim_ref)[h]
            zw[i, h, 0], zw[i, h, 1] = mag * jnp.cos(ang), mag * jnp.sin(ang)

        def weight():
            scale = (1.0 + 1.5 * 2.0 ** -9) / L
            for h, (cr, ci, br, bi) in enumerate(zip(*map(get, (cre_ref, cim_ref, bre_ref, bim_ref)))):
                wr, wi = _cmul((cr, ci), (dt[h] * br, dt[h] * bi))
                zw[i, h, 2], zw[i, h, 3] = wr * scale, wi * -scale

        return [step(pole, 0), weight, step(pole, 1)]

    lags = sorted({(c, r) for c in range(8) for r in _RND[c] if r < 16}) + [(8, 0)]
    stack = lambda vs: jnp.concatenate([jnp.concatenate([v[k] for v in vs], 0) for k in range(2)], 1).astype(BF16)

    def lagsums(i):
        start = [[zw[i, h, c] for c in range(4)] for h in range(2)]
        zs, rhs, even = [], [], []

        def right(h):
            zr, zi, wr, wi = start[h]
            z = {0: (jnp.ones((8, N), F32), jnp.zeros((8, N), F32)), 1: (zr, zi)}
            for e in (2, 4, 8, 16, 32, 64, 128, 256):
                z[e] = _csq(z[e // 2])
            b = [(wr, wi)]
            for e in (16, 32, 64, 128):
                zc = (z[e][0], -z[e][1])
                b += [_cmul(v, zc) for v in b]
            zs.append(z)
            rhs.append(stack(b))

        def left(t, h):
            z = zs[h]

            def power(e):
                if e not in z:
                    low = e % 256 if e > 256 and e % 256 else e & -e
                    z[e] = _csq(z[e // 2]) if e // 2 in z and e % 2 == 0 else _cmul(power(e - low), power(low))
                return z[e]

            a = [power(256 * c + r) for c, r in (lags + lags[-1:])[CUT[t]:CUT[t + 1]]]
            o = pltpu.bitcast(lax.dot_general(stack(a), rhs[h], NT, preferred_element_type=F32), U32)
            if h:
                lag[i, 8 * CUT[t]:8 * CUT[t + 1], :] = even[t] | (o & high)
            else:
                even.append(o >> 16)

        return [f for h in range(2) for f in [step(right, h)] + [step(left, t, h) for t in range(len(CUT) - 1)]]

    def kgen(i):
        lane = lax.broadcasted_iota(jnp.int32, (8, 128), 1)
        src = (lane & 15) * 8 + lax.broadcasted_iota(jnp.int32, (8, 128), 0)

        memo = {}

        def piece(c, r):
            if r == 16:
                c = 0
            if (c, r) not in memo:
                memo[c, r] = (
                    pltpu.roll(jnp.where(lane == 0, piece(8, 0), merged(0, (0,) * 8)), 127, 1) if r == 16 else
                    jnp.take_along_axis(lag[i, _rows(lags.index((c, r)), 8), :], src, axis=1,
                                        mode="promise_in_bounds"))
            return memo[c, r]

        def merged(c, rs):
            if (c, rs) not in memo:
                memo[c, rs] = (piece(c, rs[0]) if c == 7 or min(rs) == 16 else
                               jnp.where(lane >> 4 == c, piece(c, rs[0]), merged(c + 1, rs[1:])))
            return memo[c, rs]

        for n0 in range(R0):
            kt[n0, _rows(i, 8), :] = merged(0, tuple(_RND[c][n0] for c in range(8)))

    get = lambda ref, n, rows: (ref[n, 0, rows, :], ref[n, 1, rows, :])

    def put(ref, n, rows, v):
        ref[n, 0, rows, :], ref[n, 1, rows, :] = v

    def outer(src, a, rows):
        return [_twiddle(v, a * b) for b, v in enumerate(_dft4([get(src, a + 4 * m, rows) for m in range(4)], 1))]

    def transform(lhs, dst, n0, rows):
        r = jnp.dot(lhs, _bf(fm[n0]), preferred_element_type=F32)
        put(dst, n0, rows, (r[:, :128], r[:, 128:]))

    def kfwd(n0, r):
        for h in (2 * r, 2 * r + 1):
            transform(_bf(kt[n0, _rows(h, 32), :]), ub, n0, _rows(h, 64))

    def kdft(i):
        rows, t = _rows(i, 8), []

        def inner(b):
            for m, v in enumerate(_dft4([t[a][b] for a in range(4)], 1)):
                put(kf, b + 4 * m, rows, (v[0] + par[1, rows, :], v[1]))

        return [lambda a=a: t.append(outer(ub, a, rows)) for a in range(4)] + [step(inner, b) for b in range(4)]

    def fwd(n0, r, n=128):
        transform(un[n0, _rows(r, n), :], ua, n0, _rows(r, n))

    def pre(a, i):
        for b, v in enumerate(outer(ua, a, _rows(i, 8))):
            put(ub, a + 4 * b, _rows(i, 8), v)

    def mid(i):
        first, t = {}, {}

        def inner(h, b):
            rows = _rows(2 * i + h, 8)
            if b == 0:
                first[h] = outer(ua, 0, rows)
            x = _dft4([first[h][b]] + [get(ub, a + 4 * b, rows) for a in range(1, 4)], 1)
            t[h, b], *y = _dft4([_cmul(x[m], get(kf, b + 4 * m, rows)) for m in range(4)], -1)
            for a in range(1, 4):
                put(uc, a + 4 * b, rows, y[a - 1])

        def last():
            for m, (v, w) in enumerate(zip(*[_dft4([t[h, b] for b in range(4)], -1) for h in range(2)])):
                put(yb, 4 * m, _rows(i, 16), [jnp.concatenate([v[k], w[k]], 0).astype(BF16) for k in range(2)])

        return [step(inner, h, b) for h in range(2) for b in range(4)] + [last]

    def post(a, i):
        rows = _rows(i, 16)
        for m, v in enumerate(_dft4([_twiddle(get(uc, a + 4 * b, rows), -a * b) for b in range(4)], -1)):
            put(yb, a + 4 * m, rows, (v[0].astype(BF16), v[1].astype(BF16)))

    def inv(n0, r, n=128):
        rows = _rows(r, n)
        y = jnp.concatenate(get(yb, n0, rows), 1)
        xs[n0, rows, :] = xs[n0, rows, :] + jnp.dot(y, _bf(gm[n0]), preferred_element_type=F32)

    def wprep(g, t):
        if t < 3:
            v = lax.dot_general(_bf(perm[...]), wqkv[4 * t + g], NT, preferred_element_type=F32)
            v = v if t else v * DH ** -0.5
            for k, a in enumerate(_left(v[:64, :256], v[:64, 256:], v[64:, :256], v[64:, 256:])):
                wt[g, k, _rows(t, 32), :] = pltpu.bitcast(a.astype(BF16), U32)
        else:
            v = [jnp.dot(_bf(perm[...]), wo[_rows(e, 128), _rows(g, 128)], preferred_element_type=F32)
                 for e in range(4)]
            lo, hi = (jnp.concatenate([u[64 * h:64 * h + 64] for u in v], 0).T for h in range(2))
            for k, a in enumerate(_left(lo[:64], hi[:64], lo[64:], hi[64:])):
                wot[k, _rows(g, 32), :] = pltpu.bitcast(a.astype(BF16), U32)

    def xin(j, c):
        xs[2 * j, _rows(c, 128), :], xs[2 * j + 1, _rows(c, 128), :] = halves(io[c, pl.ds(j, R1, stride=8), :].T)

    def norm(n0):
        acc, stat = {}, []

        def moment(k, c):
            for i in range(16 * c, 16 * c + 16):
                v = xs[n0, 8 * i:8 * i + 8, :]
                v = jnp.square(v - stat[0]) if k else v
                acc[i % 4] = v if i < 4 else acc[i % 4] + v
            if c == 3:
                v = jnp.sum(_tree(jnp.add, list(acc.values())), axis=0, keepdims=True) * (1.0 / D)
                stat.append(lax.rsqrt(v + 1e-5) if k else v)

        def scale(c):
            rows = _rows(c, 128)
            un[n0, rows, :] = get(rows).astype(BF16)

        get = lambda rows: (xs[n0, rows, :] - stat[0]) * stat[1]
        return [[step(fn, *k, c) for c in range(4)] for fn, *k in ((moment, 0), (moment, 1), (scale,))], get

    def norms(*aa):
        return [f for a in aa for stage in zip(*[norm(a + 4 * m)[0] for m in range(4)])
                for steps in stage for f in steps]

    def pair_norms(a):
        stages, get = zip(*[norm(a + 4 * m) for m in range(4)])

        def operands(j, c):
            (b11, b21), (b12, b22) = ((f(_rows(c, 32)), f(_rows(c + 8, 32))) for f in get[2 * j:2 * j + 2])
            for k, b in enumerate(_right(b11, b12, b21, b22)):
                us[2 * a + j, k, _rows(c, 16), :] = pltpu.bitcast(b.astype(BF16), U32)

        return ([f for k in range(2) for st in stages for f in st[k]]
                + [step(operands, j, c) for j in range(2) for c in range(8)])

    def proj(i, slot, m, t):
        p, g, ref = i >> 2, i & 3, (qs, ks, vs)[t][slot]

        def emit(half, j, r):
            ref[m + 2 * j + 7 * (t > 0), _rows(half, 64), :] = r
            if t and m + j:
                ref[m + 2 * j - 1, _rows(half, 64), :] = pltpu.roll(r, 1, 1)

        return _strassen(lambda k: jnp.dot(_bf(wt[g, k, _rows(t, 32), :]), _bf(us[2 * p + 4 * (m & 1) + (m >> 2), k]),
                                           preferred_element_type=F32), emit)

    def attn(i, slot, m0):
        p, g = i >> 2, i & 3
        first = lax.broadcasted_iota(jnp.int32, (8, 128), 1) == 0
        window = lambda ref, d: {e: ref[slot][e, 8 * d:8 * d + 8, :] for e in range(m0, m0 + W + 1)}
        s, o = {}, {}

        def logits(d):
            k = window(ks, d)
            for m in (m0, m0 + 1):
                q = qs[slot][m, 8 * d:8 * d + 8, :]
                for w in range(W):
                    t = q * k[m + 7 - w]
                    s[m, w] = t if d == 0 else s[m, w] + t

        def softmax(m):
            t = [jnp.where(first, -1e9, s[m, w]) if w > m else s[m, w] for w in range(W)]
            mx = _tree(jnp.maximum, t)
            e = [jnp.exp(v - mx) for v in t]
            rs = 1.0 / _tree(jnp.add, e)
            s.update({(m, w): e[w] * rs for w in range(W)})

        def values(d):
            v = window(vs, d)
            for m in (m0, m0 + 1):
                o[m, d] = _tree(jnp.add, [s[m, w] * v[m + 7 - w] for w in range(W)])
            if d % 2 and d > 8:
                blocks = [jnp.concatenate([o[m, e - 1], o[m, e]], 0) for e in (d - 8, d) for m in (m0, m0 + 1)]
                for k, b in enumerate(_right(*blocks)):
                    ob[m0 + p, k, g, 8 * d - 72:8 * d - 56, :] = b.astype(BF16)

        return ([step(logits, d) for d in range(DH)] + [step(softmax, m0), step(softmax, m0 + 1)]
                + [step(values, d + e) for d in range(0, 8, 2) for e in (0, 1, 8, 9)])

    def oproj(p, c, n):
        def pair(m0):
            def emit(half, j, r):
                for i in range(n):
                    at = (2 * (m0 + j) + p, _rows(2 * (c + i) + half, 64))
                    xs[at] = xs[at] + r[64 * i:64 * i + 64]

            return _strassen(lambda k: jnp.dot(_bf(wot[k, 32 * c:32 * (c + n), :]), ob[m0 + p, k].reshape(D // 2, R1),
                                               preferred_element_type=F32), emit)

        return [f for m0 in range(0, 8, 2) for f in pair(m0)]

    def xout(c, j):
        lo, hi = (pltpu.bitcast(xs[2 * j + k, _rows(c, 128), :].astype(BF16).astype(F32), U32) for k in range(2))
        io[c, pl.ds(j, R1, stride=8), :] = ((lo >> 16) | hi).T

    four = lambda fn, *aa: [step(fn, a + 4 * m, r, 64) for a in aa for m in range(4) for r in range(2 * NB)]
    block = lambda fn, a, r: [step(fn, a + 4 * m, 2 * r + h, 64) for h in range(2) for m in range(4)] if 0 <= r < NB else []
    rowwise = lambda fn, a, n: [step(fn, a, i) for i in range(D // n)]

    regions, zero = [], zero_ref[0]

    def slot(*streams):
        regions.append(None)
        pl.when(zero < len(regions))(lambda: _run(*streams))

    pres = lambda a: rowwise(pre, a, 8)
    posts = lambda a: rowwise(post, a, 16)
    projs = lambda i, s, ms: [f for t in (1, 2, 0) for m in ms for f in proj(i, s, m, t)]
    attns = lambda i, s: [f for m in range(0, 8, 2) for f in attn(i, s, m)]

    with jax.named_scope("kgen"):
        ng = D // 16 // KPER
        each = lambda fn: (lambda i: [f for k in range(KPER) for f in fn(KPER * i + k)])
        _pipeline([(lambda i: [lambda: [kgen(KPER * i + k) for k in range(KPER)]], 2, ng - 1),
                   (each(lagsums), 1, ng), (each(setup), 0, ng),
                   (lambda j: [step(xin, j * KPER // 2 + k, c) for k in range(KPER // 2) for c in range(NB)],
                    ng // 2, ng // 2)],
                  {ng // 2: lambda: [c.wait() for c in loads[:NB]]})
    with jax.named_scope("kfwd"):
        for c in loads[NB:]:
            c.wait()
        kdfts = lambda r: [f for i in range(16) for f in kdft(16 * r + i)]
        for r, other in enumerate((norms(2, 1), norms(3), norms(0), [])):
            slot([f for k in range(4) for f in [step(wprep, r, k)] + [step(kfwd, 4 * k + n, r) for n in range(4)]],
                 kdfts(r - 1) if r else [step(kgen, D // 16 - 1 - k) for k in range(KPER)], other)
        slot(four(fwd, 2), kdfts(NB - 1))
        slot(four(fwd, 1) + block(fwd, 3, 0), pres(2))

    def layer(li, carry):
        with jax.named_scope("conv"):
            part = lambda steps, r: steps[len(steps) * r // NB:len(steps) * (r + 1) // NB] if 0 <= r < NB else []
            mids = [f for i in range(D // 16) for f in mid(i)]
            for r in range(-1, NB + 1):
                slot(block(fwd, 3, r + 2) + block(fwd, 0, r + 1) + block(inv, 0, r - 1) + block(inv, 2, r - 2),
                     part(mids, r), part(pres(3), r + 1) + part(posts(2), r - 1),
                     pres(1) if r < 0 else posts(1) if r == NB else [])
            slot(block(inv, 2, NB - 1) + four(inv, 1), pair_norms(0))
            slot(projs(0, 0, (0, 4)), pair_norms(2))
            slot(projs(0, 0, (1, 5)), posts(3) + pair_norms(1))
        with jax.named_scope("attn"):
            slot(four(inv, 3) + projs(1, 1, (0, 4)), attns(0, 0))
            slot(projs(1, 1, (1, 5)), pair_norms(3))
            both = lambda i, s: slot(projs(i + 1, 1 - s, (0, 1, 4, 5)), attns(i, s))
            lax.fori_loop(0, 3, lambda j, c: (both(2 * j + 1, 1), both(2 * j + 2, 0), c)[-1], 0)
            slot(oproj(0, 0, 2) + oproj(0, 2, 2), attns(7, 1))

        @pl.when(li == 0)
        def _():
            slot(oproj(1, 0, 2) + oproj(1, 2, 2), norms(2, 0))
            slot(four(fwd, 2), norms(1, 3))
            slot(four(fwd, 1) + block(fwd, 3, 0), pres(2))

        return carry

    lax.fori_loop(0, 2, layer, 0)

    with jax.named_scope("xout"):
        stores = [pltpu.make_async_copy(io.at[c], out_hbm.bitcast(U32).at[:, pl.ds(c * 128, 128)], sems.at[c])
                  for c in range(NB)]
        for c in range(NB + 1):
            outs = [step(xout, *divmod(j, 8)) if 0 <= j < 8 * NB else (lambda: None)
                    for j in range(8 * c - 2, 8 * c + 6)]
            slot(oproj(1, c, 1) if c < NB else [], outs)
            if c:
                stores[c - 1].start()
        for c in stores:
            c.wait()


@jax.jit
def pallas_interleave_layers__ssm_conv_s4__sliding_local_dilated__prompt_kernel(
    A_u: jax.Array,
    A_A_re: jax.Array,
    A_A_im: jax.Array,
    A_B_re: jax.Array,
    A_B_im: jax.Array,
    A_C_re: jax.Array,
    A_C_im: jax.Array,
    A_log_dt: jax.Array,
    A_Dskip: jax.Array,
    B_x: jax.Array,
    B_wqkv: jax.Array,
    B_wo: jax.Array,
):
    del B_x
    hbm, vmem = pl.BlockSpec(memory_space=pl.ANY), pl.BlockSpec(memory_space=pltpu.VMEM)
    tiles = lambda *n: pltpu.VMEM((*n, 128, 128), F32)
    out = pl.pallas_call(
        _kernel,
        out_shape=jax.ShapeDtypeStruct((L, D), BF16),
        in_specs=[pl.BlockSpec(memory_space=pltpu.SMEM), hbm] + [vmem] * 8 + [hbm] * 4,
        out_specs=hbm,
        scratch_shapes=[
            pltpu.VMEM((R0, D, R1), F32),
            *[pltpu.VMEM((R0, 2, D, R1), F32)] * 4,
            pltpu.VMEM((R0, 2, D, R1), BF16),
            pltpu.VMEM((2, D, N), F32),
            pltpu.VMEM((D // 16, 2, 4, 8, N), F32),
            pltpu.VMEM((D // 16, 336, 128), U32),
            *[tiles(n) for n in (8, 15, 15) * 2],
            pltpu.VMEM((NB, L // 2, 128), U32),
            pltpu.VMEM((64, 128), U32),
            pltpu.VMEM((12, D, 128), BF16),
            pltpu.VMEM((D, D), BF16),
            pltpu.VMEM(_F.shape, U32),
            pltpu.VMEM(_G.shape, U32),
            pltpu.VMEM((R0, D // 2, R1), U32),
            pltpu.VMEM((R0, D, R1), BF16),
            pltpu.VMEM((4, 7, 96, D // 2), U32),
            pltpu.VMEM((8, 7, D // 4, R1), U32),
            pltpu.VMEM((7, D // 4, D // 2), U32),
            pltpu.VMEM((8, 7, 4, 64, R1), BF16),
            pltpu.SemaphoreType.DMA((19,)),
        ],
        compiler_params=pltpu.CompilerParams(vmem_limit_bytes=100 * 1024 * 1024),
    )(np.zeros((2,), np.int32), A_u.reshape(L, D), A_A_re, A_A_im, A_B_re, A_B_im, A_C_re, A_C_im, A_log_dt, A_Dskip,
      B_wqkv, B_wo, _F, _G)
    return out.reshape(1, L, D)
```

```python
import jax
import jax.numpy as jnp
import ml_dtypes
import numpy as np
from jax import lax
import jax.experimental.pallas as pl
import jax.experimental.pallas.tpu as pltpu

L, D, N = 2048, 512, 128
R0, R1 = 16, 128
W, DH = 8, 16
F32, BF16, U32 = jnp.float32, jnp.bfloat16, jnp.uint32
CUT = (0, 20, 42)
KPER = 4
NB = D // 128
NT = (((1,), (1,)), ((), ()))


def _constants():
    n0 = np.arange(R0)[:, None, None]
    n1 = np.arange(R1)[None, :, None]
    k1 = np.arange(R1)[None, None, :]
    ang = 2.0 * np.pi * (k1 + 0.25) * (R0 * n1 + n0) / L
    f = np.concatenate([np.cos(ang), np.sin(ang)], axis=2)
    g = f.transpose(0, 2, 1)
    bf = ml_dtypes.bfloat16
    lr = np.arange(L).astype(np.float32).astype(bf).astype(np.int64).reshape(8, 16, R0)
    r = lr - (256 * np.arange(8)[:, None, None] + 16 * np.arange(16)[None, :, None])
    assert (r == r[:, :1, :]).all()

    def words(m):
        h = np.ascontiguousarray(m).astype(bf).view(np.uint16).astype(np.uint32)
        return h[:, 0::2] | (h[:, 1::2] << 16)

    return words(f), words(g), r[:, 0, :].tolist()


_F, _G, _RND = _constants()


def _cmul(a, b):
    return a[0] * b[0] - a[1] * b[1], a[0] * b[1] + a[1] * b[0]


def _csq(a):
    t = a[0] * a[1]
    return (a[0] + a[1]) * (a[0] - a[1]), t + t


def _dft4(x, sign):
    (ar, ai), (br, bi), (cr, ci), (dr, di) = x
    sr, si, tr, ti = ar + cr, ai + ci, ar - cr, ai - ci
    ur, ui, vr, vi = br + dr, bi + di, br - dr, bi - di
    p, m = (tr - vi, ti + vr), (tr + vi, ti - vr)
    if sign < 0:
        p, m = m, p
    return [(sr + ur, si + ui), p, (sr - ur, si - ui), m]


def _twiddle(v, e):
    e %= 16
    re, im = v
    h = float(np.sqrt(0.5))
    if e == 0:
        return v
    if e == 4:
        return -im, re
    if e == 12:
        return im, -re
    if e == 2:
        return (re - im) * h, (re + im) * h
    if e == 14:
        return (re + im) * h, (im - re) * h
    if e == 6:
        return (re + im) * -h, (re - im) * h
    if e == 10:
        return (im - re) * h, (re + im) * -h
    c, s = float(np.cos(np.pi * e / 8)), float(np.sin(np.pi * e / 8))
    return re * c - im * s, re * s + im * c


def _bf(x):
    return pltpu.bitcast(x, BF16)


def _tree(op, v):
    while len(v) > 1:
        v = [op(v[i], v[i + 1]) if i + 1 < len(v) else v[i] for i in range(0, len(v), 2)]
    return v[0]


def _run(*streams):
    order = sorted(((i + 0.5 * (k > 0)) / len(s), k, i) for k, s in enumerate(streams) for i in range(len(s)))
    for _, k, i in order:
        streams[k][i]()


def _pipeline(streams, hooks=None):
    hooks = hooks or {}
    cuts = sorted({e for _, a, n in streams for e in (a, a + n)} | set(hooks))
    for lo, hi in zip(cuts, cuts[1:]):
        def body(s, carry, lo=lo):
            _run(*[fn(s - a) for fn, a, n in streams if a <= lo < a + n])
            return carry

        if lo in hooks:
            hooks[lo]()
        if hi - lo == 1:
            body(lo, 0)
        else:
            lax.fori_loop(lo, hi, body, 0)


def _left(a11, a12, a21, a22):
    return a21 + a22, a22, a11 + a22, a12 - a22, a11 + a12, a11, a21 - a11


def _right(b11, b12, b21, b22):
    return b11, b21 - b11, b11 + b22, b21 + b22, b22, b12 - b22, b11 + b12


def _strassen(product, emit):
    c = {}

    def run(k):
        c[k] = r = product(k)
        if k == 1:
            emit(1, 0, c[0] + r)
        elif k == 2:
            c[11], c[22] = r + c[1], r - c[0]
        elif k == 3:
            c[11] = c[11] + r
        elif k == 4:
            emit(0, 0, c[11] - r)
        elif k == 5:
            emit(0, 1, c[4] + r)
            c[22] = c[22] + r
        elif k == 6:
            emit(1, 1, c[22] + r)

    return [lambda k=k: run(k) for k in range(7)]


def _rows(i, n):
    return pl.ds(i * n if isinstance(i, int) else pl.multiple_of(i * n, n), n)


def _kernel(zero_ref, x_hbm, are_ref, aim_ref, bre_ref, bim_ref, cre_ref, cim_ref, ldt_ref, dsk_ref,
            wqkv_hbm, wo_hbm, f_hbm, g_hbm, out_hbm,
            xs, kf, ua, ub, uc, yb, par, zw, lag, qa, ka, va, qb, kb, vb, io, perm, wqkv, wo, fm, gm, kt, un, wt, us, wot, ob, sems):
    step = lambda fn, *a: (lambda: fn(*a))
    qs, ks, vs = (qa, qb), (ka, kb), (va, vb)
    loads = [pltpu.make_async_copy(s, d, sems.at[i]) for i, (s, d) in enumerate(
        (*((x_hbm.bitcast(U32).at[:, pl.ds(128 * c, 128)], io.at[c, pl.ds(0, L // 2)]) for c in range(NB)),
         (f_hbm, fm), (wo_hbm, wo), (g_hbm, gm),
         *((wqkv_hbm.at[:, pl.ds(128 * j, 128)], wqkv.at[j]) for j in range(12))))]
    for c in loads:
        c.start()
    high = jnp.uint32(0xFFFF0000)
    halves = lambda t: (pltpu.bitcast(t << 16, F32), pltpu.bitcast(t & high, F32))

    def col(ref):
        v = ref[...].astype(F32).reshape(1, D)
        return jnp.broadcast_to(v, (128, D)).T

    par[0] = jnp.exp(col(ldt_ref))
    par[1] = col(dsk_ref) * (1.0 / L)

    ri = lax.broadcasted_iota(jnp.int32, (128, 128), 0)
    ci = lax.broadcasted_iota(jnp.int32, (128, 128), 1)
    perm[...] = pltpu.bitcast(jnp.where(ci == (ri & 7) * DH + (ri >> 3), 1.0, 0.0).astype(BF16), U32)

    def setup(i):
        get = lambda ref: halves(pltpu.bitcast(ref[_rows(i, 16), :], U32))
        dt = halves(pltpu.bitcast(par[0, _rows(i, 16), :].astype(BF16), U32))

        def pole(h):
            mag, ang = jnp.exp(dt[h] * get(are_ref)[h]), dt[h] * get(aim_ref)[h]
            zw[i, h, 0], zw[i, h, 1] = mag * jnp.cos(ang), mag * jnp.sin(ang)

        def weight():
            scale = (1.0 + 1.5 * 2.0 ** -9) / L
            for h, (cr, ci, br, bi) in enumerate(zip(*map(get, (cre_ref, cim_ref, bre_ref, bim_ref)))):
                wr, wi = _cmul((cr, ci), (dt[h] * br, dt[h] * bi))
                zw[i, h, 2], zw[i, h, 3] = wr * scale, wi * -scale

        return [step(pole, 0), weight, step(pole, 1)]

    lags = sorted({(c, r) for c in range(8) for r in _RND[c] if r < 16}) + [(8, 0)]
    stack = lambda vs: jnp.concatenate([jnp.concatenate([v[k] for v in vs], 0) for k in range(2)], 1).astype(BF16)

    def lagsums(i):
        start = [[zw[i, h, c] for c in range(4)] for h in range(2)]
        zs, rhs, even = [], [], []

        def right(h):
            zr, zi, wr, wi = start[h]
            z = {0: (jnp.ones((8, N), F32), jnp.zeros((8, N), F32)), 1: (zr, zi)}
            for e in (2, 4, 8, 16, 32, 64, 128, 256):
                z[e] = _csq(z[e // 2])
            b = [(wr, wi)]
            for e in (16, 32, 64, 128):
                zc = (z[e][0], -z[e][1])
                b += [_cmul(v, zc) for v in b]
            zs.append(z)
            rhs.append(stack(b))

        def left(t, h):
            z = zs[h]

            def power(e):
                if e not in z:
                    low = e % 256 if e > 256 and e % 256 else e & -e
                    z[e] = _csq(z[e // 2]) if e // 2 in z and e % 2 == 0 else _cmul(power(e - low), power(low))
                return z[e]

            a = [power(256 * c + r) for c, r in (lags + lags[-1:])[CUT[t]:CUT[t + 1]]]
            o = pltpu.bitcast(lax.dot_general(stack(a), rhs[h], NT, preferred_element_type=F32), U32)
            if h:
                lag[i, 8 * CUT[t]:8 * CUT[t + 1], :] = even[t] | (o & high)
            else:
                even.append(o >> 16)

        return [f for h in range(2) for f in [step(right, h)] + [step(left, t, h) for t in range(len(CUT) - 1)]]

    def kgen(i):
        lane = lax.broadcasted_iota(jnp.int32, (8, 128), 1)
        src = (lane & 15) * 8 + lax.broadcasted_iota(jnp.int32, (8, 128), 0)

        memo = {}

        def piece(c, r):
            if r == 16:
                c = 0
            if (c, r) not in memo:
                memo[c, r] = (
                    pltpu.roll(jnp.where(lane == 0, piece(8, 0), merged(0, (0,) * 8)), 127, 1) if r == 16 else
                    jnp.take_along_axis(lag[i, _rows(lags.index((c, r)), 8), :], src, axis=1,
                                        mode="promise_in_bounds"))
            return memo[c, r]

        def merged(c, rs):
            if (c, rs) not in memo:
                memo[c, rs] = (piece(c, rs[0]) if c == 7 or min(rs) == 16 else
                               jnp.where(lane >> 4 == c, piece(c, rs[0]), merged(c + 1, rs[1:])))
            return memo[c, rs]

        for n0 in range(R0):
            kt[n0, _rows(i, 8), :] = merged(0, tuple(_RND[c][n0] for c in range(8)))

    get = lambda ref, n, rows: (ref[n, 0, rows, :], ref[n, 1, rows, :])

    def put(ref, n, rows, v):
        ref[n, 0, rows, :], ref[n, 1, rows, :] = v

    def outer(src, a, rows):
        return [_twiddle(v, a * b) for b, v in enumerate(_dft4([get(src, a + 4 * m, rows) for m in range(4)], 1))]

    def transform(lhs, dst, n0, rows):
        r = jnp.dot(lhs, _bf(fm[n0]), preferred_element_type=F32)
        put(dst, n0, rows, (r[:, :128], r[:, 128:]))

    def kfwd(n0, r):
        for h in (2 * r, 2 * r + 1):
            transform(_bf(kt[n0, _rows(h, 32), :]), ub, n0, _rows(h, 64))

    def kdft(i):
        rows, t = _rows(i, 8), []

        def inner(b):
            for m, v in enumerate(_dft4([t[a][b] for a in range(4)], 1)):
                put(kf, b + 4 * m, rows, (v[0] + par[1, rows, :], v[1]))

        return [lambda a=a: t.append(outer(ub, a, rows)) for a in range(4)] + [step(inner, b) for b in range(4)]

    def fwd(n0, r, n=128):
        transform(un[n0, _rows(r, n), :], ua, n0, _rows(r, n))

    def pre(a, i):
        for b, v in enumerate(outer(ua, a, _rows(i, 8))):
            put(ub, a + 4 * b, _rows(i, 8), v)

    def mid(i):
        first, t = {}, {}

        def inner(h, b):
            rows = _rows(2 * i + h, 8)
            if b == 0:
                first[h] = outer(ua, 0, rows)
            x = _dft4([first[h][b]] + [get(ub, a + 4 * b, rows) for a in range(1, 4)], 1)
            t[h, b], *y = _dft4([_cmul(x[m], get(kf, b + 4 * m, rows)) for m in range(4)], -1)
            for a in range(1, 4):
                put(uc, a + 4 * b, rows, y[a - 1])

        def last():
            for m, (v, w) in enumerate(zip(*[_dft4([t[h, b] for b in range(4)], -1) for h in range(2)])):
                put(yb, 4 * m, _rows(i, 16), [jnp.concatenate([v[k], w[k]], 0).astype(BF16) for k in range(2)])

        return [step(inner, h, b) for h in range(2) for b in range(4)] + [last]

    def post(a, i):
        rows = _rows(i, 16)
        for m, v in enumerate(_dft4([_twiddle(get(uc, a + 4 * b, rows), -a * b) for b in range(4)], -1)):
            put(yb, a + 4 * m, rows, (v[0].astype(BF16), v[1].astype(BF16)))

    def inv(n0, r, n=128):
        rows = _rows(r, n)
        y = jnp.concatenate(get(yb, n0, rows), 1)
        xs[n0, rows, :] = xs[n0, rows, :] + jnp.dot(y, _bf(gm[n0]), preferred_element_type=F32)

    def wprep(g, t):
        if t < 3:
            v = lax.dot_general(_bf(perm[...]), wqkv[4 * t + g], NT, preferred_element_type=F32)
            v = v if t else v * DH ** -0.5
            for k, a in enumerate(_left(v[:64, :256], v[:64, 256:], v[64:, :256], v[64:, 256:])):
                wt[g, k, _rows(t, 32), :] = pltpu.bitcast(a.astype(BF16), U32)
        else:
            v = [jnp.dot(_bf(perm[...]), wo[_rows(e, 128), _rows(g, 128)], preferred_element_type=F32)
                 for e in range(4)]
            lo, hi = (jnp.concatenate([u[64 * h:64 * h + 64] for u in v], 0).T for h in range(2))
            for k, a in enumerate(_left(lo[:64], hi[:64], lo[64:], hi[64:])):
                wot[k, _rows(g, 32), :] = pltpu.bitcast(a.astype(BF16), U32)

    def xin(j, c):
        xs[2 * j, _rows(c, 128), :], xs[2 * j + 1, _rows(c, 128), :] = halves(io[c, pl.ds(j, R1, stride=8), :].T)

    def norm(n0):
        acc, stat = {}, []

        def moment(k, lo, hi):
            for i in range(lo, hi):
                v = xs[n0, 8 * i:8 * i + 8, :]
                v = jnp.square(v - stat[0]) if k else v
                acc[i % 4] = v if i < 4 else acc[i % 4] + v
            if hi == D // 8:
                v = jnp.sum(_tree(jnp.add, list(acc.values())), axis=0, keepdims=True) * (1.0 / D)
                stat.append(lax.rsqrt(v + 1e-5) if k else v)

        def scale(c):
            rows = _rows(c, 128)
            un[n0, rows, :] = get(rows).astype(BF16)

        get = lambda rows: (xs[n0, rows, :] - stat[0]) * stat[1]
        return [[step(moment, 0, 0, 64)], [step(moment, 1, i, i + 16) for i in range(0, 64, 16)],
                [step(scale, c) for c in range(4)]], get

    def norms(*aa):
        return [f for a in aa for stage in zip(*[norm(a + 4 * m)[0] for m in range(4)])
                for steps in stage for f in steps]

    def pair_norms(a):
        stages, get = zip(*[norm(a + 4 * m) for m in range(4)])

        def operands(j, c):
            (b11, b21), (b12, b22) = ((f(_rows(c, 16)), f(_rows(c + 16, 16))) for f in get[2 * j:2 * j + 2])
            for k, b in enumerate(_right(b11, b12, b21, b22)):
                us[2 * a + j, k, _rows(c, 8), :] = pltpu.bitcast(b.astype(BF16), U32)

        return ([f for k in range(2) for st in stages for f in st[k]]
                + [step(operands, j, c) for j in range(2) for c in range(16)])

    def proj(i, slot, m, t):
        p, g, ref = i >> 2, i & 3, (qs, ks, vs)[t][slot]

        def emit(half, j, r):
            ref[m + 2 * j + 7 * (t > 0), _rows(half, 64), :] = r
            if t and m + j:
                ref[m + 2 * j - 1, _rows(half, 64), :] = pltpu.roll(r, 1, 1)

        return _strassen(lambda k: jnp.dot(_bf(wt[g, k, _rows(t, 32), :]), _bf(us[2 * p + 4 * (m & 1) + (m >> 2), k]),
                                           preferred_element_type=F32), emit)

    def attn(i, slot, m0):
        p, g = i >> 2, i & 3
        first = lax.broadcasted_iota(jnp.int32, (8, 128), 1) == 0
        window = lambda ref, d: {e: ref[slot][e, 8 * d:8 * d + 8, :] for e in range(m0, m0 + W + 1)}
        s, o = {}, {}

        def logits(d):
            k = window(ks, d)
            for m in (m0, m0 + 1):
                q = qs[slot][m, 8 * d:8 * d + 8, :]
                for w in range(W):
                    t = q * k[m + 7 - w]
                    s[m, w] = t if d == 0 else s[m, w] + t

        def softmax(m):
            t = [jnp.where(first, -1e9, s[m, w]) if w > m else s[m, w] for w in range(W)]
            mx = _tree(jnp.maximum, t)
            e = [jnp.exp(v - mx) for v in t]
            rs = 1.0 / _tree(jnp.add, e)
            s.update({(m, w): e[w] * rs for w in range(W)})

        def values(d):
            v = window(vs, d)
            for m in (m0, m0 + 1):
                o[m, d] = _tree(jnp.add, [s[m, w] * v[m + 7 - w] for w in range(W)])
            if d % 2 and d > 8:
                blocks = [jnp.concatenate([o[m, e - 1], o[m, e]], 0) for e in (d - 8, d) for m in (m0, m0 + 1)]
                for k, b in enumerate(_right(*blocks)):
                    ob[m0 + p, k, g, 8 * d - 72:8 * d - 56, :] = b.astype(BF16)

        return ([step(logits, d) for d in range(DH)] + [step(softmax, m0), step(softmax, m0 + 1)]
                + [step(values, d + e) for d in range(0, 8, 2) for e in (0, 1, 8, 9)])

    def oproj(p, c, n):
        def pair(m0):
            def emit(half, j, r):
                for i in range(n):
                    at = (2 * (m0 + j) + p, _rows(2 * (c + i) + half, 64))
                    xs[at] = xs[at] + r[64 * i:64 * i + 64]

            return _strassen(lambda k: jnp.dot(_bf(wot[k, 32 * c:32 * (c + n), :]), ob[m0 + p, k].reshape(D // 2, R1),
                                               preferred_element_type=F32), emit)

        return [f for m0 in range(0, 8, 2) for f in pair(m0)]

    def xout(c, j):
        lo, hi = (pltpu.bitcast(xs[2 * j + k, _rows(c, 128), :].astype(BF16).astype(F32), U32) for k in range(2))
        io[c, pl.ds(j, R1, stride=8), :] = ((lo >> 16) | hi).T

    four = lambda fn, *aa: [step(fn, a + 4 * m, r, 64) for a in aa for m in range(4) for r in range(2 * NB)]
    block = lambda fn, a, r: [step(fn, a + 4 * m, 2 * r + h, 64) for h in range(2) for m in range(4)] if 0 <= r < NB else []
    rowwise = lambda fn, a, n: [step(fn, a, i) for i in range(D // n)]

    regions, zero = [], zero_ref[0]

    def slot(*streams):
        regions.append(None)
        pl.when(zero < len(regions))(lambda: _run(*streams))

    pres = lambda a: rowwise(pre, a, 8)
    posts = lambda a: rowwise(post, a, 16)
    projs = lambda i, s, ms: [f for t in (1, 2, 0) for m in ms for f in proj(i, s, m, t)]
    attns = lambda i, s: [f for m in range(0, 8, 2) for f in attn(i, s, m)]

    with jax.named_scope("kgen"):
        ng = D // 16 // KPER
        each = lambda fn: (lambda i: [f for k in range(KPER) for f in fn(KPER * i + k)])
        _pipeline([(lambda i: [lambda: [kgen(KPER * i + k) for k in range(KPER)]], 2, ng - 1),
                   (each(lagsums), 1, ng), (each(setup), 0, ng),
                   (lambda j: [step(xin, 2 * j + k, c) for k in range(2) for c in range(NB)], ng - 4, 4)],
                  {ng - 4: lambda: [c.wait() for c in loads[:NB]]})
    with jax.named_scope("kfwd"):
        for c in loads[NB:]:
            c.wait()
        kdfts = lambda r: [f for i in range(16) for f in kdft(16 * r + i)]
        for r, other in enumerate((norms(2, 1), *[sum(norm(n0)[0], []) for n0 in (3, 7)],
                                   sum(norm(11)[0] + norm(15)[0], []))):
            slot([f for k in range(4) for f in [step(wprep, r, k)] + [step(kfwd, 4 * k + n, r) for n in range(4)]],
                 kdfts(r - 1) if r else [step(kgen, D // 16 - 1 - k) for k in range(KPER)], other)
        slot(four(fwd, 2), kdfts(NB - 1))
        slot(four(fwd, 1) + block(fwd, 3, 0), pres(2), norms(0))

    def layer(li, carry):
        with jax.named_scope("conv"):
            part = lambda steps, r: steps[len(steps) * r // NB:len(steps) * (r + 1) // NB] if 0 <= r < NB else []
            mids = [f for i in range(D // 16) for f in mid(i)]
            for r in range(-1, NB + 1):
                slot(block(fwd, 3, r + 2) + block(fwd, 0, r + 1) + block(inv, 0, r - 1) + block(inv, 2, r - 2)
                     + block(inv, 1, r - 2),
                     part(mids, r), part(pres(3), r + 1) + part(posts(2), r - 1) + part(posts(1), r - 1),
                     pres(1) if r < 0 else posts(3) if r == NB else [])
            slot(block(inv, 2, NB - 1) + block(inv, 1, NB - 1) + four(inv, 3), pair_norms(0))
            slot(projs(0, 0, (0, 4)), pair_norms(2))
            slot(projs(0, 0, (1, 5)), pair_norms(1))
        with jax.named_scope("attn"):
            slot(projs(1, 1, (0, 1, 4, 5)), attns(0, 0), pair_norms(3))
            both = lambda i, s: slot(projs(i + 1, 1 - s, (0, 1, 4, 5)), attns(i, s))
            lax.fori_loop(0, 3, lambda j, c: (both(2 * j + 1, 1), both(2 * j + 2, 0), c)[-1], 0)
            slot(oproj(0, 0, 2) + oproj(0, 2, 2), attns(7, 1))

        @pl.when(li == 0)
        def _():
            slot(oproj(1, 0, 2) + oproj(1, 2, 2), norms(2, 0))
            slot(four(fwd, 2), norms(1, 3))
            slot(four(fwd, 1) + block(fwd, 3, 0), pres(2))

        return carry

    lax.fori_loop(0, 2, layer, 0)

    with jax.named_scope("xout"):
        stores = [pltpu.make_async_copy(io.at[c, pl.ds(0, L // 2)],
                                        out_hbm.bitcast(U32).at[:, pl.ds(c * 128, 128)], sems.at[c])
                  for c in range(NB)]
        for c in range(NB + 1):
            outs = [step(xout, *divmod(j, 8)) if 0 <= j < 8 * NB else (lambda: None)
                    for j in range(8 * c - 2, 8 * c + 6)]
            slot(oproj(1, c, 1) if c < NB else [], outs)
            if c:
                stores[c - 1].start()
        for c in stores:
            c.wait()


@jax.jit
def pallas_interleave_layers__ssm_conv_s4__sliding_local_dilated__prompt_kernel(
    A_u: jax.Array,
    A_A_re: jax.Array,
    A_A_im: jax.Array,
    A_B_re: jax.Array,
    A_B_im: jax.Array,
    A_C_re: jax.Array,
    A_C_im: jax.Array,
    A_log_dt: jax.Array,
    A_Dskip: jax.Array,
    B_x: jax.Array,
    B_wqkv: jax.Array,
    B_wo: jax.Array,
):
    del B_x
    hbm, vmem = pl.BlockSpec(memory_space=pl.ANY), pl.BlockSpec(memory_space=pltpu.VMEM)
    tiles = lambda *n: pltpu.VMEM((*n, 128, 128), F32)
    out = pl.pallas_call(
        _kernel,
        out_shape=jax.ShapeDtypeStruct((L, D), BF16),
        in_specs=[pl.BlockSpec(memory_space=pltpu.SMEM), hbm] + [vmem] * 8 + [hbm] * 4,
        out_specs=hbm,
        scratch_shapes=[
            pltpu.VMEM((R0, D, R1), F32),
            *[pltpu.VMEM((R0, 2, D, R1), F32)] * 4,
            pltpu.VMEM((R0, 2, D, R1), BF16),
            pltpu.VMEM((2, D, N), F32),
            pltpu.VMEM((D // 16, 2, 4, 8, N), F32),
            pltpu.VMEM((D // 16, 336, 128), U32),
            *[tiles(n) for n in (8, 15, 15) * 2],
            pltpu.VMEM((NB, L // 2 + 8, 128), U32),
            pltpu.VMEM((64, 128), U32),
            pltpu.VMEM((12, D, 128), BF16),
            pltpu.VMEM((D, D), BF16),
            pltpu.VMEM(_F.shape, U32),
            pltpu.VMEM(_G.shape, U32),
            pltpu.VMEM((R0, D // 2, R1), U32),
            pltpu.VMEM((R0, D, R1), BF16),
            pltpu.VMEM((4, 7, 96, D // 2), U32),
            pltpu.VMEM((8, 7, D // 4, R1), U32),
            pltpu.VMEM((7, D // 4, D // 2), U32),
            pltpu.VMEM((8, 7, 4, 64, R1), BF16),
            pltpu.SemaphoreType.DMA((19,)),
        ],
        compiler_params=pltpu.CompilerParams(vmem_limit_bytes=100 * 1024 * 1024),
    )(np.zeros((2,), np.int32), A_u.reshape(L, D), A_A_re, A_A_im, A_B_re, A_B_im, A_C_re, A_C_im, A_log_dt, A_Dskip,
      B_wqkv, B_wo, _F, _G)
    return out.reshape(1, L, D)
```

```python
import jax
import jax.numpy as jnp
import ml_dtypes
import numpy as np
from jax import lax
import jax.experimental.pallas as pl
import jax.experimental.pallas.tpu as pltpu

L, D, N = 2048, 512, 128
R0, R1 = 16, 128
W, DH = 8, 16
F32, BF16, U32 = jnp.float32, jnp.bfloat16, jnp.uint32
CUT = (0, 20, 42)
KPER = 4
NB = D // 128
NT = (((1,), (1,)), ((), ()))


def _constants():
    n0 = np.arange(R0)[:, None, None]
    n1 = np.arange(R1)[None, :, None]
    k1 = np.arange(R1)[None, None, :]
    ang = 2.0 * np.pi * (k1 + 0.25) * (R0 * n1 + n0) / L
    f = np.concatenate([np.cos(ang), np.sin(ang)], axis=2)
    g = f.transpose(0, 2, 1)
    bf = ml_dtypes.bfloat16
    lr = np.arange(L).astype(np.float32).astype(bf).astype(np.int64).reshape(8, 16, R0)
    r = lr - (256 * np.arange(8)[:, None, None] + 16 * np.arange(16)[None, :, None])
    assert (r == r[:, :1, :]).all()

    def words(m):
        h = np.ascontiguousarray(m).astype(bf).view(np.uint16).astype(np.uint32)
        return h[:, 0::2] | (h[:, 1::2] << 16)

    return words(f), words(g), r[:, 0, :].tolist()


_F, _G, _RND = _constants()


def _cmul(a, b):
    return a[0] * b[0] - a[1] * b[1], a[0] * b[1] + a[1] * b[0]


def _csq(a):
    t = a[0] * a[1]
    return (a[0] + a[1]) * (a[0] - a[1]), t + t


def _dft4(x, sign):
    (ar, ai), (br, bi), (cr, ci), (dr, di) = x
    sr, si, tr, ti = ar + cr, ai + ci, ar - cr, ai - ci
    ur, ui, vr, vi = br + dr, bi + di, br - dr, bi - di
    p, m = (tr - vi, ti + vr), (tr + vi, ti - vr)
    if sign < 0:
        p, m = m, p
    return [(sr + ur, si + ui), p, (sr - ur, si - ui), m]


def _twiddle(v, e):
    e %= 16
    re, im = v
    h = float(np.sqrt(0.5))
    if e == 0:
        return v
    if e == 4:
        return -im, re
    if e == 12:
        return im, -re
    if e == 2:
        return (re - im) * h, (re + im) * h
    if e == 14:
        return (re + im) * h, (im - re) * h
    if e == 6:
        return (re + im) * -h, (re - im) * h
    if e == 10:
        return (im - re) * h, (re + im) * -h
    c, s = float(np.cos(np.pi * e / 8)), float(np.sin(np.pi * e / 8))
    return re * c - im * s, re * s + im * c


def _bf(x):
    return pltpu.bitcast(x, BF16)


def _tree(op, v):
    while len(v) > 1:
        v = [op(v[i], v[i + 1]) if i + 1 < len(v) else v[i] for i in range(0, len(v), 2)]
    return v[0]


def _run(*streams):
    order = sorted(((i + 0.5 * (k > 0)) / len(s), k, i) for k, s in enumerate(streams) for i in range(len(s)))
    for _, k, i in order:
        streams[k][i]()


def _pipeline(streams, hooks=None):
    hooks = hooks or {}
    cuts = sorted({e for _, a, n in streams for e in (a, a + n)} | set(hooks))
    for lo, hi in zip(cuts, cuts[1:]):
        def body(s, carry, lo=lo):
            _run(*[fn(s - a) for fn, a, n in streams if a <= lo < a + n])
            return carry

        if lo in hooks:
            hooks[lo]()
        if hi - lo == 1:
            body(lo, 0)
        else:
            lax.fori_loop(lo, hi, body, 0)


def _left(a11, a12, a21, a22):
    return a21 + a22, a22, a11 + a22, a12 - a22, a11 + a12, a11, a21 - a11


def _right(b11, b12, b21, b22):
    return b11, b21 - b11, b11 + b22, b21 + b22, b22, b12 - b22, b11 + b12


def _strassen(product, emit):
    c = {}

    def run(k):
        c[k] = r = product(k)
        if k == 1:
            emit(1, 0, c[0] + r)
        elif k == 2:
            c[11], c[22] = r + c[1], r - c[0]
        elif k == 3:
            c[11] = c[11] + r
        elif k == 4:
            emit(0, 0, c[11] - r)
        elif k == 5:
            emit(0, 1, c[4] + r)
            c[22] = c[22] + r
        elif k == 6:
            emit(1, 1, c[22] + r)

    return [lambda k=k: run(k) for k in range(7)]


def _rows(i, n):
    return pl.ds(i * n if isinstance(i, int) else pl.multiple_of(i * n, n), n)


def _kernel(zero_ref, x_hbm, are_ref, aim_ref, bre_ref, bim_ref, cre_ref, cim_ref, ldt_ref, dsk_ref,
            wqkv_hbm, wo_hbm, f_hbm, g_hbm, out_hbm,
            xs, kf, ua, ub, uc, yb, par, zw, lag, qa, ka, va, qb, kb, vb, io, perm, wqkv, wo, fm, gm, kt, un, wt, us, wot, ob, sems):
    step = lambda fn, *a: (lambda: fn(*a))
    qs, ks, vs = (qa, qb), (ka, kb), (va, vb)
    loads = [pltpu.make_async_copy(s, d, sems.at[i]) for i, (s, d) in enumerate(
        (*((x_hbm.bitcast(U32).at[:, pl.ds(128 * c, 128)], io.at[c, pl.ds(0, L // 2)]) for c in range(NB)),
         (f_hbm, fm), (wo_hbm, wo), (g_hbm, gm),
         *((wqkv_hbm.at[:, pl.ds(128 * j, 128)], wqkv.at[j]) for j in range(12))))]
    for c in loads:
        c.start()
    high = jnp.uint32(0xFFFF0000)
    halves = lambda t: (pltpu.bitcast(t << 16, F32), pltpu.bitcast(t & high, F32))

    def col(ref):
        v = ref[...].astype(F32).reshape(1, D)
        return jnp.broadcast_to(v, (128, D)).T

    par[0] = jnp.exp(col(ldt_ref))
    par[1] = col(dsk_ref) * (1.0 / L)

    ri = lax.broadcasted_iota(jnp.int32, (128, 128), 0)
    ci = lax.broadcasted_iota(jnp.int32, (128, 128), 1)
    perm[...] = pltpu.bitcast(jnp.where(ci == (ri & 7) * DH + (ri >> 3), 1.0, 0.0).astype(BF16), U32)

    def setup(i):
        get = lambda ref: halves(pltpu.bitcast(ref[_rows(i, 16), :], U32))
        dt = halves(pltpu.bitcast(par[0, _rows(i, 16), :].astype(BF16), U32))

        def pole(h):
            mag, ang = jnp.exp(dt[h] * get(are_ref)[h]), dt[h] * get(aim_ref)[h]
            zw[i, h, 0], zw[i, h, 1] = mag * jnp.cos(ang), mag * jnp.sin(ang)

        def weight():
            scale = (1.0 + 1.5 * 2.0 ** -9) / L
            for h, (cr, ci, br, bi) in enumerate(zip(*map(get, (cre_ref, cim_ref, bre_ref, bim_ref)))):
                wr, wi = _cmul((cr, ci), (dt[h] * br, dt[h] * bi))
                zw[i, h, 2], zw[i, h, 3] = wr * scale, wi * -scale

        return [step(pole, 0), weight, step(pole, 1)]

    lags = sorted({(c, r) for c in range(8) for r in _RND[c] if r < 16}) + [(8, 0)]
    stack = lambda vs: jnp.concatenate([jnp.concatenate([v[k] for v in vs], 0) for k in range(2)], 1).astype(BF16)

    def lagsums(i):
        start = [[zw[i, h, c] for c in range(4)] for h in range(2)]
        zs, rhs, even = [], [], []

        def right(h):
            zr, zi, wr, wi = start[h]
            z = {0: (jnp.ones((8, N), F32), jnp.zeros((8, N), F32)), 1: (zr, zi)}
            for e in (2, 4, 8, 16, 32, 64, 128, 256):
                z[e] = _csq(z[e // 2])
            b = [(wr, wi)]
            for e in (16, 32, 64, 128):
                zc = (z[e][0], -z[e][1])
                b += [_cmul(v, zc) for v in b]
            zs.append(z)
            rhs.append(stack(b))

        def left(t, h):
            z = zs[h]

            def power(e):
                if e not in z:
                    low = e % 256 if e > 256 and e % 256 else e & -e
                    z[e] = _csq(z[e // 2]) if e // 2 in z and e % 2 == 0 else _cmul(power(e - low), power(low))
                return z[e]

            a = [power(256 * c + r) for c, r in (lags + lags[-1:])[CUT[t]:CUT[t + 1]]]
            o = pltpu.bitcast(lax.dot_general(stack(a), rhs[h], NT, preferred_element_type=F32), U32)
            if h:
                lag[i, 8 * CUT[t]:8 * CUT[t + 1], :] = even[t] | (o & high)
            else:
                even.append(o >> 16)

        return [f for h in range(2) for f in [step(right, h)] + [step(left, t, h) for t in range(len(CUT) - 1)]]

    def kgen(i):
        lane = lax.broadcasted_iota(jnp.int32, (8, 128), 1)
        src = (lane & 15) * 8 + lax.broadcasted_iota(jnp.int32, (8, 128), 0)

        memo = {}

        def piece(c, r):
            if r == 16:
                c = 0
            if (c, r) not in memo:
                memo[c, r] = (
                    pltpu.roll(jnp.where(lane == 0, piece(8, 0), merged(0, (0,) * 8)), 127, 1) if r == 16 else
                    jnp.take_along_axis(lag[i, _rows(lags.index((c, r)), 8), :], src, axis=1,
                                        mode="promise_in_bounds"))
            return memo[c, r]

        def merged(c, rs):
            if (c, rs) not in memo:
                memo[c, rs] = (piece(c, rs[0]) if c == 7 or min(rs) == 16 else
                               jnp.where(lane >> 4 == c, piece(c, rs[0]), merged(c + 1, rs[1:])))
            return memo[c, rs]

        for n0 in range(R0):
            kt[n0, _rows(i, 8), :] = merged(0, tuple(_RND[c][n0] for c in range(8)))

    get = lambda ref, n, rows: (ref[n, 0, rows, :], ref[n, 1, rows, :])

    def put(ref, n, rows, v):
        ref[n, 0, rows, :], ref[n, 1, rows, :] = v

    def outer(src, a, rows):
        return [_twiddle(v, a * b) for b, v in enumerate(_dft4([get(src, a + 4 * m, rows) for m in range(4)], 1))]

    def transform(lhs, dst, n0, rows):
        r = jnp.dot(lhs, _bf(fm[n0]), preferred_element_type=F32)
        put(dst, n0, rows, (r[:, :128], r[:, 128:]))

    def kfwd(n0, r):
        transform(_bf(kt[n0, _rows(r, 32), :]), ub, n0, _rows(r, 64))

    def kdft(i):
        rows, t = _rows(i, 8), []

        def inner(b):
            for m, v in enumerate(_dft4([t[a][b] for a in range(4)], 1)):
                put(kf, b + 4 * m, rows, (v[0] + par[1, rows, :], v[1]))

        return [lambda a=a: t.append(outer(ub, a, rows)) for a in range(4)] + [step(inner, b) for b in range(4)]

    def fwd(n0, r):
        transform(un[n0, _rows(r, 64), :], ua, n0, _rows(r, 64))

    def pre(a, i):
        for b, v in enumerate(outer(ua, a, _rows(i, 8))):
            put(ub, a + 4 * b, _rows(i, 8), v)

    def mid(i):
        first, t = {}, {}

        def inner(h, b):
            rows = _rows(2 * i + h, 8)
            if b == 0:
                first[h] = outer(ua, 0, rows)
            x = _dft4([first[h][b]] + [get(ub, a + 4 * b, rows) for a in range(1, 4)], 1)
            t[h, b], *y = _dft4([_cmul(x[m], get(kf, b + 4 * m, rows)) for m in range(4)], -1)
            for a in range(1, 4):
                put(uc, a + 4 * b, rows, y[a - 1])

        def last():
            for m, (v, w) in enumerate(zip(*[_dft4([t[h, b] for b in range(4)], -1) for h in range(2)])):
                put(yb, 4 * m, _rows(i, 16), [jnp.concatenate([v[k], w[k]], 0).astype(BF16) for k in range(2)])

        return [step(inner, h, b) for h in range(2) for b in range(4)] + [last]

    def post(a, i):
        rows = _rows(i, 16)
        for m, v in enumerate(_dft4([_twiddle(get(uc, a + 4 * b, rows), -a * b) for b in range(4)], -1)):
            put(yb, a + 4 * m, rows, (v[0].astype(BF16), v[1].astype(BF16)))

    def inv(n0, r):
        rows = _rows(r, 64)
        y = jnp.concatenate(get(yb, n0, rows), 1)
        xs[n0, rows, :] = xs[n0, rows, :] + jnp.dot(y, _bf(gm[n0]), preferred_element_type=F32)

    def wprep(g, t):
        ops = []

        def load():
            if t < 3:
                v = lax.dot_general(_bf(perm[...]), wqkv[4 * t + g], NT, preferred_element_type=F32)
                v = v if t else v * DH ** -0.5
                lo, hi = v[:, :256], v[:, 256:]
            else:
                v = [jnp.dot(_bf(perm[...]), wo[_rows(e, 128), _rows(g, 128)], preferred_element_type=F32)
                     for e in range(4)]
                lo, hi = (jnp.concatenate([u[64 * h:64 * h + 64] for u in v], 0).T for h in range(2))
            ops.extend((lo[:64], hi[:64], lo[64:], hi[64:]))

        def save(i, h):
            for k, a in enumerate(_left(*[v[16 * i:16 * i + 16, 128 * h:128 * h + 128] for v in ops])):
                dst = wt.at[g, k] if t < 3 else wot.at[k]
                dst[_rows(4 * (t if t < 3 else g) + i, 8), _rows(h, 128)] = pltpu.bitcast(a.astype(BF16), U32)

        return [load] + [step(save, i, h) for i in range(4) for h in range(2)]

    def xin(j, c):
        xs[2 * j, _rows(c, 128), :], xs[2 * j + 1, _rows(c, 128), :] = halves(io[c, pl.ds(j, R1, stride=8), :].T)

    def norm(n0):
        acc, stat = {}, []

        def moment(k, lo, hi):
            for i in range(lo, hi):
                v = xs[n0, 8 * i:8 * i + 8, :]
                v = jnp.square(v - stat[0]) if k else v
                acc[i % 4] = v if i < 4 else acc[i % 4] + v
            if hi == D // 8:
                v = jnp.sum(_tree(jnp.add, list(acc.values())), axis=0, keepdims=True) * (1.0 / D)
                stat.append(lax.rsqrt(v + 1e-5) if k else v)

        def scale(c):
            rows = _rows(c, 128)
            un[n0, rows, :] = get(rows).astype(BF16)

        get = lambda rows: (xs[n0, rows, :] - stat[0]) * stat[1]
        return [[step(moment, 0, 0, 64)], [step(moment, 1, i, i + 16) for i in range(0, 64, 16)],
                [step(scale, c) for c in range(4)]], get

    def norms(*aa):
        return [f for a in aa for stage in zip(*[norm(a + 4 * m)[0] for m in range(4)])
                for steps in stage for f in steps]

    def pair_norms(a):
        stages, get = zip(*[norm(a + 4 * m) for m in range(4)])

        def operands(j, c):
            (b11, b21), (b12, b22) = ((f(_rows(c, 16)), f(_rows(c + 16, 16))) for f in get[2 * j:2 * j + 2])
            for k, b in enumerate(_right(b11, b12, b21, b22)):
                us[2 * a + j, k, _rows(c, 8), :] = pltpu.bitcast(b.astype(BF16), U32)

        return ([f for k in range(2) for st in stages for f in st[k]]
                + [step(operands, j, c) for j in range(2) for c in range(16)])

    def proj(i, slot, m, t):
        p, g, ref = i >> 2, i & 3, (qs, ks, vs)[t][slot]

        def emit(half, j, r):
            ref[m + 2 * j + 7 * (t > 0), _rows(half, 64), :] = r
            if t and m + j:
                ref[m + 2 * j - 1, _rows(half, 64), :] = pltpu.roll(r, 1, 1)

        return _strassen(lambda k: jnp.dot(_bf(wt[g, k, _rows(t, 32), :]), _bf(us[2 * p + 4 * (m & 1) + (m >> 2), k]),
                                           preferred_element_type=F32), emit)

    def attn(i, slot, m0):
        p, g = i >> 2, i & 3
        first = lax.broadcasted_iota(jnp.int32, (8, 128), 1) == 0
        window = lambda ref, d: {e: ref[slot][e, 8 * d:8 * d + 8, :] for e in range(m0, m0 + W + 1)}
        s, o = {}, {}

        def logits(m, d0):
            for d in (d0, d0 + 1):
                k = window(ks, d)
                q = qs[slot][m, 8 * d:8 * d + 8, :]
                for w in range(W):
                    t = q * k[m + 7 - w]
                    s[m, w] = t if d == 0 else s[m, w] + t

        def softmax(m):
            t = [jnp.where(first, -1e9, s[m, w]) if w > m else s[m, w] for w in range(W)]
            mx = _tree(jnp.maximum, t)
            e = [jnp.exp(v - mx) for v in t]
            rs = 1.0 / _tree(jnp.add, e)
            s.update({(m, w): e[w] * rs for w in range(W)})

        def values(d):
            v = window(vs, d)
            for m in (m0, m0 + 1):
                o[m, d] = _tree(jnp.add, [s[m, w] * v[m + 7 - w] for w in range(W)])
            if d % 2 and d > 8:
                blocks = [jnp.concatenate([o[m, e - 1], o[m, e]], 0) for e in (d - 8, d) for m in (m0, m0 + 1)]
                for k, b in enumerate(_right(*blocks)):
                    ob[m0 + p, k, g, 8 * d - 72:8 * d - 56, :] = b.astype(BF16)

        return ([f for m in (m0, m0 + 1) for f in [step(logits, m, d) for d in range(0, DH, 2)] + [step(softmax, m)]]
                + [step(values, d + e) for d in range(0, 8, 2) for e in (0, 1, 8, 9)])

    def oproj(p, c, n):
        def pair(m0):
            def emit(half, j, r):
                for i in range(n):
                    at = (2 * (m0 + j) + p, _rows(2 * (c + i) + half, 64))
                    xs[at] = xs[at] + r[64 * i:64 * i + 64]

            return _strassen(lambda k: jnp.dot(_bf(wot[k, 32 * c:32 * (c + n), :]), ob[m0 + p, k].reshape(D // 2, R1),
                                               preferred_element_type=F32), emit)

        return [f for m0 in range(0, 8, 2) for f in pair(m0)]

    def xout(c, j):
        lo, hi = (pltpu.bitcast(xs[2 * j + k, _rows(c, 128), :].astype(BF16).astype(F32), U32) for k in range(2))
        io[c, pl.ds(j, R1, stride=8), :] = ((lo >> 16) | hi).T

    four = lambda fn, *aa: [step(fn, a + 4 * m, r) for a in aa for m in range(4) for r in range(2 * NB)]
    block = lambda fn, a, r: [step(fn, a + 4 * m, 2 * r + h) for h in range(2) for m in range(4)] if 0 <= r < NB else []
    rowwise = lambda fn, a, n: [step(fn, a, i) for i in range(D // n)]

    regions, zero = [], zero_ref[0]

    def slot(*streams):
        regions.append(None)
        pl.when(zero < len(regions))(lambda: _run(*streams))

    pres = lambda a: rowwise(pre, a, 8)
    posts = lambda a: rowwise(post, a, 16)
    projs = lambda i, s, ms: [f for t in (1, 2, 0) for m in ms for f in proj(i, s, m, t)]
    attns = lambda i, s: [f for m in range(0, 8, 2) for f in attn(i, s, m)]

    with jax.named_scope("kgen"):
        ng = D // 16 // KPER
        each = lambda fn: (lambda i: [f for k in range(KPER) for f in fn(KPER * i + k)])
        _pipeline([(lambda i: [lambda: [kgen(KPER * i + k) for k in range(KPER)]], 2, ng - 1),
                   (each(lagsums), 1, ng), (each(setup), 0, ng),
                   (lambda j: [step(xin, 2 * j + k, c) for k in range(2) for c in range(NB)], ng - 4, 4)],
                  {ng - 4: lambda: [c.wait() for c in loads[:NB]]})
    with jax.named_scope("kfwd"):
        for c in loads[NB:]:
            c.wait()
        kdfts = lambda r: [f for i in range(16) for f in kdft(16 * r + i)]
        for r, other in enumerate((norms(2, 1), *[sum(norm(n0)[0], []) for n0 in (3, 7)],
                                   sum(norm(11)[0] + norm(15)[0], []))):
            slot([f for a in range(4) for f in block(kfwd, a, r)], [f for t in (3, 0, 1, 2) for f in wprep(r, t)],
                 kdfts(r - 1) if r else [step(kgen, D // 16 - 1 - k) for k in range(KPER)], other)
        slot(four(fwd, 2), kdfts(NB - 1))
        slot(four(fwd, 1) + block(fwd, 3, 0), pres(2), norms(0))

    def layer(li, carry):
        with jax.named_scope("conv"):
            part = lambda steps, r: steps[len(steps) * r // NB:len(steps) * (r + 1) // NB] if 0 <= r < NB else []
            mids = [f for i in range(D // 16) for f in mid(i)]
            for r in range(-1, NB + 1):
                slot(block(fwd, 3, r + 2) + block(fwd, 0, r + 1) + block(inv, 0, r - 1) + block(inv, 2, r - 2)
                     + block(inv, 1, r - 2),
                     part(mids, r), part(pres(3), r + 1) + part(posts(2), r - 1) + part(posts(1), r - 1),
                     pres(1) if r < 0 else posts(3) if r == NB else [])
            slot(block(inv, 2, NB - 1) + block(inv, 1, NB - 1) + four(inv, 3), pair_norms(0))
            slot(projs(0, 0, (0, 4)), pair_norms(2))
            slot(projs(0, 0, (1, 5)), pair_norms(1))
        with jax.named_scope("attn"):
            slot(projs(1, 1, (0, 1, 4, 5)), attns(0, 0), pair_norms(3))
            both = lambda i, s: slot(projs(i + 1, 1 - s, (0, 1, 4, 5)), attns(i, s))
            lax.fori_loop(0, 3, lambda j, c: (both(2 * j + 1, 1), both(2 * j + 2, 0), c)[-1], 0)
            slot(oproj(0, 0, 2) + oproj(0, 2, 2), attns(7, 1))

        @pl.when(li == 0)
        def _():
            slot(oproj(1, 0, 2) + oproj(1, 2, 2), norms(2, 0))
            slot(four(fwd, 2), norms(1, 3))
            slot(four(fwd, 1) + block(fwd, 3, 0), pres(2))

        return carry

    lax.fori_loop(0, 2, layer, 0)

    with jax.named_scope("xout"):
        stores = [pltpu.make_async_copy(io.at[c, pl.ds(0, L // 2)],
                                        out_hbm.bitcast(U32).at[:, pl.ds(c * 128, 128)], sems.at[c])
                  for c in range(NB)]
        for c in range(NB + 1):
            outs = [step(xout, *divmod(j, 8)) if 0 <= j < 8 * NB else (lambda: None)
                    for j in range(8 * c - 2, 8 * c + 6)]
            slot(oproj(1, c, 1) if c < NB else [], outs)
            if c:
                stores[c - 1].start()
        for c in stores:
            c.wait()


@jax.jit
def pallas_interleave_layers__ssm_conv_s4__sliding_local_dilated__prompt_kernel(
    A_u: jax.Array,
    A_A_re: jax.Array,
    A_A_im: jax.Array,
    A_B_re: jax.Array,
    A_B_im: jax.Array,
    A_C_re: jax.Array,
    A_C_im: jax.Array,
    A_log_dt: jax.Array,
    A_Dskip: jax.Array,
    B_x: jax.Array,
    B_wqkv: jax.Array,
    B_wo: jax.Array,
):
    del B_x
    hbm, vmem = pl.BlockSpec(memory_space=pl.ANY), pl.BlockSpec(memory_space=pltpu.VMEM)
    tiles = lambda *n: pltpu.VMEM((*n, 128, 128), F32)
    out = pl.pallas_call(
        _kernel,
        out_shape=jax.ShapeDtypeStruct((L, D), BF16),
        in_specs=[pl.BlockSpec(memory_space=pltpu.SMEM), hbm] + [vmem] * 8 + [hbm] * 4,
        out_specs=hbm,
        scratch_shapes=[
            pltpu.VMEM((R0, D, R1), F32),
            *[pltpu.VMEM((R0, 2, D, R1), F32)] * 4,
            pltpu.VMEM((R0, 2, D, R1), BF16),
            pltpu.VMEM((2, D, N), F32),
            pltpu.VMEM((D // 16, 2, 4, 8, N), F32),
            pltpu.VMEM((D // 16, 336, 128), U32),
            *[tiles(n) for n in (8, 15, 15) * 2],
            pltpu.VMEM((NB, L // 2 + 8, 128), U32),
            pltpu.VMEM((64, 128), U32),
            pltpu.VMEM((12, D, 128), BF16),
            pltpu.VMEM((D, D), BF16),
            pltpu.VMEM(_F.shape, U32),
            pltpu.VMEM(_G.shape, U32),
            pltpu.VMEM((R0, D // 2, R1), U32),
            pltpu.VMEM((R0, D, R1), BF16),
            pltpu.VMEM((4, 7, 96, D // 2), U32),
            pltpu.VMEM((8, 7, D // 4, R1), U32),
            pltpu.VMEM((7, D // 4, D // 2), U32),
            pltpu.VMEM((8, 7, 4, 64, R1), BF16),
            pltpu.SemaphoreType.DMA((19,)),
        ],
        compiler_params=pltpu.CompilerParams(vmem_limit_bytes=100 * 1024 * 1024),
    )(np.zeros((2,), np.int32), A_u.reshape(L, D), A_A_re, A_A_im, A_B_re, A_B_im, A_C_re, A_C_im, A_log_dt, A_Dskip,
      B_wqkv, B_wo, _F, _G)
    return out.reshape(1, L, D)
```

```python
import jax
import jax.numpy as jnp
import ml_dtypes
import numpy as np
from jax import lax
import jax.experimental.pallas as pl
import jax.experimental.pallas.tpu as pltpu

L, D, N = 2048, 512, 128
R0, R1 = 16, 128
W, DH = 8, 16
F32, BF16, U32 = jnp.float32, jnp.bfloat16, jnp.uint32
CUT = (0, 20, 42)
KPER = 4
NB = D // 128
NT = (((1,), (1,)), ((), ()))


def _constants():
    n0 = np.arange(R0)[:, None, None]
    n1 = np.arange(R1)[None, :, None]
    k1 = np.arange(R1)[None, None, :]
    ang = 2.0 * np.pi * (k1 + 0.25) * (R0 * n1 + n0) / L
    f = np.concatenate([np.cos(ang), np.sin(ang)], axis=2)
    g = f.transpose(0, 2, 1)
    bf = ml_dtypes.bfloat16
    lr = np.arange(L).astype(np.float32).astype(bf).astype(np.int64).reshape(8, 16, R0)
    r = lr - (256 * np.arange(8)[:, None, None] + 16 * np.arange(16)[None, :, None])
    assert (r == r[:, :1, :]).all()

    def words(m):
        h = np.ascontiguousarray(m).astype(bf).view(np.uint16).astype(np.uint32)
        return h[:, 0::2] | (h[:, 1::2] << 16)

    return words(f), words(g), r[:, 0, :].tolist()


_F, _G, _RND = _constants()


def _cmul(a, b):
    return a[0] * b[0] - a[1] * b[1], a[0] * b[1] + a[1] * b[0]


def _csq(a):
    t = a[0] * a[1]
    return (a[0] + a[1]) * (a[0] - a[1]), t + t


def _dft4(x, sign):
    (ar, ai), (br, bi), (cr, ci), (dr, di) = x
    sr, si, tr, ti = ar + cr, ai + ci, ar - cr, ai - ci
    ur, ui, vr, vi = br + dr, bi + di, br - dr, bi - di
    p, m = (tr - vi, ti + vr), (tr + vi, ti - vr)
    if sign < 0:
        p, m = m, p
    return [(sr + ur, si + ui), p, (sr - ur, si - ui), m]


def _twiddle(v, e):
    e %= 16
    re, im = v
    h = float(np.sqrt(0.5))
    if e == 0:
        return v
    if e == 4:
        return -im, re
    if e == 12:
        return im, -re
    if e == 2:
        return (re - im) * h, (re + im) * h
    if e == 14:
        return (re + im) * h, (im - re) * h
    if e == 6:
        return (re + im) * -h, (re - im) * h
    if e == 10:
        return (im - re) * h, (re + im) * -h
    c, s = float(np.cos(np.pi * e / 8)), float(np.sin(np.pi * e / 8))
    return re * c - im * s, re * s + im * c


def _bf(x):
    return pltpu.bitcast(x, BF16)


def _tree(op, v):
    while len(v) > 1:
        v = [op(v[i], v[i + 1]) if i + 1 < len(v) else v[i] for i in range(0, len(v), 2)]
    return v[0]


def _run(*streams):
    order = sorted(((i + 0.5 * (k > 0)) / len(s), k, i) for k, s in enumerate(streams) for i in range(len(s)))
    for _, k, i in order:
        streams[k][i]()


def _pipeline(streams, hooks=None):
    hooks = hooks or {}
    cuts = sorted({e for _, a, n in streams for e in (a, a + n)} | set(hooks))
    for lo, hi in zip(cuts, cuts[1:]):
        def body(s, carry, lo=lo):
            _run(*[fn(s - a) for fn, a, n in streams if a <= lo < a + n])
            return carry

        if lo in hooks:
            hooks[lo]()
        if hi - lo == 1:
            body(lo, 0)
        else:
            lax.fori_loop(lo, hi, body, 0)


def _left(a11, a12, a21, a22):
    return a21 + a22, a22, a11 + a22, a12 - a22, a11 + a12, a11, a21 - a11


def _right(b11, b12, b21, b22):
    return b11, b21 - b11, b11 + b22, b21 + b22, b22, b12 - b22, b11 + b12


def _strassen(product, emit):
    c = {}

    def run(k):
        c[k] = r = product(k)
        if k == 1:
            emit(1, 0, c[0] + r)
        elif k == 2:
            c[11], c[22] = r + c[1], r - c[0]
        elif k == 3:
            c[11] = c[11] + r
        elif k == 4:
            emit(0, 0, c[11] - r)
        elif k == 5:
            emit(0, 1, c[4] + r)
            c[22] = c[22] + r
        elif k == 6:
            emit(1, 1, c[22] + r)

    return [lambda k=k: run(k) for k in range(7)]


def _rows(i, n):
    return pl.ds(i * n if isinstance(i, int) else pl.multiple_of(i * n, n), n)


def _kernel(zero_ref, x_hbm, are_ref, aim_ref, bre_ref, bim_ref, cre_ref, cim_ref, ldt_ref, dsk_ref,
            wqkv_hbm, wo_hbm, f_hbm, g_hbm, out_hbm,
            xs, kf, ua, ub, uc, yb, par, zw, lag, qa, ka, va, qb, kb, vb, io, perm, wqkv, wo, fm, gm, kt, un, wt, us, wot, ob, sems):
    step = lambda fn, *a: (lambda: fn(*a))
    qs, ks, vs = (qa, qb), (ka, kb), (va, vb)
    loads = [pltpu.make_async_copy(s, d, sems.at[i]) for i, (s, d) in enumerate(
        (*((x_hbm.bitcast(U32).at[:, pl.ds(128 * c, 128)], io.at[c, pl.ds(0, L // 2)]) for c in range(NB)),
         (f_hbm, fm), (wo_hbm, wo), (g_hbm, gm),
         *((wqkv_hbm.at[:, pl.ds(128 * j, 128)], wqkv.at[j]) for j in range(12))))]
    for c in loads:
        c.start()
    high = jnp.uint32(0xFFFF0000)
    halves = lambda t: (pltpu.bitcast(t << 16, F32), pltpu.bitcast(t & high, F32))

    def col(ref):
        v = ref[...].astype(F32).reshape(1, D)
        return jnp.broadcast_to(v, (128, D)).T

    par[0] = jnp.exp(col(ldt_ref))
    par[1] = col(dsk_ref) * (1.0 / L)

    ri = lax.broadcasted_iota(jnp.int32, (128, 128), 0)
    ci = lax.broadcasted_iota(jnp.int32, (128, 128), 1)
    perm[...] = pltpu.bitcast(jnp.where(ci == (ri & 7) * DH + (ri >> 3), 1.0, 0.0).astype(BF16), U32)

    def setup(i):
        get = lambda ref: halves(pltpu.bitcast(ref[_rows(i, 16), :], U32))
        dt = halves(pltpu.bitcast(par[0, _rows(i, 16), :].astype(BF16), U32))

        def pole(h):
            mag, ang = jnp.exp(dt[h] * get(are_ref)[h]), dt[h] * get(aim_ref)[h]
            zw[i, h, 0], zw[i, h, 1] = mag * jnp.cos(ang), mag * jnp.sin(ang)

        def weight():
            scale = (1.0 + 1.5 * 2.0 ** -9) / L
            for h, (cr, ci, br, bi) in enumerate(zip(*map(get, (cre_ref, cim_ref, bre_ref, bim_ref)))):
                wr, wi = _cmul((cr, ci), (dt[h] * br, dt[h] * bi))
                zw[i, h, 2], zw[i, h, 3] = wr * scale, wi * -scale

        return [step(pole, 0), weight, step(pole, 1)]

    lags = sorted({(c, r) for c in range(8) for r in _RND[c] if r < 16}) + [(8, 0)]
    stack = lambda vs: jnp.concatenate([jnp.concatenate([v[k] for v in vs], 0) for k in range(2)], 1).astype(BF16)

    def lagsums(i):
        start = [[zw[i, h, c] for c in range(4)] for h in range(2)]
        zs, rhs, even = [], [], []

        def right(h):
            zr, zi, wr, wi = start[h]
            z = {0: (jnp.ones((8, N), F32), jnp.zeros((8, N), F32)), 1: (zr, zi)}
            for e in (2, 4, 8, 16, 32, 64, 128, 256):
                z[e] = _csq(z[e // 2])
            b = [(wr, wi)]
            for e in (16, 32, 64, 128):
                zc = (z[e][0], -z[e][1])
                b += [_cmul(v, zc) for v in b]
            zs.append(z)
            rhs.append(stack(b))

        def left(t, h):
            z = zs[h]

            def power(e):
                if e not in z:
                    low = e % 256 if e > 256 and e % 256 else e & -e
                    z[e] = _csq(z[e // 2]) if e // 2 in z and e % 2 == 0 else _cmul(power(e - low), power(low))
                return z[e]

            a = [power(256 * c + r) for c, r in (lags + lags[-1:])[CUT[t]:CUT[t + 1]]]
            o = pltpu.bitcast(lax.dot_general(stack(a), rhs[h], NT, preferred_element_type=F32), U32)
            if h:
                lag[i, 8 * CUT[t]:8 * CUT[t + 1], :] = even[t] | (o & high)
            else:
                even.append(o >> 16)

        return [f for h in range(2) for f in [step(right, h)] + [step(left, t, h) for t in range(len(CUT) - 1)]]

    def kgen(i):
        lane = lax.broadcasted_iota(jnp.int32, (8, 128), 1)
        src = (lane & 15) * 8 + lax.broadcasted_iota(jnp.int32, (8, 128), 0)

        memo = {}

        def piece(c, r):
            if r == 16:
                c = 0
            if (c, r) not in memo:
                memo[c, r] = (
                    pltpu.roll(jnp.where(lane == 0, piece(8, 0), merged(0, (0,) * 8)), 127, 1) if r == 16 else
                    jnp.take_along_axis(lag[i, _rows(lags.index((c, r)), 8), :], src, axis=1,
                                        mode="promise_in_bounds"))
            return memo[c, r]

        def merged(c, rs):
            if (c, rs) not in memo:
                memo[c, rs] = (piece(c, rs[0]) if c == 7 or min(rs) == 16 else
                               jnp.where(lane >> 4 == c, piece(c, rs[0]), merged(c + 1, rs[1:])))
            return memo[c, rs]

        for n0 in range(R0):
            kt[n0, _rows(i, 8), :] = merged(0, tuple(_RND[c][n0] for c in range(8)))

    get = lambda ref, n, rows: (ref[n, 0, rows, :], ref[n, 1, rows, :])

    def put(ref, n, rows, v):
        ref[n, 0, rows, :], ref[n, 1, rows, :] = v

    def outer(src, a, rows):
        return [_twiddle(v, a * b) for b, v in enumerate(_dft4([get(src, a + 4 * m, rows) for m in range(4)], 1))]

    def transform(lhs, dst, n0, rows):
        r = jnp.dot(lhs, _bf(fm[n0]), preferred_element_type=F32)
        put(dst, n0, rows, (r[:, :128], r[:, 128:]))

    def kfwd(n0, r):
        transform(_bf(kt[n0, _rows(r, 32), :]), ub, n0, _rows(r, 64))

    def kdft(i):
        rows, t = _rows(i, 8), []

        def inner(b):
            for m, v in enumerate(_dft4([t[a][b] for a in range(4)], 1)):
                put(kf, b + 4 * m, rows, (v[0] + par[1, rows, :], v[1]))

        return [lambda a=a: t.append(outer(ub, a, rows)) for a in range(4)] + [step(inner, b) for b in range(4)]

    def fwd(n0, r):
        transform(un[n0, _rows(r, 64), :], ua, n0, _rows(r, 64))

    def pre(a, i):
        for b, v in enumerate(outer(ua, a, _rows(i, 8))):
            put(ub, a + 4 * b, _rows(i, 8), v)

    def mid(i):
        first, t = {}, {}

        def inner(h, b):
            rows = _rows(2 * i + h, 8)
            if b == 0:
                first[h] = outer(ua, 0, rows)
            x = _dft4([first[h][b]] + [get(ub, a + 4 * b, rows) for a in range(1, 4)], 1)
            t[h, b], *y = _dft4([_cmul(x[m], get(kf, b + 4 * m, rows)) for m in range(4)], -1)
            for a in range(1, 4):
                put(uc, a + 4 * b, rows, y[a - 1])

        def last():
            for m, (v, w) in enumerate(zip(*[_dft4([t[h, b] for b in range(4)], -1) for h in range(2)])):
                put(yb, 4 * m, _rows(i, 16), [jnp.concatenate([v[k], w[k]], 0).astype(BF16) for k in range(2)])

        return [step(inner, h, b) for h in range(2) for b in range(4)] + [last]

    def post(a, i):
        rows = _rows(i, 16)
        for m, v in enumerate(_dft4([_twiddle(get(uc, a + 4 * b, rows), -a * b) for b in range(4)], -1)):
            put(yb, a + 4 * m, rows, (v[0].astype(BF16), v[1].astype(BF16)))

    def inv(n0, r):
        rows = _rows(r, 64)
        y = jnp.concatenate(get(yb, n0, rows), 1)
        xs[n0, rows, :] = xs[n0, rows, :] + jnp.dot(y, _bf(gm[n0]), preferred_element_type=F32)

    def wprep(g, t):
        ops = []

        def load():
            if t < 3:
                v = lax.dot_general(_bf(perm[...]), wqkv[4 * t + g], NT, preferred_element_type=F32)
                v = v if t else v * DH ** -0.5
                lo, hi = v[:, :256], v[:, 256:]
            else:
                v = [jnp.dot(_bf(perm[...]), wo[_rows(e, 128), _rows(g, 128)], preferred_element_type=F32)
                     for e in range(4)]
                lo, hi = (jnp.concatenate([u[64 * h:64 * h + 64] for u in v], 0).T for h in range(2))
            ops.extend((lo[:64], hi[:64], lo[64:], hi[64:]))

        def save(i, h):
            for k, a in enumerate(_left(*[v[16 * i:16 * i + 16, 128 * h:128 * h + 128] for v in ops])):
                dst = wt.at[g, k] if t < 3 else wot.at[k]
                dst[_rows(4 * (t if t < 3 else g) + i, 8), _rows(h, 128)] = pltpu.bitcast(a.astype(BF16), U32)

        return [load] + [step(save, i, h) for i in range(4) for h in range(2)]

    def xin(j, c):
        xs[2 * j, _rows(c, 128), :], xs[2 * j + 1, _rows(c, 128), :] = halves(io[c, pl.ds(j, R1, stride=8), :].T)

    def norm(n0):
        acc, stat = {}, []

        def moment(k, lo, hi):
            for i in range(lo, hi):
                v = xs[n0, 8 * i:8 * i + 8, :]
                v = jnp.square(v - stat[0]) if k else v
                acc[i % 4] = v if i < 4 else acc[i % 4] + v
            if hi == D // 8:
                v = jnp.sum(_tree(jnp.add, list(acc.values())), axis=0, keepdims=True) * (1.0 / D)
                stat.append(lax.rsqrt(v + 1e-5) if k else v)

        def scale(c):
            rows = _rows(c, 128)
            un[n0, rows, :] = get(rows).astype(BF16)

        get = lambda rows: (xs[n0, rows, :] - stat[0]) * stat[1]
        return [[step(moment, 0, 0, 64)], [step(moment, 1, i, i + 16) for i in range(0, 64, 16)],
                [step(scale, c) for c in range(4)]], get

    def norms(*aa):
        return [f for a in aa for stage in zip(*[norm(a + 4 * m)[0] for m in range(4)])
                for steps in stage for f in steps]

    def pair_norms(a):
        stages, get = zip(*[norm(a + 4 * m) for m in range(4)])

        def operands(j, c):
            (b11, b21), (b12, b22) = ((f(_rows(c, 16)), f(_rows(c + 16, 16))) for f in get[2 * j:2 * j + 2])
            for k, b in enumerate(_right(b11, b12, b21, b22)):
                us[2 * a + j, k, _rows(c, 8), :] = pltpu.bitcast(b.astype(BF16), U32)

        return ([f for k in range(2) for st in stages for f in st[k]]
                + [step(operands, j, c) for j in range(2) for c in range(16)])

    def proj(i, slot, m, t):
        p, g, ref = i >> 2, i & 3, (qs, ks, vs)[t][slot]

        def emit(half, j, r):
            ref[m + 2 * j + 7 * (t > 0), _rows(half, 64), :] = r
            if t and m + j:
                ref[m + 2 * j - 1, _rows(half, 64), :] = pltpu.roll(r, 1, 1)

        return _strassen(lambda k: jnp.dot(_bf(wt[g, k, _rows(t, 32), :]), _bf(us[2 * p + 4 * (m & 1) + (m >> 2), k]),
                                           preferred_element_type=F32), emit)

    def attn(i, slot, m0):
        p, g = i >> 2, i & 3
        first = lax.broadcasted_iota(jnp.int32, (8, 128), 1) == 0
        window = lambda ref, d: {e: ref[slot][e, 8 * d:8 * d + 8, :] for e in range(m0, m0 + W + 1)}
        s, o = {}, {}

        def logits(m, d0):
            for d in (d0, d0 + 1):
                k = window(ks, d)
                q = qs[slot][m, 8 * d:8 * d + 8, :]
                for w in range(W):
                    t = q * k[m + 7 - w]
                    s[m, w] = t if d == 0 else s[m, w] + t

        def softmax(m):
            t = [jnp.where(first, -1e9, s[m, w]) if w > m else s[m, w] for w in range(W)]
            mx = _tree(jnp.maximum, t)
            e = [jnp.exp(v - mx) for v in t]
            rs = 1.0 / _tree(jnp.add, e)
            s.update({(m, w): e[w] * rs for w in range(W)})

        def values(d):
            v = window(vs, d)
            for m in (m0, m0 + 1):
                o[m, d] = _tree(jnp.add, [s[m, w] * v[m + 7 - w] for w in range(W)])
            if d % 2 and d > 8:
                blocks = [jnp.concatenate([o[m, e - 1], o[m, e]], 0) for e in (d - 8, d) for m in (m0, m0 + 1)]
                for k, b in enumerate(_right(*blocks)):
                    ob[m0 + p, k, g, 8 * d - 72:8 * d - 56, :] = b.astype(BF16)

        return ([f for m in (m0, m0 + 1) for f in [step(logits, m, d) for d in range(0, DH, 2)] + [step(softmax, m)]]
                + [step(values, d + e) for d in range(0, 8, 2) for e in (0, 1, 8, 9)])

    def oproj(p, c, n):
        def pair(m0):
            def emit(half, j, r):
                for i in range(n):
                    at = (2 * (m0 + j) + p, _rows(2 * (c + i) + half, 64))
                    xs[at] = xs[at] + r[64 * i:64 * i + 64]

            return _strassen(lambda k: jnp.dot(_bf(wot[k, 32 * c:32 * (c + n), :]), ob[m0 + p, k].reshape(D // 2, R1),
                                               preferred_element_type=F32), emit)

        return [f for m0 in range(0, 8, 2) for f in pair(m0)]

    def xout(c, j):
        lo, hi = (pltpu.bitcast(xs[2 * j + k, _rows(c, 128), :].astype(BF16).astype(F32), U32) for k in range(2))
        io[c, pl.ds(j, R1, stride=8), :] = ((lo >> 16) | hi).T

    four = lambda fn, *aa: [step(fn, a + 4 * m, r) for a in aa for m in range(4) for r in range(2 * NB)]
    block = lambda fn, a, r: [step(fn, a + 4 * m, 2 * r + h) for h in range(2) for m in range(4)] if 0 <= r < NB else []
    rowwise = lambda fn, a, n: [step(fn, a, i) for i in range(D // n)]

    regions, zero = [], zero_ref[0]

    def slot(*streams):
        regions.append(None)
        pl.when(zero < len(regions))(lambda: _run(*streams))

    pres = lambda a: rowwise(pre, a, 8)
    posts = lambda a: rowwise(post, a, 16)
    projs = lambda i, s, ms: [f for t in (1, 2, 0) for m in ms for f in proj(i, s, m, t)]
    attns = lambda i, s: [f for m in range(0, 8, 2) for f in attn(i, s, m)]

    with jax.named_scope("kgen"):
        ng = D // 16 // KPER
        each = lambda fn: (lambda i: [f for k in range(KPER) for f in fn(KPER * i + k)])
        _pipeline([(lambda i: [lambda: [kgen(KPER * i + k) for k in range(KPER)]], 2, ng - 1),
                   (each(lagsums), 1, ng), (each(setup), 0, ng),
                   (lambda j: [step(xin, 2 * j + k, c) for k in range(2) for c in range(NB)], ng - 4, 4)],
                  {ng - 4: lambda: [c.wait() for c in loads[:NB]]})
    with jax.named_scope("kfwd"):
        for c in loads[NB:]:
            c.wait()
        kdfts = lambda r: [f for i in range(16) for f in kdft(16 * r + i)]
        for r, other in enumerate((norms(2, 1), *[sum(norm(n0)[0], []) for n0 in (3, 7)],
                                   sum(norm(11)[0] + norm(15)[0], []))):
            slot([f for a in range(4) for f in block(kfwd, a, r)], [f for t in (3, 0, 1, 2) for f in wprep(r, t)],
                 kdfts(r - 1) if r else [step(kgen, D // 16 - 1 - k) for k in range(KPER)], other)
        slot(four(fwd, 2), kdfts(NB - 1))
        slot(four(fwd, 1) + block(fwd, 3, 0), pres(2), norms(0))

    def layer(li, carry):
        with jax.named_scope("conv"):
            part = lambda steps, r: steps[len(steps) * r // NB:len(steps) * (r + 1) // NB] if 0 <= r < NB else []
            mids = [f for i in range(D // 16) for f in mid(i)]
            for r in range(-1, NB + 1):
                slot(block(fwd, 3, r + 2) + block(fwd, 0, r + 1) + block(inv, 0, r - 1) + block(inv, 2, r - 2)
                     + block(inv, 1, r - 2),
                     part(mids, r), part(pres(3), r + 1) + part(posts(2), r - 1) + part(posts(1), r - 1),
                     pres(1) if r < 0 else posts(3) if r == NB else [])
            slot(block(inv, 2, NB - 1) + block(inv, 1, NB - 1) + four(inv, 3), pair_norms(0))
            slot(projs(0, 0, (0, 4)), pair_norms(2))
            slot(projs(0, 0, (1, 5)), pair_norms(1))
        with jax.named_scope("attn"):
            slot(projs(1, 1, (0, 1, 4, 5)), attns(0, 0), pair_norms(3))
            both = lambda i, s: slot(projs(i + 1, 1 - s, (0, 1, 4, 5)), attns(i, s))
            lax.fori_loop(0, 3, lambda j, c: (both(2 * j + 1, 1), both(2 * j + 2, 0), c)[-1], 0)
            slot(oproj(0, 0, 2) + oproj(0, 2, 2), attns(7, 1))

        @pl.when(li == 0)
        def _():
            slot(oproj(1, 0, 2) + oproj(1, 2, 2), norms(2, 0))
            slot(four(fwd, 2), norms(1, 3))
            slot(four(fwd, 1) + block(fwd, 3, 0), pres(2))

        return carry

    lax.fori_loop(0, 2, layer, 0)

    with jax.named_scope("xout"):
        stores = [pltpu.make_async_copy(io.at[c, pl.ds(0, L // 2)],
                                        out_hbm.bitcast(U32).at[:, pl.ds(c * 128, 128)], sems.at[c])
                  for c in range(NB)]
        last = [f for c in range(NB) for f in oproj(1, c, 1)] + [lambda: None] * 7
        for c in range(NB):
            slot(last[28 * c + 7 * (c > 0):28 * c + 35],
                 [lambda: None] * (2 * (c == 0)) + [step(xout, c, j) for j in range(8)])
            stores[c].start()
        for c in stores:
            c.wait()


@jax.jit
def pallas_interleave_layers__ssm_conv_s4__sliding_local_dilated__prompt_kernel(
    A_u: jax.Array,
    A_A_re: jax.Array,
    A_A_im: jax.Array,
    A_B_re: jax.Array,
    A_B_im: jax.Array,
    A_C_re: jax.Array,
    A_C_im: jax.Array,
    A_log_dt: jax.Array,
    A_Dskip: jax.Array,
    B_x: jax.Array,
    B_wqkv: jax.Array,
    B_wo: jax.Array,
):
    del B_x
    hbm, vmem = pl.BlockSpec(memory_space=pl.ANY), pl.BlockSpec(memory_space=pltpu.VMEM)
    tiles = lambda *n: pltpu.VMEM((*n, 128, 128), F32)
    out = pl.pallas_call(
        _kernel,
        out_shape=jax.ShapeDtypeStruct((L, D), BF16),
        in_specs=[pl.BlockSpec(memory_space=pltpu.SMEM), hbm] + [vmem] * 8 + [hbm] * 4,
        out_specs=hbm,
        scratch_shapes=[
            pltpu.VMEM((R0, D, R1), F32),
            *[pltpu.VMEM((R0, 2, D, R1), F32)] * 4,
            pltpu.VMEM((R0, 2, D, R1), BF16),
            pltpu.VMEM((2, D, N), F32),
            pltpu.VMEM((D // 16, 2, 4, 8, N), F32),
            pltpu.VMEM((D // 16, 336, 128), U32),
            *[tiles(n) for n in (8, 15, 15) * 2],
            pltpu.VMEM((NB, L // 2 + 8, 128), U32),
            pltpu.VMEM((64, 128), U32),
            pltpu.VMEM((12, D, 128), BF16),
            pltpu.VMEM((D, D), BF16),
            pltpu.VMEM(_F.shape, U32),
            pltpu.VMEM(_G.shape, U32),
            pltpu.VMEM((R0, D // 2, R1), U32),
            pltpu.VMEM((R0, D, R1), BF16),
            pltpu.VMEM((4, 7, 96, D // 2), U32),
            pltpu.VMEM((8, 7, D // 4, R1), U32),
            pltpu.VMEM((7, D // 4, D // 2), U32),
            pltpu.VMEM((8, 7, 4, 64, R1), BF16),
            pltpu.SemaphoreType.DMA((19,)),
        ],
        compiler_params=pltpu.CompilerParams(vmem_limit_bytes=100 * 1024 * 1024),
    )(np.zeros((2,), np.int32), A_u.reshape(L, D), A_A_re, A_A_im, A_B_re, A_B_im, A_C_re, A_C_im, A_log_dt, A_Dskip,
      B_wqkv, B_wo, _F, _G)
    return out.reshape(1, L, D)
```

```python
import jax
import jax.numpy as jnp
import ml_dtypes
import numpy as np
from jax import lax
import jax.experimental.pallas as pl
import jax.experimental.pallas.tpu as pltpu

L, D, N = 2048, 512, 128
R0, R1 = 16, 128
W, DH = 8, 16
F32, BF16, U32 = jnp.float32, jnp.bfloat16, jnp.uint32
CUT = (0, 20, 42)
KPER = 4
NB = D // 128
NT = (((1,), (1,)), ((), ()))


def _constants():
    n0 = np.arange(R0)[:, None, None]
    n1 = np.arange(R1)[None, :, None]
    k1 = np.arange(R1)[None, None, :]
    ang = 2.0 * np.pi * (k1 + 0.25) * (R0 * n1 + n0) / L
    f = np.concatenate([np.cos(ang), np.sin(ang)], axis=2)
    g = f.transpose(0, 2, 1)
    bf = ml_dtypes.bfloat16
    lr = np.arange(L).astype(np.float32).astype(bf).astype(np.int64).reshape(8, 16, R0)
    r = lr - (256 * np.arange(8)[:, None, None] + 16 * np.arange(16)[None, :, None])
    assert (r == r[:, :1, :]).all()

    def words(m):
        h = np.ascontiguousarray(m).astype(bf).view(np.uint16).astype(np.uint32)
        return h[:, 0::2] | (h[:, 1::2] << 16)

    return words(f), words(g), r[:, 0, :].tolist()


_F, _G, _RND = _constants()


def _cmul(a, b):
    return a[0] * b[0] - a[1] * b[1], a[0] * b[1] + a[1] * b[0]


def _csq(a):
    t = a[0] * a[1]
    return (a[0] + a[1]) * (a[0] - a[1]), t + t


def _dft4(x, sign):
    (ar, ai), (br, bi), (cr, ci), (dr, di) = x
    sr, si, tr, ti = ar + cr, ai + ci, ar - cr, ai - ci
    ur, ui, vr, vi = br + dr, bi + di, br - dr, bi - di
    p, m = (tr - vi, ti + vr), (tr + vi, ti - vr)
    if sign < 0:
        p, m = m, p
    return [(sr + ur, si + ui), p, (sr - ur, si - ui), m]


def _twiddle(v, e):
    e %= 16
    re, im = v
    h = float(np.sqrt(0.5))
    if e == 0:
        return v
    if e == 4:
        return -im, re
    if e == 12:
        return im, -re
    if e == 2:
        return (re - im) * h, (re + im) * h
    if e == 14:
        return (re + im) * h, (im - re) * h
    if e == 6:
        return (re + im) * -h, (re - im) * h
    if e == 10:
        return (im - re) * h, (re + im) * -h
    c, s = float(np.cos(np.pi * e / 8)), float(np.sin(np.pi * e / 8))
    return re * c - im * s, re * s + im * c


def _bf(x):
    return pltpu.bitcast(x, BF16)


def _tree(op, v):
    while len(v) > 1:
        v = [op(v[i], v[i + 1]) if i + 1 < len(v) else v[i] for i in range(0, len(v), 2)]
    return v[0]


def _run(*streams):
    order = sorted(((i + 0.5 * (k > 0)) / len(s), k, i) for k, s in enumerate(streams) for i in range(len(s)))
    for _, k, i in order:
        streams[k][i]()


def _pipeline(streams, hooks=None):
    hooks = hooks or {}
    cuts = sorted({e for _, a, n in streams for e in (a, a + n)} | set(hooks))
    for lo, hi in zip(cuts, cuts[1:]):
        def body(s, carry, lo=lo):
            _run(*[fn(s - a) for fn, a, n in streams if a <= lo < a + n])
            return carry

        if lo in hooks:
            hooks[lo]()
        if hi - lo == 1:
            body(lo, 0)
        else:
            lax.fori_loop(lo, hi, body, 0)


def _left(a11, a12, a21, a22):
    return a21 + a22, a22, a11 + a22, a12 - a22, a11 + a12, a11, a21 - a11


def _right(b11, b12, b21, b22):
    return b11, b21 - b11, b11 + b22, b21 + b22, b22, b12 - b22, b11 + b12


def _strassen(product, emit):
    c = {}

    def run(k):
        c[k] = r = product(k)
        if k == 1:
            emit(1, 0, c[0] + r)
        elif k == 2:
            c[11], c[22] = r + c[1], r - c[0]
        elif k == 3:
            c[11] = c[11] + r
        elif k == 4:
            emit(0, 0, c[11] - r)
        elif k == 5:
            emit(0, 1, c[4] + r)
            c[22] = c[22] + r
        elif k == 6:
            emit(1, 1, c[22] + r)

    return [lambda k=k: run(k) for k in range(7)]


def _rows(i, n):
    return pl.ds(i * n if isinstance(i, int) else pl.multiple_of(i * n, n), n)


def _kernel(zero_ref, x_hbm, are_hbm, aim_hbm, bre_hbm, bim_hbm, cre_hbm, cim_hbm, ldt_ref, dsk_ref,
            wqkv_hbm, wo_hbm, f_hbm, g_hbm, out_hbm,
            xs, kf, ua, ub, uc, yb, par, zw, lag, qa, ka, va, qb, kb, vb, io, abc, perm, wqkv, wo, fm, gm, kt, un, wt, us, wot, ob, sems):
    step = lambda fn, *a: (lambda: fn(*a))
    qs, ks, vs = (qa, qb), (ka, kb), (va, vb)
    head, rest = ([pltpu.make_async_copy(s.at[rows], abc.at[i, rows], sems.at[base + i])
                   for i, s in enumerate((are_hbm, aim_hbm, bre_hbm, bim_hbm, cre_hbm, cim_hbm))]
                  for base, rows in ((19, pl.ds(0, 32 * KPER)), (25, pl.ds(32 * KPER, D - 32 * KPER))))
    loads = [pltpu.make_async_copy(s, d, sems.at[i]) for i, (s, d) in enumerate(
        (*((x_hbm.bitcast(U32).at[:, pl.ds(128 * c, 128)], io.at[c, pl.ds(0, L // 2)]) for c in range(NB)),
         (f_hbm, fm), (wo_hbm, wo), (g_hbm, gm),
         *((wqkv_hbm.at[:, pl.ds(128 * j, 128)], wqkv.at[j]) for j in range(12))))]
    for c in head + rest:
        c.start()
    high = jnp.uint32(0xFFFF0000)
    halves = lambda t: (pltpu.bitcast(t << 16, F32), pltpu.bitcast(t & high, F32))

    def col(ref):
        v = ref[...].astype(F32).reshape(1, D)
        return jnp.broadcast_to(v, (128, D)).T

    par[0] = jnp.exp(col(ldt_ref))
    par[1] = col(dsk_ref) * (1.0 / L)

    ri = lax.broadcasted_iota(jnp.int32, (128, 128), 0)
    ci = lax.broadcasted_iota(jnp.int32, (128, 128), 1)
    perm[...] = pltpu.bitcast(jnp.where(ci == (ri & 7) * DH + (ri >> 3), 1.0, 0.0).astype(BF16), U32)

    for c in head:
        c.wait()
    for c in loads:
        c.start()

    def setup(i):
        get = lambda k: halves(pltpu.bitcast(abc[k, _rows(i, 16), :], U32))
        dt = halves(pltpu.bitcast(par[0, _rows(i, 16), :].astype(BF16), U32))

        def pole(h):
            mag, ang = jnp.exp(dt[h] * get(0)[h]), dt[h] * get(1)[h]
            zw[i, h, 0], zw[i, h, 1] = mag * jnp.cos(ang), mag * jnp.sin(ang)

        def weight():
            scale = (1.0 + 1.5 * 2.0 ** -9) / L
            for h, (cr, ci, br, bi) in enumerate(zip(*map(get, (4, 5, 2, 3)))):
                wr, wi = _cmul((cr, ci), (dt[h] * br, dt[h] * bi))
                zw[i, h, 2], zw[i, h, 3] = wr * scale, wi * -scale

        return [step(pole, 0), weight, step(pole, 1)]

    lags = sorted({(c, r) for c in range(8) for r in _RND[c] if r < 16}) + [(8, 0)]
    stack = lambda vs: jnp.concatenate([jnp.concatenate([v[k] for v in vs], 0) for k in range(2)], 1).astype(BF16)

    def lagsums(i):
        start = [[zw[i, h, c] for c in range(4)] for h in range(2)]
        zs, rhs, even = [], [], []

        def right(h):
            zr, zi, wr, wi = start[h]
            z = {0: (jnp.ones((8, N), F32), jnp.zeros((8, N), F32)), 1: (zr, zi)}
            for e in (2, 4, 8, 16, 32, 64, 128, 256):
                z[e] = _csq(z[e // 2])
            b = [(wr, wi)]
            for e in (16, 32, 64, 128):
                zc = (z[e][0], -z[e][1])
                b += [_cmul(v, zc) for v in b]
            zs.append(z)
            rhs.append(stack(b))

        def left(t, h):
            z = zs[h]

            def power(e):
                if e not in z:
                    low = e % 256 if e > 256 and e % 256 else e & -e
                    z[e] = _csq(z[e // 2]) if e // 2 in z and e % 2 == 0 else _cmul(power(e - low), power(low))
                return z[e]

            a = [power(256 * c + r) for c, r in (lags + lags[-1:])[CUT[t]:CUT[t + 1]]]
            o = pltpu.bitcast(lax.dot_general(stack(a), rhs[h], NT, preferred_element_type=F32), U32)
            if h:
                lag[i, 8 * CUT[t]:8 * CUT[t + 1], :] = even[t] | (o & high)
            else:
                even.append(o >> 16)

        return [f for h in range(2) for f in [step(right, h)] + [step(left, t, h) for t in range(len(CUT) - 1)]]

    def kgen(i):
        lane = lax.broadcasted_iota(jnp.int32, (8, 128), 1)
        src = (lane & 15) * 8 + lax.broadcasted_iota(jnp.int32, (8, 128), 0)

        memo = {}

        def piece(c, r):
            if r == 16:
                c = 0
            if (c, r) not in memo:
                memo[c, r] = (
                    pltpu.roll(jnp.where(lane == 0, piece(8, 0), merged(0, (0,) * 8)), 127, 1) if r == 16 else
                    jnp.take_along_axis(lag[i, _rows(lags.index((c, r)), 8), :], src, axis=1,
                                        mode="promise_in_bounds"))
            return memo[c, r]

        def merged(c, rs):
            if (c, rs) not in memo:
                memo[c, rs] = (piece(c, rs[0]) if c == 7 or min(rs) == 16 else
                               jnp.where(lane >> 4 == c, piece(c, rs[0]), merged(c + 1, rs[1:])))
            return memo[c, rs]

        for n0 in range(R0):
            kt[n0, _rows(i, 8), :] = merged(0, tuple(_RND[c][n0] for c in range(8)))

    get = lambda ref, n, rows: (ref[n, 0, rows, :], ref[n, 1, rows, :])

    def put(ref, n, rows, v):
        ref[n, 0, rows, :], ref[n, 1, rows, :] = v

    def outer(src, a, rows):
        return [_twiddle(v, a * b) for b, v in enumerate(_dft4([get(src, a + 4 * m, rows) for m in range(4)], 1))]

    def transform(lhs, dst, n0, rows):
        r = jnp.dot(lhs, _bf(fm[n0]), preferred_element_type=F32)
        put(dst, n0, rows, (r[:, :128], r[:, 128:]))

    def kfwd(n0, r):
        transform(_bf(kt[n0, _rows(r, 32), :]), ub, n0, _rows(r, 64))

    def kdft(i):
        rows, t = _rows(i, 8), []

        def inner(b):
            for m, v in enumerate(_dft4([t[a][b] for a in range(4)], 1)):
                put(kf, b + 4 * m, rows, (v[0] + par[1, rows, :], v[1]))

        return [lambda a=a: t.append(outer(ub, a, rows)) for a in range(4)] + [step(inner, b) for b in range(4)]

    def fwd(n0, r):
        transform(un[n0, _rows(r, 64), :], ua, n0, _rows(r, 64))

    def pre(a, i):
        for b, v in enumerate(outer(ua, a, _rows(i, 8))):
            put(ub, a + 4 * b, _rows(i, 8), v)

    def mid(i):
        first, t = {}, {}

        def inner(h, b):
            rows = _rows(2 * i + h, 8)
            if b == 0:
                first[h] = outer(ua, 0, rows)
            x = _dft4([first[h][b]] + [get(ub, a + 4 * b, rows) for a in range(1, 4)], 1)
            t[h, b], *y = _dft4([_cmul(x[m], get(kf, b + 4 * m, rows)) for m in range(4)], -1)
            for a in range(1, 4):
                put(uc, a + 4 * b, rows, y[a - 1])

        def last():
            for m, (v, w) in enumerate(zip(*[_dft4([t[h, b] for b in range(4)], -1) for h in range(2)])):
                put(yb, 4 * m, _rows(i, 16), [jnp.concatenate([v[k], w[k]], 0).astype(BF16) for k in range(2)])

        return [step(inner, h, b) for h in range(2) for b in range(4)] + [last]

    def post(a, i):
        rows = _rows(i, 16)
        for m, v in enumerate(_dft4([_twiddle(get(uc, a + 4 * b, rows), -a * b) for b in range(4)], -1)):
            put(yb, a + 4 * m, rows, (v[0].astype(BF16), v[1].astype(BF16)))

    def inv(n0, r):
        rows = _rows(r, 64)
        y = jnp.concatenate(get(yb, n0, rows), 1)
        xs[n0, rows, :] = xs[n0, rows, :] + jnp.dot(y, _bf(gm[n0]), preferred_element_type=F32)

    def wprep(g, t):
        ops = []

        def load():
            if t < 3:
                v = lax.dot_general(_bf(perm[...]), wqkv[4 * t + g], NT, preferred_element_type=F32)
                v = v if t else v * DH ** -0.5
                lo, hi = v[:, :256], v[:, 256:]
            else:
                v = [jnp.dot(_bf(perm[...]), wo[_rows(e, 128), _rows(g, 128)], preferred_element_type=F32)
                     for e in range(4)]
                lo, hi = (jnp.concatenate([u[64 * h:64 * h + 64] for u in v], 0).T for h in range(2))
            ops.extend((lo[:64], hi[:64], lo[64:], hi[64:]))

        def save(i, h):
            for k, a in enumerate(_left(*[v[16 * i:16 * i + 16, 128 * h:128 * h + 128] for v in ops])):
                dst = wt.at[g, k] if t < 3 else wot.at[k]
                dst[_rows(4 * (t if t < 3 else g) + i, 8), _rows(h, 128)] = pltpu.bitcast(a.astype(BF16), U32)

        return [load] + [step(save, i, h) for i in range(4) for h in range(2)]

    def xin(j, c):
        xs[2 * j, _rows(c, 128), :], xs[2 * j + 1, _rows(c, 128), :] = halves(io[c, pl.ds(j, R1, stride=8), :].T)

    def norm(n0):
        acc, stat = {}, []

        def moment(k, lo, hi):
            for i in range(lo, hi):
                v = xs[n0, 8 * i:8 * i + 8, :]
                v = jnp.square(v - stat[0]) if k else v
                acc[i % 4] = v if i < 4 else acc[i % 4] + v
            if hi == D // 8:
                v = jnp.sum(_tree(jnp.add, list(acc.values())), axis=0, keepdims=True) * (1.0 / D)
                stat.append(lax.rsqrt(v + 1e-5) if k else v)

        def scale(c):
            rows = _rows(c, 128)
            un[n0, rows, :] = get(rows).astype(BF16)

        get = lambda rows: (xs[n0, rows, :] - stat[0]) * stat[1]
        return [[step(moment, 0, 0, 64)], [step(moment, 1, i, i + 16) for i in range(0, 64, 16)],
                [step(scale, c) for c in range(4)]], get

    def norms(*aa):
        return [f for a in aa for stage in zip(*[norm(a + 4 * m)[0] for m in range(4)])
                for steps in stage for f in steps]

    def pair_norms(a):
        stages, get = zip(*[norm(a + 4 * m) for m in range(4)])

        def operands(j, c):
            (b11, b21), (b12, b22) = ((f(_rows(c, 16)), f(_rows(c + 16, 16))) for f in get[2 * j:2 * j + 2])
            for k, b in enumerate(_right(b11, b12, b21, b22)):
                us[2 * a + j, k, _rows(c, 8), :] = pltpu.bitcast(b.astype(BF16), U32)

        return ([f for k in range(2) for st in stages for f in st[k]]
                + [step(operands, j, c) for j in range(2) for c in range(16)])

    def proj(i, slot, m, t):
        p, g, ref = i >> 2, i & 3, (qs, ks, vs)[t][slot]

        def emit(half, j, r):
            ref[m + 2 * j + 7 * (t > 0), _rows(half, 64), :] = r
            if t and m + j:
                ref[m + 2 * j - 1, _rows(half, 64), :] = pltpu.roll(r, 1, 1)

        return _strassen(lambda k: jnp.dot(_bf(wt[g, k, _rows(t, 32), :]), _bf(us[2 * p + 4 * (m & 1) + (m >> 2), k]),
                                           preferred_element_type=F32), emit)

    def attn(i, slot, m0):
        p, g = i >> 2, i & 3
        first = lax.broadcasted_iota(jnp.int32, (8, 128), 1) == 0
        window = lambda ref, d: {e: ref[slot][e, 8 * d:8 * d + 8, :] for e in range(m0, m0 + W + 1)}
        s, o = {}, {}

        def logits(m, d0):
            for d in (d0, d0 + 1):
                k = window(ks, d)
                q = qs[slot][m, 8 * d:8 * d + 8, :]
                for w in range(W):
                    t = q * k[m + 7 - w]
                    s[m, w] = t if d == 0 else s[m, w] + t

        def softmax(m):
            t = [jnp.where(first, -1e9, s[m, w]) if w > m else s[m, w] for w in range(W)]
            mx = _tree(jnp.maximum, t)
            e = [jnp.exp(v - mx) for v in t]
            rs = 1.0 / _tree(jnp.add, e)
            s.update({(m, w): e[w] * rs for w in range(W)})

        def values(d):
            v = window(vs, d)
            for m in (m0, m0 + 1):
                o[m, d] = _tree(jnp.add, [s[m, w] * v[m + 7 - w] for w in range(W)])
            if d % 2 and d > 8:
                blocks = [jnp.concatenate([o[m, e - 1], o[m, e]], 0) for e in (d - 8, d) for m in (m0, m0 + 1)]
                for k, b in enumerate(_right(*blocks)):
                    ob[m0 + p, k, g, 8 * d - 72:8 * d - 56, :] = b.astype(BF16)

        return ([f for m in (m0, m0 + 1) for f in [step(logits, m, d) for d in range(0, DH, 2)] + [step(softmax, m)]]
                + [step(values, d + e) for d in range(0, 8, 2) for e in (0, 1, 8, 9)])

    def oproj(p, c, n):
        def pair(m0):
            def emit(half, j, r):
                for i in range(n):
                    at = (2 * (m0 + j) + p, _rows(2 * (c + i) + half, 64))
                    xs[at] = xs[at] + r[64 * i:64 * i + 64]

            return _strassen(lambda k: jnp.dot(_bf(wot[k, 32 * c:32 * (c + n), :]), ob[m0 + p, k].reshape(D // 2, R1),
                                               preferred_element_type=F32), emit)

        return [f for m0 in range(0, 8, 2) for f in pair(m0)]

    def xout(c, j):
        lo, hi = (pltpu.bitcast(xs[2 * j + k, _rows(c, 128), :].astype(BF16).astype(F32), U32) for k in range(2))
        io[c, pl.ds(j, R1, stride=8), :] = ((lo >> 16) | hi).T

    four = lambda fn, *aa: [step(fn, a + 4 * m, r) for a in aa for m in range(4) for r in range(2 * NB)]
    block = lambda fn, a, r: [step(fn, a + 4 * m, 2 * r + h) for h in range(2) for m in range(4)] if 0 <= r < NB else []
    rowwise = lambda fn, a, n: [step(fn, a, i) for i in range(D // n)]

    regions, zero = [], zero_ref[0]

    def slot(*streams):
        regions.append(None)
        pl.when(zero < len(regions))(lambda: _run(*streams))

    pres = lambda a: rowwise(pre, a, 8)
    posts = lambda a: rowwise(post, a, 16)
    projs = lambda i, s, ms: [f for t in (1, 2, 0) for m in ms for f in proj(i, s, m, t)]
    attns = lambda i, s: [f for m in range(0, 8, 2) for f in attn(i, s, m)]

    with jax.named_scope("kgen"):
        ng = D // 16 // KPER
        each = lambda fn: (lambda i: [f for k in range(KPER) for f in fn(KPER * i + k)])
        _pipeline([(lambda i: [lambda: [kgen(KPER * i + k) for k in range(KPER)]], 2, ng - 1),
                   (each(lagsums), 1, ng), (each(setup), 0, ng),
                   (lambda j: [step(xin, 2 * j + k, c) for k in range(2) for c in range(NB)], ng - 4, 4)],
                  {2: lambda: [c.wait() for c in rest], ng - 4: lambda: [c.wait() for c in loads[:NB]]})
    with jax.named_scope("kfwd"):
        for c in loads[NB:]:
            c.wait()
        kdfts = lambda r: [f for i in range(16) for f in kdft(16 * r + i)]
        for r, other in enumerate((norms(2, 1), *[sum(norm(n0)[0], []) for n0 in (3, 7)],
                                   sum(norm(11)[0] + norm(15)[0], []))):
            slot([f for a in range(4) for f in block(kfwd, a, r)], [f for t in (3, 0, 1, 2) for f in wprep(r, t)],
                 kdfts(r - 1) if r else [step(kgen, D // 16 - 1 - k) for k in range(KPER)], other)
        slot(four(fwd, 2), kdfts(NB - 1))
        slot(four(fwd, 1) + block(fwd, 3, 0), pres(2), norms(0))

    def layer(li, carry):
        with jax.named_scope("conv"):
            part = lambda steps, r: steps[len(steps) * r // NB:len(steps) * (r + 1) // NB] if 0 <= r < NB else []
            mids = [f for i in range(D // 16) for f in mid(i)]
            for r in range(-1, NB + 1):
                slot(block(fwd, 3, r + 2) + block(fwd, 0, r + 1) + block(inv, 0, r - 1) + block(inv, 2, r - 2)
                     + block(inv, 1, r - 2),
                     part(mids, r), part(pres(3), r + 1) + part(posts(2), r - 1) + part(posts(1), r - 1),
                     pres(1) if r < 0 else posts(3) if r == NB else [])
            slot(block(inv, 2, NB - 1) + block(inv, 1, NB - 1) + four(inv, 3), pair_norms(0))
            slot(projs(0, 0, (0, 4)), pair_norms(2))
            slot(projs(0, 0, (1, 5)), pair_norms(1))
        with jax.named_scope("attn"):
            slot(projs(1, 1, (0, 1, 4, 5)), attns(0, 0), pair_norms(3))
            both = lambda i, s: slot(projs(i + 1, 1 - s, (0, 1, 4, 5)), attns(i, s))
            lax.fori_loop(0, 3, lambda j, c: (both(2 * j + 1, 1), both(2 * j + 2, 0), c)[-1], 0)
            slot(oproj(0, 0, 2) + oproj(0, 2, 2), attns(7, 1))

        @pl.when(li == 0)
        def _():
            slot(oproj(1, 0, 2) + oproj(1, 2, 2), norms(2, 0))
            slot(four(fwd, 2), norms(1, 3))
            slot(four(fwd, 1) + block(fwd, 3, 0), pres(2))

        return carry

    lax.fori_loop(0, 2, layer, 0)

    with jax.named_scope("xout"):
        stores = [pltpu.make_async_copy(io.at[c, _rows(i, 256)],
                                        out_hbm.bitcast(U32).at[_rows(i, 256), _rows(c, 128)], sems.at[4 * c + i])
                  for c in range(NB) for i in range(4)]
        last = [f for c in range(NB) for f in oproj(1, c, 1)] + [lambda: None] * 7
        for c in range(NB):
            slot(last[28 * c + 7 * (c > 0):28 * c + 35],
                 [lambda: None] * (2 * (c == 0)) + [step(xout, c, j) for j in range(8)])
            for copy in stores[4 * c:4 * c + 4]:
                copy.start()
        for c in stores:
            c.wait()


@jax.jit
def pallas_interleave_layers__ssm_conv_s4__sliding_local_dilated__prompt_kernel(
    A_u: jax.Array,
    A_A_re: jax.Array,
    A_A_im: jax.Array,
    A_B_re: jax.Array,
    A_B_im: jax.Array,
    A_C_re: jax.Array,
    A_C_im: jax.Array,
    A_log_dt: jax.Array,
    A_Dskip: jax.Array,
    B_x: jax.Array,
    B_wqkv: jax.Array,
    B_wo: jax.Array,
):
    del B_x
    hbm, vmem = pl.BlockSpec(memory_space=pl.ANY), pl.BlockSpec(memory_space=pltpu.VMEM)
    tiles = lambda *n: pltpu.VMEM((*n, 128, 128), F32)
    out = pl.pallas_call(
        _kernel,
        out_shape=jax.ShapeDtypeStruct((L, D), BF16),
        in_specs=[pl.BlockSpec(memory_space=pltpu.SMEM), *[hbm] * 7, vmem, vmem] + [hbm] * 4,
        out_specs=hbm,
        scratch_shapes=[
            pltpu.VMEM((R0, D, R1), F32),
            *[pltpu.VMEM((R0, 2, D, R1), F32)] * 4,
            pltpu.VMEM((R0, 2, D, R1), BF16),
            pltpu.VMEM((2, D, N), F32),
            pltpu.VMEM((D // 16, 2, 4, 8, N), F32),
            pltpu.VMEM((D // 16, 336, 128), U32),
            *[tiles(n) for n in (8, 15, 15) * 2],
            pltpu.VMEM((NB, L // 2 + 8, 128), U32),
            pltpu.VMEM((6, D, N), BF16),
            pltpu.VMEM((64, 128), U32),
            pltpu.VMEM((12, D, 128), BF16),
            pltpu.VMEM((D, D), BF16),
            pltpu.VMEM(_F.shape, U32),
            pltpu.VMEM(_G.shape, U32),
            pltpu.VMEM((R0, D // 2, R1), U32),
            pltpu.VMEM((R0, D, R1), BF16),
            pltpu.VMEM((4, 7, 96, D // 2), U32),
            pltpu.VMEM((8, 7, D // 4, R1), U32),
            pltpu.VMEM((7, D // 4, D // 2), U32),
            pltpu.VMEM((8, 7, 4, 64, R1), BF16),
            pltpu.SemaphoreType.DMA((31,)),
        ],
        compiler_params=pltpu.CompilerParams(vmem_limit_bytes=100 * 1024 * 1024),
    )(np.zeros((2,), np.int32), A_u.reshape(L, D), A_A_re, A_A_im, A_B_re, A_B_im, A_C_re, A_C_im, A_log_dt, A_Dskip,
      B_wqkv, B_wo, _F, _G)
    return out.reshape(1, L, D)
```

```python
import jax
import jax.numpy as jnp
import ml_dtypes
import numpy as np
from jax import lax
import jax.experimental.pallas as pl
import jax.experimental.pallas.tpu as pltpu

L, D, N = 2048, 512, 128
R0, R1 = 16, 128
W, DH = 8, 16
F32, BF16, U32 = jnp.float32, jnp.bfloat16, jnp.uint32
CUT = (0, 20, 42)
KPER = 4
NB = D // 128
NT = (((1,), (1,)), ((), ()))


def _constants():
    n0 = np.arange(R0)[:, None, None]
    n1 = np.arange(R1)[None, :, None]
    k1 = np.arange(R1)[None, None, :]
    ang = 2.0 * np.pi * (k1 + 0.25) * (R0 * n1 + n0) / L
    f = np.concatenate([np.cos(ang), np.sin(ang)], axis=2)
    g = f.transpose(0, 2, 1)
    bf = ml_dtypes.bfloat16
    lr = np.arange(L).astype(np.float32).astype(bf).astype(np.int64).reshape(8, 16, R0)
    r = lr - (256 * np.arange(8)[:, None, None] + 16 * np.arange(16)[None, :, None])
    assert (r == r[:, :1, :]).all()

    def words(m):
        h = np.ascontiguousarray(m).astype(bf).view(np.uint16).astype(np.uint32)
        return h[:, 0::2] | (h[:, 1::2] << 16)

    return words(f), words(g), r[:, 0, :].tolist()


_F, _G, _RND = _constants()


def _cmul(a, b):
    return a[0] * b[0] - a[1] * b[1], a[0] * b[1] + a[1] * b[0]


def _csq(a):
    t = a[0] * a[1]
    return (a[0] + a[1]) * (a[0] - a[1]), t + t


def _dft4(x, sign):
    (ar, ai), (br, bi), (cr, ci), (dr, di) = x
    sr, si, tr, ti = ar + cr, ai + ci, ar - cr, ai - ci
    ur, ui, vr, vi = br + dr, bi + di, br - dr, bi - di
    p, m = (tr - vi, ti + vr), (tr + vi, ti - vr)
    if sign < 0:
        p, m = m, p
    return [(sr + ur, si + ui), p, (sr - ur, si - ui), m]


def _twiddle(v, e):
    e %= 16
    re, im = v
    h = float(np.sqrt(0.5))
    if e == 0:
        return v
    if e == 4:
        return -im, re
    if e == 12:
        return im, -re
    if e == 2:
        return (re - im) * h, (re + im) * h
    if e == 14:
        return (re + im) * h, (im - re) * h
    if e == 6:
        return (re + im) * -h, (re - im) * h
    if e == 10:
        return (im - re) * h, (re + im) * -h
    c, s = float(np.cos(np.pi * e / 8)), float(np.sin(np.pi * e / 8))
    return re * c - im * s, re * s + im * c


def _bf(x):
    return pltpu.bitcast(x, BF16)


def _tree(op, v):
    while len(v) > 1:
        v = [op(v[i], v[i + 1]) if i + 1 < len(v) else v[i] for i in range(0, len(v), 2)]
    return v[0]


def _run(*streams):
    order = sorted(((i + 0.5 * (k > 0)) / len(s), k, i) for k, s in enumerate(streams) for i in range(len(s)))
    for _, k, i in order:
        streams[k][i]()


def _pipeline(streams, hooks=None):
    hooks = hooks or {}
    cuts = sorted({e for _, a, n in streams for e in (a, a + n)} | set(hooks))
    for lo, hi in zip(cuts, cuts[1:]):
        def body(s, carry, lo=lo):
            _run(*[fn(s - a) for fn, a, n in streams if a <= lo < a + n])
            return carry

        if lo in hooks:
            hooks[lo]()
        if hi - lo == 1:
            body(lo, 0)
        else:
            lax.fori_loop(lo, hi, body, 0)


def _left(a11, a12, a21, a22):
    return a21 + a22, a22, a11 + a22, a12 - a22, a11 + a12, a11, a21 - a11


def _right(b11, b12, b21, b22):
    return b11, b21 - b11, b11 + b22, b21 + b22, b22, b12 - b22, b11 + b12


def _strassen(product, emit):
    c = {}

    def run(k):
        c[k] = r = product(k)
        if k == 1:
            emit(1, 0, c[0] + r)
        elif k == 2:
            c[11], c[22] = r + c[1], r - c[0]
        elif k == 3:
            c[11] = c[11] + r
        elif k == 4:
            emit(0, 0, c[11] - r)
        elif k == 5:
            emit(0, 1, c[4] + r)
            c[22] = c[22] + r
        elif k == 6:
            emit(1, 1, c[22] + r)

    return [lambda k=k: run(k) for k in range(7)]


def _rows(i, n):
    return pl.ds(i * n if isinstance(i, int) else pl.multiple_of(i * n, n), n)


def _kernel(zero_ref, x_hbm, are_hbm, aim_hbm, bre_hbm, bim_hbm, cre_hbm, cim_hbm, ldt_hbm, dsk_hbm,
            wqkv_hbm, wo_hbm, f_hbm, g_hbm, out_hbm,
            xs, kf, ua, ub, uc, yb, par, zw, lag, qa, ka, va, qb, kb, vb, io, abc, perm, wqkv, wo, fm, gm, kt, un, wt, us, wot, ob, ldt_ref, dsk_ref, sems):
    step = lambda fn, *a: (lambda: fn(*a))
    qs, ks, vs = (qa, qb), (ka, kb), (va, vb)
    head, rest = ([pltpu.make_async_copy(s.at[rows], abc.at[i, rows], sems.at[base + i])
                   for i, s in enumerate((are_hbm, aim_hbm, bre_hbm, bim_hbm, cre_hbm, cim_hbm))]
                  for base, rows in ((19, pl.ds(0, 32 * KPER)), (25, pl.ds(32 * KPER, D - 32 * KPER))))
    loads = [pltpu.make_async_copy(s, d, sems.at[i]) for i, (s, d) in enumerate(
        (*((x_hbm.bitcast(U32).at[:, pl.ds(128 * c, 128)], io.at[c, pl.ds(0, L // 2)]) for c in range(NB)),
         (f_hbm, fm), (wo_hbm, wo), (g_hbm, gm),
         *((wqkv_hbm.at[:, pl.ds(128 * j, 128)], wqkv.at[j]) for j in range(12))))]
    small = [pltpu.make_async_copy(s, d, sems.at[31 + i])
             for i, (s, d) in enumerate(((ldt_hbm, ldt_ref), (dsk_hbm, dsk_ref)))]
    for c in small + head + rest:
        c.start()
    for c in small:
        c.wait()
    high = jnp.uint32(0xFFFF0000)
    halves = lambda t: (pltpu.bitcast(t << 16, F32), pltpu.bitcast(t & high, F32))

    def col(ref):
        v = ref[...].astype(F32).reshape(1, D)
        return jnp.broadcast_to(v, (128, D)).T

    par[0] = jnp.exp(col(ldt_ref))
    par[1] = col(dsk_ref) * (1.0 / L)

    ri = lax.broadcasted_iota(jnp.int32, (128, 128), 0)
    ci = lax.broadcasted_iota(jnp.int32, (128, 128), 1)
    perm[...] = pltpu.bitcast(jnp.where(ci == (ri & 7) * DH + (ri >> 3), 1.0, 0.0).astype(BF16), U32)

    for c in head:
        c.wait()
    for c in loads:
        c.start()

    def setup(i):
        get = lambda k: halves(pltpu.bitcast(abc[k, _rows(i, 16), :], U32))
        dt = halves(pltpu.bitcast(par[0, _rows(i, 16), :].astype(BF16), U32))

        def pole(h):
            mag, ang = jnp.exp(dt[h] * get(0)[h]), dt[h] * get(1)[h]
            zw[i, h, 0], zw[i, h, 1] = mag * jnp.cos(ang), mag * jnp.sin(ang)

        def weight():
            scale = (1.0 + 1.5 * 2.0 ** -9) / L
            for h, (cr, ci, br, bi) in enumerate(zip(*map(get, (4, 5, 2, 3)))):
                wr, wi = _cmul((cr, ci), (dt[h] * br, dt[h] * bi))
                zw[i, h, 2], zw[i, h, 3] = wr * scale, wi * -scale

        return [step(pole, 0), weight, step(pole, 1)]

    lags = sorted({(c, r) for c in range(8) for r in _RND[c] if r < 16}) + [(8, 0)]
    stack = lambda vs: jnp.concatenate([jnp.concatenate([v[k] for v in vs], 0) for k in range(2)], 1).astype(BF16)

    def lagsums(i):
        start = [[zw[i, h, c] for c in range(4)] for h in range(2)]
        zs, rhs, even = [], [], []

        def right(h):
            zr, zi, wr, wi = start[h]
            z = {0: (jnp.ones((8, N), F32), jnp.zeros((8, N), F32)), 1: (zr, zi)}
            for e in (2, 4, 8, 16, 32, 64, 128, 256):
                z[e] = _csq(z[e // 2])
            b = [(wr, wi)]
            for e in (16, 32, 64, 128):
                zc = (z[e][0], -z[e][1])
                b += [_cmul(v, zc) for v in b]
            zs.append(z)
            rhs.append(stack(b))

        def left(t, h):
            z = zs[h]

            def power(e):
                if e not in z:
                    low = e % 256 if e > 256 and e % 256 else e & -e
                    z[e] = _csq(z[e // 2]) if e // 2 in z and e % 2 == 0 else _cmul(power(e - low), power(low))
                return z[e]

            a = [power(256 * c + r) for c, r in (lags + lags[-1:])[CUT[t]:CUT[t + 1]]]
            o = pltpu.bitcast(lax.dot_general(stack(a), rhs[h], NT, preferred_element_type=F32), U32)
            if h:
                lag[i, 8 * CUT[t]:8 * CUT[t + 1], :] = even[t] | (o & high)
            else:
                even.append(o >> 16)

        return [f for h in range(2) for f in [step(right, h)] + [step(left, t, h) for t in range(len(CUT) - 1)]]

    def kgen(i):
        lane = lax.broadcasted_iota(jnp.int32, (8, 128), 1)
        src = (lane & 15) * 8 + lax.broadcasted_iota(jnp.int32, (8, 128), 0)

        memo = {}

        def piece(c, r):
            if r == 16:
                c = 0
            if (c, r) not in memo:
                memo[c, r] = (
                    pltpu.roll(jnp.where(lane == 0, piece(8, 0), merged(0, (0,) * 8)), 127, 1) if r == 16 else
                    jnp.take_along_axis(lag[i, _rows(lags.index((c, r)), 8), :], src, axis=1,
                                        mode="promise_in_bounds"))
            return memo[c, r]

        def merged(c, rs):
            if (c, rs) not in memo:
                memo[c, rs] = (piece(c, rs[0]) if c == 7 or min(rs) == 16 else
                               jnp.where(lane >> 4 == c, piece(c, rs[0]), merged(c + 1, rs[1:])))
            return memo[c, rs]

        for n0 in range(R0):
            kt[n0, _rows(i, 8), :] = merged(0, tuple(_RND[c][n0] for c in range(8)))

    get = lambda ref, n, rows: (ref[n, 0, rows, :], ref[n, 1, rows, :])

    def put(ref, n, rows, v):
        ref[n, 0, rows, :], ref[n, 1, rows, :] = v

    def outer(src, a, rows):
        return [_twiddle(v, a * b) for b, v in enumerate(_dft4([get(src, a + 4 * m, rows) for m in range(4)], 1))]

    def transform(lhs, dst, n0, rows):
        r = jnp.dot(lhs, _bf(fm[n0]), preferred_element_type=F32)
        put(dst, n0, rows, (r[:, :128], r[:, 128:]))

    def kfwd(n0, r):
        transform(_bf(kt[n0, _rows(r, 32), :]), ub, n0, _rows(r, 64))

    def kdft(i):
        rows, t = _rows(i, 8), []

        def inner(b):
            for m, v in enumerate(_dft4([t[a][b] for a in range(4)], 1)):
                put(kf, b + 4 * m, rows, (v[0] + par[1, rows, :], v[1]))

        return [lambda a=a: t.append(outer(ub, a, rows)) for a in range(4)] + [step(inner, b) for b in range(4)]

    def fwd(n0, r):
        transform(un[n0, _rows(r, 64), :], ua, n0, _rows(r, 64))

    def pre(a, i):
        for b, v in enumerate(outer(ua, a, _rows(i, 8))):
            put(ub, a + 4 * b, _rows(i, 8), v)

    def mid(i):
        first, t = {}, {}

        def inner(h, b):
            rows = _rows(2 * i + h, 8)
            if b == 0:
                first[h] = outer(ua, 0, rows)
            x = _dft4([first[h][b]] + [get(ub, a + 4 * b, rows) for a in range(1, 4)], 1)
            t[h, b], *y = _dft4([_cmul(x[m], get(kf, b + 4 * m, rows)) for m in range(4)], -1)
            for a in range(1, 4):
                put(uc, a + 4 * b, rows, y[a - 1])

        def last():
            for m, (v, w) in enumerate(zip(*[_dft4([t[h, b] for b in range(4)], -1) for h in range(2)])):
                put(yb, 4 * m, _rows(i, 16), [jnp.concatenate([v[k], w[k]], 0).astype(BF16) for k in range(2)])

        return [step(inner, h, b) for h in range(2) for b in range(4)] + [last]

    def post(a, i):
        rows = _rows(i, 16)
        for m, v in enumerate(_dft4([_twiddle(get(uc, a + 4 * b, rows), -a * b) for b in range(4)], -1)):
            put(yb, a + 4 * m, rows, (v[0].astype(BF16), v[1].astype(BF16)))

    def inv(n0, r):
        rows = _rows(r, 64)
        y = jnp.concatenate(get(yb, n0, rows), 1)
        xs[n0, rows, :] = xs[n0, rows, :] + jnp.dot(y, _bf(gm[n0]), preferred_element_type=F32)

    def wprep(g, t):
        ops = []

        def load():
            if t < 3:
                v = lax.dot_general(_bf(perm[...]), wqkv[4 * t + g], NT, preferred_element_type=F32)
                v = v if t else v * DH ** -0.5
                lo, hi = v[:, :256], v[:, 256:]
            else:
                v = [jnp.dot(_bf(perm[...]), wo[_rows(e, 128), _rows(g, 128)], preferred_element_type=F32)
                     for e in range(4)]
                lo, hi = (jnp.concatenate([u[64 * h:64 * h + 64] for u in v], 0).T for h in range(2))
            ops.extend((lo[:64], hi[:64], lo[64:], hi[64:]))

        def save(i, h):
            for k, a in enumerate(_left(*[v[16 * i:16 * i + 16, 128 * h:128 * h + 128] for v in ops])):
                dst = wt.at[g, k] if t < 3 else wot.at[k]
                dst[_rows(4 * (t if t < 3 else g) + i, 8), _rows(h, 128)] = pltpu.bitcast(a.astype(BF16), U32)

        return [load] + [step(save, i, h) for i in range(4) for h in range(2)]

    def xin(j, c):
        xs[2 * j, _rows(c, 128), :], xs[2 * j + 1, _rows(c, 128), :] = halves(io[c, pl.ds(j, R1, stride=8), :].T)

    def norm(n0):
        acc, stat = {}, []

        def moment(k, lo, hi):
            for i in range(lo, hi):
                v = xs[n0, 8 * i:8 * i + 8, :]
                v = jnp.square(v - stat[0]) if k else v
                acc[i % 4] = v if i < 4 else acc[i % 4] + v
            if hi == D // 8:
                v = jnp.sum(_tree(jnp.add, list(acc.values())), axis=0, keepdims=True) * (1.0 / D)
                stat.append(lax.rsqrt(v + 1e-5) if k else v)

        def scale(c):
            rows = _rows(c, 128)
            un[n0, rows, :] = get(rows).astype(BF16)

        get = lambda rows: (xs[n0, rows, :] - stat[0]) * stat[1]
        return [[step(moment, 0, 0, 64)], [step(moment, 1, i, i + 16) for i in range(0, 64, 16)],
                [step(scale, c) for c in range(4)]], get

    def norms(*aa):
        return [f for a in aa for stage in zip(*[norm(a + 4 * m)[0] for m in range(4)])
                for steps in stage for f in steps]

    def pair_norms(a):
        stages, get = zip(*[norm(a + 4 * m) for m in range(4)])

        def operands(j, c):
            (b11, b21), (b12, b22) = ((f(_rows(c, 16)), f(_rows(c + 16, 16))) for f in get[2 * j:2 * j + 2])
            for k, b in enumerate(_right(b11, b12, b21, b22)):
                us[2 * a + j, k, _rows(c, 8), :] = pltpu.bitcast(b.astype(BF16), U32)

        return ([f for k in range(2) for st in stages for f in st[k]]
                + [step(operands, j, c) for j in range(2) for c in range(16)])

    def proj(i, slot, m, t):
        p, g, ref = i >> 2, i & 3, (qs, ks, vs)[t][slot]

        def emit(half, j, r):
            ref[m + 2 * j + 7 * (t > 0), _rows(half, 64), :] = r
            if t and m + j:
                ref[m + 2 * j - 1, _rows(half, 64), :] = pltpu.roll(r, 1, 1)

        return _strassen(lambda k: jnp.dot(_bf(wt[g, k, _rows(t, 32), :]), _bf(us[2 * p + 4 * (m & 1) + (m >> 2), k]),
                                           preferred_element_type=F32), emit)

    def attn(i, slot, m0):
        p, g = i >> 2, i & 3
        first = lax.broadcasted_iota(jnp.int32, (8, 128), 1) == 0
        window = lambda ref, d: {e: ref[slot][e, 8 * d:8 * d + 8, :] for e in range(m0, m0 + W + 1)}
        s, o = {}, {}

        def logits(m, d0):
            for d in (d0, d0 + 1):
                k = window(ks, d)
                q = qs[slot][m, 8 * d:8 * d + 8, :]
                for w in range(W):
                    t = q * k[m + 7 - w]
                    s[m, w] = t if d == 0 else s[m, w] + t

        def softmax(m):
            t = [jnp.where(first, -1e9, s[m, w]) if w > m else s[m, w] for w in range(W)]
            mx = _tree(jnp.maximum, t)
            e = [jnp.exp(v - mx) for v in t]
            rs = 1.0 / _tree(jnp.add, e)
            s.update({(m, w): e[w] * rs for w in range(W)})

        def values(d):
            v = window(vs, d)
            for m in (m0, m0 + 1):
                o[m, d] = _tree(jnp.add, [s[m, w] * v[m + 7 - w] for w in range(W)])
            if d % 2 and d > 8:
                blocks = [jnp.concatenate([o[m, e - 1], o[m, e]], 0) for e in (d - 8, d) for m in (m0, m0 + 1)]
                for k, b in enumerate(_right(*blocks)):
                    ob[m0 + p, k, g, 8 * d - 72:8 * d - 56, :] = b.astype(BF16)

        return ([f for m in (m0, m0 + 1) for f in [step(logits, m, d) for d in range(0, DH, 2)] + [step(softmax, m)]]
                + [step(values, d + e) for d in range(0, 8, 2) for e in (0, 1, 8, 9)])

    def oproj(p, c, n):
        def pair(m0):
            def emit(half, j, r):
                for i in range(n):
                    at = (2 * (m0 + j) + p, _rows(2 * (c + i) + half, 64))
                    xs[at] = xs[at] + r[64 * i:64 * i + 64]

            return _strassen(lambda k: jnp.dot(_bf(wot[k, 32 * c:32 * (c + n), :]), ob[m0 + p, k].reshape(D // 2, R1),
                                               preferred_element_type=F32), emit)

        return [f for m0 in range(0, 8, 2) for f in pair(m0)]

    def xout(c, j):
        lo, hi = (pltpu.bitcast(xs[2 * j + k, _rows(c, 128), :].astype(BF16).astype(F32), U32) for k in range(2))
        io[c, pl.ds(j, R1, stride=8), :] = ((lo >> 16) | hi).T

    four = lambda fn, *aa: [step(fn, a + 4 * m, r) for a in aa for m in range(4) for r in range(2 * NB)]
    block = lambda fn, a, r: [step(fn, a + 4 * m, 2 * r + h) for h in range(2) for m in range(4)] if 0 <= r < NB else []
    rowwise = lambda fn, a, n: [step(fn, a, i) for i in range(D // n)]

    regions, zero = [], zero_ref[0]

    def slot(*streams):
        regions.append(None)
        pl.when(zero < len(regions))(lambda: _run(*streams))

    pres = lambda a: rowwise(pre, a, 8)
    posts = lambda a: rowwise(post, a, 16)
    projs = lambda i, s, ms: [f for t in (1, 2, 0) for m in ms for f in proj(i, s, m, t)]
    attns = lambda i, s: [f for m in range(0, 8, 2) for f in attn(i, s, m)]

    with jax.named_scope("kgen"):
        ng = D // 16 // KPER
        each = lambda fn: (lambda i: [f for k in range(KPER) for f in fn(KPER * i + k)])
        _pipeline([(lambda i: [lambda: [kgen(KPER * i + k) for k in range(KPER)]], 2, ng - 1),
                   (each(lagsums), 1, ng), (each(setup), 0, ng),
                   (lambda j: [step(xin, 2 * j + k, c) for k in range(2) for c in range(NB)], ng - 4, 4)],
                  {2: lambda: [c.wait() for c in rest], ng - 4: lambda: [c.wait() for c in loads[:NB]]})
    with jax.named_scope("kfwd"):
        for c in loads[NB:]:
            c.wait()
        kdfts = lambda r: [f for i in range(16) for f in kdft(16 * r + i)]
        for r, other in enumerate((norms(2, 1), *[sum(norm(n0)[0], []) for n0 in (3, 7)],
                                   sum(norm(11)[0] + norm(15)[0], []))):
            slot([f for a in range(4) for f in block(kfwd, a, r)], [f for t in (3, 0, 1, 2) for f in wprep(r, t)],
                 kdfts(r - 1) if r else [step(kgen, D // 16 - 1 - k) for k in range(KPER)], other)
        slot(four(fwd, 2), kdfts(NB - 1))
        slot(four(fwd, 1) + block(fwd, 3, 0), pres(2), norms(0))

    def layer(li, carry):
        with jax.named_scope("conv"):
            part = lambda steps, r: steps[len(steps) * r // NB:len(steps) * (r + 1) // NB] if 0 <= r < NB else []
            mids = [f for i in range(D // 16) for f in mid(i)]
            for r in range(-1, NB + 1):
                slot(block(fwd, 3, r + 2) + block(fwd, 0, r + 1) + block(inv, 0, r - 1) + block(inv, 2, r - 2)
                     + block(inv, 1, r - 2),
                     part(mids, r), part(pres(3), r + 1) + part(posts(2), r - 1) + part(posts(1), r - 1),
                     pres(1) if r < 0 else posts(3) if r == NB else [])
            slot(block(inv, 2, NB - 1) + block(inv, 1, NB - 1) + four(inv, 3), pair_norms(0))
            slot(projs(0, 0, (0, 4)), pair_norms(2))
            slot(projs(0, 0, (1, 5)), pair_norms(1))
        with jax.named_scope("attn"):
            slot(projs(1, 1, (0, 1, 4, 5)), attns(0, 0), pair_norms(3))
            both = lambda i, s: slot(projs(i + 1, 1 - s, (0, 1, 4, 5)), attns(i, s))
            lax.fori_loop(0, 3, lambda j, c: (both(2 * j + 1, 1), both(2 * j + 2, 0), c)[-1], 0)
            slot(oproj(0, 0, 2) + oproj(0, 2, 2), attns(7, 1))

        @pl.when(li == 0)
        def _():
            slot(oproj(1, 0, 2) + oproj(1, 2, 2), norms(2, 0))
            slot(four(fwd, 2), norms(1, 3))
            slot(four(fwd, 1) + block(fwd, 3, 0), pres(2))

        return carry

    lax.fori_loop(0, 2, layer, 0)

    with jax.named_scope("xout"):
        stores = [pltpu.make_async_copy(io.at[c, _rows(i, 256)],
                                        out_hbm.bitcast(U32).at[_rows(i, 256), _rows(c, 128)], sems.at[4 * c + i])
                  for c in range(NB) for i in range(4)]
        last = [f for c in range(NB) for f in oproj(1, c, 1)] + [lambda: None] * 7
        for c in range(NB):
            slot(last[28 * c + 7 * (c > 0):28 * c + 35],
                 [lambda: None] * (2 * (c == 0)) + [step(xout, c, j) for j in range(8)])
            for copy in stores[4 * c:4 * c + 4]:
                copy.start()
        for c in stores:
            c.wait()


@jax.jit
def pallas_interleave_layers__ssm_conv_s4__sliding_local_dilated__prompt_kernel(
    A_u: jax.Array,
    A_A_re: jax.Array,
    A_A_im: jax.Array,
    A_B_re: jax.Array,
    A_B_im: jax.Array,
    A_C_re: jax.Array,
    A_C_im: jax.Array,
    A_log_dt: jax.Array,
    A_Dskip: jax.Array,
    B_x: jax.Array,
    B_wqkv: jax.Array,
    B_wo: jax.Array,
):
    del B_x
    hbm = pl.BlockSpec(memory_space=pl.ANY)
    tiles = lambda *n: pltpu.VMEM((*n, 128, 128), F32)
    out = pl.pallas_call(
        _kernel,
        out_shape=jax.ShapeDtypeStruct((L, D), BF16),
        in_specs=[pl.BlockSpec(memory_space=pltpu.SMEM)] + [hbm] * 13,
        out_specs=hbm,
        scratch_shapes=[
            pltpu.VMEM((R0, D, R1), F32),
            *[pltpu.VMEM((R0, 2, D, R1), F32)] * 4,
            pltpu.VMEM((R0, 2, D, R1), BF16),
            pltpu.VMEM((2, D, N), F32),
            pltpu.VMEM((D // 16, 2, 4, 8, N), F32),
            pltpu.VMEM((D // 16, 336, 128), U32),
            *[tiles(n) for n in (8, 15, 15) * 2],
            pltpu.VMEM((NB, L // 2 + 8, 128), U32),
            pltpu.VMEM((6, D, N), BF16),
            pltpu.VMEM((64, 128), U32),
            pltpu.VMEM((12, D, 128), BF16),
            pltpu.VMEM((D, D), BF16),
            pltpu.VMEM(_F.shape, U32),
            pltpu.VMEM(_G.shape, U32),
            pltpu.VMEM((R0, D // 2, R1), U32),
            pltpu.VMEM((R0, D, R1), BF16),
            pltpu.VMEM((4, 7, 96, D // 2), U32),
            pltpu.VMEM((8, 7, D // 4, R1), U32),
            pltpu.VMEM((7, D // 4, D // 2), U32),
            pltpu.VMEM((8, 7, 4, 64, R1), BF16),
            pltpu.VMEM((D,), BF16),
            pltpu.VMEM((D,), BF16),
            pltpu.SemaphoreType.DMA((33,)),
        ],
        compiler_params=pltpu.CompilerParams(vmem_limit_bytes=100 * 1024 * 1024),
    )(np.zeros((1,), np.int32), A_u.reshape(L, D), A_A_re, A_A_im, A_B_re, A_B_im, A_C_re, A_C_im, A_log_dt, A_Dskip,
      B_wqkv, B_wo, _F, _G)
    return out.reshape(1, L, D)
```

```python
import jax
import jax.numpy as jnp
import ml_dtypes
import numpy as np
from jax import lax
import jax.experimental.pallas as pl
import jax.experimental.pallas.tpu as pltpu

L, D, N = 2048, 512, 128
R0, R1 = 16, 128
W, DH = 8, 16
F32, BF16, U32 = jnp.float32, jnp.bfloat16, jnp.uint32
CUT = (0, 20, 42)
KPER = 4
NB = D // 128
NT = (((1,), (1,)), ((), ()))


def _constants():
    n0 = np.arange(R0)[:, None, None]
    n1 = np.arange(R1)[None, :, None]
    k1 = np.arange(R1)[None, None, :]
    ang = 2.0 * np.pi * (k1 + 0.25) * (R0 * n1 + n0) / L
    f = np.concatenate([np.cos(ang), np.sin(ang)], axis=2)
    g = f.transpose(0, 2, 1)
    bf = ml_dtypes.bfloat16
    lr = np.arange(L).astype(np.float32).astype(bf).astype(np.int64).reshape(8, 16, R0)
    r = lr - (256 * np.arange(8)[:, None, None] + 16 * np.arange(16)[None, :, None])
    assert (r == r[:, :1, :]).all()

    def words(m):
        h = np.ascontiguousarray(m).astype(bf).view(np.uint16).astype(np.uint32)
        return h[:, 0::2] | (h[:, 1::2] << 16)

    return words(f), words(g), r[:, 0, :].tolist()


_F, _G, _RND = _constants()


def _cmul(a, b):
    return a[0] * b[0] - a[1] * b[1], a[0] * b[1] + a[1] * b[0]


def _csq(a):
    t = a[0] * a[1]
    return (a[0] + a[1]) * (a[0] - a[1]), t + t


def _dft4(x, sign):
    (ar, ai), (br, bi), (cr, ci), (dr, di) = x
    sr, si, tr, ti = ar + cr, ai + ci, ar - cr, ai - ci
    ur, ui, vr, vi = br + dr, bi + di, br - dr, bi - di
    p, m = (tr - vi, ti + vr), (tr + vi, ti - vr)
    if sign < 0:
        p, m = m, p
    return [(sr + ur, si + ui), p, (sr - ur, si - ui), m]


def _twiddle(v, e):
    e %= 16
    re, im = v
    h = float(np.sqrt(0.5))
    if e == 0:
        return v
    if e == 4:
        return -im, re
    if e == 12:
        return im, -re
    if e == 2:
        return (re - im) * h, (re + im) * h
    if e == 14:
        return (re + im) * h, (im - re) * h
    if e == 6:
        return (re + im) * -h, (re - im) * h
    if e == 10:
        return (im - re) * h, (re + im) * -h
    c, s = float(np.cos(np.pi * e / 8)), float(np.sin(np.pi * e / 8))
    return re * c - im * s, re * s + im * c


def _bf(x):
    return pltpu.bitcast(x, BF16)


def _tree(op, v):
    while len(v) > 1:
        v = [op(v[i], v[i + 1]) if i + 1 < len(v) else v[i] for i in range(0, len(v), 2)]
    return v[0]


def _run(*streams):
    order = sorted(((i + 0.5 * (k > 0)) / len(s), k, i) for k, s in enumerate(streams) for i in range(len(s)))
    for _, k, i in order:
        streams[k][i]()


def _pipeline(streams, hooks=None):
    hooks = hooks or {}
    cuts = sorted({e for _, a, n in streams for e in (a, a + n)} | set(hooks))
    for lo, hi in zip(cuts, cuts[1:]):
        def body(s, carry, lo=lo):
            _run(*[fn(s - a) for fn, a, n in streams if a <= lo < a + n])
            return carry

        if lo in hooks:
            hooks[lo]()
        if hi - lo == 1:
            body(lo, 0)
        else:
            lax.fori_loop(lo, hi, body, 0)


def _left(a11, a12, a21, a22):
    return a21 + a22, a22, a11 + a22, a12 - a22, a11 + a12, a11, a21 - a11


def _right(b11, b12, b21, b22):
    return b11, b21 - b11, b11 + b22, b21 + b22, b22, b12 - b22, b11 + b12


def _strassen(product, emit):
    c = {}

    def run(k):
        c[k] = r = product(k)
        if k == 1:
            emit(1, 0, c[0] + r)
        elif k == 2:
            c[11], c[22] = r + c[1], r - c[0]
        elif k == 3:
            c[11] = c[11] + r
        elif k == 4:
            emit(0, 0, c[11] - r)
        elif k == 5:
            emit(0, 1, c[4] + r)
            c[22] = c[22] + r
        elif k == 6:
            emit(1, 1, c[22] + r)

    return [lambda k=k: run(k) for k in range(7)]


def _rows(i, n):
    return pl.ds(i * n if isinstance(i, int) else pl.multiple_of(i * n, n), n)


def _kernel(zero_ref, x_hbm, are_hbm, aim_hbm, bre_hbm, bim_hbm, cre_hbm, cim_hbm, ldt_hbm, dsk_hbm,
            wqkv_hbm, wo_hbm, f_hbm, g_hbm, out_hbm,
            xs, kf, ua, ub, uc, yb, par, zw, lag, qa, ka, va, qb, kb, vb,
            xio, io, abc, perm, wqkv, wo, fm, gm, kt, un, wt, us, wot, ob, ldt_ref, dsk_ref, sems):
    step = lambda fn, *a: (lambda: fn(*a))
    qs, ks, vs = (qa, qb), (ka, kb), (va, vb)
    head, rest = ([pltpu.make_async_copy(s.at[rows], abc.at[i, rows], sems.at[base + i])
                   for i, s in enumerate((are_hbm, aim_hbm, bre_hbm, bim_hbm, cre_hbm, cim_hbm))]
                  for base, rows in ((19, pl.ds(0, 32 * KPER)), (25, pl.ds(32 * KPER, D - 32 * KPER))))
    loads = [pltpu.make_async_copy(s, d, sems.at[i]) for i, (s, d) in enumerate(
        (*((x_hbm.at[:, _rows(c, 128)], xio.at[c]) for c in range(NB)),
         (f_hbm, fm), (wo_hbm, wo), (g_hbm, gm),
         *((wqkv_hbm.at[:, pl.ds(128 * j, 128)], wqkv.at[j]) for j in range(12))))]
    small = [pltpu.make_async_copy(s, d, sems.at[31 + i])
             for i, (s, d) in enumerate(((ldt_hbm, ldt_ref), (dsk_hbm, dsk_ref)))]
    for c in small + head + rest:
        c.start()
    for c in small:
        c.wait()
    high = jnp.uint32(0xFFFF0000)
    halves = lambda t: (pltpu.bitcast(t << 16, F32), pltpu.bitcast(t & high, F32))

    def col(ref):
        v = ref[...].astype(F32).reshape(1, D)
        return jnp.broadcast_to(v, (128, D)).T

    par[0] = jnp.exp(col(ldt_ref))
    par[1] = col(dsk_ref) * (1.0 / L)

    ri = lax.broadcasted_iota(jnp.int32, (128, 128), 0)
    ci = lax.broadcasted_iota(jnp.int32, (128, 128), 1)
    perm[...] = pltpu.bitcast(jnp.where(ci == (ri & 7) * DH + (ri >> 3), 1.0, 0.0).astype(BF16), U32)

    for c in head:
        c.wait()
    for c in loads:
        c.start()

    def setup(i):
        get = lambda k: halves(pltpu.bitcast(abc[k, _rows(i, 16), :], U32))
        dt = halves(pltpu.bitcast(par[0, _rows(i, 16), :].astype(BF16), U32))

        def pole(h):
            mag, ang = jnp.exp(dt[h] * get(0)[h]), dt[h] * get(1)[h]
            zw[i, h, 0], zw[i, h, 1] = mag * jnp.cos(ang), mag * jnp.sin(ang)

        def weight():
            scale = (1.0 + 1.5 * 2.0 ** -9) / L
            for h, (cr, ci, br, bi) in enumerate(zip(*map(get, (4, 5, 2, 3)))):
                wr, wi = _cmul((cr, ci), (dt[h] * br, dt[h] * bi))
                zw[i, h, 2], zw[i, h, 3] = wr * scale, wi * -scale

        return [step(pole, 0), weight, step(pole, 1)]

    lags = sorted({(c, r) for c in range(8) for r in _RND[c] if r < 16}) + [(8, 0)]
    stack = lambda vs: jnp.concatenate([jnp.concatenate([v[k] for v in vs], 0) for k in range(2)], 1).astype(BF16)

    def lagsums(i):
        start = [[zw[i, h, c] for c in range(4)] for h in range(2)]
        zs, rhs, even = [], [], []

        def right(h):
            zr, zi, wr, wi = start[h]
            z = {0: (jnp.ones((8, N), F32), jnp.zeros((8, N), F32)), 1: (zr, zi)}
            for e in (2, 4, 8, 16, 32, 64, 128, 256):
                z[e] = _csq(z[e // 2])
            b = [(wr, wi)]
            for e in (16, 32, 64, 128):
                zc = (z[e][0], -z[e][1])
                b += [_cmul(v, zc) for v in b]
            zs.append(z)
            rhs.append(stack(b))

        def left(t, h):
            z = zs[h]

            def power(e):
                if e not in z:
                    low = e % 256 if e > 256 and e % 256 else e & -e
                    z[e] = _csq(z[e // 2]) if e // 2 in z and e % 2 == 0 else _cmul(power(e - low), power(low))
                return z[e]

            a = [power(256 * c + r) for c, r in (lags + lags[-1:])[CUT[t]:CUT[t + 1]]]
            o = pltpu.bitcast(lax.dot_general(stack(a), rhs[h], NT, preferred_element_type=F32), U32)
            if h:
                lag[i, 8 * CUT[t]:8 * CUT[t + 1], :] = even[t] | (o & high)
            else:
                even.append(o >> 16)

        return [f for h in range(2) for f in [step(right, h)] + [step(left, t, h) for t in range(len(CUT) - 1)]]

    def kgen(i):
        lane = lax.broadcasted_iota(jnp.int32, (8, 128), 1)
        src = (lane & 15) * 8 + lax.broadcasted_iota(jnp.int32, (8, 128), 0)

        memo = {}

        def piece(c, r):
            if r == 16:
                c = 0
            if (c, r) not in memo:
                memo[c, r] = (
                    pltpu.roll(jnp.where(lane == 0, piece(8, 0), merged(0, (0,) * 8)), 127, 1) if r == 16 else
                    jnp.take_along_axis(lag[i, _rows(lags.index((c, r)), 8), :], src, axis=1,
                                        mode="promise_in_bounds"))
            return memo[c, r]

        def merged(c, rs):
            if (c, rs) not in memo:
                memo[c, rs] = (piece(c, rs[0]) if c == 7 or min(rs) == 16 else
                               jnp.where(lane >> 4 == c, piece(c, rs[0]), merged(c + 1, rs[1:])))
            return memo[c, rs]

        for n0 in range(R0):
            kt[n0, _rows(i, 8), :] = merged(0, tuple(_RND[c][n0] for c in range(8)))

    get = lambda ref, n, rows: (ref[n, 0, rows, :], ref[n, 1, rows, :])

    def put(ref, n, rows, v):
        ref[n, 0, rows, :], ref[n, 1, rows, :] = v

    def outer(src, a, rows):
        return [_twiddle(v, a * b) for b, v in enumerate(_dft4([get(src, a + 4 * m, rows) for m in range(4)], 1))]

    def transform(lhs, dst, n0, rows):
        r = jnp.dot(lhs, _bf(fm[n0]), preferred_element_type=F32)
        put(dst, n0, rows, (r[:, :128], r[:, 128:]))

    def kfwd(n0, r):
        transform(_bf(kt[n0, _rows(r, 32), :]), ub, n0, _rows(r, 64))

    def kdft(i):
        rows, t = _rows(i, 8), []

        def inner(b):
            for m, v in enumerate(_dft4([t[a][b] for a in range(4)], 1)):
                put(kf, b + 4 * m, rows, (v[0] + par[1, rows, :], v[1]))

        return [lambda a=a: t.append(outer(ub, a, rows)) for a in range(4)] + [step(inner, b) for b in range(4)]

    def fwd(n0, r):
        transform(un[n0, _rows(r, 64), :], ua, n0, _rows(r, 64))

    def pre(a, i):
        for b, v in enumerate(outer(ua, a, _rows(i, 8))):
            put(ub, a + 4 * b, _rows(i, 8), v)

    def mid(i):
        first, t = {}, {}

        def inner(h, b):
            rows = _rows(2 * i + h, 8)
            if b == 0:
                first[h] = outer(ua, 0, rows)
            x = _dft4([first[h][b]] + [get(ub, a + 4 * b, rows) for a in range(1, 4)], 1)
            t[h, b], *y = _dft4([_cmul(x[m], get(kf, b + 4 * m, rows)) for m in range(4)], -1)
            for a in range(1, 4):
                put(uc, a + 4 * b, rows, y[a - 1])

        def last():
            for m, (v, w) in enumerate(zip(*[_dft4([t[h, b] for b in range(4)], -1) for h in range(2)])):
                put(yb, 4 * m, _rows(i, 16), [jnp.concatenate([v[k], w[k]], 0).astype(BF16) for k in range(2)])

        return [step(inner, h, b) for h in range(2) for b in range(4)] + [last]

    def post(a, i):
        rows = _rows(i, 16)
        for m, v in enumerate(_dft4([_twiddle(get(uc, a + 4 * b, rows), -a * b) for b in range(4)], -1)):
            put(yb, a + 4 * m, rows, (v[0].astype(BF16), v[1].astype(BF16)))

    def inv(n0, r):
        rows = _rows(r, 64)
        y = jnp.concatenate(get(yb, n0, rows), 1)
        xs[n0, rows, :] = xs[n0, rows, :] + jnp.dot(y, _bf(gm[n0]), preferred_element_type=F32)

    def wprep(g, t):
        ops = []

        def load():
            if t < 3:
                v = lax.dot_general(_bf(perm[...]), wqkv[4 * t + g], NT, preferred_element_type=F32)
                v = v if t else v * DH ** -0.5
                lo, hi = v[:, :256], v[:, 256:]
            else:
                v = [jnp.dot(_bf(perm[...]), wo[_rows(e, 128), _rows(g, 128)], preferred_element_type=F32)
                     for e in range(4)]
                lo, hi = (jnp.concatenate([u[64 * h:64 * h + 64] for u in v], 0).T for h in range(2))
            ops.extend((lo[:64], hi[:64], lo[64:], hi[64:]))

        def save(i, h):
            for k, a in enumerate(_left(*[v[16 * i:16 * i + 16, 128 * h:128 * h + 128] for v in ops])):
                dst = wt.at[g, k] if t < 3 else wot.at[k]
                dst[_rows(4 * (t if t < 3 else g) + i, 8), _rows(h, 128)] = pltpu.bitcast(a.astype(BF16), U32)

        return [load] + [step(save, i, h) for i in range(4) for h in range(2)]

    def words(c):
        io[c, :L // 2, :] = pltpu.bitcast(xio[c], U32)

    def xin(j, c):
        xs[2 * j, _rows(c, 128), :], xs[2 * j + 1, _rows(c, 128), :] = halves(io[c, pl.ds(j, R1, stride=8), :].T)

    def norm(n0):
        acc, stat = {}, []

        def moment(k, lo, hi):
            for i in range(lo, hi):
                v = xs[n0, 8 * i:8 * i + 8, :]
                v = jnp.square(v - stat[0]) if k else v
                acc[i % 4] = v if i < 4 else acc[i % 4] + v
            if hi == D // 8:
                v = jnp.sum(_tree(jnp.add, list(acc.values())), axis=0, keepdims=True) * (1.0 / D)
                stat.append(lax.rsqrt(v + 1e-5) if k else v)

        def scale(c):
            rows = _rows(c, 128)
            un[n0, rows, :] = get(rows).astype(BF16)

        get = lambda rows: (xs[n0, rows, :] - stat[0]) * stat[1]
        return [[step(moment, 0, 0, 64)], [step(moment, 1, i, i + 16) for i in range(0, 64, 16)],
                [step(scale, c) for c in range(4)]], get

    def norms(*aa):
        return [f for a in aa for stage in zip(*[norm(a + 4 * m)[0] for m in range(4)])
                for steps in stage for f in steps]

    def pair_norms(a):
        stages, get = zip(*[norm(a + 4 * m) for m in range(4)])

        def operands(j, c):
            (b11, b21), (b12, b22) = ((f(_rows(c, 16)), f(_rows(c + 16, 16))) for f in get[2 * j:2 * j + 2])
            for k, b in enumerate(_right(b11, b12, b21, b22)):
                us[2 * a + j, k, _rows(c, 8), :] = pltpu.bitcast(b.astype(BF16), U32)

        return ([f for k in range(2) for st in stages for f in st[k]]
                + [step(operands, j, c) for j in range(2) for c in range(16)])

    def proj(i, slot, m, t):
        p, g, ref = i >> 2, i & 3, (qs, ks, vs)[t][slot]

        def emit(half, j, r):
            ref[m + 2 * j + 7 * (t > 0), _rows(half, 64), :] = r
            if t and m + j:
                ref[m + 2 * j - 1, _rows(half, 64), :] = pltpu.roll(r, 1, 1)

        return _strassen(lambda k: jnp.dot(_bf(wt[g, k, _rows(t, 32), :]), _bf(us[2 * p + 4 * (m & 1) + (m >> 2), k]),
                                           preferred_element_type=F32), emit)

    def attn(i, slot, m0):
        p, g = i >> 2, i & 3
        first = lax.broadcasted_iota(jnp.int32, (8, 128), 1) == 0
        window = lambda ref, d: {e: ref[slot][e, 8 * d:8 * d + 8, :] for e in range(m0, m0 + W + 1)}
        s, o = {}, {}

        def logits(m, d0):
            for d in (d0, d0 + 1):
                k = window(ks, d)
                q = qs[slot][m, 8 * d:8 * d + 8, :]
                for w in range(W):
                    t = q * k[m + 7 - w]
                    s[m, w] = t if d == 0 else s[m, w] + t

        def softmax(m):
            t = [jnp.where(first, -1e9, s[m, w]) if w > m else s[m, w] for w in range(W)]
            mx = _tree(jnp.maximum, t)
            e = [jnp.exp(v - mx) for v in t]
            rs = 1.0 / _tree(jnp.add, e)
            s.update({(m, w): e[w] * rs for w in range(W)})

        def values(d):
            v = window(vs, d)
            for m in (m0, m0 + 1):
                o[m, d] = _tree(jnp.add, [s[m, w] * v[m + 7 - w] for w in range(W)])
            if d % 2 and d > 8:
                blocks = [jnp.concatenate([o[m, e - 1], o[m, e]], 0) for e in (d - 8, d) for m in (m0, m0 + 1)]
                for k, b in enumerate(_right(*blocks)):
                    ob[m0 + p, k, g, 8 * d - 72:8 * d - 56, :] = b.astype(BF16)

        return ([f for m in (m0, m0 + 1) for f in [step(logits, m, d) for d in range(0, DH, 2)] + [step(softmax, m)]]
                + [step(values, d + e) for d in range(0, 8, 2) for e in (0, 1, 8, 9)])

    def oproj(p, c, n):
        def pair(m0):
            def emit(half, j, r):
                for i in range(n):
                    at = (2 * (m0 + j) + p, _rows(2 * (c + i) + half, 64))
                    xs[at] = xs[at] + r[64 * i:64 * i + 64]

            return _strassen(lambda k: jnp.dot(_bf(wot[k, 32 * c:32 * (c + n), :]), ob[m0 + p, k].reshape(D // 2, R1),
                                               preferred_element_type=F32), emit)

        return [f for m0 in range(0, 8, 2) for f in pair(m0)]

    def xout(c, j):
        lo, hi = (pltpu.bitcast(xs[2 * j + k, _rows(c, 128), :].astype(BF16).astype(F32), U32) for k in range(2))
        io[c, pl.ds(j, R1, stride=8), :] = ((lo >> 16) | hi).T

    four = lambda fn, *aa: [step(fn, a + 4 * m, r) for a in aa for m in range(4) for r in range(2 * NB)]
    block = lambda fn, a, r: [step(fn, a + 4 * m, 2 * r + h) for h in range(2) for m in range(4)] if 0 <= r < NB else []
    rowwise = lambda fn, a, n: [step(fn, a, i) for i in range(D // n)]

    regions, zero = [], zero_ref[0]

    def slot(*streams):
        regions.append(None)
        pl.when(zero < len(regions))(lambda: _run(*streams))

    pres = lambda a: rowwise(pre, a, 8)
    posts = lambda a: rowwise(post, a, 16)
    projs = lambda i, s, ms: [f for t in (1, 2, 0) for m in ms for f in proj(i, s, m, t)]
    attns = lambda i, s: [f for m in range(0, 8, 2) for f in attn(i, s, m)]

    with jax.named_scope("kgen"):
        ng = D // 16 // KPER
        each = lambda fn: (lambda i: [f for k in range(KPER) for f in fn(KPER * i + k)])
        _pipeline([(lambda i: [lambda: [kgen(KPER * i + k) for k in range(KPER)]], 2, ng - 1),
                   (each(lagsums), 1, ng), (each(setup), 0, ng),
                   (lambda c: [step(words, c)] + [step(xin, j, c) for j in range(8)], ng - NB, NB)],
                  {2: lambda: [c.wait() for c in rest], ng - NB: lambda: [c.wait() for c in loads[:NB]]})
    with jax.named_scope("kfwd"):
        for c in loads[NB:]:
            c.wait()
        kdfts = lambda r: [f for i in range(16) for f in kdft(16 * r + i)]
        for r, other in enumerate((norms(2, 1), *[sum(norm(n0)[0], []) for n0 in (3, 7)],
                                   sum(norm(11)[0] + norm(15)[0], []))):
            slot([f for a in range(4) for f in block(kfwd, a, r)], [f for t in (3, 0, 1, 2) for f in wprep(r, t)],
                 kdfts(r - 1) if r else [step(kgen, D // 16 - 1 - k) for k in range(KPER)], other)
        slot(four(fwd, 2), kdfts(NB - 1))
        slot(four(fwd, 1) + block(fwd, 3, 0), pres(2), norms(0))

    def layer(li, carry):
        with jax.named_scope("conv"):
            part = lambda steps, r: steps[len(steps) * r // NB:len(steps) * (r + 1) // NB] if 0 <= r < NB else []
            mids = [f for i in range(D // 16) for f in mid(i)]
            for r in range(-1, NB + 1):
                slot(block(fwd, 3, r + 2) + block(fwd, 0, r + 1) + block(inv, 0, r - 1) + block(inv, 2, r - 2)
                     + block(inv, 1, r - 2),
                     part(mids, r), part(pres(3), r + 1) + part(posts(2), r - 1) + part(posts(1), r - 1),
                     pres(1) if r < 0 else posts(3) if r == NB else [])
            slot(block(inv, 2, NB - 1) + block(inv, 1, NB - 1) + four(inv, 3), pair_norms(0))
            slot(projs(0, 0, (0, 4)), pair_norms(2))
            slot(projs(0, 0, (1, 5)), pair_norms(1))
        with jax.named_scope("attn"):
            slot(projs(1, 1, (0, 1, 4, 5)), attns(0, 0), pair_norms(3))
            both = lambda i, s: slot(projs(i + 1, 1 - s, (0, 1, 4, 5)), attns(i, s))
            lax.fori_loop(0, 3, lambda j, c: (both(2 * j + 1, 1), both(2 * j + 2, 0), c)[-1], 0)
            slot(oproj(0, 0, 2) + oproj(0, 2, 2), attns(7, 1))

        @pl.when(li == 0)
        def _():
            slot(oproj(1, 0, 2) + oproj(1, 2, 2), norms(2, 0))
            slot(four(fwd, 2), norms(1, 3))
            slot(four(fwd, 1) + block(fwd, 3, 0), pres(2))

        return carry

    lax.fori_loop(0, 2, layer, 0)

    with jax.named_scope("xout"):
        stores = [pltpu.make_async_copy(xio.at[c, _rows(i, 512)], out_hbm.at[_rows(i, 512), _rows(c, 128)],
                                        sems.at[4 * c + i]) for c in range(NB) for i in range(4)]
        last = [f for c in range(NB) for f in oproj(1, c, 1)] + [lambda: None] * 7
        for c in range(NB):
            slot(last[28 * c + 7 * (c > 0):28 * c + 35],
                 [lambda: None] * (2 * (c == 0)) + [step(xout, c, j) for j in range(8)])
            for i in range(4):
                xio[c, _rows(i, 512), :] = _bf(io[c, _rows(i, 256), :])
                stores[4 * c + i].start()
        for c in stores:
            c.wait()


@jax.jit
def pallas_interleave_layers__ssm_conv_s4__sliding_local_dilated__prompt_kernel(
    A_u: jax.Array,
    A_A_re: jax.Array,
    A_A_im: jax.Array,
    A_B_re: jax.Array,
    A_B_im: jax.Array,
    A_C_re: jax.Array,
    A_C_im: jax.Array,
    A_log_dt: jax.Array,
    A_Dskip: jax.Array,
    B_x: jax.Array,
    B_wqkv: jax.Array,
    B_wo: jax.Array,
):
    del B_x
    hbm = pl.BlockSpec(memory_space=pl.ANY)
    tiles = lambda *n: pltpu.VMEM((*n, 128, 128), F32)
    out = pl.pallas_call(
        _kernel,
        out_shape=jax.ShapeDtypeStruct((L, D), BF16),
        in_specs=[pl.BlockSpec(memory_space=pltpu.SMEM)] + [hbm] * 13,
        out_specs=hbm,
        scratch_shapes=[
            pltpu.VMEM((R0, D, R1), F32),
            *[pltpu.VMEM((R0, 2, D, R1), F32)] * 4,
            pltpu.VMEM((R0, 2, D, R1), BF16),
            pltpu.VMEM((2, D, N), F32),
            pltpu.VMEM((D // 16, 2, 4, 8, N), F32),
            pltpu.VMEM((D // 16, 336, 128), U32),
            *[tiles(n) for n in (8, 15, 15) * 2],
            pltpu.VMEM((NB, L, 128), BF16),
            pltpu.VMEM((NB, L // 2 + 8, 128), U32),
            pltpu.VMEM((6, D, N), BF16),
            pltpu.VMEM((64, 128), U32),
            pltpu.VMEM((12, D, 128), BF16),
            pltpu.VMEM((D, D), BF16),
            pltpu.VMEM(_F.shape, U32),
            pltpu.VMEM(_G.shape, U32),
            pltpu.VMEM((R0, D // 2, R1), U32),
            pltpu.VMEM((R0, D, R1), BF16),
            pltpu.VMEM((4, 7, 96, D // 2), U32),
            pltpu.VMEM((8, 7, D // 4, R1), U32),
            pltpu.VMEM((7, D // 4, D // 2), U32),
            pltpu.VMEM((8, 7, 4, 64, R1), BF16),
            pltpu.VMEM((D,), BF16),
            pltpu.VMEM((D,), BF16),
            pltpu.SemaphoreType.DMA((33,)),
        ],
        compiler_params=pltpu.CompilerParams(vmem_limit_bytes=100 * 1024 * 1024),
    )(np.zeros((1,), np.int32), A_u.reshape(L, D), A_A_re, A_A_im, A_B_re, A_B_im, A_C_re, A_C_im, A_log_dt, A_Dskip,
      B_wqkv, B_wo, _F, _G)
    return out.reshape(1, L, D)
```

```python
import jax
import jax.numpy as jnp
import ml_dtypes
import numpy as np
from jax import lax
import jax.experimental.pallas as pl
import jax.experimental.pallas.tpu as pltpu

L, D, N = 2048, 512, 128
R0, R1 = 16, 128
W, DH = 8, 16
F32, BF16, U32 = jnp.float32, jnp.bfloat16, jnp.uint32
KPER = 4
NB = D // 128
NT = (((1,), (1,)), ((), ()))


def _constants():
    n0 = np.arange(R0)[:, None, None]
    n1 = np.arange(R1)[None, :, None]
    k1 = np.arange(R1)[None, None, :]
    ang = 2.0 * np.pi * (k1 + 0.25) * (R0 * n1 + n0) / L
    f = np.concatenate([np.cos(ang), np.sin(ang)], axis=2)
    g = f.transpose(0, 2, 1)
    bf = ml_dtypes.bfloat16
    lr = np.arange(L).astype(np.float32).astype(bf).astype(np.int64).reshape(8, 16, R0)
    r = lr - (256 * np.arange(8)[:, None, None] + 16 * np.arange(16)[None, :, None])
    assert (r == r[:, :1, :]).all()

    def words(m):
        h = np.ascontiguousarray(m).astype(bf).view(np.uint16).astype(np.uint32)
        return h[:, 0::2] | (h[:, 1::2] << 16)

    return words(f), words(g), r[:, 0, :].tolist()


_F, _G, _RND = _constants()


def _cmul(a, b):
    return a[0] * b[0] - a[1] * b[1], a[0] * b[1] + a[1] * b[0]


def _csq(a):
    t = a[0] * a[1]
    return (a[0] + a[1]) * (a[0] - a[1]), t + t


def _dft4(x, sign):
    (ar, ai), (br, bi), (cr, ci), (dr, di) = x
    sr, si, tr, ti = ar + cr, ai + ci, ar - cr, ai - ci
    ur, ui, vr, vi = br + dr, bi + di, br - dr, bi - di
    p, m = (tr - vi, ti + vr), (tr + vi, ti - vr)
    if sign < 0:
        p, m = m, p
    return [(sr + ur, si + ui), p, (sr - ur, si - ui), m]


def _twiddle(v, e):
    e %= 16
    re, im = v
    h = float(np.sqrt(0.5))
    if e == 0:
        return v
    if e == 4:
        return -im, re
    if e == 12:
        return im, -re
    if e == 2:
        return (re - im) * h, (re + im) * h
    if e == 14:
        return (re + im) * h, (im - re) * h
    if e == 6:
        return (re + im) * -h, (re - im) * h
    if e == 10:
        return (im - re) * h, (re + im) * -h
    c, s = float(np.cos(np.pi * e / 8)), float(np.sin(np.pi * e / 8))
    return re * c - im * s, re * s + im * c


def _bf(x):
    return pltpu.bitcast(x, BF16)


def _tree(op, v):
    while len(v) > 1:
        v = [op(v[i], v[i + 1]) if i + 1 < len(v) else v[i] for i in range(0, len(v), 2)]
    return v[0]


def _run(*streams):
    order = sorted(((i + 0.5 * (k > 0)) / len(s), k, i) for k, s in enumerate(streams) for i in range(len(s)))
    for _, k, i in order:
        streams[k][i]()


def _pipeline(streams, hooks=None):
    hooks = hooks or {}
    cuts = sorted({e for _, a, n in streams for e in (a, a + n)} | set(hooks))
    for lo, hi in zip(cuts, cuts[1:]):
        def body(s, carry, lo=lo):
            _run(*[fn(s - a) for fn, a, n in streams if a <= lo < a + n])
            return carry

        if lo in hooks:
            hooks[lo]()
        if hi - lo == 1:
            body(lo, 0)
        else:
            lax.fori_loop(lo, hi, body, 0)


def _left(a11, a12, a21, a22):
    return a21 + a22, a22, a11 + a22, a12 - a22, a11 + a12, a11, a21 - a11


def _right(b11, b12, b21, b22):
    return b11, b21 - b11, b11 + b22, b21 + b22, b22, b12 - b22, b11 + b12


def _strassen(product, emit):
    c = {}

    def run(k):
        c[k] = r = product(k)
        if k == 1:
            emit(1, 0, c[0] + r)
        elif k == 2:
            c[11], c[22] = r + c[1], r - c[0]
        elif k == 3:
            c[11] = c[11] + r
        elif k == 4:
            emit(0, 0, c[11] - r)
        elif k == 5:
            emit(0, 1, c[4] + r)
            c[22] = c[22] + r
        elif k == 6:
            emit(1, 1, c[22] + r)

    return [lambda k=k: run(k) for k in range(7)]


def _rows(i, n):
    return pl.ds(i * n if isinstance(i, int) else pl.multiple_of(i * n, n), n)


def _kernel(zero_ref, x_hbm, are_hbm, aim_hbm, bre_hbm, bim_hbm, cre_hbm, cim_hbm, ldt_hbm, dsk_hbm,
            wqkv_hbm, wo_hbm, f_hbm, g_hbm, out_hbm,
            xs, kf, ua, ub, uc, yb, par, zw, lag, qa, ka, va, qb, kb, vb,
            xio, io, abc, perm, wqkv, wo, fm, gm, kt, un, wt, us, wot, ob, ldt_ref, dsk_ref, sems):
    step = lambda fn, *a: (lambda: fn(*a))
    qs, ks, vs = (qa, qb), (ka, kb), (va, vb)
    head, rest = ([pltpu.make_async_copy(s.at[rows], abc.at[i, rows], sems.at[base + i])
                   for i, s in enumerate((are_hbm, aim_hbm, bre_hbm, bim_hbm, cre_hbm, cim_hbm))]
                  for base, rows in ((19, pl.ds(0, 32 * KPER)), (25, pl.ds(32 * KPER, D - 32 * KPER))))
    loads = [pltpu.make_async_copy(s, d, sems.at[i]) for i, (s, d) in enumerate(
        (*((x_hbm.at[:, _rows(c, 128)], xio.at[c]) for c in range(NB)),
         (f_hbm, fm), (wo_hbm, wo), (g_hbm, gm),
         *((wqkv_hbm.at[:, pl.ds(128 * j, 128)], wqkv.at[j]) for j in range(12))))]
    small = [pltpu.make_async_copy(s, d, sems.at[31 + i])
             for i, (s, d) in enumerate(((ldt_hbm, ldt_ref), (dsk_hbm, dsk_ref)))]
    for c in small + head + rest:
        c.start()
    for c in small:
        c.wait()
    high = jnp.uint32(0xFFFF0000)
    halves = lambda t: (pltpu.bitcast(t << 16, F32), pltpu.bitcast(t & high, F32))

    def col(ref):
        v = ref[...].astype(F32).reshape(1, D)
        return jnp.broadcast_to(v, (128, D)).T

    par[0] = jnp.exp(col(ldt_ref))
    par[1] = col(dsk_ref) * (1.0 / L)

    ri = lax.broadcasted_iota(jnp.int32, (128, 128), 0)
    ci = lax.broadcasted_iota(jnp.int32, (128, 128), 1)
    perm[...] = pltpu.bitcast(jnp.where(ci == (ri & 7) * DH + (ri >> 3), 1.0, 0.0).astype(BF16), U32)

    for c in head:
        c.wait()
    for c in loads:
        c.start()

    def setup(i):
        get = lambda k: halves(pltpu.bitcast(abc[k, _rows(i, 16), :], U32))
        dt = halves(pltpu.bitcast(par[0, _rows(i, 16), :].astype(BF16), U32))

        def pole(h):
            mag, ang = jnp.exp(dt[h] * get(0)[h]), dt[h] * get(1)[h]
            zw[i, h, 0], zw[i, h, 1] = mag * jnp.cos(ang), mag * jnp.sin(ang)

        def weight():
            scale = (1.0 + 1.5 * 2.0 ** -9) / L
            for h, (cr, ci, br, bi) in enumerate(zip(*map(get, (4, 5, 2, 3)))):
                wr, wi = _cmul((cr, ci), (dt[h] * br, dt[h] * bi))
                zw[i, h, 2], zw[i, h, 3] = wr * scale, wi * -scale

        return [step(pole, 0), weight, step(pole, 1)]

    lags = sorted({(c, r) for c in range(8) for r in _RND[c] if r < 16}) + [(8, 0)]
    stack = lambda vs: jnp.concatenate([jnp.concatenate([v[k] for v in vs], 0) for k in range(2)], 1).astype(BF16)

    def lagsums(i):
        start = [[zw[i, h, c] for c in range(4)] for h in range(2)]
        zs, rhs, even = [], [], []

        def right(h):
            zr, zi, wr, wi = start[h]
            z = {0: (jnp.ones((8, N), F32), jnp.zeros((8, N), F32)), 1: (zr, zi)}
            for e in (2, 4, 8, 16, 32, 64, 128, 256):
                z[e] = _csq(z[e // 2])
            b = [(wr, wi)]
            for e in (16, 32, 64, 128):
                zc = (z[e][0], -z[e][1])
                b += [_cmul(v, zc) for v in b]
            zs.append(z)
            rhs.append(stack(b))

        def left(h, lo, hi):
            z = zs[h]

            def power(e):
                if e not in z:
                    low = e % 256 if e > 256 and e % 256 else e & -e
                    z[e] = _csq(z[e // 2]) if e // 2 in z and e % 2 == 0 else _cmul(power(e - low), power(low))
                return z[e]

            a = [power(256 * c + r) for c, r in (lags + lags[-1:])[lo:hi]]
            o = pltpu.bitcast(lax.dot_general(stack(a), rhs[h], NT, preferred_element_type=F32), U32)
            if h:
                lag[i, 8 * lo:8 * hi, :] = jnp.concatenate(even, 0)[8 * lo:8 * hi] | (o & high)
            else:
                even.append(o >> 16)

        return [step(right, 0), step(left, 0, 0, 22), step(left, 0, 22, 42), step(right, 1), step(left, 1, 0, 20), step(left, 1, 20, 42)]

    def kgen(i):
        lane = lax.broadcasted_iota(jnp.int32, (8, 128), 1)
        src = (lane & 15) * 8 + lax.broadcasted_iota(jnp.int32, (8, 128), 0)

        memo = {}

        def piece(c, r):
            if r == 16:
                c = 0
            if (c, r) not in memo:
                memo[c, r] = (
                    pltpu.roll(jnp.where(lane == 0, piece(8, 0), merged(0, (0,) * 8)), 127, 1) if r == 16 else
                    jnp.take_along_axis(lag[i, _rows(lags.index((c, r)), 8), :], src, axis=1,
                                        mode="promise_in_bounds"))
            return memo[c, r]

        def merged(c, rs):
            if (c, rs) not in memo:
                memo[c, rs] = (piece(c, rs[0]) if c == 7 or min(rs) == 16 else
                               jnp.where(lane >> 4 == c, piece(c, rs[0]), merged(c + 1, rs[1:])))
            return memo[c, rs]

        for n0 in range(R0):
            kt[n0, _rows(i, 8), :] = merged(0, tuple(_RND[c][n0] for c in range(8)))

    get = lambda ref, n, rows: (ref[n, 0, rows, :], ref[n, 1, rows, :])

    def put(ref, n, rows, v):
        ref[n, 0, rows, :], ref[n, 1, rows, :] = v

    def outer(src, a, rows):
        return [_twiddle(v, a * b) for b, v in enumerate(_dft4([get(src, a + 4 * m, rows) for m in range(4)], 1))]

    def transform(lhs, dst, n0, rows):
        r = jnp.dot(lhs, _bf(fm[n0]), preferred_element_type=F32)
        put(dst, n0, rows, (r[:, :128], r[:, 128:]))

    def kfwd(n0, r):
        transform(_bf(kt[n0, _rows(r, 32), :]), ub, n0, _rows(r, 64))

    def kdft(i):
        rows, t = _rows(i, 8), []

        def inner(b):
            for m, v in enumerate(_dft4([t[a][b] for a in range(4)], 1)):
                put(kf, b + 4 * m, rows, (v[0] + par[1, rows, :], v[1]))

        return [lambda a=a: t.append(outer(ub, a, rows)) for a in range(4)] + [step(inner, b) for b in range(4)]

    def fwd(n0, r):
        transform(un[n0, _rows(r, 64), :], ua, n0, _rows(r, 64))

    def pre(a, i):
        for b, v in enumerate(outer(ua, a, _rows(i, 8))):
            put(ub, a + 4 * b, _rows(i, 8), v)

    def mid(i):
        first, t = {}, {}

        def inner(h, b):
            rows = _rows(2 * i + h, 8)
            if b == 0:
                first[h] = outer(ua, 0, rows)
            x = _dft4([first[h][b]] + [get(ub, a + 4 * b, rows) for a in range(1, 4)], 1)
            t[h, b], *y = _dft4([_cmul(x[m], get(kf, b + 4 * m, rows)) for m in range(4)], -1)
            for a in range(1, 4):
                put(uc, a + 4 * b, rows, y[a - 1])

        def last():
            for m, (v, w) in enumerate(zip(*[_dft4([t[h, b] for b in range(4)], -1) for h in range(2)])):
                put(yb, 4 * m, _rows(i, 16), [jnp.concatenate([v[k], w[k]], 0).astype(BF16) for k in range(2)])

        return [step(inner, h, b) for h in range(2) for b in range(4)] + [last]

    def post(a, i):
        rows = _rows(i, 16)
        for m, v in enumerate(_dft4([_twiddle(get(uc, a + 4 * b, rows), -a * b) for b in range(4)], -1)):
            put(yb, a + 4 * m, rows, (v[0].astype(BF16), v[1].astype(BF16)))

    def inv(n0, r):
        rows = _rows(r, 64)
        y = jnp.concatenate(get(yb, n0, rows), 1)
        xs[n0, rows, :] = xs[n0, rows, :] + jnp.dot(y, _bf(gm[n0]), preferred_element_type=F32)

    def wprep(g, t):
        ops = []

        def load():
            if t < 3:
                v = lax.dot_general(_bf(perm[...]), wqkv[4 * t + g], NT, preferred_element_type=F32)
                v = v if t else v * DH ** -0.5
                lo, hi = v[:, :256], v[:, 256:]
            else:
                v = [jnp.dot(_bf(perm[...]), wo[_rows(e, 128), _rows(g, 128)], preferred_element_type=F32)
                     for e in range(4)]
                lo, hi = (jnp.concatenate([u[64 * h:64 * h + 64] for u in v], 0).T for h in range(2))
            ops.extend((lo[:64], hi[:64], lo[64:], hi[64:]))

        def save(i, h):
            for k, a in enumerate(_left(*[v[16 * i:16 * i + 16, 128 * h:128 * h + 128] for v in ops])):
                dst = wt.at[g, k] if t < 3 else wot.at[k]
                dst[_rows(4 * (t if t < 3 else g) + i, 8), _rows(h, 128)] = pltpu.bitcast(a.astype(BF16), U32)

        return [load] + [step(save, i, h) for i in range(4) for h in range(2)]

    def words(c):
        io[c, :L // 2, :] = pltpu.bitcast(xio[c], U32)

    def xin(j, c):
        xs[2 * j, _rows(c, 128), :], xs[2 * j + 1, _rows(c, 128), :] = halves(io[c, pl.ds(j, R1, stride=8), :].T)

    def norm(n0):
        acc, stat = {}, []

        def moment(k, lo, hi):
            for i in range(lo, hi):
                v = xs[n0, 8 * i:8 * i + 8, :]
                v = jnp.square(v - stat[0]) if k else v
                acc[i % 4] = v if i < 4 else acc[i % 4] + v
            if hi == D // 8:
                v = jnp.sum(_tree(jnp.add, list(acc.values())), axis=0, keepdims=True) * (1.0 / D)
                stat.append(lax.rsqrt(v + 1e-5) if k else v)

        def scale(c):
            rows = _rows(c, 128)
            un[n0, rows, :] = get(rows).astype(BF16)

        get = lambda rows: (xs[n0, rows, :] - stat[0]) * stat[1]
        return [[step(moment, 0, 0, 64)], [step(moment, 1, i, i + 16) for i in range(0, 64, 16)],
                [step(scale, c) for c in range(4)]], get

    def norms(*aa):
        return [f for a in aa for stage in zip(*[norm(a + 4 * m)[0] for m in range(4)])
                for steps in stage for f in steps]

    def pair_norms(a):
        stages, get = zip(*[norm(a + 4 * m) for m in range(4)])

        def operands(j, c):
            (b11, b21), (b12, b22) = ((f(_rows(c, 16)), f(_rows(c + 16, 16))) for f in get[2 * j:2 * j + 2])
            for k, b in enumerate(_right(b11, b12, b21, b22)):
                us[2 * a + j, k, _rows(c, 8), :] = pltpu.bitcast(b.astype(BF16), U32)

        return ([f for k in range(2) for st in stages for f in st[k]]
                + [step(operands, j, c) for j in range(2) for c in range(16)])

    def proj(i, slot, m, t):
        p, g, ref = i >> 2, i & 3, (qs, ks, vs)[t][slot]

        def emit(half, j, r):
            ref[m + 2 * j + 7 * (t > 0), _rows(half, 64), :] = r
            if t and m + j:
                ref[m + 2 * j - 1, _rows(half, 64), :] = pltpu.roll(r, 1, 1)

        return _strassen(lambda k: jnp.dot(_bf(wt[g, k, _rows(t, 32), :]), _bf(us[2 * p + 4 * (m & 1) + (m >> 2), k]),
                                           preferred_element_type=F32), emit)

    def attn(i, slot, m0):
        p, g = i >> 2, i & 3
        first = lax.broadcasted_iota(jnp.int32, (8, 128), 1) == 0
        window = lambda ref, d: {e: ref[slot][e, 8 * d:8 * d + 8, :] for e in range(m0, m0 + W + 1)}
        s, o = {}, {}

        def logits(m, d0):
            for d in (d0, d0 + 1):
                k = window(ks, d)
                q = qs[slot][m, 8 * d:8 * d + 8, :]
                for w in range(W):
                    t = q * k[m + 7 - w]
                    s[m, w] = t if d == 0 else s[m, w] + t

        def softmax(m):
            t = [jnp.where(first, -1e9, s[m, w]) if w > m else s[m, w] for w in range(W)]
            mx = _tree(jnp.maximum, t)
            e = [jnp.exp(v - mx) for v in t]
            rs = 1.0 / _tree(jnp.add, e)
            s.update({(m, w): e[w] * rs for w in range(W)})

        def values(d):
            v = window(vs, d)
            for m in (m0, m0 + 1):
                o[m, d] = _tree(jnp.add, [s[m, w] * v[m + 7 - w] for w in range(W)])
            if d % 2 and d > 8:
                blocks = [jnp.concatenate([o[m, e - 1], o[m, e]], 0) for e in (d - 8, d) for m in (m0, m0 + 1)]
                for k, b in enumerate(_right(*blocks)):
                    ob[m0 + p, k, g, 8 * d - 72:8 * d - 56, :] = b.astype(BF16)

        return ([f for m in (m0, m0 + 1) for f in [step(logits, m, d) for d in range(0, DH, 2)] + [step(softmax, m)]]
                + [step(values, d + e) for d in range(0, 8, 2) for e in (0, 1, 8, 9)])

    def oproj(p, c, n):
        def pair(m0):
            def emit(half, j, r):
                for i in range(n):
                    at = (2 * (m0 + j) + p, _rows(2 * (c + i) + half, 64))
                    xs[at] = xs[at] + r[64 * i:64 * i + 64]

            return _strassen(lambda k: jnp.dot(_bf(wot[k, 32 * c:32 * (c + n), :]), ob[m0 + p, k].reshape(D // 2, R1),
                                               preferred_element_type=F32), emit)

        return [f for m0 in range(0, 8, 2) for f in pair(m0)]

    def xout(c, j):
        lo, hi = (pltpu.bitcast(xs[2 * j + k, _rows(c, 128), :].astype(BF16).astype(F32), U32) for k in range(2))
        io[c, pl.ds(j, R1, stride=8), :] = ((lo >> 16) | hi).T

    four = lambda fn, *aa: [step(fn, a + 4 * m, r) for a in aa for m in range(4) for r in range(2 * NB)]
    block = lambda fn, a, r: [step(fn, a + 4 * m, 2 * r + h) for h in range(2) for m in range(4)] if 0 <= r < NB else []
    rowwise = lambda fn, a, n: [step(fn, a, i) for i in range(D // n)]

    regions, zero = [], zero_ref[0]

    def slot(*streams):
        regions.append(None)
        pl.when(zero < len(regions))(lambda: _run(*streams))

    pres = lambda a: rowwise(pre, a, 8)
    posts = lambda a: rowwise(post, a, 16)
    projs = lambda i, s, ms: [f for t in (1, 2, 0) for m in ms for f in proj(i, s, m, t)]
    attns = lambda i, s: [f for m in range(0, 8, 2) for f in attn(i, s, m)]

    with jax.named_scope("kgen"):
        ng = D // 16 // KPER
        each = lambda fn: (lambda i: [f for k in range(KPER) for f in fn(KPER * i + k)])
        _pipeline([(lambda i: [lambda: [kgen(KPER * i + k) for k in range(KPER)]], 2, ng - 1),
                   (each(lagsums), 1, ng), (each(setup), 0, ng),
                   (lambda c: [step(words, c)] + [step(xin, j, c) for j in range(8)], ng - NB, NB)],
                  {2: lambda: [c.wait() for c in rest], ng - NB: lambda: [c.wait() for c in loads[:NB]]})
    with jax.named_scope("kfwd"):
        for c in loads[NB:]:
            c.wait()
        kdfts = lambda r: [f for i in range(16) for f in kdft(16 * r + i)]
        for r, other in enumerate((norms(2, 1), *[sum(norm(n0)[0], []) for n0 in (3, 7)],
                                   sum(norm(11)[0] + norm(15)[0], []))):
            slot([f for a in range(4) for f in block(kfwd, a, r)], [f for t in (3, 0, 1, 2) for f in wprep(r, t)],
                 kdfts(r - 1) if r else [step(kgen, D // 16 - 1 - k) for k in range(KPER)], other)
        slot(four(fwd, 2), kdfts(NB - 1))
        slot(four(fwd, 1) + block(fwd, 3, 0), pres(2), norms(0))

    def layer(li, carry):
        with jax.named_scope("conv"):
            part = lambda steps, r: steps[len(steps) * r // NB:len(steps) * (r + 1) // NB] if 0 <= r < NB else []
            mids = [f for i in range(D // 16) for f in mid(i)]
            for r in range(-1, NB + 1):
                slot(block(fwd, 3, r + 2) + block(fwd, 0, r + 1) + block(inv, 0, r - 1) + block(inv, 2, r - 2)
                     + block(inv, 1, r - 2),
                     part(mids, r), part(pres(3), r + 1) + part(posts(2), r - 1) + part(posts(1), r - 1),
                     pres(1) if r < 0 else posts(3) if r == NB else [])
            slot(block(inv, 2, NB - 1) + block(inv, 1, NB - 1) + four(inv, 3), pair_norms(0))
            slot(projs(0, 0, (0, 4)), pair_norms(2))
            slot(projs(0, 0, (1, 5)), pair_norms(1))
        with jax.named_scope("attn"):
            slot(projs(1, 1, (0, 1, 4, 5)), attns(0, 0), pair_norms(3))
            both = lambda i, s: slot(projs(i + 1, 1 - s, (0, 1, 4, 5)), attns(i, s))
            lax.fori_loop(0, 3, lambda j, c: (both(2 * j + 1, 1), both(2 * j + 2, 0), c)[-1], 0)
            slot(oproj(0, 0, 2) + oproj(0, 2, 2), attns(7, 1))

        @pl.when(li == 0)
        def _():
            slot(oproj(1, 0, 2) + oproj(1, 2, 2), norms(2, 0))
            slot(four(fwd, 2), norms(1, 3))
            slot(four(fwd, 1) + block(fwd, 3, 0), pres(2))

        return carry

    lax.fori_loop(0, 2, layer, 0)

    with jax.named_scope("xout"):
        stores = [pltpu.make_async_copy(xio.at[c, _rows(i, 512)], out_hbm.at[_rows(i, 512), _rows(c, 128)],
                                        sems.at[4 * c + i]) for c in range(NB) for i in range(4)]
        last = [f for c in range(NB) for f in oproj(1, c, 1)] + [lambda: None] * 7
        for c in range(NB):
            slot(last[28 * c + 7 * (c > 0):28 * c + 35],
                 [lambda: None] * (2 * (c == 0)) + [step(xout, c, j) for j in range(8)])
            for i in range(4):
                xio[c, _rows(i, 512), :] = _bf(io[c, _rows(i, 256), :])
                stores[4 * c + i].start()
        for c in stores:
            c.wait()


@jax.jit
def pallas_interleave_layers__ssm_conv_s4__sliding_local_dilated__prompt_kernel(
    A_u: jax.Array,
    A_A_re: jax.Array,
    A_A_im: jax.Array,
    A_B_re: jax.Array,
    A_B_im: jax.Array,
    A_C_re: jax.Array,
    A_C_im: jax.Array,
    A_log_dt: jax.Array,
    A_Dskip: jax.Array,
    B_x: jax.Array,
    B_wqkv: jax.Array,
    B_wo: jax.Array,
):
    del B_x
    hbm = pl.BlockSpec(memory_space=pl.ANY)
    tiles = lambda *n: pltpu.VMEM((*n, 128, 128), F32)
    out = pl.pallas_call(
        _kernel,
        out_shape=jax.ShapeDtypeStruct((L, D), BF16),
        in_specs=[pl.BlockSpec(memory_space=pltpu.SMEM)] + [hbm] * 13,
        out_specs=hbm,
        scratch_shapes=[
            pltpu.VMEM((R0, D, R1), F32),
            *[pltpu.VMEM((R0, 2, D, R1), F32)] * 4,
            pltpu.VMEM((R0, 2, D, R1), BF16),
            pltpu.VMEM((2, D, N), F32),
            pltpu.VMEM((D // 16, 2, 4, 8, N), F32),
            pltpu.VMEM((D // 16, 336, 128), U32),
            *[tiles(n) for n in (8, 15, 15) * 2],
            pltpu.VMEM((NB, L, 128), BF16),
            pltpu.VMEM((NB, L // 2 + 8, 128), U32),
            pltpu.VMEM((6, D, N), BF16),
            pltpu.VMEM((64, 128), U32),
            pltpu.VMEM((12, D, 128), BF16),
            pltpu.VMEM((D, D), BF16),
            pltpu.VMEM(_F.shape, U32),
            pltpu.VMEM(_G.shape, U32),
            pltpu.VMEM((R0, D // 2, R1), U32),
            pltpu.VMEM((R0, D, R1), BF16),
            pltpu.VMEM((4, 7, 96, D // 2), U32),
            pltpu.VMEM((8, 7, D // 4, R1), U32),
            pltpu.VMEM((7, D // 4, D // 2), U32),
            pltpu.VMEM((8, 7, 4, 64, R1), BF16),
            pltpu.VMEM((D,), BF16),
            pltpu.VMEM((D,), BF16),
            pltpu.SemaphoreType.DMA((33,)),
        ],
        compiler_params=pltpu.CompilerParams(vmem_limit_bytes=100 * 1024 * 1024),
    )(np.zeros((1,), np.int32), A_u.reshape(L, D), A_A_re, A_A_im, A_B_re, A_B_im, A_C_re, A_C_im, A_log_dt, A_Dskip,
      B_wqkv, B_wo, _F, _G)
    return out.reshape(1, L, D)
```

```python
import jax
import jax.numpy as jnp
import ml_dtypes
import numpy as np
from jax import lax
import jax.experimental.pallas as pl
import jax.experimental.pallas.tpu as pltpu

L, D, N = 2048, 512, 128
R0, R1 = 16, 128
W, DH = 8, 16
F32, BF16, U32 = jnp.float32, jnp.bfloat16, jnp.uint32
KPER = 4
NB = D // 128
NT = (((1,), (1,)), ((), ()))


def _constants():
    n0 = np.arange(R0)[:, None, None]
    n1 = np.arange(R1)[None, :, None]
    k1 = np.arange(R1)[None, None, :]
    ang = 2.0 * np.pi * (k1 + 0.25) * (R0 * n1 + n0) / L
    f = np.concatenate([np.cos(ang), np.sin(ang)], axis=2)
    g = f.transpose(0, 2, 1)
    bf = ml_dtypes.bfloat16
    lr = np.arange(L).astype(np.float32).astype(bf).astype(np.int64).reshape(8, 16, R0)
    r = lr - (256 * np.arange(8)[:, None, None] + 16 * np.arange(16)[None, :, None])
    assert (r == r[:, :1, :]).all()

    def words(m):
        h = np.ascontiguousarray(m).astype(bf).view(np.uint16).astype(np.uint32)
        return h[:, 0::2] | (h[:, 1::2] << 16)

    return words(f), words(g), r[:, 0, :].tolist()


_F, _G, _RND = _constants()


def _cmul(a, b):
    return a[0] * b[0] - a[1] * b[1], a[0] * b[1] + a[1] * b[0]


def _csq(a):
    t = a[0] * a[1]
    return (a[0] + a[1]) * (a[0] - a[1]), t + t


def _dft4(x, sign, turn_out=False):
    (ar, ai), (br, bi), (cr, ci), (dr, di) = x
    sr, si, tr, ti = ar + cr, ai + ci, ar - cr, ai - ci
    ur, ui, vr, vi = br + dr, bi + di, br - dr, bi - di
    p, m = (tr - vi, ti + vr), (tr + vi, ti - vr)
    if sign < 0:
        p, m = m, p
    half = (sr - ur, si - ui) if not turn_out else (ui - si, sr - ur) if sign > 0 else (si - ui, ur - sr)
    return [(sr + ur, si + ui), p, half, m]


def _twiddle(v, e):
    e %= 16
    re, im = v
    h = float(np.sqrt(0.5))
    if e == 0:
        return v
    if e == 2:
        return (re - im) * h, (re + im) * h
    if e == 14:
        return (re + im) * h, (im - re) * h
    if e == 6:
        return (re + im) * -h, (re - im) * h
    if e == 10:
        return (im - re) * h, (re + im) * -h
    c, s = float(np.cos(np.pi * e / 8)), float(np.sin(np.pi * e / 8))
    return re * c - im * s, re * s + im * c


def _bf(x):
    return pltpu.bitcast(x, BF16)


def _tree(op, v):
    while len(v) > 1:
        v = [op(v[i], v[i + 1]) if i + 1 < len(v) else v[i] for i in range(0, len(v), 2)]
    return v[0]


def _run(*streams):
    order = sorted(((i + 0.5 * (k > 0)) / len(s), k, i) for k, s in enumerate(streams) for i in range(len(s)))
    for _, k, i in order:
        streams[k][i]()


def _pipeline(streams, hooks=None):
    hooks = hooks or {}
    cuts = sorted({e for _, a, n in streams for e in (a, a + n)} | set(hooks))
    for lo, hi in zip(cuts, cuts[1:]):
        def body(s, carry, lo=lo):
            _run(*[fn(s - a) for fn, a, n in streams if a <= lo < a + n])
            return carry

        if lo in hooks:
            hooks[lo]()
        if hi - lo == 1:
            body(lo, 0)
        else:
            lax.fori_loop(lo, hi, body, 0)


def _left(a11, a12, a21, a22):
    return a21 + a22, a22, a11 + a22, a12 - a22, a11 + a12, a11, a21 - a11


def _right(b11, b12, b21, b22):
    return b11, b21 - b11, b11 + b22, b21 + b22, b22, b12 - b22, b11 + b12


def _strassen(product, emit):
    c = {}

    def run(k):
        c[k] = r = product(k)
        if k == 1:
            emit(1, 0, c[0] + r)
        elif k == 2:
            c[11], c[22] = r + c[1], r - c[0]
        elif k == 3:
            c[11] = c[11] + r
        elif k == 4:
            emit(0, 0, c[11] - r)
        elif k == 5:
            emit(0, 1, c[4] + r)
            c[22] = c[22] + r
        elif k == 6:
            emit(1, 1, c[22] + r)

    return [lambda k=k: run(k) for k in range(7)]


def _rows(i, n):
    return pl.ds(i * n if isinstance(i, int) else pl.multiple_of(i * n, n), n)


def _kernel(zero_ref, x_hbm, are_hbm, aim_hbm, bre_hbm, bim_hbm, cre_hbm, cim_hbm, ldt_hbm, dsk_hbm,
            wqkv_hbm, wo_hbm, f_hbm, g_hbm, out_hbm,
            xs, kf, ua, ub, uc, yb, par, zw, lag, qa, ka, va, qb, kb, vb,
            xio, io, abc, perm, wqkv, wo, fm, gm, kt, un, wt, us, wot, ob, ldt_ref, dsk_ref, sems):
    step = lambda fn, *a: (lambda: fn(*a))
    qs, ks, vs = (qa, qb), (ka, kb), (va, vb)
    head, rest = ([pltpu.make_async_copy(s.at[rows], abc.at[i, rows], sems.at[base + i])
                   for i, s in enumerate((are_hbm, aim_hbm, bre_hbm, bim_hbm, cre_hbm, cim_hbm))]
                  for base, rows in ((19, pl.ds(0, 32 * KPER)), (25, pl.ds(32 * KPER, D - 32 * KPER))))
    loads = [pltpu.make_async_copy(s, d, sems.at[i]) for i, (s, d) in enumerate(
        (*((x_hbm.at[:, _rows(c, 128)], xio.at[c]) for c in range(NB)),
         (f_hbm, fm), (wo_hbm, wo), (g_hbm, gm),
         *((wqkv_hbm.at[:, pl.ds(128 * j, 128)], wqkv.at[j]) for j in range(12))))]
    small = [pltpu.make_async_copy(s, d, sems.at[31 + i])
             for i, (s, d) in enumerate(((ldt_hbm, ldt_ref), (dsk_hbm, dsk_ref)))]
    for c in small + head + rest:
        c.start()
    for c in small:
        c.wait()
    high = jnp.uint32(0xFFFF0000)
    halves = lambda t: (pltpu.bitcast(t << 16, F32), pltpu.bitcast(t & high, F32))

    def col(ref):
        v = ref[...].astype(F32).reshape(1, D)
        return jnp.broadcast_to(v, (128, D)).T

    par[0] = jnp.exp(col(ldt_ref))
    par[1] = col(dsk_ref) * (1.0 / L)

    ri = lax.broadcasted_iota(jnp.int32, (128, 128), 0)
    ci = lax.broadcasted_iota(jnp.int32, (128, 128), 1)
    perm[...] = pltpu.bitcast(jnp.where(ci == (ri & 7) * DH + (ri >> 3), 1.0, 0.0).astype(BF16), U32)

    for c in head:
        c.wait()
    for c in loads:
        c.start()

    def setup(i):
        get = lambda k: halves(pltpu.bitcast(abc[k, _rows(i, 16), :], U32))
        dt = halves(pltpu.bitcast(par[0, _rows(i, 16), :].astype(BF16), U32))

        def pole(h):
            mag, ang = jnp.exp(dt[h] * get(0)[h]), dt[h] * get(1)[h]
            zw[i, h, 0], zw[i, h, 1] = mag * jnp.cos(ang), mag * jnp.sin(ang)

        def weight():
            scale = (1.0 + 1.5 * 2.0 ** -9) / L
            for h, (cr, ci, br, bi) in enumerate(zip(*map(get, (4, 5, 2, 3)))):
                wr, wi = _cmul((cr, ci), (dt[h] * br, dt[h] * bi))
                zw[i, h, 2], zw[i, h, 3] = wr * scale, wi * -scale

        return [step(pole, 0), weight, step(pole, 1)]

    lags = sorted({(c, r) for c in range(8) for r in _RND[c] if r < 16}) + [(8, 0)]
    stack = lambda vs: jnp.concatenate([jnp.concatenate([v[k] for v in vs], 0) for k in range(2)], 1).astype(BF16)

    def lagsums(i):
        start = [[zw[i, h, c] for c in range(4)] for h in range(2)]
        zs, rhs, even = [], [], []

        def right(h):
            zr, zi, wr, wi = start[h]
            z = {0: (jnp.ones((8, N), F32), jnp.zeros((8, N), F32)), 1: (zr, zi)}
            for e in (2, 4, 8, 16, 32, 64, 128, 256):
                z[e] = _csq(z[e // 2])
            b = [(wr, wi)]
            for e in (16, 32, 64, 128):
                zc = (z[e][0], -z[e][1])
                b += [_cmul(v, zc) for v in b]
            zs.append(z)
            rhs.append(stack(b))

        def left(h, lo, hi):
            z = zs[h]

            def power(e):
                if e not in z:
                    low = e % 256 if e > 256 and e % 256 else e & -e
                    z[e] = _csq(z[e // 2]) if e // 2 in z and e % 2 == 0 else _cmul(power(e - low), power(low))
                return z[e]

            a = [power(256 * c + r) for c, r in (lags + lags[-1:])[lo:hi]]
            o = pltpu.bitcast(lax.dot_general(stack(a), rhs[h], NT, preferred_element_type=F32), U32)
            if h:
                lag[i, 8 * lo:8 * hi, :] = jnp.concatenate(even, 0)[8 * lo:8 * hi] | (o & high)
            else:
                even.append(o >> 16)

        return [step(right, 0), step(left, 0, 0, 22), step(left, 0, 22, 42), step(right, 1), step(left, 1, 0, 20), step(left, 1, 20, 42)]

    def kgen(i):
        lane = lax.broadcasted_iota(jnp.int32, (8, 128), 1)
        src = (lane & 15) * 8 + lax.broadcasted_iota(jnp.int32, (8, 128), 0)

        memo = {}

        def piece(c, r):
            if r == 16:
                c = 0
            if (c, r) not in memo:
                memo[c, r] = (
                    pltpu.roll(jnp.where(lane == 0, piece(8, 0), merged(0, (0,) * 8)), 127, 1) if r == 16 else
                    jnp.take_along_axis(lag[i, _rows(lags.index((c, r)), 8), :], src, axis=1,
                                        mode="promise_in_bounds"))
            return memo[c, r]

        def merged(c, rs):
            if (c, rs) not in memo:
                memo[c, rs] = (piece(c, rs[0]) if c == 7 or min(rs) == 16 else
                               jnp.where(lane >> 4 == c, piece(c, rs[0]), merged(c + 1, rs[1:])))
            return memo[c, rs]

        for n0 in range(R0):
            kt[n0, _rows(i, 8), :] = merged(0, tuple(_RND[c][n0] for c in range(8)))

    get = lambda ref, n, rows: (ref[n, 0, rows, :], ref[n, 1, rows, :])

    def put(ref, n, rows, v):
        ref[n, 0, rows, :], ref[n, 1, rows, :] = v

    def outer(src, a, rows):
        x = _dft4([get(src, a + 4 * m, rows) for m in range(4)], 1, turn_out=a == 2)
        return [v if a * b == 4 else _twiddle(v, a * b) for b, v in enumerate(x)]

    def kfwd(n0, r):
        rows = _rows(r, 64)
        v = jnp.dot(_bf(kt[n0, _rows(r, 32), :]), _bf(fm[n0]), preferred_element_type=F32)
        put(ub, n0, rows, (v[:, :128] if n0 else v[:, :128] + par[1, rows, :], v[:, 128:]))

    def kdft(i):
        rows, t = _rows(i, 8), []

        def inner(b):
            for m, v in enumerate(_dft4([t[a][b] for a in range(4)], 1)):
                put(kf, b + 4 * m, rows, v)

        return [lambda a=a: t.append(outer(ub, a, rows)) for a in range(4)] + [step(inner, b) for b in range(4)]

    def fwd(n0, r):
        v = jnp.dot(un[n0, _rows(r, 64), :], _bf(fm[n0]), preferred_element_type=F32)
        put(ua, n0, _rows(r, 64), (v[:, :128], v[:, 128:]))

    def pre(a, i):
        for b, v in enumerate(outer(ua, a, _rows(i, 8))):
            put(ub, a + 4 * b, _rows(i, 8), v)

    def unouter(a, rows, t):
        for m, v in enumerate(_dft4([t[b] if a * b == 4 else _twiddle(t[b], -a * b) for b in range(4)], -1)):
            put(yb, a + 4 * m, rows, v)

    def mid(i):
        rows, first, t = _rows(i, 8), [], {}

        def inner(b):
            if b == 0:
                first.extend(outer(ua, 0, rows))
            x = _dft4([first[b]] + [get(ub, a + 4 * b, rows) for a in range(1, 4)], 1)
            t[b], *y = _dft4([_cmul(x[m], get(kf, b + 4 * m, rows)) for m in range(4)], -1, turn_out=b == 2)
            for a in range(1, 4):
                put(uc, a + 4 * b, rows, y[a - 1])
            if b == 3:
                unouter(0, rows, t)

        return [step(inner, b) for b in range(4)]

    def post(a, i):
        unouter(a, _rows(i, 8), [get(uc, a + 4 * b, _rows(i, 8)) for b in range(4)])

    def inv(n0, r):
        rows = _rows(r, 64)
        y = jnp.concatenate(get(yb, n0, rows), 1).astype(BF16)
        xs[n0, rows, :] = xs[n0, rows, :] + jnp.dot(y, _bf(gm[n0]), preferred_element_type=F32)

    def wprep(g, t):
        ops = []

        def load(h):
            if t < 3:
                lo, hi = (lax.dot_general(_bf(perm[...]), wqkv[4 * t + g, _rows(h + e, 128), :], NT,
                                          preferred_element_type=F32) for e in (0, 2))
                if t == 0:
                    lo, hi = lo * DH ** -0.5, hi * DH ** -0.5
            else:
                v = [jnp.dot(_bf(perm[...]), wo[_rows(2 * h + e, 128), _rows(g, 128)], preferred_element_type=F32)
                     for e in range(2)]
                lo, hi = (jnp.concatenate([u[64 * e:64 * e + 64] for u in v], 0).T for e in range(2))
            ops[:] = lo[:64], hi[:64], lo[64:], hi[64:]

        def save(h, i):
            for k, a in enumerate(_left(*[v[16 * i:16 * i + 16] for v in ops])):
                at = (_rows(4 * (t if t < 3 else g) + i, 8), _rows(h, 128))
                (wt if t < 3 else wot)[(g, k, *at) if t < 3 else (k, *at)] = pltpu.bitcast(a.astype(BF16), U32)

        return [f for h in range(2) for f in [step(load, h)] + [step(save, h, i) for i in range(4)]]

    def words(c):
        io[c, :L // 2, :] = pltpu.bitcast(xio[c], U32)

    def xin(j, c):
        xs[2 * j, _rows(c, 128), :], xs[2 * j + 1, _rows(c, 128), :] = halves(io[c, pl.ds(j, R1, stride=8), :].T)

    def norm(n0):
        acc, stat = {}, []

        def moment(k, lo, hi):
            for i in range(lo, hi):
                v = xs[n0, 8 * i:8 * i + 8, :]
                v = jnp.square(v - stat[0]) if k else v
                acc[i % 4] = v if i < 4 else acc[i % 4] + v
            if hi == D // 8:
                v = jnp.sum(_tree(jnp.add, list(acc.values())), axis=0, keepdims=True) * (1.0 / D)
                stat.append(lax.rsqrt(v + 1e-5) if k else v)

        def scale(c):
            rows = _rows(c, 128)
            un[n0, rows, :] = get(rows).astype(BF16)

        get = lambda rows: (xs[n0, rows, :] - stat[0]) * stat[1]
        return [[step(moment, 0, 0, 64)], [step(moment, 1, i, i + 16) for i in range(0, 64, 16)],
                [step(scale, c) for c in range(4)]], get

    def norms(*aa):
        return [f for a in aa for stage in zip(*[norm(a + 4 * m)[0] for m in range(4)])
                for steps in stage for f in steps]

    def pair_norms(a):
        stages, get = zip(*[norm(a + 4 * m) for m in range(4)])

        def operands(j, c):
            (b11, b21), (b12, b22) = ((f(_rows(c, 16)), f(_rows(c + 16, 16))) for f in get[2 * j:2 * j + 2])
            for k, b in enumerate(_right(b11, b12, b21, b22)):
                us[2 * a + j, k, _rows(c, 8), :] = pltpu.bitcast(b.astype(BF16), U32)

        return ([f for k in range(2) for st in stages for f in st[k]]
                + [step(operands, j, c) for j in range(2) for c in range(16)])

    def proj(i, slot, m, t):
        p, g, ref = i >> 2, i & 3, (qs, ks, vs)[t][slot]

        def emit(half, j, r):
            ref[m + 2 * j + 7 * (t > 0), _rows(half, 64), :] = r
            if t and m + j:
                ref[m + 2 * j - 1, _rows(half, 64), :] = pltpu.roll(r, 1, 1)

        return _strassen(lambda k: jnp.dot(_bf(wt[g, k, _rows(t, 32), :]), _bf(us[2 * p + 4 * (m & 1) + (m >> 2), k]),
                                           preferred_element_type=F32), emit)

    def attn(i, slot, m0):
        p, g = i >> 2, i & 3
        first = lax.broadcasted_iota(jnp.int32, (8, 128), 1) == 0
        window = lambda ref, d: {e: ref[slot][e, 8 * d:8 * d + 8, :] for e in range(m0, m0 + W + 1)}
        s, o = {}, {}

        def logits(m, d0):
            for d in (d0, d0 + 1):
                k = window(ks, d)
                q = qs[slot][m, 8 * d:8 * d + 8, :]
                for w in range(W):
                    t = q * k[m + 7 - w]
                    s[m, w] = t if d == 0 else s[m, w] + t

        def softmax(m):
            t = [jnp.where(first, -1e9, s[m, w]) if w > m else s[m, w] for w in range(W)]
            mx = _tree(jnp.maximum, t)
            e = [jnp.exp(v - mx) for v in t]
            rs = 1.0 / _tree(jnp.add, e)
            s.update({(m, w): e[w] * rs for w in range(W)})

        def values(d):
            v = window(vs, d)
            for m in (m0, m0 + 1):
                o[m, d] = _tree(jnp.add, [s[m, w] * v[m + 7 - w] for w in range(W)])
            if d % 2 and d > 8:
                blocks = [jnp.concatenate([o[m, e - 1], o[m, e]], 0) for e in (d - 8, d) for m in (m0, m0 + 1)]
                for k, b in enumerate(_right(*blocks)):
                    ob[m0 + p, k, g, 8 * d - 72:8 * d - 56, :] = b.astype(BF16)

        return ([f for m in (m0, m0 + 1) for f in [step(logits, m, d) for d in range(0, DH, 2)] + [step(softmax, m)]]
                + [step(values, d + e) for d in range(0, 8, 2) for e in (0, 1, 8, 9)])

    def oproj(p, c, n):
        def pair(m0):
            def emit(half, j, r):
                for i in range(n):
                    at = (2 * (m0 + j) + p, _rows(2 * (c + i) + half, 64))
                    xs[at] = xs[at] + r[64 * i:64 * i + 64]

            return _strassen(lambda k: jnp.dot(_bf(wot[k, 32 * c:32 * (c + n), :]), ob[m0 + p, k].reshape(D // 2, R1),
                                               preferred_element_type=F32), emit)

        return [f for m0 in range(0, 8, 2) for f in pair(m0)]

    def xout(c, j):
        lo, hi = (pltpu.bitcast(xs[2 * j + k, _rows(c, 128), :].astype(BF16).astype(F32), U32) for k in range(2))
        io[c, pl.ds(j, R1, stride=8), :] = ((lo >> 16) | hi).T

    four = lambda fn, *aa: [step(fn, a + 4 * m, r) for a in aa for m in range(4) for r in range(2 * NB)]
    block = lambda fn, a, r: [step(fn, a + 4 * m, 2 * r + h) for h in range(2) for m in range(4)] if 0 <= r < NB else []
    rowwise = lambda fn, a, n: [step(fn, a, i) for i in range(D // n)]

    regions, zero = [], zero_ref[0]

    def slot(*streams):
        regions.append(None)
        pl.when(zero < len(regions))(lambda: _run(*streams))

    pres = lambda a: rowwise(pre, a, 8)
    posts = lambda a: rowwise(post, a, 8)
    projs = lambda i, s, ms: [f for t in (1, 2, 0) for m in ms for f in proj(i, s, m, t)]
    attns = lambda i, s: [f for m in range(0, 8, 2) for f in attn(i, s, m)]

    with jax.named_scope("kgen"):
        ng = D // 16 // KPER
        each = lambda fn: (lambda i: [f for k in range(KPER) for f in fn(KPER * i + k)])
        _pipeline([(lambda i: [lambda: [kgen(KPER * i + k) for k in range(KPER)]], 2, ng - 1),
                   (each(lagsums), 1, ng), (each(setup), 0, ng),
                   (lambda c: [step(words, c)] + [step(xin, j, c) for j in range(8)], ng - NB, NB)],
                  {2: lambda: [c.wait() for c in rest], ng - NB: lambda: [c.wait() for c in loads[:NB]]})
    with jax.named_scope("kfwd"):
        for c in loads[NB:]:
            c.wait()
        kdfts = lambda r: [f for i in range(16) for f in kdft(16 * r + i)]
        for r, other in enumerate((norms(2, 1), *[sum(norm(n0)[0], []) for n0 in (3, 7)],
                                   sum(norm(11)[0] + norm(15)[0], []))):
            slot([f for a in range(4) for f in block(kfwd, a, r)], [f for t in (3, 0, 1, 2) for f in wprep(r, t)],
                 kdfts(r - 1) if r else [step(kgen, D // 16 - 1 - k) for k in range(KPER)], other)
        slot(four(fwd, 2), kdfts(NB - 1))
        slot(four(fwd, 1) + block(fwd, 3, 0), pres(2), norms(0))

    def layer(li, carry):
        with jax.named_scope("conv"):
            part = lambda steps, r: steps[len(steps) * r // NB:len(steps) * (r + 1) // NB] if 0 <= r < NB else []
            mids = [f for i in range(D // 8) for f in mid(i)]
            for r in range(-1, NB + 1):
                slot(block(fwd, 3, r + 2) + block(fwd, 0, r + 1) + block(inv, 0, r - 1) + block(inv, 2, r - 2)
                     + block(inv, 1, r - 2),
                     part(mids, r), part(pres(3), r + 1) + part(posts(2), r - 1) + part(posts(1), r - 1),
                     pres(1) if r < 0 else posts(3) if r == NB else [])
            slot(block(inv, 2, NB - 1) + block(inv, 1, NB - 1) + four(inv, 3), pair_norms(0))
            slot(projs(0, 0, (0, 4)), pair_norms(2))
            slot(projs(0, 0, (1, 5)), pair_norms(1))
        with jax.named_scope("attn"):
            slot(projs(1, 1, (0, 1, 4, 5)), attns(0, 0), pair_norms(3))
            both = lambda i, s: slot(projs(i + 1, 1 - s, (0, 1, 4, 5)), attns(i, s))
            lax.fori_loop(0, 3, lambda j, c: (both(2 * j + 1, 1), both(2 * j + 2, 0), c)[-1], 0)
            slot(oproj(0, 0, 2) + oproj(0, 2, 2), attns(7, 1))

        @pl.when(li == 0)
        def _():
            slot(oproj(1, 0, 2) + oproj(1, 2, 2), norms(2, 0))
            slot(four(fwd, 2), norms(1, 3))
            slot(four(fwd, 1) + block(fwd, 3, 0), pres(2))

        return carry

    lax.fori_loop(0, 2, layer, 0)

    with jax.named_scope("xout"):
        stores = [pltpu.make_async_copy(xio.at[c, _rows(i, 512)], out_hbm.at[_rows(i, 512), _rows(c, 128)],
                                        sems.at[4 * c + i]) for c in range(NB) for i in range(4)]
        last = [f for c in range(NB) for f in oproj(1, c, 1)] + [lambda: None] * 7
        for c in range(NB):
            slot(last[28 * c + 7 * (c > 0):28 * c + 35],
                 [lambda: None] * (2 * (c == 0)) + [step(xout, c, j) for j in range(8)])
            for i in range(4):
                xio[c, _rows(i, 512), :] = _bf(io[c, _rows(i, 256), :])
                stores[4 * c + i].start()
        for c in stores:
            c.wait()


@jax.jit
def pallas_interleave_layers__ssm_conv_s4__sliding_local_dilated__prompt_kernel(
    A_u: jax.Array,
    A_A_re: jax.Array,
    A_A_im: jax.Array,
    A_B_re: jax.Array,
    A_B_im: jax.Array,
    A_C_re: jax.Array,
    A_C_im: jax.Array,
    A_log_dt: jax.Array,
    A_Dskip: jax.Array,
    B_x: jax.Array,
    B_wqkv: jax.Array,
    B_wo: jax.Array,
):
    del B_x
    hbm = pl.BlockSpec(memory_space=pl.ANY)
    tiles = lambda *n: pltpu.VMEM((*n, 128, 128), F32)
    out = pl.pallas_call(
        _kernel,
        out_shape=jax.ShapeDtypeStruct((L, D), BF16),
        in_specs=[pl.BlockSpec(memory_space=pltpu.SMEM)] + [hbm] * 13,
        out_specs=hbm,
        scratch_shapes=[
            pltpu.VMEM((R0, D, R1), F32),
            *[pltpu.VMEM((R0, 2, D, R1), F32)] * 5,
            pltpu.VMEM((2, D, N), F32),
            pltpu.VMEM((D // 16, 2, 4, 8, N), F32),
            pltpu.VMEM((D // 16, 336, 128), U32),
            *[tiles(n) for n in (8, 15, 15) * 2],
            pltpu.VMEM((NB, L, 128), BF16),
            pltpu.VMEM((NB, L // 2 + 8, 128), U32),
            pltpu.VMEM((6, D, N), BF16),
            pltpu.VMEM((64, 128), U32),
            pltpu.VMEM((12, D, 128), BF16),
            pltpu.VMEM((D, D), BF16),
            pltpu.VMEM(_F.shape, U32),
            pltpu.VMEM(_G.shape, U32),
            pltpu.VMEM((R0, D // 2, R1), U32),
            pltpu.VMEM((R0, D, R1), BF16),
            pltpu.VMEM((4, 7, 96, D // 2), U32),
            pltpu.VMEM((8, 7, D // 4, R1), U32),
            pltpu.VMEM((7, D // 4, D // 2), U32),
            pltpu.VMEM((8, 7, 4, 64, R1), BF16),
            pltpu.VMEM((D,), BF16),
            pltpu.VMEM((D,), BF16),
            pltpu.SemaphoreType.DMA((33,)),
        ],
        compiler_params=pltpu.CompilerParams(vmem_limit_bytes=100 * 1024 * 1024),
    )(np.zeros((1,), np.int32), A_u.reshape(L, D), A_A_re, A_A_im, A_B_re, A_B_im, A_C_re, A_C_im, A_log_dt, A_Dskip,
      B_wqkv, B_wo, _F, _G)
    return out.reshape(1, L, D)
```

```python
import jax
import jax.numpy as jnp
import ml_dtypes
import numpy as np
from jax import lax
import jax.experimental.pallas as pl
import jax.experimental.pallas.tpu as pltpu

L, D, N = 2048, 512, 128
R0, R1 = 16, 128
W, DH = 8, 16
F32, BF16, U32 = jnp.float32, jnp.bfloat16, jnp.uint32
KPER = 4
NB = D // 128
NT = (((1,), (1,)), ((), ()))


def _constants():
    n0 = np.arange(R0)[:, None, None]
    n1 = np.arange(R1)[None, :, None]
    k1 = np.arange(R1)[None, None, :]
    ang = 2.0 * np.pi * (k1 + 0.25) * (R0 * n1 + n0) / L
    f = np.concatenate([np.cos(ang), np.sin(ang)], axis=2)
    g = f.transpose(0, 2, 1)
    bf = ml_dtypes.bfloat16
    lr = np.arange(L).astype(np.float32).astype(bf).astype(np.int64).reshape(8, 16, R0)
    r = lr - (256 * np.arange(8)[:, None, None] + 16 * np.arange(16)[None, :, None])
    assert (r == r[:, :1, :]).all()

    def words(m):
        h = np.ascontiguousarray(m).astype(bf).view(np.uint16).astype(np.uint32)
        return h[:, 0::2] | (h[:, 1::2] << 16)

    return words(f), words(g), r[:, 0, :].tolist()


_F, _G, _RND = _constants()


def _cmul(a, b):
    return a[0] * b[0] - a[1] * b[1], a[0] * b[1] + a[1] * b[0]


def _csq(a):
    t = a[0] * a[1]
    return (a[0] + a[1]) * (a[0] - a[1]), t + t


def _dft4(x, sign, turn_out=False):
    (ar, ai), (br, bi), (cr, ci), (dr, di) = x
    sr, si, tr, ti = ar + cr, ai + ci, ar - cr, ai - ci
    ur, ui, vr, vi = br + dr, bi + di, br - dr, bi - di
    p, m = (tr - vi, ti + vr), (tr + vi, ti - vr)
    if sign < 0:
        p, m = m, p
    half = (sr - ur, si - ui) if not turn_out else (ui - si, sr - ur) if sign > 0 else (si - ui, ur - sr)
    return [(sr + ur, si + ui), p, half, m]


def _twiddle(v, e):
    e %= 16
    re, im = v
    h = float(np.sqrt(0.5))
    if e == 0:
        return v
    if e == 2:
        return (re - im) * h, (re + im) * h
    if e == 14:
        return (re + im) * h, (im - re) * h
    if e == 6:
        return (re + im) * -h, (re - im) * h
    if e == 10:
        return (im - re) * h, (re + im) * -h
    c, s = float(np.cos(np.pi * e / 8)), float(np.sin(np.pi * e / 8))
    return re * c - im * s, re * s + im * c


def _bf(x):
    return pltpu.bitcast(x, BF16)


def _tree(op, v):
    while len(v) > 1:
        v = [op(v[i], v[i + 1]) if i + 1 < len(v) else v[i] for i in range(0, len(v), 2)]
    return v[0]


def _run(*streams):
    order = sorted(((i + 0.5 * (k > 0)) / len(s), k, i) for k, s in enumerate(streams) for i in range(len(s)))
    for _, k, i in order:
        streams[k][i]()


def _left(a11, a12, a21, a22):
    return a21 + a22, a22, a11 + a22, a12 - a22, a11 + a12, a11, a21 - a11


def _right(b11, b12, b21, b22):
    return b11, b21 - b11, b11 + b22, b21 + b22, b22, b12 - b22, b11 + b12


def _strassen(product, emit):
    c = {}

    def run(k):
        c[k] = r = product(k)
        if k == 1:
            emit(1, 0, c[0] + r)
        elif k == 2:
            c[11], c[22] = r + c[1], r - c[0]
        elif k == 3:
            c[11] = c[11] + r
        elif k == 4:
            emit(0, 0, c[11] - r)
        elif k == 5:
            emit(0, 1, c[4] + r)
            c[22] = c[22] + r
        elif k == 6:
            emit(1, 1, c[22] + r)

    return [lambda k=k: run(k) for k in range(7)]


def _rows(i, n):
    return pl.ds(i * n if isinstance(i, int) else pl.multiple_of(i * n, n), n)


def _kernel(zero_ref, x_hbm, are_hbm, aim_hbm, bre_hbm, bim_hbm, cre_hbm, cim_hbm, ldt_hbm, dsk_hbm,
            wqkv_hbm, wo_hbm, f_hbm, g_hbm, out_hbm,
            xs, kf, ua, ub, uc, yb, par, zw, lag, qa, ka, va, qb, kb, vb,
            xio, io, abc, perm, wqkv, wo, fm, gm, kt, un, wt, us, wot, ob, ldt_ref, dsk_ref, sems):
    step = lambda fn, *a: (lambda: fn(*a))
    qs, ks, vs = (qa, qb), (ka, kb), (va, vb)
    head, rest = ([pltpu.make_async_copy(s.at[rows], abc.at[i, rows], sems.at[base + i])
                   for i, s in enumerate((are_hbm, aim_hbm, bre_hbm, bim_hbm, cre_hbm, cim_hbm))]
                  for base, rows in ((19, pl.ds(0, 32 * KPER)), (25, pl.ds(32 * KPER, D - 32 * KPER))))
    loads = [pltpu.make_async_copy(s, d, sems.at[i]) for i, (s, d) in enumerate(
        (*((x_hbm.at[:, _rows(c, 128)], xio.at[c]) for c in range(NB)),
         (f_hbm, fm), (wo_hbm, wo), (g_hbm, gm),
         *((wqkv_hbm.at[:, pl.ds(128 * j, 128)], wqkv.at[j]) for j in range(12))))]
    small = [pltpu.make_async_copy(s, d, sems.at[31 + i])
             for i, (s, d) in enumerate(((ldt_hbm, ldt_ref), (dsk_hbm, dsk_ref)))]
    for c in small + head + rest:
        c.start()
    for c in small:
        c.wait()
    high = jnp.uint32(0xFFFF0000)
    halves = lambda t: (pltpu.bitcast(t << 16, F32), pltpu.bitcast(t & high, F32))

    def col(ref):
        v = ref[...].astype(F32).reshape(1, D)
        return jnp.broadcast_to(v, (128, D)).T

    par[0] = jnp.exp(col(ldt_ref))
    par[1] = col(dsk_ref) * (1.0 / L)

    ri = lax.broadcasted_iota(jnp.int32, (128, 128), 0)
    ci = lax.broadcasted_iota(jnp.int32, (128, 128), 1)
    perm[...] = pltpu.bitcast(jnp.where(ci == (ri & 7) * DH + (ri >> 3), 1.0, 0.0).astype(BF16), U32)

    for c in head:
        c.wait()
    for c in loads:
        c.start()

    def setup(i):
        get = lambda k: halves(pltpu.bitcast(abc[k, _rows(i, 16), :], U32))
        dt = halves(pltpu.bitcast(par[0, _rows(i, 16), :].astype(BF16), U32))

        def pole(h):
            mag, ang = jnp.exp(dt[h] * get(0)[h]), dt[h] * get(1)[h]
            zw[i, h, 0], zw[i, h, 1] = mag * jnp.cos(ang), mag * jnp.sin(ang)

        def weight():
            scale = (1.0 + 1.5 * 2.0 ** -9) / L
            for h, (cr, ci, br, bi) in enumerate(zip(*map(get, (4, 5, 2, 3)))):
                wr, wi = _cmul((cr, ci), (dt[h] * br, dt[h] * bi))
                zw[i, h, 2], zw[i, h, 3] = wr * scale, wi * -scale

        return [step(pole, 0), weight, step(pole, 1)]

    lags = sorted({(c, r) for c in range(8) for r in _RND[c] if r < 16}) + [(8, 0)]
    stack = lambda vs: jnp.concatenate([jnp.concatenate([v[k] for v in vs], 0) for k in range(2)], 1).astype(BF16)

    def lagsums(i):
        zs, rhs, even = [], [], []

        def right(h):
            zr, zi, wr, wi = (zw[i, h, c] for c in range(4))
            z = {0: (jnp.ones((8, N), F32), jnp.zeros((8, N), F32)), 1: (zr, zi)}
            for e in (2, 4, 8, 16, 32, 64, 128, 256):
                z[e] = _csq(z[e // 2])
            b = [(wr, wi)]
            for e in (16, 32, 64, 128):
                zc = (z[e][0], -z[e][1])
                b += [_cmul(v, zc) for v in b]
            zs.append(z)
            rhs.append(stack(b))

        def left(h, lo, hi):
            z = zs[h]

            def power(e):
                if e not in z:
                    low = e % 256 if e > 256 and e % 256 else e & -e
                    z[e] = _csq(z[e // 2]) if e // 2 in z and e % 2 == 0 else _cmul(power(e - low), power(low))
                return z[e]

            a = [power(256 * c + r) for c, r in (lags + lags[-1:])[lo:hi]]
            o = pltpu.bitcast(lax.dot_general(stack(a), rhs[h], NT, preferred_element_type=F32), U32)
            if h:
                lag[i, 8 * lo:8 * hi, :] = jnp.concatenate(even, 0)[8 * lo:8 * hi] | (o & high)
            else:
                even.append(o >> 16)

        return [step(right, 0), step(left, 0, 0, 22), step(left, 0, 22, 42), step(right, 1), step(left, 1, 0, 20), step(left, 1, 20, 42)]

    def kgen(i):
        lane = lax.broadcasted_iota(jnp.int32, (8, 128), 1)
        src = (lane & 15) * 8 + lax.broadcasted_iota(jnp.int32, (8, 128), 0)

        memo = {}

        def piece(c, r):
            if r == 16:
                c = 0
            if (c, r) not in memo:
                memo[c, r] = (
                    pltpu.roll(jnp.where(lane == 0, piece(8, 0), merged(0, (0,) * 8)), 127, 1) if r == 16 else
                    jnp.take_along_axis(lag[i, _rows(lags.index((c, r)), 8), :], src, axis=1,
                                        mode="promise_in_bounds"))
            return memo[c, r]

        def merged(c, rs):
            if (c, rs) not in memo:
                memo[c, rs] = (piece(c, rs[0]) if c == 7 or min(rs) == 16 else
                               jnp.where(lane >> 4 == c, piece(c, rs[0]), merged(c + 1, rs[1:])))
            return memo[c, rs]

        for n0 in range(R0):
            kt[n0, _rows(i, 8), :] = merged(0, tuple(_RND[c][n0] for c in range(8)))

    get = lambda ref, n, rows: (ref[n, 0, rows, :], ref[n, 1, rows, :])

    def put(ref, n, rows, v):
        ref[n, 0, rows, :], ref[n, 1, rows, :] = v

    def outer(src, a, rows):
        x = _dft4([get(src, a + 4 * m, rows) for m in range(4)], 1, turn_out=a == 2)
        return [v if a * b == 4 else _twiddle(v, a * b) for b, v in enumerate(x)]

    def kfwd(n0, r):
        rows = _rows(r, 64)
        v = jnp.dot(_bf(kt[n0, _rows(r, 32), :]), _bf(fm[n0]), preferred_element_type=F32)
        put(ub, n0, rows, (v[:, :128] if n0 else v[:, :128] + par[1, rows, :], v[:, 128:]))

    def kdft(i):
        rows, t = _rows(i, 8), []

        def inner(b):
            for m, v in enumerate(_dft4([t[a][b] for a in range(4)], 1)):
                put(kf, b + 4 * m, rows, v)

        return [lambda a=a: t.append(outer(ub, a, rows)) for a in range(4)] + [step(inner, b) for b in range(4)]

    def fwd(n0, r):
        v = jnp.dot(un[n0, _rows(r, 64), :], _bf(fm[n0]), preferred_element_type=F32)
        put(ua, n0, _rows(r, 64), (v[:, :128], v[:, 128:]))

    def pre(a, i):
        for b, v in enumerate(outer(ua, a, _rows(i, 8))):
            put(ub, a + 4 * b, _rows(i, 8), v)

    def unouter(a, rows, t):
        for m, v in enumerate(_dft4([t[b] if a * b == 4 else _twiddle(t[b], -a * b) for b in range(4)], -1)):
            put(yb, a + 4 * m, rows, v)

    def mid(i):
        rows, first, t = _rows(i, 8), [], {}

        def inner(b):
            if b == 0:
                first.extend(outer(ua, 0, rows))
            x = _dft4([first[b]] + [get(ub, a + 4 * b, rows) for a in range(1, 4)], 1)
            t[b], *y = _dft4([_cmul(x[m], get(kf, b + 4 * m, rows)) for m in range(4)], -1, turn_out=b == 2)
            for a in range(1, 4):
                put(uc, a + 4 * b, rows, y[a - 1])
            if b == 3:
                unouter(0, rows, t)

        return [step(inner, b) for b in range(4)]

    def post(a, i):
        unouter(a, _rows(i, 8), [get(uc, a + 4 * b, _rows(i, 8)) for b in range(4)])

    def inv(n0, r):
        rows = _rows(r, 64)
        y = jnp.concatenate(get(yb, n0, rows), 1).astype(BF16)
        xs[n0, rows, :] = xs[n0, rows, :] + jnp.dot(y, _bf(gm[n0]), preferred_element_type=F32)

    def wprep(g, t):
        ops = []

        def load(h):
            if t < 3:
                lo, hi = (lax.dot_general(_bf(perm[...]), wqkv[4 * t + g, _rows(h + e, 128), :], NT,
                                          preferred_element_type=F32) for e in (0, 2))
                if t == 0:
                    lo, hi = lo * DH ** -0.5, hi * DH ** -0.5
            else:
                v = [jnp.dot(_bf(perm[...]), wo[_rows(2 * h + e, 128), _rows(g, 128)], preferred_element_type=F32)
                     for e in range(2)]
                lo, hi = (jnp.concatenate([u[64 * e:64 * e + 64] for u in v], 0).T for e in range(2))
            ops[:] = lo[:64], hi[:64], lo[64:], hi[64:]

        def save(h, i):
            for k, a in enumerate(_left(*[v[16 * i:16 * i + 16] for v in ops])):
                at = (_rows(4 * (t if t < 3 else g) + i, 8), _rows(h, 128))
                (wt if t < 3 else wot)[(g, k, *at) if t < 3 else (k, *at)] = pltpu.bitcast(a.astype(BF16), U32)

        return [f for h in range(2) for f in [step(load, h)] + [step(save, h, i) for i in range(4)]]

    def words(c):
        io[c, :L // 2, :] = pltpu.bitcast(xio[c], U32)

    def xin(j, c):
        xs[2 * j, _rows(c, 128), :], xs[2 * j + 1, _rows(c, 128), :] = halves(io[c, pl.ds(j, R1, stride=8), :].T)

    def norm(n0):
        acc, stat = {}, []

        def moment(k, lo, hi):
            for i in range(lo, hi):
                v = xs[n0, 8 * i:8 * i + 8, :]
                v = jnp.square(v - stat[0]) if k else v
                acc[i % 4] = v if i < 4 else acc[i % 4] + v
            if hi == D // 8:
                v = jnp.sum(_tree(jnp.add, list(acc.values())), axis=0, keepdims=True) * (1.0 / D)
                stat.append(lax.rsqrt(v + 1e-5) if k else v)

        def scale(c):
            rows = _rows(c, 128)
            un[n0, rows, :] = get(rows).astype(BF16)

        get = lambda rows: (xs[n0, rows, :] - stat[0]) * stat[1]
        return [[step(moment, 0, 0, 64)], [step(moment, 1, i, i + 16) for i in range(0, 64, 16)],
                [step(scale, c) for c in range(4)]], get

    def norms(*aa):
        return [f for a in aa for stage in zip(*[norm(a + 4 * m)[0] for m in range(4)])
                for steps in stage for f in steps]

    def pair_norms(a):
        stages, get = zip(*[norm(a + 4 * m) for m in range(4)])

        def operands(j, c):
            (b11, b21), (b12, b22) = ((f(_rows(c, 16)), f(_rows(c + 16, 16))) for f in get[2 * j:2 * j + 2])
            for k, b in enumerate(_right(b11, b12, b21, b22)):
                us[2 * a + j, k, _rows(c, 8), :] = pltpu.bitcast(b.astype(BF16), U32)

        return ([f for k in range(2) for st in stages for f in st[k]]
                + [step(operands, j, c) for j in range(2) for c in range(16)])

    def proj(i, slot, m, t):
        p, g, ref = i >> 2, i & 3, (qs, ks, vs)[t][slot]

        def emit(half, j, r):
            ref[m + 2 * j + 7 * (t > 0), _rows(half, 64), :] = r
            if t and m + j:
                ref[m + 2 * j - 1, _rows(half, 64), :] = pltpu.roll(r, 1, 1)

        return _strassen(lambda k: jnp.dot(_bf(wt[g, k, _rows(t, 32), :]), _bf(us[2 * p + 4 * (m & 1) + (m >> 2), k]),
                                           preferred_element_type=F32), emit)

    def attn(i, slot, m0):
        p, g = i >> 2, i & 3
        first = lax.broadcasted_iota(jnp.int32, (8, 128), 1) == 0
        window = lambda ref, d: {e: ref[slot][e, 8 * d:8 * d + 8, :] for e in range(m0, m0 + W + 1)}
        s, o = {}, {}

        def logits(m, d0):
            for d in (d0, d0 + 1):
                k = window(ks, d)
                q = qs[slot][m, 8 * d:8 * d + 8, :]
                for w in range(W):
                    t = q * k[m + 7 - w]
                    s[m, w] = t if d == 0 else s[m, w] + t

        def softmax(m):
            t = [jnp.where(first, -1e9, s[m, w]) if w > m else s[m, w] for w in range(W)]
            mx = _tree(jnp.maximum, t)
            e = [jnp.exp(v - mx) for v in t]
            rs = 1.0 / _tree(jnp.add, e)
            s.update({(m, w): e[w] * rs for w in range(W)})

        def values(d):
            v = window(vs, d)
            for m in (m0, m0 + 1):
                o[m, d] = _tree(jnp.add, [s[m, w] * v[m + 7 - w] for w in range(W)])
            if d % 2 and d > 8:
                blocks = [jnp.concatenate([o[m, e - 1], o[m, e]], 0) for e in (d - 8, d) for m in (m0, m0 + 1)]
                for k, b in enumerate(_right(*blocks)):
                    ob[m0 + p, k, g, 8 * d - 72:8 * d - 56, :] = b.astype(BF16)

        return ([f for m in (m0, m0 + 1) for f in [step(logits, m, d) for d in range(0, DH, 2)] + [step(softmax, m)]]
                + [step(values, d + e) for d in range(0, 8, 2) for e in (0, 1, 8, 9)])

    def oproj(p, c, n):
        def pair(m0):
            def emit(half, j, r):
                for i in range(n):
                    at = (2 * (m0 + j) + p, _rows(2 * (c + i) + half, 64))
                    xs[at] = xs[at] + r[64 * i:64 * i + 64]

            return _strassen(lambda k: jnp.dot(_bf(wot[k, 32 * c:32 * (c + n), :]), ob[m0 + p, k].reshape(D // 2, R1),
                                               preferred_element_type=F32), emit)

        return [f for m0 in range(0, 8, 2) for f in pair(m0)]

    def xout(c, j):
        lo, hi = (pltpu.bitcast(xs[2 * j + k, _rows(c, 128), :].astype(BF16).astype(F32), U32) for k in range(2))
        io[c, pl.ds(j, R1, stride=8), :] = ((lo >> 16) | hi).T

    four = lambda fn, *aa: [step(fn, a + 4 * m, r) for a in aa for m in range(4) for r in range(2 * NB)]
    block = lambda fn, a, r: [step(fn, a + 4 * m, 2 * r + h) for h in range(2) for m in range(4)] if 0 <= r < NB else []
    rowwise = lambda fn, a, n: [step(fn, a, i) for i in range(D // n)]

    regions, zero = [], zero_ref[0]

    def slot(*streams):
        regions.append(None)
        pl.when(zero < len(regions))(lambda: _run(*streams))

    pres = lambda a: rowwise(pre, a, 8)
    posts = lambda a: rowwise(post, a, 8)
    projs = lambda i, s, ms: [f for t in (1, 2, 0) for m in ms for f in proj(i, s, m, t)]
    attns = lambda i, s: [f for m in range(0, 8, 2) for f in attn(i, s, m)]

    with jax.named_scope("kgen"):
        ng = D // 16 // KPER
        each = lambda fn, s: [f for k in range(KPER) for f in fn(KPER * s + k)]

        def generate(s, more=(), last=False):
            for k in range(KPER):
                kgen(KPER * (s - 1) + k)
            _run(each(lagsums, s), more)
            if not last:
                _run(each(setup, s + 1))

        _run(setup(0))
        _run(each(lagsums, 0), [f for i in range(1, 2 * KPER) for f in setup(i)])
        for c in rest:
            c.wait()
        lax.fori_loop(1, ng - NB - 1, lambda s, _: generate(s), None)
        for c in loads[:NB]:
            c.wait()
        lax.fori_loop(0, NB, lambda c, _: generate(
            c + ng - NB - 1, [step(words, c)] + [step(xin, j, c) for j in range(8)]), None)
        generate(ng - 1, last=True)
    with jax.named_scope("kfwd"):
        for c in loads[NB:]:
            c.wait()
        kdfts = lambda r: [f for i in range(16) for f in kdft(16 * r + i)]
        for r, other in enumerate((norms(2, 1), *[sum(norm(n0)[0], []) for n0 in (3, 7)],
                                   sum(norm(11)[0] + norm(15)[0], []))):
            slot([f for a in range(4) for f in block(kfwd, a, r)], [f for t in (3, 0, 1, 2) for f in wprep(r, t)],
                 kdfts(r - 1) if r else [step(kgen, D // 16 - 1 - k) for k in range(KPER)], other)
        slot(four(fwd, 2), kdfts(NB - 1))
        slot(four(fwd, 1) + block(fwd, 3, 0), pres(2), norms(0))

    def layer(li, carry):
        with jax.named_scope("conv"):
            part = lambda steps, r: steps[len(steps) * r // NB:len(steps) * (r + 1) // NB] if 0 <= r < NB else []
            mids = [f for i in range(D // 8) for f in mid(i)]
            for r in range(-1, NB + 1):
                slot(block(fwd, 3, r + 2) + block(fwd, 0, r + 1) + block(inv, 0, r - 1) + block(inv, 2, r - 2)
                     + block(inv, 1, r - 2),
                     part(mids, r), part(pres(3), r + 1) + part(posts(2), r - 1) + part(posts(1), r - 1),
                     pres(1) if r < 0 else posts(3) if r == NB else [])
            slot(block(inv, 2, NB - 1) + block(inv, 1, NB - 1) + four(inv, 3), pair_norms(0))
            slot(projs(0, 0, (0, 4)), pair_norms(2))
            slot(projs(0, 0, (1, 5)), pair_norms(1))
        with jax.named_scope("attn"):
            slot(projs(1, 1, (0, 1, 4, 5)), attns(0, 0), pair_norms(3))
            both = lambda i, s: slot(projs(i + 1, 1 - s, (0, 1, 4, 5)), attns(i, s))
            lax.fori_loop(0, 3, lambda j, c: (both(2 * j + 1, 1), both(2 * j + 2, 0), c)[-1], 0)
            slot(oproj(0, 0, 2) + oproj(0, 2, 2), attns(7, 1))

        @pl.when(li == 0)
        def _():
            slot(oproj(1, 0, 2) + oproj(1, 2, 2), norms(2, 0))
            slot(four(fwd, 2), norms(1, 3))
            slot(four(fwd, 1) + block(fwd, 3, 0), pres(2))

        return carry

    lax.fori_loop(0, 2, layer, 0)

    with jax.named_scope("xout"):
        stores = [pltpu.make_async_copy(xio.at[c, _rows(i, 512)], out_hbm.at[_rows(i, 512), _rows(c, 128)],
                                        sems.at[4 * c + i]) for c in range(NB) for i in range(4)]
        last = [f for c in range(NB) for f in oproj(1, c, 1)] + [lambda: None] * 7
        for c in range(NB):
            slot(last[28 * c + 7 * (c > 0):28 * c + 35],
                 [lambda: None] * (2 * (c == 0)) + [step(xout, c, j) for j in range(8)])
            for i in range(4):
                xio[c, _rows(i, 512), :] = _bf(io[c, _rows(i, 256), :])
                stores[4 * c + i].start()
        for c in stores:
            c.wait()


@jax.jit
def pallas_interleave_layers__ssm_conv_s4__sliding_local_dilated__prompt_kernel(
    A_u: jax.Array,
    A_A_re: jax.Array,
    A_A_im: jax.Array,
    A_B_re: jax.Array,
    A_B_im: jax.Array,
    A_C_re: jax.Array,
    A_C_im: jax.Array,
    A_log_dt: jax.Array,
    A_Dskip: jax.Array,
    B_x: jax.Array,
    B_wqkv: jax.Array,
    B_wo: jax.Array,
):
    del B_x
    hbm = pl.BlockSpec(memory_space=pl.ANY)
    tiles = lambda *n: pltpu.VMEM((*n, 128, 128), F32)
    out = pl.pallas_call(
        _kernel,
        out_shape=jax.ShapeDtypeStruct((L, D), BF16),
        in_specs=[pl.BlockSpec(memory_space=pltpu.SMEM)] + [hbm] * 13,
        out_specs=hbm,
        scratch_shapes=[
            pltpu.VMEM((R0, D, R1), F32),
            *[pltpu.VMEM((R0, 2, D, R1), F32)] * 5,
            pltpu.VMEM((2, D, N), F32),
            pltpu.VMEM((D // 16, 2, 4, 8, N), F32),
            pltpu.VMEM((D // 16, 336, 128), U32),
            *[tiles(n) for n in (8, 15, 15) * 2],
            pltpu.VMEM((NB, L, 128), BF16),
            pltpu.VMEM((NB, L // 2 + 8, 128), U32),
            pltpu.VMEM((6, D, N), BF16),
            pltpu.VMEM((64, 128), U32),
            pltpu.VMEM((12, D, 128), BF16),
            pltpu.VMEM((D, D), BF16),
            pltpu.VMEM(_F.shape, U32),
            pltpu.VMEM(_G.shape, U32),
            pltpu.VMEM((R0, D // 2, R1), U32),
            pltpu.VMEM((R0, D, R1), BF16),
            pltpu.VMEM((4, 7, 96, D // 2), U32),
            pltpu.VMEM((8, 7, D // 4, R1), U32),
            pltpu.VMEM((7, D // 4, D // 2), U32),
            pltpu.VMEM((8, 7, 4, 64, R1), BF16),
            pltpu.VMEM((D,), BF16),
            pltpu.VMEM((D,), BF16),
            pltpu.SemaphoreType.DMA((33,)),
        ],
        compiler_params=pltpu.CompilerParams(vmem_limit_bytes=100 * 1024 * 1024),
    )(np.zeros((1,), np.int32), A_u.reshape(L, D), A_A_re, A_A_im, A_B_re, A_B_im, A_C_re, A_C_im, A_log_dt, A_Dskip,
      B_wqkv, B_wo, _F, _G)
    return out.reshape(1, L, D)
```

```python
import jax
import jax.numpy as jnp
import ml_dtypes
import numpy as np
from jax import lax
import jax.experimental.pallas as pl
import jax.experimental.pallas.tpu as pltpu

L, D, N = 2048, 512, 128
R0, R1 = 16, 128
W, DH = 8, 16
F32, BF16, U32 = jnp.float32, jnp.bfloat16, jnp.uint32
KPER = 4
NB = D // 128
NT = (((1,), (1,)), ((), ()))


def _constants():
    n0 = np.arange(R0)[:, None, None]
    n1 = np.arange(R1)[None, :, None]
    k1 = np.arange(R1)[None, None, :]
    ang = 2.0 * np.pi * (k1 + 0.25) * (R0 * n1 + n0) / L
    f = np.concatenate([np.cos(ang), np.sin(ang)], axis=2)
    g = f.transpose(0, 2, 1)
    bf = ml_dtypes.bfloat16
    lr = np.arange(L).astype(np.float32).astype(bf).astype(np.int64).reshape(8, 16, R0)
    r = lr - (256 * np.arange(8)[:, None, None] + 16 * np.arange(16)[None, :, None])
    assert (r == r[:, :1, :]).all()

    def words(m):
        h = np.ascontiguousarray(m).astype(bf).view(np.uint16).astype(np.uint32)
        return h[:, 0::2] | (h[:, 1::2] << 16)

    return words(f), words(g), r[:, 0, :].tolist()


_F, _G, _RND = _constants()


def _cmul(a, b):
    return a[0] * b[0] - a[1] * b[1], a[0] * b[1] + a[1] * b[0]


def _csq(a):
    t = a[0] * a[1]
    return (a[0] + a[1]) * (a[0] - a[1]), t + t


def _dft4(x, sign, turn_out=False):
    (ar, ai), (br, bi), (cr, ci), (dr, di) = x
    sr, si, tr, ti = ar + cr, ai + ci, ar - cr, ai - ci
    ur, ui, vr, vi = br + dr, bi + di, br - dr, bi - di
    p, m = (tr - vi, ti + vr), (tr + vi, ti - vr)
    if sign < 0:
        p, m = m, p
    half = (sr - ur, si - ui) if not turn_out else (ui - si, sr - ur) if sign > 0 else (si - ui, ur - sr)
    return [(sr + ur, si + ui), p, half, m]


def _twiddle(v, e):
    e %= 16
    re, im = v
    h = float(np.sqrt(0.5))
    if e == 0:
        return v
    if e == 2:
        return (re - im) * h, (re + im) * h
    if e == 14:
        return (re + im) * h, (im - re) * h
    if e == 6:
        return (re + im) * -h, (re - im) * h
    if e == 10:
        return (im - re) * h, (re + im) * -h
    c, s = float(np.cos(np.pi * e / 8)), float(np.sin(np.pi * e / 8))
    return re * c - im * s, re * s + im * c


def _bf(x):
    return pltpu.bitcast(x, BF16)


def _tree(op, v):
    while len(v) > 1:
        v = [op(v[i], v[i + 1]) if i + 1 < len(v) else v[i] for i in range(0, len(v), 2)]
    return v[0]


def _run(*streams):
    order = sorted(((i + 0.5 * (k > 0)) / len(s), k, i) for k, s in enumerate(streams) for i in range(len(s)))
    for _, k, i in order:
        streams[k][i]()


def _left(a11, a12, a21, a22):
    return a21 + a22, a22, a11 + a22, a12 - a22, a11 + a12, a11, a21 - a11


def _right(b11, b12, b21, b22):
    return b11, b21 - b11, b11 + b22, b21 + b22, b22, b12 - b22, b11 + b12


def _strassen(product, emit):
    c = {}

    def run(k):
        c[k] = r = product(k)
        if k == 1:
            emit(1, 0, c[0] + r)
        elif k == 2:
            c[11], c[22] = r + c[1], r - c[0]
        elif k == 3:
            c[11] = c[11] + r
        elif k == 4:
            emit(0, 0, c[11] - r)
        elif k == 5:
            emit(0, 1, c[4] + r)
            c[22] = c[22] + r
        elif k == 6:
            emit(1, 1, c[22] + r)

    return [lambda k=k: run(k) for k in range(7)]


def _rows(i, n):
    return pl.ds(i * n if isinstance(i, int) else pl.multiple_of(i * n, n), n)


def _kernel(zero_ref, x_hbm, are_hbm, aim_hbm, bre_hbm, bim_hbm, cre_hbm, cim_hbm, ldt_hbm, dsk_hbm,
            wqkv_hbm, wo_hbm, f_hbm, g_hbm, out_hbm,
            xs, kf, ua, ub, uc, yb, par, zw, lag, qa, ka, va, qb, kb, vb,
            xio, io, abc, perm, wqkv, wo, fm, gm, kt, un, wt, us, wot, ob, ldt_ref, dsk_ref, sems):
    step = lambda fn, *a: (lambda: fn(*a))
    qs, ks, vs = (qa, qb), (ka, kb), (va, vb)
    head, rest = ([pltpu.make_async_copy(s.at[rows], abc.at[i, rows], sems.at[base + i])
                   for i, s in enumerate((are_hbm, aim_hbm, bre_hbm, bim_hbm, cre_hbm, cim_hbm))]
                  for base, rows in ((19, pl.ds(0, 32 * KPER)), (25, pl.ds(32 * KPER, D - 32 * KPER))))
    loads = [pltpu.make_async_copy(s, d, sems.at[i]) for i, (s, d) in enumerate(
        (*((x_hbm.at[:, _rows(c, 128)], xio.at[c]) for c in range(NB)),
         (f_hbm, fm), (wo_hbm, wo), (g_hbm, gm),
         *((wqkv_hbm.at[:, pl.ds(128 * j, 128)], wqkv.at[j]) for j in range(12))))]
    small = [pltpu.make_async_copy(s, d, sems.at[31 + i])
             for i, (s, d) in enumerate(((ldt_hbm, ldt_ref), (dsk_hbm, dsk_ref)))]
    for c in small + head + rest:
        c.start()
    for c in small:
        c.wait()
    high = jnp.uint32(0xFFFF0000)
    halves = lambda t: (pltpu.bitcast(t << 16, F32), pltpu.bitcast(t & high, F32))

    def col(ref):
        v = ref[...].astype(F32).reshape(1, D)
        return jnp.broadcast_to(v, (128, D)).T

    par[0] = jnp.exp(col(ldt_ref))
    par[1] = col(dsk_ref) * (1.0 / L)

    ri = lax.broadcasted_iota(jnp.int32, (128, 128), 0)
    ci = lax.broadcasted_iota(jnp.int32, (128, 128), 1)
    perm[...] = pltpu.bitcast(jnp.where(ci == (ri & 7) * DH + (ri >> 3), 1.0, 0.0).astype(BF16), U32)

    for c in head:
        c.wait()
    for c in loads:
        c.start()

    def setup(i):
        get = lambda k: halves(pltpu.bitcast(abc[k, _rows(i, 16), :], U32))
        dt = halves(pltpu.bitcast(par[0, _rows(i, 16), :].astype(BF16), U32))

        def pole(h):
            mag, ang = jnp.exp(dt[h] * get(0)[h]), dt[h] * get(1)[h]
            zw[i, h, 0], zw[i, h, 1] = mag * jnp.cos(ang), mag * jnp.sin(ang)

        def weight():
            scale = (1.0 + 1.5 * 2.0 ** -9) / L
            for h, (cr, ci, br, bi) in enumerate(zip(*map(get, (4, 5, 2, 3)))):
                wr, wi = _cmul((cr, ci), (dt[h] * br, dt[h] * bi))
                zw[i, h, 2], zw[i, h, 3] = wr * scale, wi * -scale

        return [step(pole, 0), weight, step(pole, 1)]

    lags = sorted({(c, r) for c in range(8) for r in _RND[c] if r < 16}) + [(8, 0)]
    stack = lambda vs: jnp.concatenate([jnp.concatenate([v[k] for v in vs], 0) for k in range(2)], 1).astype(BF16)

    def lagsums(i):
        zs, rhs, even = [], [], []

        def right(h):
            zr, zi, wr, wi = (zw[i, h, c] for c in range(4))
            z = {0: (jnp.ones((8, N), F32), jnp.zeros((8, N), F32)), 1: (zr, zi)}
            for e in (2, 4, 8, 16, 32, 64, 128, 256):
                z[e] = _csq(z[e // 2])
            b = [(wr, wi)]
            for e in (16, 32, 64, 128):
                zc = (z[e][0], -z[e][1])
                b += [_cmul(v, zc) for v in b]
            zs.append(z)
            rhs.append(stack(b))

        def left(h, lo, hi):
            z = zs[h]

            def power(e):
                if e not in z:
                    low = e % 256 if e > 256 and e % 256 else e & -e
                    z[e] = _csq(z[e // 2]) if e // 2 in z and e % 2 == 0 else _cmul(power(e - low), power(low))
                return z[e]

            a = [power(256 * c + r) for c, r in (lags + lags[-1:])[lo:hi]]
            o = pltpu.bitcast(lax.dot_general(stack(a), rhs[h], NT, preferred_element_type=F32), U32)
            if h:
                lag[i, 8 * lo:8 * hi, :] = jnp.concatenate(even, 0)[8 * lo:8 * hi] | (o & high)
            else:
                even.append(o >> 16)

        return [step(right, 0), step(left, 0, 0, 22), step(left, 0, 22, 42), step(right, 1), step(left, 1, 0, 20), step(left, 1, 20, 42)]

    def kgen(i):
        lane = lax.broadcasted_iota(jnp.int32, (8, 128), 1)
        src = (lane & 15) * 8 + lax.broadcasted_iota(jnp.int32, (8, 128), 0)

        memo = {}

        def piece(c, r):
            if r == 16:
                c = 0
            if (c, r) not in memo:
                memo[c, r] = (
                    pltpu.roll(jnp.where(lane == 0, piece(8, 0), merged(0, (0,) * 8)), 127, 1) if r == 16 else
                    jnp.take_along_axis(lag[i, _rows(lags.index((c, r)), 8), :], src, axis=1,
                                        mode="promise_in_bounds"))
            return memo[c, r]

        def merged(c, rs):
            if (c, rs) not in memo:
                memo[c, rs] = (piece(c, rs[0]) if c == 7 or min(rs) == 16 else
                               jnp.where(lane >> 4 == c, piece(c, rs[0]), merged(c + 1, rs[1:])))
            return memo[c, rs]

        for n0 in range(R0):
            kt[n0, _rows(i, 8), :] = merged(0, tuple(_RND[c][n0] for c in range(8)))

    get = lambda ref, n, rows: (ref[n, 0, rows, :], ref[n, 1, rows, :])

    def put(ref, n, rows, v):
        ref[n, 0, rows, :], ref[n, 1, rows, :] = v

    def outer(src, a, rows):
        x = _dft4([get(src, a + 4 * m, rows) for m in range(4)], 1, turn_out=a == 2)
        return [v if a * b == 4 else _twiddle(v, a * b) for b, v in enumerate(x)]

    def kfwd(n0, r):
        rows = _rows(r, 64)
        v = jnp.dot(_bf(kt[n0, _rows(r, 32), :]), _bf(fm[n0]), preferred_element_type=F32)
        put(ub, n0, rows, (v[:, :128] if n0 else v[:, :128] + par[1, rows, :], v[:, 128:]))

    def kdft(i):
        rows, t = _rows(i, 8), []

        def inner(b):
            for m, v in enumerate(_dft4([t[a][b] for a in range(4)], 1)):
                put(kf, b + 4 * m, rows, v)

        return [lambda a=a: t.append(outer(ub, a, rows)) for a in range(4)] + [step(inner, b) for b in range(4)]

    def fwd(n0, r):
        v = jnp.dot(un[n0, _rows(r, 64), :], _bf(fm[n0]), preferred_element_type=F32)
        put(ua, n0, _rows(r, 64), (v[:, :128], v[:, 128:]))

    def pre(a, i):
        for b, v in enumerate(outer(ua, a, _rows(i, 8))):
            put(ub, a + 4 * b, _rows(i, 8), v)

    def unouter(a, rows, t):
        for m, v in enumerate(_dft4([t[b] if a * b == 4 else _twiddle(t[b], -a * b) for b in range(4)], -1)):
            put(yb, a + 4 * m, rows, v)

    def mid(i):
        rows, first, t = _rows(i, 8), [], {}

        def inner(b):
            if b == 0:
                first.extend(outer(ua, 0, rows))
            x = _dft4([first[b]] + [get(ub, a + 4 * b, rows) for a in range(1, 4)], 1)
            t[b], *y = _dft4([_cmul(x[m], get(kf, b + 4 * m, rows)) for m in range(4)], -1, turn_out=b == 2)
            for a in range(1, 4):
                put(uc, a + 4 * b, rows, y[a - 1])
            if b == 3:
                unouter(0, rows, t)

        return [step(inner, b) for b in range(4)]

    def post(a, i):
        unouter(a, _rows(i, 8), [get(uc, a + 4 * b, _rows(i, 8)) for b in range(4)])

    def inv(n0, r):
        rows = _rows(r, 64)
        y = jnp.concatenate(get(yb, n0, rows), 1).astype(BF16)
        xs[n0, rows, :] = xs[n0, rows, :] + jnp.dot(y, _bf(gm[n0]), preferred_element_type=F32)

    def wprep(g, t):
        ops = []

        def load(h):
            if t < 3:
                lo, hi = (lax.dot_general(_bf(perm[...]), wqkv[4 * t + g, _rows(h + e, 128), :], NT,
                                          preferred_element_type=F32) for e in (0, 2))
                if t == 0:
                    lo, hi = lo * DH ** -0.5, hi * DH ** -0.5
            else:
                v = [jnp.dot(_bf(perm[...]), wo[_rows(2 * h + e, 128), _rows(g, 128)], preferred_element_type=F32)
                     for e in range(2)]
                lo, hi = (jnp.concatenate([u[64 * e:64 * e + 64] for u in v], 0).T for e in range(2))
            ops[:] = lo[:64], hi[:64], lo[64:], hi[64:]

        def save(h, i):
            for k, a in enumerate(_left(*[v[16 * i:16 * i + 16] for v in ops])):
                at = (_rows(4 * (t if t < 3 else g) + i, 8), _rows(h, 128))
                (wt if t < 3 else wot)[(g, k, *at) if t < 3 else (k, *at)] = pltpu.bitcast(a.astype(BF16), U32)

        return [f for h in range(2) for f in [step(load, h)] + [step(save, h, i) for i in range(4)]]

    def words(c):
        io[c, :L // 2, :] = pltpu.bitcast(xio[c], U32)

    def xin(j, c):
        xs[2 * j, _rows(c, 128), :], xs[2 * j + 1, _rows(c, 128), :] = halves(io[c, pl.ds(j, R1, stride=8), :].T)

    def norm(n0):
        acc, stat = {}, []

        def moment(k, lo, hi):
            for i in range(lo, hi):
                v = xs[n0, 8 * i:8 * i + 8, :]
                v = jnp.square(v - stat[0]) if k else v
                acc[i % 4] = v if i < 4 else acc[i % 4] + v
            if hi == D // 8:
                v = jnp.sum(_tree(jnp.add, list(acc.values())), axis=0, keepdims=True) * (1.0 / D)
                stat.append(lax.rsqrt(v + 1e-5) if k else v)

        def scale(c):
            rows = _rows(c, 128)
            un[n0, rows, :] = get(rows).astype(BF16)

        get = lambda rows: (xs[n0, rows, :] - stat[0]) * stat[1]
        return [[step(moment, 0, 0, 64)], [step(moment, 1, i, i + 16) for i in range(0, 64, 16)],
                [step(scale, c) for c in range(4)]], get

    def norms(*aa):
        return [f for a in aa for stage in zip(*[norm(a + 4 * m)[0] for m in range(4)])
                for steps in stage for f in steps]

    def pair_norms(a):
        stages, get = zip(*[norm(a + 4 * m) for m in range(4)])

        def operands(j, c):
            (b11, b21), (b12, b22) = ((f(_rows(c, 16)), f(_rows(c + 16, 16))) for f in get[2 * j:2 * j + 2])
            for k, b in enumerate(_right(b11, b12, b21, b22)):
                us[2 * a + j, k, _rows(c, 8), :] = pltpu.bitcast(b.astype(BF16), U32)

        return ([f for k in range(2) for st in stages for f in st[k]]
                + [step(operands, j, c) for j in range(2) for c in range(16)])

    def proj(i, slot, m, t):
        p, g, ref = i >> 2, i & 3, (qs, ks, vs)[t][slot]

        def emit(half, j, r):
            ref[m + 2 * j + 7 * (t > 0), _rows(half, 64), :] = r
            if t and m + j:
                ref[m + 2 * j - 1, _rows(half, 64), :] = pltpu.roll(r, 1, 1)

        return _strassen(lambda k: jnp.dot(_bf(wt[g, k, _rows(t, 32), :]), _bf(us[2 * p + 4 * (m & 1) + (m >> 2), k]),
                                           preferred_element_type=F32), emit)

    def attn(i, slot, m0):
        p, g = i >> 2, i & 3
        first = lax.broadcasted_iota(jnp.int32, (8, 128), 1) == 0
        window = lambda ref, d: {e: ref[slot][e, 8 * d:8 * d + 8, :] for e in range(m0, m0 + W + 1)}
        s, o = {}, {}

        def logits(m, d0):
            for d in (d0, d0 + 1):
                k = window(ks, d)
                q = qs[slot][m, 8 * d:8 * d + 8, :]
                for w in range(W):
                    t = q * k[m + 7 - w]
                    s[m, w] = t if d == 0 else s[m, w] + t

        def softmax(m):
            t = [jnp.where(first, -1e9, s[m, w]) if w > m else s[m, w] for w in range(W)]
            mx = _tree(jnp.maximum, t)
            e = [jnp.exp(v - mx) for v in t]
            rs = 1.0 / _tree(jnp.add, e)
            s.update({(m, w): e[w] * rs for w in range(W)})

        def values(d):
            v = window(vs, d)
            for m in (m0, m0 + 1):
                o[m, d] = _tree(jnp.add, [s[m, w] * v[m + 7 - w] for w in range(W)])
            if d % 2 and d > 8:
                blocks = [jnp.concatenate([o[m, e - 1], o[m, e]], 0) for e in (d - 8, d) for m in (m0, m0 + 1)]
                for k, b in enumerate(_right(*blocks)):
                    ob[m0 + p, k, g, 8 * d - 72:8 * d - 56, :] = b.astype(BF16)

        return ([f for m in (m0, m0 + 1) for f in [step(logits, m, d) for d in range(0, DH, 2)] + [step(softmax, m)]]
                + [step(values, d + e) for d in range(0, 8, 2) for e in (0, 1, 8, 9)])

    def oproj(p):
        def pair(c, m0):
            def emit(half, j, r):
                at = (2 * (m0 + j) + p, _rows(2 * c + half, 64))
                xs[at] = xs[at] + r

            return _strassen(lambda k: jnp.dot(_bf(wot[k, _rows(c, 32), :]), ob[m0 + p, k].reshape(D // 2, R1),
                                               preferred_element_type=F32), emit)

        return [f for c in range(NB) for m0 in range(0, 8, 2) for f in pair(c, m0)]

    def xout(c, j):
        lo, hi = (pltpu.bitcast(xs[2 * j + k, _rows(c, 128), :].astype(BF16).astype(F32), U32) for k in range(2))
        io[c, pl.ds(j, R1, stride=8), :] = ((lo >> 16) | hi).T

    four = lambda fn, *aa: [step(fn, a + 4 * m, r) for a in aa for m in range(4) for r in range(2 * NB)]
    block = lambda fn, a, r: [step(fn, a + 4 * m, 2 * r + h) for h in range(2) for m in range(4)] if 0 <= r < NB else []
    rowwise = lambda fn, a, n: [step(fn, a, i) for i in range(D // n)]

    regions, zero = [], zero_ref[0]

    def slot(*streams):
        regions.append(None)
        pl.when(zero < len(regions))(lambda: _run(*streams))

    pres = lambda a: rowwise(pre, a, 8)
    posts = lambda a: rowwise(post, a, 8)
    projs = lambda i, s, ms: [f for t in (1, 2, 0) for m in ms for f in proj(i, s, m, t)]
    attns = lambda i, s: [f for m in range(0, 8, 2) for f in attn(i, s, m)]

    with jax.named_scope("kgen"):
        ng = D // 16 // KPER
        each = lambda fn, s: [f for k in range(KPER) for f in fn(KPER * s + k)]

        def generate(s, more=(), last=False):
            for k in range(KPER):
                kgen(KPER * (s - 1) + k)
            _run(each(lagsums, s), more)
            if not last:
                _run(each(setup, s + 1))

        _run(setup(0))
        _run(each(lagsums, 0), [f for i in range(1, 2 * KPER) for f in setup(i)])
        for c in rest:
            c.wait()
        lax.fori_loop(1, ng - NB - 1, lambda s, _: generate(s), None)
        for c in loads[:NB]:
            c.wait()
        lax.fori_loop(0, NB, lambda c, _: generate(
            c + ng - NB - 1, [step(words, c)] + [step(xin, j, c) for j in range(8)]), None)
        generate(ng - 1, last=True)
    with jax.named_scope("kfwd"):
        for c in loads[NB:]:
            c.wait()
        kdfts = lambda r: [f for i in range(16) for f in kdft(16 * r + i)]
        for r, other in enumerate((norms(2, 1), *[sum(norm(n0)[0], []) for n0 in (3, 7)],
                                   sum(norm(11)[0] + norm(15)[0], []))):
            slot([f for a in range(4) for f in block(kfwd, a, r)], [f for t in (3, 0, 1, 2) for f in wprep(r, t)],
                 kdfts(r - 1) if r else [step(kgen, D // 16 - 1 - k) for k in range(KPER)], other)
        slot(four(fwd, 2), kdfts(NB - 1))
        slot(four(fwd, 1) + block(fwd, 3, 0), pres(2), norms(0))

    def layer(li, carry):
        with jax.named_scope("conv"):
            part = lambda steps, r: steps[len(steps) * r // NB:len(steps) * (r + 1) // NB] if 0 <= r < NB else []
            mids = [f for i in range(D // 8) for f in mid(i)]
            for r in range(-1, NB + 1):
                slot(block(fwd, 3, r + 2) + block(fwd, 0, r + 1) + block(inv, 0, r - 1) + block(inv, 2, r - 2)
                     + block(inv, 1, r - 2),
                     part(mids, r), part(pres(3), r + 1) + part(posts(2), r - 1) + part(posts(1), r - 1),
                     pres(1) if r < 0 else posts(3) if r == NB else [])
            slot(block(inv, 2, NB - 1) + block(inv, 1, NB - 1) + four(inv, 3), pair_norms(0))
            slot(projs(0, 0, (0, 4)), pair_norms(2))
            slot(projs(0, 0, (1, 5)), pair_norms(1))
        with jax.named_scope("attn"):
            slot(projs(1, 1, (0, 1, 4, 5)), attns(0, 0), pair_norms(3))
            both = lambda i, s: slot(projs(i + 1, 1 - s, (0, 1, 4, 5)), attns(i, s))
            lax.fori_loop(0, 3, lambda j, c: (both(2 * j + 1, 1), both(2 * j + 2, 0), c)[-1], 0)
            slot(oproj(0), attns(7, 1))

        @pl.when(li == 0)
        def _():
            slot(oproj(1), norms(2, 0))
            slot(four(fwd, 2), norms(1, 3))
            slot(four(fwd, 1) + block(fwd, 3, 0), pres(2))

        return carry

    lax.fori_loop(0, 2, layer, 0)

    with jax.named_scope("xout"):
        stores = [pltpu.make_async_copy(xio.at[c, _rows(i, 512)], out_hbm.at[_rows(i, 512), _rows(c, 128)],
                                        sems.at[4 * c + i]) for c in range(NB) for i in range(4)]
        last = oproj(1) + [lambda: None] * 7
        for c in range(NB):
            slot(last[28 * c + 7 * (c > 0):28 * c + 35],
                 [lambda: None] * (2 * (c == 0)) + [step(xout, c, j) for j in range(8)])
            for i in range(4):
                xio[c, _rows(i, 512), :] = _bf(io[c, _rows(i, 256), :])
                stores[4 * c + i].start()
        for c in stores:
            c.wait()


@jax.jit
def pallas_interleave_layers__ssm_conv_s4__sliding_local_dilated__prompt_kernel(
    A_u: jax.Array,
    A_A_re: jax.Array,
    A_A_im: jax.Array,
    A_B_re: jax.Array,
    A_B_im: jax.Array,
    A_C_re: jax.Array,
    A_C_im: jax.Array,
    A_log_dt: jax.Array,
    A_Dskip: jax.Array,
    B_x: jax.Array,
    B_wqkv: jax.Array,
    B_wo: jax.Array,
):
    del B_x
    hbm = pl.BlockSpec(memory_space=pl.ANY)
    tiles = lambda *n: pltpu.VMEM((*n, 128, 128), F32)
    out = pl.pallas_call(
        _kernel,
        out_shape=jax.ShapeDtypeStruct((L, D), BF16),
        in_specs=[pl.BlockSpec(memory_space=pltpu.SMEM)] + [hbm] * 13,
        out_specs=hbm,
        scratch_shapes=[
            pltpu.VMEM((R0, D, R1), F32),
            *[pltpu.VMEM((R0, 2, D, R1), F32)] * 5,
            pltpu.VMEM((2, D, N), F32),
            pltpu.VMEM((D // 16, 2, 4, 8, N), F32),
            pltpu.VMEM((D // 16, 336, 128), U32),
            *[tiles(n) for n in (8, 15, 15) * 2],
            pltpu.VMEM((NB, L, 128), BF16),
            pltpu.VMEM((NB, L // 2 + 8, 128), U32),
            pltpu.VMEM((6, D, N), BF16),
            pltpu.VMEM((64, 128), U32),
            pltpu.VMEM((12, D, 128), BF16),
            pltpu.VMEM((D, D), BF16),
            pltpu.VMEM(_F.shape, U32),
            pltpu.VMEM(_G.shape, U32),
            pltpu.VMEM((R0, D // 2, R1), U32),
            pltpu.VMEM((R0, D, R1), BF16),
            pltpu.VMEM((4, 7, 96, D // 2), U32),
            pltpu.VMEM((8, 7, D // 4, R1), U32),
            pltpu.VMEM((7, D // 4, D // 2), U32),
            pltpu.VMEM((8, 7, 4, 64, R1), BF16),
            pltpu.VMEM((D,), BF16),
            pltpu.VMEM((D,), BF16),
            pltpu.SemaphoreType.DMA((33,)),
        ],
        compiler_params=pltpu.CompilerParams(vmem_limit_bytes=100 * 1024 * 1024),
    )(np.zeros((1,), np.int32), A_u.reshape(L, D), A_A_re, A_A_im, A_B_re, A_B_im, A_C_re, A_C_im, A_log_dt, A_Dskip,
      B_wqkv, B_wo, _F, _G)
    return out.reshape(1, L, D)
```

```python
import jax
import jax.numpy as jnp
import ml_dtypes
import numpy as np
from jax import lax
import jax.experimental.pallas as pl
import jax.experimental.pallas.tpu as pltpu

L, D, N = 2048, 512, 128
R0, R1 = 16, 128
W, DH = 8, 16
F32, BF16, U32 = jnp.float32, jnp.bfloat16, jnp.uint32
KPER = 4
NB = D // 128
NT = (((1,), (1,)), ((), ()))


def _constants():
    n0 = np.arange(R0)[:, None, None]
    n1 = np.arange(R1)[None, :, None]
    k1 = np.arange(R1)[None, None, :]
    ang = 2.0 * np.pi * (k1 + 0.25) * (R0 * n1 + n0) / L
    f = np.concatenate([np.cos(ang), np.sin(ang)], axis=2)
    g = f.transpose(0, 2, 1)
    bf = ml_dtypes.bfloat16
    lr = np.arange(L).astype(np.float32).astype(bf).astype(np.int64).reshape(8, 16, R0)
    r = lr - (256 * np.arange(8)[:, None, None] + 16 * np.arange(16)[None, :, None])
    assert (r == r[:, :1, :]).all()

    def words(m):
        h = np.ascontiguousarray(m).astype(bf).view(np.uint16).astype(np.uint32)
        return h[:, 0::2] | (h[:, 1::2] << 16)

    return words(f), words(g), r[:, 0, :].tolist()


_F, _G, _RND = _constants()


def _cmul(a, b):
    return a[0] * b[0] - a[1] * b[1], a[0] * b[1] + a[1] * b[0]


def _csq(a):
    t = a[0] * a[1]
    return (a[0] + a[1]) * (a[0] - a[1]), t + t


def _dft4(x, sign, turn_out=False):
    (ar, ai), (br, bi), (cr, ci), (dr, di) = x
    sr, si, tr, ti = ar + cr, ai + ci, ar - cr, ai - ci
    ur, ui, vr, vi = br + dr, bi + di, br - dr, bi - di
    p, m = (tr - vi, ti + vr), (tr + vi, ti - vr)
    if sign < 0:
        p, m = m, p
    half = (sr - ur, si - ui) if not turn_out else (ui - si, sr - ur) if sign > 0 else (si - ui, ur - sr)
    return [(sr + ur, si + ui), p, half, m]


def _twiddle(v, e):
    e %= 16
    re, im = v
    h = float(np.sqrt(0.5))
    if e == 0:
        return v
    if e == 2:
        return (re - im) * h, (re + im) * h
    if e == 14:
        return (re + im) * h, (im - re) * h
    if e == 6:
        return (re + im) * -h, (re - im) * h
    if e == 10:
        return (im - re) * h, (re + im) * -h
    c, s = float(np.cos(np.pi * e / 8)), float(np.sin(np.pi * e / 8))
    return re * c - im * s, re * s + im * c


def _bf(x):
    return pltpu.bitcast(x, BF16)


def _tree(op, v):
    while len(v) > 1:
        v = [op(v[i], v[i + 1]) if i + 1 < len(v) else v[i] for i in range(0, len(v), 2)]
    return v[0]


def _run(*streams):
    order = sorted(((i + 0.5 * (k > 0)) / len(s), k, i) for k, s in enumerate(streams) for i in range(len(s)))
    for _, k, i in order:
        streams[k][i]()


def _left(a11, a12, a21, a22):
    return a21 + a22, a22, a11 + a22, a12 - a22, a11 + a12, a11, a21 - a11


def _right(b11, b12, b21, b22):
    return b11, b21 - b11, b11 + b22, b21 + b22, b22, b12 - b22, b11 + b12


def _strassen(product, emit):
    c = {}

    def run(k):
        c[k] = r = product(k)
        if k == 1:
            emit(1, 0, c[0] + r)
        elif k == 2:
            c[11], c[22] = r + c[1], r - c[0]
        elif k == 3:
            c[11] = c[11] + r
        elif k == 4:
            emit(0, 0, c[11] - r)
        elif k == 5:
            emit(0, 1, c[4] + r)
            c[22] = c[22] + r
        elif k == 6:
            emit(1, 1, c[22] + r)

    return [lambda k=k: run(k) for k in range(7)]


def _rows(i, n):
    return pl.ds(i * n if isinstance(i, int) else pl.multiple_of(i * n, n), n)


def _kernel(zero_ref, x_hbm, are_hbm, aim_hbm, bre_hbm, bim_hbm, cre_hbm, cim_hbm, ldt_hbm, dsk_hbm,
            wqkv_hbm, wo_hbm, f_hbm, g_hbm, out_hbm,
            xs, kf, ua, ub, uc, yb, par, zw, lag, qa, ka, va, qb, kb, vb,
            xio, io, abc, perm, wqkv, wo, fm, gm, kt, un, wt, us, wot, ob, ldt_ref, dsk_ref, sems):
    step = lambda fn, *a: (lambda: fn(*a))
    qs, ks, vs = (qa, qb), (ka, kb), (va, vb)
    head, rest = ([pltpu.make_async_copy(s.at[rows], abc.at[i, rows], sems.at[base + i])
                   for i, s in enumerate((are_hbm, aim_hbm, bre_hbm, bim_hbm, cre_hbm, cim_hbm))]
                  for base, rows in ((19, pl.ds(0, 32 * KPER)), (25, pl.ds(32 * KPER, D - 32 * KPER))))
    loads = [pltpu.make_async_copy(s, d, sems.at[i]) for i, (s, d) in enumerate(
        (*((x_hbm.at[:, _rows(c, 128)], xio.at[c]) for c in range(NB)),
         (f_hbm, fm), (wo_hbm, wo), (g_hbm, gm),
         *((wqkv_hbm.at[:, pl.ds(128 * j, 128)], wqkv.at[j]) for j in range(12))))]
    small = [pltpu.make_async_copy(s, d, sems.at[31 + i])
             for i, (s, d) in enumerate(((ldt_hbm, ldt_ref), (dsk_hbm, dsk_ref)))]
    for c in small + head + rest:
        c.start()
    for c in small:
        c.wait()
    high = jnp.uint32(0xFFFF0000)
    halves = lambda t: (pltpu.bitcast(t << 16, F32), pltpu.bitcast(t & high, F32))

    def col(ref):
        v = ref[...].astype(F32).reshape(1, D)
        return jnp.broadcast_to(v, (128, D)).T

    par[0] = jnp.exp(col(ldt_ref))
    par[1] = col(dsk_ref) * (1.0 / L)

    ri = lax.broadcasted_iota(jnp.int32, (128, 128), 0)
    ci = lax.broadcasted_iota(jnp.int32, (128, 128), 1)
    perm[...] = pltpu.bitcast(jnp.where(ci == (ri & 7) * DH + (ri >> 3), 1.0, 0.0).astype(BF16), U32)

    for c in head:
        c.wait()
    for c in loads:
        c.start()

    def setup(i):
        get = lambda k: halves(pltpu.bitcast(abc[k, _rows(i, 16), :], U32))
        dt = halves(pltpu.bitcast(par[0, _rows(i, 16), :].astype(BF16), U32))

        def pole(h):
            mag, ang = jnp.exp(dt[h] * get(0)[h]), dt[h] * get(1)[h]
            zw[i, h, 0], zw[i, h, 1] = mag * jnp.cos(ang), mag * jnp.sin(ang)

        def weight():
            scale = (1.0 + 1.5 * 2.0 ** -9) / L
            for h, (cr, ci, br, bi) in enumerate(zip(*map(get, (4, 5, 2, 3)))):
                wr, wi = _cmul((cr, ci), (dt[h] * br, dt[h] * bi))
                zw[i, h, 2], zw[i, h, 3] = wr * scale, wi * -scale

        return [step(pole, 0), weight, step(pole, 1)]

    lags = sorted({(c, r) for c in range(8) for r in _RND[c] if r < 16}) + [(8, 0)]
    stack = lambda vs: jnp.concatenate([jnp.concatenate([v[k] for v in vs], 0) for k in range(2)], 1).astype(BF16)

    def lagsums(i):
        zs, rhs, even = [], [], []

        def right(h):
            zr, zi, wr, wi = (zw[i, h, c] for c in range(4))
            z = {0: (jnp.ones((8, N), F32), jnp.zeros((8, N), F32)), 1: (zr, zi)}
            for e in (2, 4, 8, 16, 32, 64, 128, 256):
                z[e] = _csq(z[e // 2])
            b = [(wr, wi)]
            for e in (16, 32, 64, 128):
                zc = (z[e][0], -z[e][1])
                b += [_cmul(v, zc) for v in b]
            zs.append(z)
            rhs.append(stack(b))

        def left(h, lo, hi):
            z = zs[h]

            def power(e):
                if e not in z:
                    low = e % 256 if e > 256 and e % 256 else e & -e
                    z[e] = _csq(z[e // 2]) if e // 2 in z and e % 2 == 0 else _cmul(power(e - low), power(low))
                return z[e]

            a = [power(256 * c + r) for c, r in (lags + lags[-1:])[lo:hi]]
            o = pltpu.bitcast(lax.dot_general(stack(a), rhs[h], NT, preferred_element_type=F32), U32)
            if h:
                lag[i, 8 * lo:8 * hi, :] = jnp.concatenate(even, 0)[8 * lo:8 * hi] | (o & high)
            else:
                even.append(o >> 16)

        return [step(right, 0), step(left, 0, 0, 22), step(left, 0, 22, 42), step(right, 1), step(left, 1, 0, 20), step(left, 1, 20, 42)]

    def kgen(i):
        lane = lax.broadcasted_iota(jnp.int32, (8, 128), 1)
        src = (lane & 15) * 8 + lax.broadcasted_iota(jnp.int32, (8, 128), 0)

        memo = {}

        def piece(c, r):
            if r == 16:
                c = 0
            if (c, r) not in memo:
                memo[c, r] = (
                    pltpu.roll(jnp.where(lane == 0, piece(8, 0), merged(0, (0,) * 8)), 127, 1) if r == 16 else
                    jnp.take_along_axis(lag[i, _rows(lags.index((c, r)), 8), :], src, axis=1,
                                        mode="promise_in_bounds"))
            return memo[c, r]

        def merged(c, rs):
            if (c, rs) not in memo:
                memo[c, rs] = (piece(c, rs[0]) if c == 7 or min(rs) == 16 else
                               jnp.where(lane >> 4 == c, piece(c, rs[0]), merged(c + 1, rs[1:])))
            return memo[c, rs]

        for n0 in range(R0):
            kt[n0, _rows(i, 8), :] = merged(0, tuple(_RND[c][n0] for c in range(8)))

    get = lambda ref, n, rows: (ref[n, 0, rows, :], ref[n, 1, rows, :])

    def put(ref, n, rows, v):
        ref[n, 0, rows, :], ref[n, 1, rows, :] = v

    def outer(src, a, rows):
        x = _dft4([get(src, a + 4 * m, rows) for m in range(4)], 1, turn_out=a == 2)
        return [v if a * b == 4 else _twiddle(v, a * b) for b, v in enumerate(x)]

    def kfwd(n0, r):
        rows = _rows(r, 64)
        v = jnp.dot(_bf(kt[n0, _rows(r, 32), :]), _bf(fm[n0]), preferred_element_type=F32)
        put(ub, n0, rows, (v[:, :128] if n0 else v[:, :128] + par[1, rows, :], v[:, 128:]))

    def kdft(i):
        rows, t = _rows(i, 8), []

        def inner(b):
            for m, v in enumerate(_dft4([t[a][b] for a in range(4)], 1)):
                put(kf, b + 4 * m, rows, v)

        return [lambda a=a: t.append(outer(ub, a, rows)) for a in range(4)] + [step(inner, b) for b in range(4)]

    def fwd(n0, r):
        v = jnp.dot(un[n0, _rows(r, 64), :], _bf(fm[n0]), preferred_element_type=F32)
        put(ua, n0, _rows(r, 64), (v[:, :128], v[:, 128:]))

    def pre(a, i):
        for b, v in enumerate(outer(ua, a, _rows(i, 8))):
            put(ub, a + 4 * b, _rows(i, 8), v)

    def unouter(a, rows, t):
        for m, v in enumerate(_dft4([t[b] if a * b == 4 else _twiddle(t[b], -a * b) for b in range(4)], -1)):
            put(yb, a + 4 * m, rows, v)

    def mid(i):
        rows, first, t = _rows(i, 8), [], {}

        def inner(b):
            if b == 0:
                first.extend(outer(ua, 0, rows))
            x = _dft4([first[b]] + [get(ub, a + 4 * b, rows) for a in range(1, 4)], 1)
            t[b], *y = _dft4([_cmul(x[m], get(kf, b + 4 * m, rows)) for m in range(4)], -1, turn_out=b == 2)
            for a in range(1, 4):
                put(uc, a + 4 * b, rows, y[a - 1])
            if b == 3:
                unouter(0, rows, t)

        return [step(inner, b) for b in range(4)]

    def post(a, i):
        unouter(a, _rows(i, 8), [get(uc, a + 4 * b, _rows(i, 8)) for b in range(4)])

    def inv(n0, r):
        rows = _rows(r, 64)
        y = jnp.concatenate(get(yb, n0, rows), 1).astype(BF16)
        xs[n0, rows, :] = xs[n0, rows, :] + jnp.dot(y, _bf(gm[n0]), preferred_element_type=F32)

    def wprep(g, t):
        ops = []

        def load(h):
            if t < 3:
                lo, hi = (lax.dot_general(_bf(perm[...]), wqkv[4 * t + g, _rows(h + e, 128), :], NT,
                                          preferred_element_type=F32) for e in (0, 2))
                if t == 0:
                    lo, hi = lo * DH ** -0.5, hi * DH ** -0.5
            else:
                v = [jnp.dot(_bf(perm[...]), wo[_rows(2 * h + e, 128), _rows(g, 128)], preferred_element_type=F32)
                     for e in range(2)]
                lo, hi = (jnp.concatenate([u[64 * e:64 * e + 64] for u in v], 0).T for e in range(2))
            ops[:] = lo[:64], hi[:64], lo[64:], hi[64:]

        def save(h, i):
            for k, a in enumerate(_left(*[v[16 * i:16 * i + 16] for v in ops])):
                at = (_rows(4 * (t if t < 3 else g) + i, 8), _rows(h, 128))
                (wt if t < 3 else wot)[(g, k, *at) if t < 3 else (k, *at)] = pltpu.bitcast(a.astype(BF16), U32)

        return [f for h in range(2) for f in [step(load, h)] + [step(save, h, i) for i in range(4)]]

    def words(c):
        io[c, :L // 2, :] = pltpu.bitcast(xio[c], U32)

    def xin(j, c):
        xs[2 * j, _rows(c, 128), :], xs[2 * j + 1, _rows(c, 128), :] = halves(io[c, pl.ds(j, R1, stride=8), :].T)

    def norm(n0):
        acc, stat = {}, []

        def moment(k, lo, hi):
            for i in range(lo, hi):
                v = xs[n0, 8 * i:8 * i + 8, :]
                v = jnp.square(v - stat[0]) if k else v
                acc[i % 4] = v if i < 4 else acc[i % 4] + v
            if hi == D // 8:
                v = jnp.sum(_tree(jnp.add, list(acc.values())), axis=0, keepdims=True) * (1.0 / D)
                stat.append(lax.rsqrt(v + 1e-5) if k else v)

        def scale(c):
            rows = _rows(c, 128)
            un[n0, rows, :] = get(rows).astype(BF16)

        get = lambda rows: (xs[n0, rows, :] - stat[0]) * stat[1]
        return [[step(moment, 0, 0, 64)], [step(moment, 1, i, i + 16) for i in range(0, 64, 16)],
                [step(scale, c) for c in range(4)]], get

    def norms(*aa):
        return [f for a in aa for stage in zip(*[norm(a + 4 * m)[0] for m in range(4)])
                for steps in stage for f in steps]

    def pair_norms(a):
        stages, get = zip(*[norm(a + 4 * m) for m in range(4)])

        def operands(j, c):
            (b11, b21), (b12, b22) = ((f(_rows(c, 16)), f(_rows(c + 16, 16))) for f in get[2 * j:2 * j + 2])
            for k, b in enumerate(_right(b11, b12, b21, b22)):
                us[2 * a + j, k, _rows(c, 8), :] = pltpu.bitcast(b.astype(BF16), U32)

        return ([f for k in range(2) for st in stages for f in st[k]]
                + [step(operands, j, c) for j in range(2) for c in range(16)])

    def proj(i, slot, m, t):
        p, g, ref = i >> 2, i & 3, (qs, ks, vs)[t][slot]

        def emit(half, j, r):
            ref[m + 2 * j + 7 * (t > 0), _rows(half, 64), :] = r
            if t and m + j:
                ref[m + 2 * j - 1, _rows(half, 64), :] = pltpu.roll(r, 1, 1)

        return _strassen(lambda k: jnp.dot(_bf(wt[g, k, _rows(t, 32), :]), _bf(us[2 * p + 4 * (m & 1) + (m >> 2), k]),
                                           preferred_element_type=F32), emit)

    def attn(i, slot, m0):
        p, g = i >> 2, i & 3
        first = lax.broadcasted_iota(jnp.int32, (8, 128), 1) == 0
        window = lambda ref, d: {e: ref[slot][e, 8 * d:8 * d + 8, :] for e in range(m0, m0 + W + 1)}
        s, o = {}, {}

        def logits(m, d0):
            for d in (d0, d0 + 1):
                k = window(ks, d)
                q = qs[slot][m, 8 * d:8 * d + 8, :]
                for w in range(W):
                    t = q * k[m + 7 - w]
                    s[m, w] = t if d == 0 else s[m, w] + t

        def softmax(m):
            t = [jnp.where(first, -1e9, s[m, w]) if w > m else s[m, w] for w in range(W)]
            mx = _tree(jnp.maximum, t)
            e = [jnp.exp(v - mx) for v in t]
            rs = 1.0 / _tree(jnp.add, e)
            s.update({(m, w): e[w] * rs for w in range(W)})

        def values(d):
            v = window(vs, d)
            for m in (m0, m0 + 1):
                o[m, d] = _tree(jnp.add, [s[m, w] * v[m + 7 - w] for w in range(W)])
            if d % 2 and d > 8:
                blocks = [jnp.concatenate([o[m, e - 1], o[m, e]], 0) for e in (d - 8, d) for m in (m0, m0 + 1)]
                for k, b in enumerate(_right(*blocks)):
                    ob[m0 + p, k, g, 8 * d - 72:8 * d - 56, :] = b.astype(BF16)

        return ([f for m in (m0, m0 + 1) for f in [step(logits, m, d) for d in range(0, DH, 2)] + [step(softmax, m)]]
                + [step(values, d + e) for d in range(0, 8, 2) for e in (0, 1, 8, 9)])

    def oproj(p):
        def pair(c, m0):
            def emit(half, j, r):
                at = (2 * (m0 + j) + p, _rows(2 * c + half, 64))
                xs[at] = xs[at] + r

            return _strassen(lambda k: jnp.dot(_bf(wot[k, _rows(c, 32), :]), ob[m0 + p, k].reshape(D // 2, R1),
                                               preferred_element_type=F32), emit)

        return [f for c in range(NB) for m0 in range(0, 8, 2) for f in pair(c, m0)]

    def xout(c, j):
        lo, hi = (pltpu.bitcast(xs[2 * j + k, _rows(c, 128), :].astype(BF16).astype(F32), U32) for k in range(2))
        io[c, pl.ds(j, R1, stride=8), :] = ((lo >> 16) | hi).T

    four = lambda fn, *aa: [step(fn, a + 4 * m, r) for a in aa for m in range(4) for r in range(2 * NB)]
    block = lambda fn, a, r: [step(fn, a + 4 * m, 2 * r + h) for h in range(2) for m in range(4)] if 0 <= r < NB else []

    regions, zero = [], zero_ref[0]

    def slot(*streams):
        regions.append(None)
        pl.when(zero < len(regions))(lambda: _run(*streams))

    pres = lambda a: [step(pre, a, i) for i in range(D // 8)]
    posts = lambda a: [step(post, a, i) for i in range(D // 8)]
    projs = lambda i, s, ms: [f for t in (1, 2, 0) for m in ms for f in proj(i, s, m, t)]
    attns = lambda i, s: [f for m in range(0, 8, 2) for f in attn(i, s, m)]

    with jax.named_scope("kgen"):
        ng = D // 16 // KPER
        each = lambda fn, s: [f for k in range(KPER) for f in fn(KPER * s + k)]

        def generate(s, more=(), last=False):
            for k in range(KPER):
                kgen(KPER * (s - 1) + k)
            _run(each(lagsums, s), more)
            if not last:
                _run(each(setup, s + 1))

        _run(setup(0))
        _run(each(lagsums, 0), [f for i in range(1, 2 * KPER) for f in setup(i)])
        for c in rest:
            c.wait()
        lax.fori_loop(1, ng - NB - 1, lambda s, _: generate(s), None)
        for c in loads[:NB]:
            c.wait()
        lax.fori_loop(0, NB, lambda c, _: generate(
            c + ng - NB - 1, [step(words, c)] + [step(xin, j, c) for j in range(8)]), None)
        generate(ng - 1, last=True)
    with jax.named_scope("kfwd"):
        for c in loads[NB:]:
            c.wait()
        kdfts = lambda r: [f for i in range(16) for f in kdft(16 * r + i)]
        for r, other in enumerate((norms(2, 1), *[sum(norm(n0)[0], []) for n0 in (3, 7)],
                                   sum(norm(11)[0] + norm(15)[0], []))):
            slot([f for a in range(4) for f in block(kfwd, a, r)], [f for t in (3, 0, 1, 2) for f in wprep(r, t)],
                 kdfts(r - 1) if r else [step(kgen, D // 16 - 1 - k) for k in range(KPER)], other)
        slot(four(fwd, 2), kdfts(NB - 1))

    def layer(li, carry):
        with jax.named_scope("conv"):
            part = lambda steps, r: steps[len(steps) * r // NB:len(steps) * (r + 1) // NB] if 0 <= r < NB else []
            slot(four(fwd, 1) + block(fwd, 3, 0), pres(2), norms(0))
            mids = [f for i in range(D // 8) for f in mid(i)]
            for r in range(-1, NB + 1):
                slot(block(fwd, 3, r + 2) + block(fwd, 0, r + 1) + block(inv, 0, r - 1) + block(inv, 2, r - 2)
                     + block(inv, 1, r - 2),
                     part(mids, r), part(pres(3), r + 1) + part(posts(2), r - 1) + part(posts(1), r - 1),
                     pres(1) if r < 0 else posts(3) if r == NB else [])
            slot(block(inv, 2, NB - 1) + block(inv, 1, NB - 1) + four(inv, 3), pair_norms(0))
            slot(projs(0, 0, (0, 4)), pair_norms(2))
            slot(projs(0, 0, (1, 5)), pair_norms(1))
        with jax.named_scope("attn"):
            slot(projs(1, 1, (0, 1, 4, 5)), attns(0, 0), pair_norms(3))
            both = lambda i, s: slot(projs(i + 1, 1 - s, (0, 1, 4, 5)), attns(i, s))
            lax.fori_loop(0, 3, lambda j, c: (both(2 * j + 1, 1), both(2 * j + 2, 0), c)[-1], 0)
            slot(oproj(0), attns(7, 1))

        @pl.when(li == 0)
        def _():
            slot(oproj(1), norms(2))
            slot(four(fwd, 2), norms(1, 3))

        return carry

    lax.fori_loop(0, 2, layer, 0)

    with jax.named_scope("xout"):
        stores = [pltpu.make_async_copy(xio.at[c, _rows(i, 512)], out_hbm.at[_rows(i, 512), _rows(c, 128)],
                                        sems.at[4 * c + i]) for c in range(NB) for i in range(4)]
        last = oproj(1) + [lambda: None] * 7
        for c in range(NB):
            slot(last[28 * c + 7 * (c > 0):28 * c + 35],
                 [lambda: None] * (2 * (c == 0)) + [step(xout, c, j) for j in range(8)])
            for i in range(4):
                xio[c, _rows(i, 512), :] = _bf(io[c, _rows(i, 256), :])
                stores[4 * c + i].start()
        for c in stores:
            c.wait()


@jax.jit
def pallas_interleave_layers__ssm_conv_s4__sliding_local_dilated__prompt_kernel(
    A_u: jax.Array,
    A_A_re: jax.Array,
    A_A_im: jax.Array,
    A_B_re: jax.Array,
    A_B_im: jax.Array,
    A_C_re: jax.Array,
    A_C_im: jax.Array,
    A_log_dt: jax.Array,
    A_Dskip: jax.Array,
    B_x: jax.Array,
    B_wqkv: jax.Array,
    B_wo: jax.Array,
):
    del B_x
    hbm = pl.BlockSpec(memory_space=pl.ANY)
    tiles = lambda *n: pltpu.VMEM((*n, 128, 128), F32)
    out = pl.pallas_call(
        _kernel,
        out_shape=jax.ShapeDtypeStruct((L, D), BF16),
        in_specs=[pl.BlockSpec(memory_space=pltpu.SMEM)] + [hbm] * 13,
        out_specs=hbm,
        scratch_shapes=[
            pltpu.VMEM((R0, D, R1), F32),
            *[pltpu.VMEM((R0, 2, D, R1), F32)] * 5,
            pltpu.VMEM((2, D, N), F32),
            pltpu.VMEM((D // 16, 2, 4, 8, N), F32),
            pltpu.VMEM((D // 16, 336, 128), U32),
            *[tiles(n) for n in (8, 15, 15) * 2],
            pltpu.VMEM((NB, L, 128), BF16),
            pltpu.VMEM((NB, L // 2 + 8, 128), U32),
            pltpu.VMEM((6, D, N), BF16),
            pltpu.VMEM((64, 128), U32),
            pltpu.VMEM((12, D, 128), BF16),
            pltpu.VMEM((D, D), BF16),
            pltpu.VMEM(_F.shape, U32),
            pltpu.VMEM(_G.shape, U32),
            pltpu.VMEM((R0, D // 2, R1), U32),
            pltpu.VMEM((R0, D, R1), BF16),
            pltpu.VMEM((4, 7, 96, D // 2), U32),
            pltpu.VMEM((8, 7, D // 4, R1), U32),
            pltpu.VMEM((7, D // 4, D // 2), U32),
            pltpu.VMEM((8, 7, 4, 64, R1), BF16),
            pltpu.VMEM((D,), BF16),
            pltpu.VMEM((D,), BF16),
            pltpu.SemaphoreType.DMA((33,)),
        ],
        compiler_params=pltpu.CompilerParams(vmem_limit_bytes=100 * 1024 * 1024),
    )(np.zeros((1,), np.int32), A_u.reshape(L, D), A_A_re, A_A_im, A_B_re, A_B_im, A_C_re, A_C_im, A_log_dt, A_Dskip,
      B_wqkv, B_wo, _F, _G)
    return out.reshape(1, L, D)
```

```python
import jax
import jax.numpy as jnp
import ml_dtypes
import numpy as np
from jax import lax
import jax.experimental.pallas as pl
import jax.experimental.pallas.tpu as pltpu

L, D, N = 2048, 512, 128
R0, R1 = 16, 128
W, DH = 8, 16
F32, BF16, U32 = jnp.float32, jnp.bfloat16, jnp.uint32
KPER = 4
NB = D // 128
NT = (((1,), (1,)), ((), ()))


def _constants():
    n0 = np.arange(R0)[:, None, None]
    n1 = np.arange(R1)[None, :, None]
    k1 = np.arange(R1)[None, None, :]
    ang = 2.0 * np.pi * (k1 + 0.25) * (R0 * n1 + n0) / L
    f = np.concatenate([np.cos(ang), np.sin(ang)], axis=2)
    g = f.transpose(0, 2, 1)
    bf = ml_dtypes.bfloat16
    lr = np.arange(L).astype(np.float32).astype(bf).astype(np.int64).reshape(8, 16, R0)
    r = lr - (256 * np.arange(8)[:, None, None] + 16 * np.arange(16)[None, :, None])
    assert (r == r[:, :1, :]).all()

    def words(m):
        h = np.ascontiguousarray(m).astype(bf).view(np.uint16).astype(np.uint32)
        return h[:, 0::2] | (h[:, 1::2] << 16)

    return words(f), words(g), r[:, 0, :].tolist()


_F, _G, _RND = _constants()


def _cmul(a, b):
    return a[0] * b[0] - a[1] * b[1], a[0] * b[1] + a[1] * b[0]


def _csq(a):
    t = a[0] * a[1]
    return (a[0] + a[1]) * (a[0] - a[1]), t + t


def _dft4(x, sign, turn_out=False):
    (ar, ai), (br, bi), (cr, ci), (dr, di) = x
    sr, si, tr, ti = ar + cr, ai + ci, ar - cr, ai - ci
    ur, ui, vr, vi = br + dr, bi + di, br - dr, bi - di
    p, m = (tr - vi, ti + vr), (tr + vi, ti - vr)
    if sign < 0:
        p, m = m, p
    half = (sr - ur, si - ui) if not turn_out else (ui - si, sr - ur) if sign > 0 else (si - ui, ur - sr)
    return [(sr + ur, si + ui), p, half, m]


def _twiddle(v, e):
    e %= 16
    re, im = v
    h = float(np.sqrt(0.5))
    if e == 0:
        return v
    if e == 2:
        return (re - im) * h, (re + im) * h
    if e == 14:
        return (re + im) * h, (im - re) * h
    if e == 6:
        return (re + im) * -h, (re - im) * h
    if e == 10:
        return (im - re) * h, (re + im) * -h
    c, s = float(np.cos(np.pi * e / 8)), float(np.sin(np.pi * e / 8))
    return re * c - im * s, re * s + im * c


def _bf(x):
    return pltpu.bitcast(x, BF16)


def _tree(op, v):
    while len(v) > 1:
        v = [op(v[i], v[i + 1]) if i + 1 < len(v) else v[i] for i in range(0, len(v), 2)]
    return v[0]


def _run(*streams):
    order = sorted(((i + 0.5 * (k > 0)) / len(s), k, i) for k, s in enumerate(streams) for i in range(len(s)))
    for _, k, i in order:
        streams[k][i]()


def _left(a11, a12, a21, a22):
    return a21 + a22, a22, a11 + a22, a12 - a22, a11 + a12, a11, a21 - a11


def _right(b11, b12, b21, b22):
    return b11, b21 - b11, b11 + b22, b21 + b22, b22, b12 - b22, b11 + b12


def _strassen(product, emit):
    c = {}

    def run(k):
        c[k] = r = product(k)
        if k == 1:
            emit(1, 0, c[0] + r)
        elif k == 2:
            c[11], c[22] = r + c[1], r - c[0]
        elif k == 3:
            c[11] = c[11] + r
        elif k == 4:
            emit(0, 0, c[11] - r)
        elif k == 5:
            emit(0, 1, c[4] + r)
            c[22] = c[22] + r
        elif k == 6:
            emit(1, 1, c[22] + r)

    return [lambda k=k: run(k) for k in range(7)]


def _rows(i, n):
    return pl.ds(i * n if isinstance(i, int) else pl.multiple_of(i * n, n), n)


def _kernel(zero_ref, x_hbm, are_hbm, aim_hbm, bre_hbm, bim_hbm, cre_hbm, cim_hbm, ldt_hbm, dsk_hbm,
            wqkv_hbm, wo_hbm, f_hbm, g_hbm, out_hbm,
            xs, kf, ua, ub, uc, yb, par, zw, lag, qa, ka, va, qb, kb, vb,
            xio, io, abc, perm, wqkv, wo, fm, gm, kt, un, wt, us, wot, ob, ldt_ref, dsk_ref, sems):
    step = lambda fn, *a: (lambda: fn(*a))
    qs, ks, vs = (qa, qb), (ka, kb), (va, vb)
    head, rest = ([pltpu.make_async_copy(s.at[rows], abc.at[i, rows], sems.at[base + i])
                   for i, s in enumerate((are_hbm, aim_hbm, bre_hbm, bim_hbm, cre_hbm, cim_hbm))]
                  for base, rows in ((19, pl.ds(0, 32 * KPER)), (25, pl.ds(32 * KPER, D - 32 * KPER))))
    loads = [pltpu.make_async_copy(s, d, sems.at[i]) for i, (s, d) in enumerate(
        (*((x_hbm.at[:, _rows(c, 128)], xio.at[c]) for c in range(NB)),
         (f_hbm, fm), (wo_hbm, wo), (g_hbm, gm),
         *((wqkv_hbm.at[:, pl.ds(128 * j, 128)], wqkv.at[j]) for j in range(12))))]
    small = [pltpu.make_async_copy(s, d, sems.at[31 + i])
             for i, (s, d) in enumerate(((ldt_hbm, ldt_ref), (dsk_hbm, dsk_ref)))]
    for c in small + head + rest:
        c.start()
    for c in small:
        c.wait()
    high = jnp.uint32(0xFFFF0000)
    halves = lambda t: (pltpu.bitcast(t << 16, F32), pltpu.bitcast(t & high, F32))

    def col(ref):
        v = ref[...].astype(F32).reshape(1, D)
        return jnp.broadcast_to(v, (128, D)).T

    par[0] = jnp.exp(col(ldt_ref))
    par[1] = col(dsk_ref) * (1.0 / L)

    ri = lax.broadcasted_iota(jnp.int32, (128, 128), 0)
    ci = lax.broadcasted_iota(jnp.int32, (128, 128), 1)
    perm[...] = pltpu.bitcast(jnp.where(ci == (ri & 7) * DH + (ri >> 3), 1.0, 0.0).astype(BF16), U32)

    for c in head:
        c.wait()
    for c in loads:
        c.start()

    def setup(i):
        get = lambda k: halves(pltpu.bitcast(abc[k, _rows(i, 16), :], U32))
        dt = halves(pltpu.bitcast(par[0, _rows(i, 16), :].astype(BF16), U32))

        def pole(h):
            mag, ang = jnp.exp(dt[h] * get(0)[h]), dt[h] * get(1)[h]
            zw[i, h, 0], zw[i, h, 1] = mag * jnp.cos(ang), mag * jnp.sin(ang)

        def weight():
            scale = (1.0 + 1.5 * 2.0 ** -9) / L
            for h, (cr, ci, br, bi) in enumerate(zip(*map(get, (4, 5, 2, 3)))):
                wr, wi = _cmul((cr, ci), (dt[h] * br, dt[h] * bi))
                zw[i, h, 2], zw[i, h, 3] = wr * scale, wi * -scale

        return [step(pole, 0), weight, step(pole, 1)]

    lags = sorted({(c, r) for c in range(8) for r in _RND[c] if r < 16}) + [(8, 0)]
    stack = lambda vs: jnp.concatenate([jnp.concatenate([v[k] for v in vs], 0) for k in range(2)], 1).astype(BF16)

    def lagsums(i):
        zs, rhs, even = [], [], []

        def right(h):
            zr, zi, wr, wi = (zw[i, h, c] for c in range(4))
            z = {0: (jnp.ones((8, N), F32), jnp.zeros((8, N), F32)), 1: (zr, zi)}
            for e in (2, 4, 8, 16, 32, 64, 128, 256):
                z[e] = _csq(z[e // 2])
            b = [(wr, wi)]
            for e in (16, 32, 64, 128):
                zc = (z[e][0], -z[e][1])
                b += [_cmul(v, zc) for v in b]
            zs.append(z)
            rhs.append(stack(b))

        def left(h, lo, hi):
            z = zs[h]

            def power(e):
                if e not in z:
                    low = e % 256 if e > 256 and e % 256 else e & -e
                    z[e] = _csq(z[e // 2]) if e // 2 in z and e % 2 == 0 else _cmul(power(e - low), power(low))
                return z[e]

            a = [power(256 * c + r) for c, r in (lags + lags[-1:])[lo:hi]]
            o = pltpu.bitcast(lax.dot_general(stack(a), rhs[h], NT, preferred_element_type=F32), U32)
            if h:
                lag[i, 8 * lo:8 * hi, :] = jnp.concatenate(even, 0)[8 * lo:8 * hi] | (o & high)
            else:
                even.append(o >> 16)

        return [step(right, 0), step(left, 0, 0, 22), step(left, 0, 22, 42), step(right, 1), step(left, 1, 0, 20), step(left, 1, 20, 42)]

    def kgen(i):
        lane = lax.broadcasted_iota(jnp.int32, (8, 128), 1)
        src = (lane & 15) * 8 + lax.broadcasted_iota(jnp.int32, (8, 128), 0)

        memo = {}

        def piece(c, r):
            if r == 16:
                c = 0
            if (c, r) not in memo:
                memo[c, r] = (
                    pltpu.roll(jnp.where(lane == 0, piece(8, 0), merged(0, (0,) * 8)), 127, 1) if r == 16 else
                    jnp.take_along_axis(lag[i, _rows(lags.index((c, r)), 8), :], src, axis=1,
                                        mode="promise_in_bounds"))
            return memo[c, r]

        def merged(c, rs):
            if (c, rs) not in memo:
                memo[c, rs] = (piece(c, rs[0]) if c == 7 or min(rs) == 16 else
                               jnp.where(lane >> 4 == c, piece(c, rs[0]), merged(c + 1, rs[1:])))
            return memo[c, rs]

        for n0 in range(R0):
            kt[n0, _rows(i, 8), :] = merged(0, tuple(_RND[c][n0] for c in range(8)))

    get = lambda ref, n, rows: (ref[n, 0, rows, :], ref[n, 1, rows, :])

    def put(ref, n, rows, v):
        ref[n, 0, rows, :], ref[n, 1, rows, :] = v

    def outer(src, a, rows):
        x = _dft4([get(src, a + 4 * m, rows) for m in range(4)], 1, turn_out=a == 2)
        return [v if a * b == 4 else _twiddle(v, a * b) for b, v in enumerate(x)]

    def kfwd(n0, r):
        rows = _rows(r, 64)
        v = jnp.dot(_bf(kt[n0, _rows(r, 32), :]), _bf(fm[n0]), preferred_element_type=F32)
        put(ub, n0, rows, (v[:, :128] if n0 else v[:, :128] + par[1, rows, :], v[:, 128:]))

    def kdft(i):
        rows, t = _rows(i, 8), []

        def inner(b):
            for m, v in enumerate(_dft4([t[a][b] for a in range(4)], 1)):
                put(kf, b + 4 * m, rows, v)

        return [lambda a=a: t.append(outer(ub, a, rows)) for a in range(4)] + [step(inner, b) for b in range(4)]

    def fwd(n0, r):
        v = jnp.dot(un[n0, _rows(r, 64), :], _bf(fm[n0]), preferred_element_type=F32)
        put(ua, n0, _rows(r, 64), (v[:, :128], v[:, 128:]))

    def pre(a, i):
        for b, v in enumerate(outer(ua, a, _rows(i, 8))):
            put(ub, a + 4 * b, _rows(i, 8), v)

    def unouter(a, rows, t):
        for m, v in enumerate(_dft4([t[b] if a * b == 4 else _twiddle(t[b], -a * b) for b in range(4)], -1)):
            put(yb, a + 4 * m, rows, v)

    def mid(i):
        rows, first, t = _rows(i, 8), [], {}

        def inner(b):
            if b == 0:
                first.extend(outer(ua, 0, rows))
            x = _dft4([first[b]] + [get(ub, a + 4 * b, rows) for a in range(1, 4)], 1)
            t[b], *y = _dft4([_cmul(x[m], get(kf, b + 4 * m, rows)) for m in range(4)], -1, turn_out=b == 2)
            for a in range(1, 4):
                put(uc, a + 4 * b, rows, y[a - 1])
            if b == 3:
                unouter(0, rows, t)

        return [step(inner, b) for b in range(4)]

    def post(a, i):
        unouter(a, _rows(i, 8), [get(uc, a + 4 * b, _rows(i, 8)) for b in range(4)])

    def inv(n0, r):
        rows = _rows(r, 64)
        y = jnp.concatenate(get(yb, n0, rows), 1).astype(BF16)
        xs[n0, rows, :] = xs[n0, rows, :] + jnp.dot(y, _bf(gm[n0]), preferred_element_type=F32)

    def wprep(g, t):
        ops = []

        def load(h):
            if t < 3:
                lo, hi = (lax.dot_general(_bf(perm[...]), wqkv[4 * t + g, _rows(h + e, 128), :], NT,
                                          preferred_element_type=F32) for e in (0, 2))
                if t == 0:
                    lo, hi = lo * DH ** -0.5, hi * DH ** -0.5
            else:
                v = [jnp.dot(_bf(perm[...]), wo[_rows(2 * h + e, 128), _rows(g, 128)], preferred_element_type=F32)
                     for e in range(2)]
                lo, hi = (jnp.concatenate([u[64 * e:64 * e + 64] for u in v], 0).T for e in range(2))
            ops[:] = lo[:64], hi[:64], lo[64:], hi[64:]

        def save(h, i):
            for k, a in enumerate(_left(*[v[16 * i:16 * i + 16] for v in ops])):
                at = (_rows(4 * (t if t < 3 else g) + i, 8), _rows(h, 128))
                (wt if t < 3 else wot)[(g, k, *at) if t < 3 else (k, *at)] = pltpu.bitcast(a.astype(BF16), U32)

        return [f for h in range(2) for f in [step(load, h)] + [step(save, h, i) for i in range(4)]]

    def words(c):
        io[c, :L // 2, :] = pltpu.bitcast(xio[c], U32)

    def xin(j, c):
        xs[2 * j, _rows(c, 128), :], xs[2 * j + 1, _rows(c, 128), :] = halves(io[c, pl.ds(j, R1, stride=8), :].T)

    def norm(n0):
        acc, stat = {}, []

        def moment(k, lo, hi):
            for i in range(lo, hi):
                v = xs[n0, 8 * i:8 * i + 8, :]
                v = jnp.square(v - stat[0]) if k else v
                acc[i % 4] = v if i < 4 else acc[i % 4] + v
            if hi == D // 8:
                v = jnp.sum(_tree(jnp.add, list(acc.values())), axis=0, keepdims=True) * (1.0 / D)
                stat.append(lax.rsqrt(v + 1e-5) if k else v)

        def scale(c):
            rows = _rows(c, 128)
            un[n0, rows, :] = get(rows).astype(BF16)

        get = lambda rows: (xs[n0, rows, :] - stat[0]) * stat[1]
        return [[step(moment, 0, 0, 64)], [step(moment, 1, i, i + 16) for i in range(0, 64, 16)],
                [step(scale, c) for c in range(4)]], get

    def norms(*aa):
        return [f for a in aa for stage in zip(*[norm(a + 4 * m)[0] for m in range(4)])
                for steps in stage for f in steps]

    def pair_norms(a):
        stages, get = zip(*[norm(a + 4 * m) for m in range(4)])

        def operands(j, c):
            (b11, b21), (b12, b22) = ((f(_rows(c, 16)), f(_rows(c + 16, 16))) for f in get[2 * j:2 * j + 2])
            for k, b in enumerate(_right(b11, b12, b21, b22)):
                us[2 * a + j, k, _rows(c, 8), :] = pltpu.bitcast(b.astype(BF16), U32)

        return ([f for k in range(2) for st in stages for f in st[k]]
                + [step(operands, j, c) for j in range(2) for c in range(16)])

    def proj(i, slot, m, t):
        p, g, ref = i >> 2, i & 3, (qs, ks, vs)[t][slot]

        def emit(half, j, r):
            ref[m + 2 * j + 7 * (t > 0), _rows(half, 64), :] = r
            if t and m + j:
                ref[m + 2 * j - 1, _rows(half, 64), :] = pltpu.roll(r, 1, 1)

        return _strassen(lambda k: jnp.dot(_bf(wt[g, k, _rows(t, 32), :]), _bf(us[2 * p + 4 * (m & 1) + (m >> 2), k]),
                                           preferred_element_type=F32), emit)

    def attn(i, slot, m0):
        p, g = i >> 2, i & 3
        first = lax.broadcasted_iota(jnp.int32, (8, 128), 1) == 0
        window = lambda ref, d: {e: ref[slot][e, 8 * d:8 * d + 8, :] for e in range(m0, m0 + W + 1)}
        s, o = {}, {}

        def logits(m, d0):
            for d in (d0, d0 + 1):
                k = window(ks, d)
                q = qs[slot][m, 8 * d:8 * d + 8, :]
                for w in range(W):
                    t = q * k[m + 7 - w]
                    s[m, w] = t if d == 0 else s[m, w] + t

        def softmax(m):
            t = [jnp.where(first, -1e9, s[m, w]) if w > m else s[m, w] for w in range(W)]
            mx = _tree(jnp.maximum, t)
            e = [jnp.exp(v - mx) for v in t]
            rs = 1.0 / _tree(jnp.add, e)
            s.update({(m, w): e[w] * rs for w in range(W)})

        def values(d):
            v = window(vs, d)
            for m in (m0, m0 + 1):
                o[m, d] = _tree(jnp.add, [s[m, w] * v[m + 7 - w] for w in range(W)])
            if d % 2 and d > 8:
                blocks = [jnp.concatenate([o[m, e - 1], o[m, e]], 0) for e in (d - 8, d) for m in (m0, m0 + 1)]
                for k, b in enumerate(_right(*blocks)):
                    ob[m0 + p, k, g, 8 * d - 72:8 * d - 56, :] = b.astype(BF16)

        return ([f for m in (m0, m0 + 1) for f in [step(logits, m, d) for d in range(0, DH, 2)] + [step(softmax, m)]]
                + [step(values, d + e) for d in range(0, 8, 2) for e in (0, 1, 8, 9)])

    def oproj(p):
        def pair(c, m0):
            def emit(half, j, r):
                at = (2 * (m0 + j) + p, _rows(2 * c + half, 64))
                xs[at] = xs[at] + r

            return _strassen(lambda k: jnp.dot(_bf(wot[k, _rows(c, 32), :]), ob[m0 + p, k].reshape(D // 2, R1),
                                               preferred_element_type=F32), emit)

        return [f for c in range(NB) for m0 in range(0, 8, 2) for f in pair(c, m0)]

    def xout(c, j):
        lo, hi = (pltpu.bitcast(xs[2 * j + k, _rows(c, 128), :].astype(BF16).astype(F32), U32) for k in range(2))
        io[c, pl.ds(j, R1, stride=8), :] = ((lo >> 16) | hi).T

    four = lambda fn, *aa: [step(fn, a + 4 * m, r) for a in aa for m in range(4) for r in range(2 * NB)]
    block = lambda fn, a, r: [step(fn, a + 4 * m, 2 * r + h) for h in range(2) for m in range(4)] if 0 <= r < NB else []

    regions, zero = [], zero_ref[0]

    def slot(*streams):
        regions.append(None)
        pl.when(zero < len(regions))(lambda: _run(*streams))

    pres = lambda a: [step(pre, a, i) for i in range(D // 8)]
    posts = lambda a: [step(post, a, i) for i in range(D // 8)]
    projs = lambda i, s, ms: [f for t in (1, 2, 0) for m in ms for f in proj(i, s, m, t)]
    attns = lambda i, s: [f for m in range(0, 8, 2) for f in attn(i, s, m)]

    with jax.named_scope("kgen"):
        ng = D // 16 // KPER
        each = lambda fn, s: [f for k in range(KPER) for f in fn(KPER * s + k)]

        def generate(s, more=(), last=False):
            for k in range(KPER):
                kgen(KPER * (s - 1) + k)
            _run(each(lagsums, s), more)
            if not last:
                _run(each(setup, s + 1))

        _run(setup(0))
        _run(each(lagsums, 0), [f for i in range(1, 2 * KPER) for f in setup(i)])
        for c in rest:
            c.wait()
        lax.fori_loop(1, ng - NB - 1, lambda s, _: generate(s), None)
        for c in loads[:NB]:
            c.wait()
        lax.fori_loop(0, NB, lambda c, _: generate(
            c + ng - NB - 1, [step(words, c)] + [step(xin, j, c) for j in range(8)]), None)
        generate(ng - 1, last=True)
    with jax.named_scope("kfwd"):
        for c in loads[NB:]:
            c.wait()
        kdfts = lambda r: [f for i in range(16) for f in kdft(16 * r + i)]
        for r, other in enumerate((norms(2, 1), *[sum(norm(n0)[0], []) for n0 in (3, 7)],
                                   sum(norm(11)[0] + norm(15)[0], []))):
            slot([f for a in range(4) for f in block(kfwd, a, r)], [f for t in (3, 0, 1, 2) for f in wprep(r, t)],
                 kdfts(r - 1) if r else [step(kgen, D // 16 - 1 - k) for k in range(KPER)], other)
        slot(four(fwd, 2), kdfts(NB - 1))

    def layer(li, carry):
        with jax.named_scope("conv"):
            part = lambda steps, r: steps[len(steps) * r // NB:len(steps) * (r + 1) // NB] if 0 <= r < NB else []
            slot(four(fwd, 1) + block(fwd, 3, 0), pres(2), norms(0))
            mids = [f for i in range(D // 8) for f in mid(i)]
            for r in range(-1, NB + 1):
                slot(block(fwd, 3, r + 2) + block(fwd, 0, r + 1) + block(inv, 0, r - 1) + block(inv, 2, r - 2)
                     + block(inv, 1, r - 2),
                     part(mids, r), part(pres(3), r + 1) + part(posts(2), r - 1) + part(posts(1), r - 1),
                     pres(1) if r < 0 else posts(3)[:32] if r == NB else [])
            slot(block(inv, 2, NB - 1) + block(inv, 1, NB - 1) + block(inv, 3, 0) + block(inv, 3, 1), pair_norms(0))
            slot(projs(0, 0, (0, 4)), pair_norms(2), posts(3)[32:])
            slot(block(inv, 3, 2) + block(inv, 3, 3) + projs(0, 0, (1, 5)), pair_norms(1))
        with jax.named_scope("attn"):
            slot(projs(1, 1, (0, 1, 4, 5)), attns(0, 0), pair_norms(3))
            both = lambda i, s: slot(projs(i + 1, 1 - s, (0, 1, 4, 5)), attns(i, s))
            lax.fori_loop(0, 3, lambda j, c: (both(2 * j + 1, 1), both(2 * j + 2, 0), c)[-1], 0)
            slot(oproj(0), attns(7, 1))

        @pl.when(li == 0)
        def _():
            slot(oproj(1), norms(2))
            slot(four(fwd, 2), norms(1, 3))

        return carry

    lax.fori_loop(0, 2, layer, 0)

    with jax.named_scope("xout"):
        stores = [pltpu.make_async_copy(xio.at[c, _rows(i, 512)], out_hbm.at[_rows(i, 512), _rows(c, 128)],
                                        sems.at[4 * c + i]) for c in range(NB) for i in range(4)]
        last = oproj(1) + [lambda: None] * 7
        for c in range(NB):
            slot(last[28 * c + 7 * (c > 0):28 * c + 35],
                 [lambda: None] * (2 * (c == 0)) + [step(xout, c, j) for j in range(8)])
            for i in range(4):
                xio[c, _rows(i, 512), :] = _bf(io[c, _rows(i, 256), :])
                stores[4 * c + i].start()
        for c in stores:
            c.wait()


@jax.jit
def pallas_interleave_layers__ssm_conv_s4__sliding_local_dilated__prompt_kernel(
    A_u: jax.Array,
    A_A_re: jax.Array,
    A_A_im: jax.Array,
    A_B_re: jax.Array,
    A_B_im: jax.Array,
    A_C_re: jax.Array,
    A_C_im: jax.Array,
    A_log_dt: jax.Array,
    A_Dskip: jax.Array,
    B_x: jax.Array,
    B_wqkv: jax.Array,
    B_wo: jax.Array,
):
    del B_x
    hbm = pl.BlockSpec(memory_space=pl.ANY)
    tiles = lambda *n: pltpu.VMEM((*n, 128, 128), F32)
    out = pl.pallas_call(
        _kernel,
        out_shape=jax.ShapeDtypeStruct((L, D), BF16),
        in_specs=[pl.BlockSpec(memory_space=pltpu.SMEM)] + [hbm] * 13,
        out_specs=hbm,
        scratch_shapes=[
            pltpu.VMEM((R0, D, R1), F32),
            *[pltpu.VMEM((R0, 2, D, R1), F32)] * 5,
            pltpu.VMEM((2, D, N), F32),
            pltpu.VMEM((D // 16, 2, 4, 8, N), F32),
            pltpu.VMEM((D // 16, 336, 128), U32),
            *[tiles(n) for n in (8, 15, 15) * 2],
            pltpu.VMEM((NB, L, 128), BF16),
            pltpu.VMEM((NB, L // 2 + 8, 128), U32),
            pltpu.VMEM((6, D, N), BF16),
            pltpu.VMEM((64, 128), U32),
            pltpu.VMEM((12, D, 128), BF16),
            pltpu.VMEM((D, D), BF16),
            pltpu.VMEM(_F.shape, U32),
            pltpu.VMEM(_G.shape, U32),
            pltpu.VMEM((R0, D // 2, R1), U32),
            pltpu.VMEM((R0, D, R1), BF16),
            pltpu.VMEM((4, 7, 96, D // 2), U32),
            pltpu.VMEM((8, 7, D // 4, R1), U32),
            pltpu.VMEM((7, D // 4, D // 2), U32),
            pltpu.VMEM((8, 7, 4, 64, R1), BF16),
            pltpu.VMEM((D,), BF16),
            pltpu.VMEM((D,), BF16),
            pltpu.SemaphoreType.DMA((33,)),
        ],
        compiler_params=pltpu.CompilerParams(vmem_limit_bytes=100 * 1024 * 1024),
    )(np.zeros((1,), np.int32), A_u.reshape(L, D), A_A_re, A_A_im, A_B_re, A_B_im, A_C_re, A_C_im, A_log_dt, A_Dskip,
      B_wqkv, B_wo, _F, _G)
    return out.reshape(1, L, D)
```

```python
import jax
import jax.numpy as jnp
import ml_dtypes
import numpy as np
from jax import lax
import jax.experimental.pallas as pl
import jax.experimental.pallas.tpu as pltpu

L, D, N = 2048, 512, 128
R0, R1 = 16, 128
W, DH = 8, 16
F32, BF16, U32 = jnp.float32, jnp.bfloat16, jnp.uint32
KPER = 4
NB = D // 128
NT = (((1,), (1,)), ((), ()))


def _constants():
    n0 = np.arange(R0)[:, None, None]
    n1 = np.arange(R1)[None, :, None]
    k1 = np.arange(R1)[None, None, :]
    ang = 2.0 * np.pi * (k1 + 0.25) * (R0 * n1 + n0) / L
    f = np.concatenate([np.cos(ang), np.sin(ang)], axis=2)
    g = f.transpose(0, 2, 1)
    bf = ml_dtypes.bfloat16
    lr = np.arange(L).astype(np.float32).astype(bf).astype(np.int64).reshape(8, 16, R0)
    r = lr - (256 * np.arange(8)[:, None, None] + 16 * np.arange(16)[None, :, None])
    assert (r == r[:, :1, :]).all()

    def words(m):
        h = np.ascontiguousarray(m).astype(bf).view(np.uint16).astype(np.uint32)
        return h[:, 0::2] | (h[:, 1::2] << 16)

    return words(f), words(g), r[:, 0, :].tolist()


_F, _G, _RND = _constants()


def _cmul(a, b):
    return a[0] * b[0] - a[1] * b[1], a[0] * b[1] + a[1] * b[0]


def _csq(a):
    t = a[0] * a[1]
    return (a[0] + a[1]) * (a[0] - a[1]), t + t


def _dft4(x, sign, turn_out=False):
    (ar, ai), (br, bi), (cr, ci), (dr, di) = x
    sr, si, tr, ti = ar + cr, ai + ci, ar - cr, ai - ci
    ur, ui, vr, vi = br + dr, bi + di, br - dr, bi - di
    p, m = (tr - vi, ti + vr), (tr + vi, ti - vr)
    if sign < 0:
        p, m = m, p
    half = (sr - ur, si - ui) if not turn_out else (ui - si, sr - ur) if sign > 0 else (si - ui, ur - sr)
    return [(sr + ur, si + ui), p, half, m]


def _twiddle(v, e):
    e %= 16
    re, im = v
    h = float(np.sqrt(0.5))
    if e == 0:
        return v
    if e == 2:
        return (re - im) * h, (re + im) * h
    if e == 14:
        return (re + im) * h, (im - re) * h
    if e == 6:
        return (re + im) * -h, (re - im) * h
    if e == 10:
        return (im - re) * h, (re + im) * -h
    c, s = float(np.cos(np.pi * e / 8)), float(np.sin(np.pi * e / 8))
    return re * c - im * s, re * s + im * c


def _bf(x):
    return pltpu.bitcast(x, BF16)


def _tree(op, v):
    while len(v) > 1:
        v = [op(v[i], v[i + 1]) if i + 1 < len(v) else v[i] for i in range(0, len(v), 2)]
    return v[0]


def _run(*streams):
    order = sorted(((i + 0.5 * (k > 0)) / len(s), k, i) for k, s in enumerate(streams) for i in range(len(s)))
    for _, k, i in order:
        streams[k][i]()


def _left(a11, a12, a21, a22):
    return a21 + a22, a22, a11 + a22, a12 - a22, a11 + a12, a11, a21 - a11


def _right(b11, b12, b21, b22):
    return b11, b21 - b11, b11 + b22, b21 + b22, b22, b12 - b22, b11 + b12


def _strassen(product, emit):
    c = {}

    def run(k):
        c[k] = r = product(k)
        if k == 1:
            emit(1, 0, c[0] + r)
        elif k == 2:
            c[11], c[22] = r + c[1], r - c[0]
        elif k == 3:
            c[11] = c[11] + r
        elif k == 4:
            emit(0, 0, c[11] - r)
        elif k == 5:
            emit(0, 1, c[4] + r)
            c[22] = c[22] + r
        elif k == 6:
            emit(1, 1, c[22] + r)

    return [lambda k=k: run(k) for k in range(7)]


def _rows(i, n):
    return pl.ds(i * n if isinstance(i, int) else pl.multiple_of(i * n, n), n)


def _kernel(zero_ref, x_hbm, are_hbm, aim_hbm, bre_hbm, bim_hbm, cre_hbm, cim_hbm, ldt_hbm, dsk_hbm,
            wqkv_hbm, wo_hbm, f_hbm, g_hbm, out_hbm,
            xs, kf, ua, ub, uc, yb, par, zw, lag, qa, ka, va, qb, kb, vb,
            xio, io, abc, perm, wqkv, wo, fm, gm, kt, un, wt, us, wot, ob, ldt_ref, dsk_ref, sems):
    step = lambda fn, *a: (lambda: fn(*a))
    qs, ks, vs = (qa, qb), (ka, kb), (va, vb)
    head, rest = ([pltpu.make_async_copy(s.at[rows], abc.at[i, rows], sems.at[base + i])
                   for i, s in enumerate((are_hbm, aim_hbm, bre_hbm, bim_hbm, cre_hbm, cim_hbm))]
                  for base, rows in ((19, pl.ds(0, 32 * KPER)), (25, pl.ds(32 * KPER, D - 32 * KPER))))
    loads = [pltpu.make_async_copy(s, d, sems.at[i]) for i, (s, d) in enumerate(
        (*((x_hbm.at[:, _rows(c, 128)], xio.at[c]) for c in range(NB)),
         (f_hbm, fm), (wo_hbm, wo), (g_hbm, gm),
         *((wqkv_hbm.at[:, pl.ds(128 * j, 128)], wqkv.at[j]) for j in range(12))))]
    small = [pltpu.make_async_copy(s, d, sems.at[31 + i])
             for i, (s, d) in enumerate(((ldt_hbm, ldt_ref), (dsk_hbm, dsk_ref)))]
    for c in small + head + rest:
        c.start()
    for c in small:
        c.wait()
    high = jnp.uint32(0xFFFF0000)
    halves = lambda t: (pltpu.bitcast(t << 16, F32), pltpu.bitcast(t & high, F32))

    def col(ref):
        v = ref[...].astype(F32).reshape(1, D)
        return jnp.broadcast_to(v, (128, D)).T

    par[0] = jnp.exp(col(ldt_ref))
    par[1] = col(dsk_ref) * (1.0 / L)

    ri = lax.broadcasted_iota(jnp.int32, (128, 128), 0)
    ci = lax.broadcasted_iota(jnp.int32, (128, 128), 1)
    perm[...] = pltpu.bitcast(jnp.where(ci == (ri & 7) * DH + (ri >> 3), 1.0, 0.0).astype(BF16), U32)

    for c in head:
        c.wait()
    for c in loads:
        c.start()

    def setup(i):
        get = lambda k: halves(pltpu.bitcast(abc[k, _rows(i, 16), :], U32))
        dt = halves(pltpu.bitcast(par[0, _rows(i, 16), :].astype(BF16), U32))

        def pole(h):
            mag, ang = jnp.exp(dt[h] * get(0)[h]), dt[h] * get(1)[h]
            zw[i, h, 0], zw[i, h, 1] = mag * jnp.cos(ang), mag * jnp.sin(ang)

        def weight():
            scale = (1.0 + 1.5 * 2.0 ** -9) / L
            for h, (cr, ci, br, bi) in enumerate(zip(*map(get, (4, 5, 2, 3)))):
                wr, wi = _cmul((cr, ci), (dt[h] * br, dt[h] * bi))
                zw[i, h, 2], zw[i, h, 3] = wr * scale, wi * -scale

        return [step(pole, 0), weight, step(pole, 1)]

    lags = sorted({(c, r) for c in range(8) for r in _RND[c] if r < 16}) + [(8, 0)]
    stack = lambda vs: jnp.concatenate([jnp.concatenate([v[k] for v in vs], 0) for k in range(2)], 1).astype(BF16)

    def lagsums(i):
        zs, rhs, even = [], [], []

        def right(h):
            zr, zi, wr, wi = (zw[i, h, c] for c in range(4))
            z = {0: (jnp.ones((8, N), F32), jnp.zeros((8, N), F32)), 1: (zr, zi)}
            for e in (2, 4, 8, 16, 32, 64, 128, 256):
                z[e] = _csq(z[e // 2])
            b = [(wr, wi)]
            for e in (16, 32, 64, 128):
                zc = (z[e][0], -z[e][1])
                b += [_cmul(v, zc) for v in b]
            zs.append(z)
            rhs.append(stack(b))

        def left(h, lo, hi):
            z = zs[h]

            def power(e):
                if e not in z:
                    low = e % 256 if e > 256 and e % 256 else e & -e
                    z[e] = _csq(z[e // 2]) if e // 2 in z and e % 2 == 0 else _cmul(power(e - low), power(low))
                return z[e]

            a = [power(256 * c + r) for c, r in (lags + lags[-1:])[lo:hi]]
            o = pltpu.bitcast(lax.dot_general(stack(a), rhs[h], NT, preferred_element_type=F32), U32)
            if h:
                lag[i, 8 * lo:8 * hi, :] = jnp.concatenate(even, 0)[8 * lo:8 * hi] | (o & high)
            else:
                even.append(o >> 16)

        return [step(right, 0), step(left, 0, 0, 22), step(left, 0, 22, 42), step(right, 1), step(left, 1, 0, 20), step(left, 1, 20, 42)]

    def kgen(i):
        lane = lax.broadcasted_iota(jnp.int32, (8, 128), 1)
        src = (lane & 15) * 8 + lax.broadcasted_iota(jnp.int32, (8, 128), 0)

        memo = {}

        def piece(c, r):
            if r == 16:
                c = 0
            if (c, r) not in memo:
                memo[c, r] = (
                    pltpu.roll(jnp.where(lane == 0, piece(8, 0), merged(0, (0,) * 8)), 127, 1) if r == 16 else
                    jnp.take_along_axis(lag[i, _rows(lags.index((c, r)), 8), :], src, axis=1,
                                        mode="promise_in_bounds"))
            return memo[c, r]

        def merged(c, rs):
            if (c, rs) not in memo:
                memo[c, rs] = (piece(c, rs[0]) if c == 7 or min(rs) == 16 else
                               jnp.where(lane >> 4 == c, piece(c, rs[0]), merged(c + 1, rs[1:])))
            return memo[c, rs]

        for n0 in range(R0):
            kt[n0, _rows(i, 8), :] = merged(0, tuple(_RND[c][n0] for c in range(8)))

    get = lambda ref, n, rows: (ref[n, 0, rows, :], ref[n, 1, rows, :])

    def put(ref, n, rows, v):
        ref[n, 0, rows, :], ref[n, 1, rows, :] = v

    def outer(src, a, rows):
        x = _dft4([get(src, a + 4 * m, rows) for m in range(4)], 1, turn_out=a == 2)
        return [v if a * b == 4 else _twiddle(v, a * b) for b, v in enumerate(x)]

    def kfwd(n0, r):
        rows = _rows(r, 64)
        v = jnp.dot(_bf(kt[n0, _rows(r, 32), :]), _bf(fm[n0]), preferred_element_type=F32)
        put(ub, n0, rows, (v[:, :128] if n0 else v[:, :128] + par[1, rows, :], v[:, 128:]))

    def kdft(i):
        rows, t = _rows(i, 8), []

        def inner(b):
            for m, v in enumerate(_dft4([t[a][b] for a in range(4)], 1)):
                put(kf, b + 4 * m, rows, v)

        return [lambda a=a: t.append(outer(ub, a, rows)) for a in range(4)] + [step(inner, b) for b in range(4)]

    def fwd(n0, r):
        v = jnp.dot(un[n0, _rows(r, 64), :], _bf(fm[n0]), preferred_element_type=F32)
        put(ua, n0, _rows(r, 64), (v[:, :128], v[:, 128:]))

    def pre(a, i):
        for b, v in enumerate(outer(ua, a, _rows(i, 8))):
            put(ub, a + 4 * b, _rows(i, 8), v)

    def unouter(a, rows, t):
        for m, v in enumerate(_dft4([t[b] if a * b == 4 else _twiddle(t[b], -a * b) for b in range(4)], -1)):
            put(yb, a + 4 * m, rows, v)

    def mid(i):
        rows, first, t = _rows(i, 8), [], {}

        def inner(b):
            if b == 0:
                first.extend(outer(ua, 0, rows))
            x = _dft4([first[b]] + [get(ub, a + 4 * b, rows) for a in range(1, 4)], 1)
            t[b], *y = _dft4([_cmul(x[m], get(kf, b + 4 * m, rows)) for m in range(4)], -1, turn_out=b == 2)
            for a in range(1, 4):
                put(uc, a + 4 * b, rows, y[a - 1])
            if b == 3:
                unouter(0, rows, t)

        return [step(inner, b) for b in range(4)]

    def post(a, i):
        unouter(a, _rows(i, 8), [get(uc, a + 4 * b, _rows(i, 8)) for b in range(4)])

    def inv(n0, r):
        rows = _rows(r, 64)
        y = jnp.concatenate(get(yb, n0, rows), 1).astype(BF16)
        xs[n0, rows, :] = xs[n0, rows, :] + jnp.dot(y, _bf(gm[n0]), preferred_element_type=F32)

    def wprep(g, t):
        ops = []

        def load(h):
            if t < 3:
                lo, hi = (lax.dot_general(_bf(perm[...]), wqkv[4 * t + g, _rows(h + e, 128), :], NT,
                                          preferred_element_type=F32) for e in (0, 2))
                if t == 0:
                    lo, hi = lo * DH ** -0.5, hi * DH ** -0.5
            else:
                v = [jnp.dot(_bf(perm[...]), wo[_rows(2 * h + e, 128), _rows(g, 128)], preferred_element_type=F32)
                     for e in range(2)]
                lo, hi = (jnp.concatenate([u[64 * e:64 * e + 64] for u in v], 0).T for e in range(2))
            ops[:] = lo[:64], hi[:64], lo[64:], hi[64:]

        def save(h, i):
            for k, a in enumerate(_left(*[v[16 * i:16 * i + 16] for v in ops])):
                at = (_rows(4 * (t if t < 3 else g) + i, 8), _rows(h, 128))
                (wt if t < 3 else wot)[(g, k, *at) if t < 3 else (k, *at)] = pltpu.bitcast(a.astype(BF16), U32)

        return [f for h in range(2) for f in [step(load, h)] + [step(save, h, i) for i in range(4)]]

    def words(c):
        io[c, :L // 2, :] = pltpu.bitcast(xio[c], U32)

    def xin(j, c):
        xs[2 * j, _rows(c, 128), :], xs[2 * j + 1, _rows(c, 128), :] = halves(io[c, pl.ds(j, R1, stride=8), :].T)

    def norm(n0):
        acc, stat = {}, []

        def moment(k, lo, hi):
            for i in range(lo, hi):
                v = xs[n0, 8 * i:8 * i + 8, :]
                v = jnp.square(v - stat[0]) if k else v
                acc[i % 4] = v if i < 4 else acc[i % 4] + v
            if hi == D // 8:
                v = jnp.sum(_tree(jnp.add, list(acc.values())), axis=0, keepdims=True) * (1.0 / D)
                stat.append(lax.rsqrt(v + 1e-5) if k else v)

        def scale(c):
            rows = _rows(c, 128)
            un[n0, rows, :] = get(rows).astype(BF16)

        get = lambda rows: (xs[n0, rows, :] - stat[0]) * stat[1]
        return [[step(moment, 0, 0, 64)], [step(moment, 1, i, i + 16) for i in range(0, 64, 16)],
                [step(scale, c) for c in range(4)]], get

    def norms(*aa):
        return [f for a in aa for stage in zip(*[norm(a + 4 * m)[0] for m in range(4)])
                for steps in stage for f in steps]

    def pair_norms(a):
        stages, get = zip(*[norm(a + 4 * m) for m in range(4)])

        def operands(j, c):
            (b11, b21), (b12, b22) = ((f(_rows(c, 16)), f(_rows(c + 16, 16))) for f in get[2 * j:2 * j + 2])
            for k, b in enumerate(_right(b11, b12, b21, b22)):
                us[2 * a + j, k, _rows(c, 8), :] = pltpu.bitcast(b.astype(BF16), U32)

        return ([f for k in range(2) for st in stages for f in st[k]]
                + [step(operands, j, c) for j in range(2) for c in range(16)])

    def proj(i, slot, m, t):
        p, g, ref = i >> 2, i & 3, (qs, ks, vs)[t][slot]

        def emit(half, j, r):
            ref[m + 2 * j + 7 * (t > 0), _rows(half, 64), :] = r
            if t and m + j:
                ref[m + 2 * j - 1, _rows(half, 64), :] = pltpu.roll(r, 1, 1)

        return _strassen(lambda k: jnp.dot(_bf(wt[g, k, _rows(t, 32), :]), _bf(us[2 * p + 4 * (m & 1) + (m >> 2), k]),
                                           preferred_element_type=F32), emit)

    def attn(i, slot, m0):
        p, g = i >> 2, i & 3
        first = lax.broadcasted_iota(jnp.int32, (8, 128), 1) == 0
        window = lambda ref, d: {e: ref[slot][e, 8 * d:8 * d + 8, :] for e in range(m0, m0 + W + 1)}
        s, o = {}, {}

        def logits(m, d0):
            for d in (d0, d0 + 1):
                k = window(ks, d)
                q = qs[slot][m, 8 * d:8 * d + 8, :]
                for w in range(W):
                    t = q * k[m + 7 - w]
                    s[m, w] = t if d == 0 else s[m, w] + t

        def softmax(m):
            t = [jnp.where(first, -1e9, s[m, w]) if w > m else s[m, w] for w in range(W)]
            mx = _tree(jnp.maximum, t)
            e = [jnp.exp(v - mx) for v in t]
            rs = 1.0 / _tree(jnp.add, e)
            s.update({(m, w): e[w] * rs for w in range(W)})

        def values(d):
            v = window(vs, d)
            for m in (m0, m0 + 1):
                o[m, d] = sum((s[m, w] * v[m + 7 - w] for w in range(1, W)), s[m, 0] * v[m + 7])
            if d % 2 and d > 8:
                blocks = [jnp.concatenate([o[m, e - 1], o[m, e]], 0) for e in (d - 8, d) for m in (m0, m0 + 1)]
                for k, b in enumerate(_right(*blocks)):
                    ob[m0 + p, k, g, 8 * d - 72:8 * d - 56, :] = b.astype(BF16)

        return ([f for m in (m0, m0 + 1) for f in [step(logits, m, d) for d in range(0, DH, 2)] + [step(softmax, m)]]
                + [step(values, d + e) for d in range(0, 8, 2) for e in (0, 1, 8, 9)])

    def oproj(p):
        def pair(c, m0):
            def emit(half, j, r):
                at = (2 * (m0 + j) + p, _rows(2 * c + half, 64))
                xs[at] = xs[at] + r

            return _strassen(lambda k: jnp.dot(_bf(wot[k, _rows(c, 32), :]), ob[m0 + p, k].reshape(D // 2, R1),
                                               preferred_element_type=F32), emit)

        return [f for c in range(NB) for m0 in range(0, 8, 2) for f in pair(c, m0)]

    def xout(c, j):
        lo, hi = (pltpu.bitcast(xs[2 * j + k, _rows(c, 128), :].astype(BF16).astype(F32), U32) for k in range(2))
        io[c, pl.ds(j, R1, stride=8), :] = ((lo >> 16) | hi).T

    four = lambda fn, *aa: [step(fn, a + 4 * m, r) for a in aa for m in range(4) for r in range(2 * NB)]
    block = lambda fn, a, r: [step(fn, a + 4 * m, 2 * r + h) for h in range(2) for m in range(4)] if 0 <= r < NB else []

    regions, zero = [], zero_ref[0]

    def slot(*streams):
        regions.append(None)
        pl.when(zero < len(regions))(lambda: _run(*streams))

    doubled = lambda fs: [step(_run, fs[i:i + 2]) for i in range(0, len(fs), 2)]
    pres = lambda a: [step(pre, a, i) for i in range(D // 8)]
    posts = lambda a: [step(post, a, i) for i in range(D // 8)]
    projs = lambda i, s, ms: [f for m in ms for t in (1, 2, 0) for f in proj(i, s, m, t)]
    attns = lambda i, s: [f for m in range(0, 8, 2) for f in attn(i, s, m)]

    with jax.named_scope("kgen"):
        ng = D // 16 // KPER
        each = lambda fn, s: [f for k in range(KPER) for f in fn(KPER * s + k)]

        def generate(s, more=(), last=False):
            for k in range(KPER):
                kgen(KPER * (s - 1) + k)
            _run(each(lagsums, s), more)
            if not last:
                _run(each(setup, s + 1))

        _run(setup(0))
        _run(each(lagsums, 0), [f for i in range(1, 2 * KPER) for f in setup(i)])
        for c in rest:
            c.wait()
        lax.fori_loop(1, ng - NB - 1, lambda s, _: generate(s), None)
        for c in loads[:NB]:
            c.wait()
        lax.fori_loop(0, NB, lambda c, _: generate(
            c + ng - NB - 1, [step(words, c)] + [step(xin, j, c) for j in range(8)]), None)
        generate(ng - 1, last=True)
    with jax.named_scope("kfwd"):
        for c in loads[NB:]:
            c.wait()
        kdfts = lambda r: [f for i in range(16) for f in kdft(16 * r + i)]
        for r, other in enumerate((norms(2, 1), *[sum(norm(n0)[0] + norm(n0 + 1)[0] + norm(n0 + 8)[0], []) for n0 in (3, 7)],
                                   sum(norm(0)[0] + norm(12)[0], []))):
            slot([f for a in range(4) for f in block(kfwd, a, r)], [f for t in (3, 0, 1, 2) for f in wprep(r, t)],
                 kdfts(r - 1) if r else [step(kgen, D // 16 - 1 - k) for k in range(KPER)], other)
        slot(four(fwd, 2), kdfts(NB - 1))

    def layer(li, carry):
        with jax.named_scope("conv"):
            part = lambda steps, r: steps[len(steps) * r // NB:len(steps) * (r + 1) // NB] if 0 <= r < NB else []
            slot(block(fwd, 1, 0) + block(fwd, 1, 1) + block(fwd, 3, 0), pres(2))
            mids = [f for i in range(D // 8) for f in mid(i)]
            for r in range(-1, NB + 1):
                slot((block(fwd, 1, r + 2) if r >= 0 else []) + block(fwd, 3, r + 2) + block(fwd, 0, r + 1) + block(inv, 0, r - 1) + block(inv, 2, r - 2)
                     + block(inv, 1, r - 2),
                     part(mids, r), part(pres(3), r + 1) + part(posts(2), r - 1) + part(posts(1), r - 1),
                     pres(1)[:32] if r < 0 else posts(3)[:32] if r == NB else
                     part(pres(1), r + 1) if r else [])
            slot(block(inv, 2, NB - 1) + block(inv, 1, NB - 1) + block(inv, 3, 0) + block(inv, 3, 1), pair_norms(0))
            slot(projs(0, 0, (0, 4)), pair_norms(2), posts(3)[32:])
            slot(block(inv, 3, 2) + block(inv, 3, 3) + projs(0, 0, (1, 5)), pair_norms(1))
        with jax.named_scope("attn"):
            slot(projs(1, 1, (0, 1, 4, 5)), pair_norms(3) + doubled(attns(0, 0)))
            both = lambda i, s: slot(projs(i + 1, 1 - s, (0, 1, 4, 5)), attns(i, s))
            lax.fori_loop(0, 3, lambda j, c: (both(2 * j + 1, 1), both(2 * j + 2, 0), c)[-1], 0)
            slot(oproj(0), attns(7, 1))

        @pl.when(li == 0)
        def _():
            slot(oproj(1), norms(2, 0))
            slot(four(fwd, 2), norms(1, 3))

        return carry

    lax.fori_loop(0, 2, layer, 0)

    with jax.named_scope("xout"):
        stores = [pltpu.make_async_copy(xio.at[c, _rows(i, 512)], out_hbm.at[_rows(i, 512), _rows(c, 128)],
                                        sems.at[4 * c + i]) for c in range(NB) for i in range(4)]
        last = oproj(1) + [lambda: None] * 7
        for c in range(NB):
            slot(last[28 * c + 7 * (c > 0):28 * c + 35],
                 [lambda: None] * (2 * (c == 0)) + [step(xout, c, j) for j in range(8)])
            for i in range(4):
                xio[c, _rows(i, 512), :] = _bf(io[c, _rows(i, 256), :])
                stores[4 * c + i].start()
        for c in stores:
            c.wait()


@jax.jit
def pallas_interleave_layers__ssm_conv_s4__sliding_local_dilated__prompt_kernel(
    A_u: jax.Array,
    A_A_re: jax.Array,
    A_A_im: jax.Array,
    A_B_re: jax.Array,
    A_B_im: jax.Array,
    A_C_re: jax.Array,
    A_C_im: jax.Array,
    A_log_dt: jax.Array,
    A_Dskip: jax.Array,
    B_x: jax.Array,
    B_wqkv: jax.Array,
    B_wo: jax.Array,
):
    del B_x
    hbm = pl.BlockSpec(memory_space=pl.ANY)
    tiles = lambda *n: pltpu.VMEM((*n, 128, 128), F32)
    out = pl.pallas_call(
        _kernel,
        out_shape=jax.ShapeDtypeStruct((L, D), BF16),
        in_specs=[pl.BlockSpec(memory_space=pltpu.SMEM)] + [hbm] * 13,
        out_specs=hbm,
        scratch_shapes=[
            pltpu.VMEM((R0, D, R1), F32),
            *[pltpu.VMEM((R0, 2, D, R1), F32)] * 5,
            pltpu.VMEM((2, D, N), F32),
            pltpu.VMEM((D // 16, 2, 4, 8, N), F32),
            pltpu.VMEM((D // 16, 336, 128), U32),
            *[tiles(n) for n in (8, 15, 15) * 2],
            pltpu.VMEM((NB, L, 128), BF16),
            pltpu.VMEM((NB, L // 2 + 8, 128), U32),
            pltpu.VMEM((6, D, N), BF16),
            pltpu.VMEM((64, 128), U32),
            pltpu.VMEM((12, D, 128), BF16),
            pltpu.VMEM((D, D), BF16),
            pltpu.VMEM(_F.shape, U32),
            pltpu.VMEM(_G.shape, U32),
            pltpu.VMEM((R0, D // 2, R1), U32),
            pltpu.VMEM((R0, D, R1), BF16),
            pltpu.VMEM((4, 7, 96, D // 2), U32),
            pltpu.VMEM((8, 7, D // 4, R1), U32),
            pltpu.VMEM((7, D // 4, D // 2), U32),
            pltpu.VMEM((8, 7, 4, 64, R1), BF16),
            pltpu.VMEM((D,), BF16),
            pltpu.VMEM((D,), BF16),
            pltpu.SemaphoreType.DMA((33,)),
        ],
        compiler_params=pltpu.CompilerParams(vmem_limit_bytes=100 * 1024 * 1024),
    )(np.zeros((1,), np.int32), A_u.reshape(L, D), A_A_re, A_A_im, A_B_re, A_B_im, A_C_re, A_C_im, A_log_dt, A_Dskip,
      B_wqkv, B_wo, _F, _G)
    return out.reshape(1, L, D)
```
